```python
import jax
import jax.numpy as jnp

def _softmax(x, axis=-1):
    return jax.nn.softmax(x, axis=axis)

def _gelu(x):
    return jax.nn.gelu(x, approximate=True)

def _silu(x):
    return jax.nn.silu(x)

def _sigmoid(x):
    return jax.nn.sigmoid(x)

def _layernorm(x, axis=-1, eps=1e-05):
    m = jnp.mean(x, axis=axis, keepdims=True)
    v = jnp.var(x, axis=axis, keepdims=True)
    return (x - m) / jnp.sqrt(v + eps)

def _scatter_add(tgt, idx, src, axis=0):
    return tgt.at[idx].add(src)

def _segment_sum(src, seg, n):
    return jax.ops.segment_sum(src, seg, n)

class _Rng:

    def __init__(self, key):
        self._k = key

    def _next(self):
        self._k, sub = jax.random.split(self._k)
        return sub

    def normal(self, shape):
        return jax.random.normal(self._next(), shape, dtype=jnp.bfloat16)

    def randint(self, lo, hi, shape):
        return jax.random.randint(self._next(), shape, lo, hi, dtype=jnp.int32)

    def uniform(self, shape, lo=0.0, hi=1.0):
        return jax.random.uniform(self._next(), shape, jnp.bfloat16, lo, hi)

    def permutation(self, n):
        return jax.random.permutation(self._next(), n)
kernel_name = 'sequential_preLN__memory_aug_infini_attn__moe_arch_mod__prompt'

def setup_inputs():
    _rng = _Rng(jax.random.key(int.from_bytes(__import__("os").urandom(4), "little")))
    _w = lambda a: (lambda t: t.astype(jnp.bfloat16) if jnp.issubdtype(t.dtype, jnp.floating) else t)(jnp.asarray(a))

    def _A_setup():
        B, S, D, H = (1, 2048, 576, 32)
        N = 4
        L = max(1, S // N)
        sc = D ** (-0.5)
        return {'x': _w((lambda *s: _rng.normal(s) * 0.05)(B, N * L, D)), 'wq': _w((lambda *s: _rng.normal(s) * 0.05)(D, D) * sc), 'wk': _w((lambda *s: _rng.normal(s) * 0.05)(D, D) * sc), 'wv': _w((lambda *s: _rng.normal(s) * 0.05)(D, D) * sc), 'wo': _w((lambda *s: _rng.normal(s) * 0.05)(D, D) * sc), 'beta': _w((lambda *s: _rng.normal(s) * 0.05)(H))}
    _A_in = _A_setup()

    def _B_setup():
        B, S, D, F, C = (1, 2048, 576, 4608, 1)
        return {'x': _w((lambda *s: _rng.normal(s) * 0.05)(B, S, D)), 'w_r': _w((lambda *s: _rng.normal(s) * 0.05)(D)), 'w_gate': _w((lambda *s: _rng.normal(s) * 0.05)(D, F)), 'w_up': _w((lambda *s: _rng.normal(s) * 0.05)(D, F)), 'w_down': _w((lambda *s: _rng.normal(s) * 0.05)(F, D))}
    _B_in = _B_setup()
    return {'A_x': _A_in['x'], 'A_wq': _A_in['wq'], 'A_wk': _A_in['wk'], 'A_wv': _A_in['wv'], 'A_wo': _A_in['wo'], 'A_beta': _A_in['beta'], 'B_x': _B_in['x'], 'B_w_r': _B_in['w_r'], 'B_w_gate': _B_in['w_gate'], 'B_w_up': _B_in['w_up'], 'B_w_down': _B_in['w_down']}

def reference(A_x, A_wq, A_wk, A_wv, A_wo, A_beta, B_x, B_w_r, B_w_gate, B_w_up, B_w_down):

    def _A_ref(x, wq, wk, wv, wo, beta):
        B, S, D = x.shape
        H = 32
        Dh = D // H
        N = 4
        L = S // N
        q = (lambda x, *d: x.transpose(*d))((x @ wq).reshape(B, S, H, Dh), 0, 2, 1, 3).reshape(B, H, N, L, Dh)
        k = (lambda x, *d: x.transpose(*d))((x @ wk).reshape(B, S, H, Dh), 0, 2, 1, 3).reshape(B, H, N, L, Dh)
        v = (lambda x, *d: x.transpose(*d))((x @ wv).reshape(B, S, H, Dh), 0, 2, 1, 3).reshape(B, H, N, L, Dh)
        phi = lambda t: jnp.where(t > 0, t + 1.0, jnp.exp(t))
        scale = Dh ** (-0.5)
        ar = jnp.arange(L)
        mask = (lambda x, dt: x.astype(dt))(ar[:, None] < ar[None, :], x.dtype) * -1000000000.0
        g = _sigmoid(beta).reshape(1, H, 1, 1)
        M = jnp.einsum('bhd,bhe->bhde', q[:, :, 0, 0, :] * 0.0, q[:, :, 0, 0, :] * 0.0)
        z = q[:, :, 0, 0, :] * 0.0
        outs = []
        for s in range(N):
            qs, ks, vs = (q[:, :, s].copy(), k[:, :, s].copy(), v[:, :, s].copy())
            logits = jnp.einsum('bhqd,bhkd->bhqk', qs, ks) * scale + mask
            p = _softmax(logits, axis=-1)
            a_dot = jnp.einsum('bhqk,bhkd->bhqd', p, vs)
            pq = phi(qs)
            num = jnp.einsum('bhld,bhde->bhle', pq, M)
            den = jnp.einsum('bhld,bhd->bhl', pq, z)[..., None] + 1e-06
            a_mem = num / den
            o = g * a_mem + (1.0 - g) * a_dot
            outs.append(o)
            pk = phi(ks)
            M = M + jnp.einsum('bhld,bhle->bhde', pk, vs)
            z = z + jnp.einsum('bhld->bhd', pk)
        o = (lambda x, *d: x.transpose(*d))(jnp.stack(outs, 2).reshape(B, H, S, Dh), 0, 2, 1, 3).reshape(B, S, D)
        return o @ wo

    def _B_ref(x, w_r, w_gate, w_up, w_down):
        B, S, D = x.shape
        C = 1
        r = x @ w_r
        idx = jnp.argsort(-r, axis=-1)[:, :C]
        idx_e = jnp.repeat(idx.reshape(B, C, 1), D, axis=2)
        x_sel = jnp.take_along_axis(x, idx_e, axis=1)
        g = _silu(x_sel @ w_gate)
        u = x_sel @ w_up
        y = g * u @ w_down
        r_sel = _sigmoid(jnp.take_along_axis(r, idx, axis=1))
        y = y * r_sel.reshape(B, C, 1)
        b_off = (jnp.arange(B) * S).reshape(B, 1)
        flat_idx = (idx + b_off).reshape(B * C)
        zero = (x * 0.0).reshape(B * S, D)
        upd = _scatter_add(zero, flat_idx, y.reshape(B * C, D), axis=0)
        return x + upd.reshape(B, S, D)
    x = A_x
    h = x + _A_ref(_layernorm(x, axis=-1), A_wq, A_wk, A_wv, A_wo, A_beta)
    h2 = h + _B_ref(_layernorm(h, axis=-1), B_w_r, B_w_gate, B_w_up, B_w_down)
    return h2
```

```python
import jax
import jax.numpy as jnp
import jax.experimental.pallas as pl
import jax.experimental.pallas.tpu as pltpu

F32 = jnp.float32
BF16 = jnp.bfloat16
U32 = jnp.uint32
I32 = jnp.int32

S = 2048
D = 576
H = 32
DH = 18
NSEG = 4
L = S // NSEG
FF = 4608
NQB = L // 128
TOFF = (0, 1, 3, 6)
NTILE = 10
NG = 5
WIN = 112
GROUP_HEADS = tuple(tuple(h for h in range(H)
                          if min(max(0, -(-(DH * h + DH - 128) // WIN)), NG - 1) == g)
                    for g in range(NG))
GROUP_OF = {h: g for g in range(NG) for h in GROUP_HEADS[g]}
GH_MAX = max(len(t) for t in GROUP_HEADS)
LN_EPS = 1e-5
LOG2E = 1.4426950408889634
QSCALE = (DH ** -0.5) * LOG2E
SAFE_LOGIT = 60.0
SAFE_V = 2.0 ** 50

NN = (((1,), (0,)), ((), ()))
NT = (((1,), (1,)), ((), ()))
TN = (((0,), (0,)), ((), ()))

for _g, _hs in enumerate(GROUP_HEADS):
    for _h in _hs:
        assert WIN * _g <= DH * _h and DH * _h + DH <= WIN * _g + 128


def _dot(a, b, dims=NN):
    return jax.lax.dot_general(a, b, dims, preferred_element_type=F32)


def _layernorm_t(x):
    m = jnp.sum(x, axis=0, keepdims=True) * (1.0 / D)
    xc = x - m
    v = jnp.sum(xc * xc, axis=0, keepdims=True) * (1.0 / D)
    return xc * jax.lax.rsqrt(v + LN_EPS)


def _phi(t):
    return jnp.where(t > 0, t + 1.0, jnp.exp(t))


def _sigmoid(t):
    return 1.0 / (1.0 + jnp.exp(-t))


def _max_col_norm(w):
    wf = w.astype(F32)
    ss = jnp.sum(wf * wf, axis=0, keepdims=True)
    return jnp.sqrt(jnp.max(ss, axis=1, keepdims=True))


def _kernel(xt_hbm, wq_hbm, wk_hbm, wv_hbm, wo_hbm, beta_ref, wr_ref, wg_hbm, wu_hbm, wdt_hbm,
            out_hbm,
            xbuf, wq_raw, wk_raw, wv_raw, wo_raw, wqt, wkt, wvt, wot, xn, kb, qt, pkt, pqt, vt32,
            pbuf, m_f32, m_bf, ot, h_all, obuf, wg_v, wu_v, wdt_v, gcol, wrcol, cmask, bestv,
            besti, stage, flag, sem_x, sem_w, sem_o):
    def x_copy(s):
        cols = pl.ds(pl.multiple_of(s * L, L), L)
        return pltpu.make_async_copy(xt_hbm.at[:, cols], xbuf.at[:, cols], sem_x.at[s])

    def out_copy(s):
        cols = pl.ds(pl.multiple_of(s * L, L), L)
        return pltpu.make_async_copy(obuf.at[:, cols], out_hbm.at[:, cols], sem_o.at[s])

    cp_wk = pltpu.make_async_copy(wk_hbm, wk_raw, sem_w.at[0])
    cp_wq = pltpu.make_async_copy(wq_hbm, wq_raw, sem_w.at[1])
    cp_wv = pltpu.make_async_copy(wv_hbm, wv_raw, sem_w.at[2])
    cp_wo = pltpu.make_async_copy(wo_hbm, wo_raw, sem_w.at[3])
    cp_wg = pltpu.make_async_copy(wg_hbm, wg_v, sem_w.at[4])
    cp_wu = pltpu.make_async_copy(wu_hbm, wu_v, sem_w.at[5])
    cp_wd = pltpu.make_async_copy(wdt_hbm, wdt_v, sem_w.at[6])

    def stage_ln1(s):
        for c in range(NQB):
            cols = pl.ds(pl.multiple_of(s * L + 128 * c, 128), 128)
            xn[:, 128 * c:128 * (c + 1)] = _layernorm_t(xbuf[:, cols].astype(F32)).astype(BF16)

    def stage_proj():
        xv = xn[...]
        kt = _dot(wkt[...], xv)
        pkt[...] = _phi(kt).astype(BF16)
        ktb = kt.astype(BF16)
        for g in range(NG):
            kb[g] = ktb[WIN * g:WIN * g + 128, :].T
        qf = _dot(wqt[...], xv)
        qt[...] = (qf * QSCALE).astype(BF16)
        pqt[...] = _phi(qf).astype(BF16)
        vt = _dot(wvt[...], xv)
        tail = jnp.concatenate([jnp.ones((1, L), F32), jnp.zeros((13, L), F32)], axis=0)
        for h in range(H):
            vt32[32 * h:32 * h + 16, :] = vt[DH * h:DH * h + 16].astype(BF16)
            vt32[32 * h + 16:32 * h + 32, :] = jnp.concatenate(
                [vt[DH * h + 16:DH * h + 18], tail], axis=0).astype(BF16)

    def masked_q(w0, i, word_mask):
        qu = pltpu.bitcast(qt[pl.ds(w0, 128), 128 * i:128 * (i + 1)], U32)
        return pltpu.bitcast(jnp.where(word_mask, qu, jnp.uint32(0)), BF16)

    def head_word_mask(lo):
        word = jax.lax.broadcasted_iota(I32, (64, 128), 0)
        return (2 * word >= lo) & (2 * word < lo + DH)

    def stage_scores_fast():
        for h in range(H):
            g = GROUP_OF[h]
            word_mask = head_word_mask(DH * h - WIN * g)
            for i in range(NQB):
                n = 128 * (i + 1)
                st = _dot(kb[g, 0:n, :], masked_q(WIN * g, i, word_mask))
                p = jnp.exp2(st)
                r0 = TOFF[i] * 64
                if i > 0:
                    pbuf[h, r0:r0 + 64 * i, :] = pltpu.bitcast(p[:n - 128].astype(BF16), U32)
                pd = pltpu.bitcast(p[n - 128:n].astype(BF16), U32)
                pbuf[h, r0 + 64 * i:r0 + 64 * (i + 1), :] = pd & cmask[...]

    def stage_scores_safe():
        causal = (jax.lax.broadcasted_iota(I32, (128, 128), 0)
                  <= jax.lax.broadcasted_iota(I32, (128, 128), 1))

        def head(h, carry):
            g = jnp.clip((DH * h + DH - 128 + WIN - 1) // WIN, 0, NG - 1)
            g = jnp.where(DH * h + DH <= 128, 0, g)
            w0 = pl.multiple_of(WIN * g, 16)
            word_mask = head_word_mask(DH * h - WIN * g)
            for i in range(NQB):
                n = 128 * (i + 1)
                st = _dot(kb[g, 0:n, :], masked_q(w0, i, word_mask))
                sd = jnp.where(causal, st[n - 128:n], -jnp.inf)
                m = jnp.max(sd, axis=0, keepdims=True)
                if i > 0:
                    m = jnp.maximum(m, jnp.max(st[:n - 128], axis=0, keepdims=True))
                r0 = TOFF[i] * 64
                if i > 0:
                    pbuf[h, r0:r0 + 64 * i, :] = pltpu.bitcast(
                        jnp.exp2(st[:n - 128] - m).astype(BF16), U32)
                pbuf[h, r0 + 64 * i:r0 + 64 * (i + 1), :] = pltpu.bitcast(
                    jnp.exp2(sd - m).astype(BF16), U32)
            return carry

        jax.lax.fori_loop(0, H, head, 0)

    def stage_pv():
        for g in range(NG):
            heads = GROUP_HEADS[g]
            nh = len(heads)
            for i in range(NQB):
                n = 128 * (i + 1)
                nm = _dot(m_bf[g, 0:32 * nh, :],
                          pqt[WIN * g:WIN * g + 128, 128 * i:128 * (i + 1)])
                for j, h in enumerate(heads):
                    r0 = TOFF[i] * 64
                    p = pltpu.bitcast(pbuf[h, r0:r0 + 64 * (i + 1), :], BF16)
                    o = _dot(vt32[32 * h:32 * h + 32, 0:n], p)
                    gate = gcol[h:h + 1, :]
                    a = (1.0 - gate) / o[DH:DH + 1, :]
                    b = gate / (nm[32 * j + DH:32 * j + DH + 1, :] + 1e-6)
                    ot[i, DH * h:DH * h + 24, :] = o[0:24] * a + nm[32 * j:32 * j + 24] * b

    def stage_mem_update():
        for g in range(NG):
            heads = GROUP_HEADS[g]
            nh = len(heads)
            upd = _dot(vt32[32 * heads[0]:32 * (heads[0] + nh), :],
                       pkt[WIN * g:WIN * g + 128, :], NT)
            row = jax.lax.broadcasted_iota(I32, (32 * nh, 128), 0)
            lane = jax.lax.broadcasted_iota(I32, (32 * nh, 128), 1)
            lo = (row >> 5) * DH + (DH * heads[0] - WIN * g)
            keep = (lane >= lo) & (lane < lo + DH)
            m_new = m_f32[g, 0:32 * nh, :] + jnp.where(keep, upd, 0.0)
            m_f32[g, 0:32 * nh, :] = m_new
            m_bf[g, 0:32 * nh, :] = m_new.astype(BF16)

    def stage_out(s):
        wo = wot[...]
        for i in range(NQB):
            cols = pl.ds(pl.multiple_of(s * L + 128 * i, 128), 128)
            attn = _dot(wo, ot[i, 0:D, :].astype(BF16))
            hh = xbuf[:, cols].astype(F32) + attn
            h_all[s * NQB + i] = hh
            hn = _layernorm_t(hh)
            obuf[:, cols] = (hh + hn).astype(BF16)
            r = jnp.sum(hn * wrcol[...], axis=0, keepdims=True)
            m = jnp.max(r, axis=1, keepdims=True)
            ids = s * L + 128 * i + jax.lax.broadcasted_iota(I32, (1, 128), 1)
            idx = jnp.min(jnp.where(r == m, ids, S), axis=1, keepdims=True)
            better = m > bestv[0:1, 0:1]
            bestv[...] = jnp.broadcast_to(jnp.where(better, m, bestv[0:1, 0:1]), (8, 128))
            besti[...] = jnp.broadcast_to(jnp.where(better, idx, besti[0:1, 0:1]), (8, 128))

    x_copy(0).start()
    cp_wk.start()
    cp_wq.start()
    cp_wv.start()
    cp_wo.start()
    for s in range(1, NSEG):
        x_copy(s).start()

    beta = beta_ref[...].astype(F32).reshape(1, H)
    gpad = jnp.concatenate([_sigmoid(beta), jnp.zeros((1, 128 - H), F32)], axis=1)
    gcol[...] = jnp.transpose(jnp.broadcast_to(gpad, (128, 128)))
    wr = jnp.concatenate([wr_ref[...].astype(F32).reshape(1, D), jnp.zeros((1, 64), F32)], axis=1)
    wrcol[...] = jnp.transpose(jnp.broadcast_to(wr, (128, D + 64)))[0:D]
    kr = 2 * jax.lax.broadcasted_iota(I32, (64, 128), 0)
    qc = jax.lax.broadcasted_iota(I32, (64, 128), 1)
    cmask[...] = (jnp.where(kr <= qc, jnp.uint32(0x0000FFFF), jnp.uint32(0))
                  | jnp.where(kr + 1 <= qc, jnp.uint32(0xFFFF0000), jnp.uint32(0)))
    m_f32[...] = jnp.zeros_like(m_f32)
    m_bf[...] = jnp.zeros_like(m_bf)
    bestv[...] = jnp.full((8, 128), -jnp.inf, F32)
    besti[...] = jnp.zeros((8, 128), I32)

    x_copy(0).wait()
    stage_ln1(0)
    cp_wk.wait()
    wk = wk_raw[...]
    wkt[...] = wk.T
    nk = _max_col_norm(wk)
    cp_wq.wait()
    wq = wq_raw[...]
    wqt[...] = wq.T
    nq = _max_col_norm(wq)
    cp_wv.wait()
    wv = wv_raw[...]
    wvt[...] = wv.T
    nv = _max_col_norm(wv)
    cp_wo.wait()
    wot[...] = wo_raw[...].T
    cp_wg.start()
    cp_wu.start()
    cp_wd.start()

    bound = (QSCALE * DH * D) * nq * nk
    safe = (bound <= SAFE_LOGIT) & (nv * (D ** 0.5) <= SAFE_V)
    flag[0] = jnp.sum(jnp.where(safe, 1, 0).astype(I32))

    def segment(s, carry):
        stage_proj()

        @pl.when(s + 1 < NSEG)
        def _():
            x_copy(s + 1).wait()

        nxt = jnp.minimum(s + 1, NSEG - 1)

        @pl.when(flag[0] == 1)
        def _():
            stage_scores_fast()
            stage_ln1(nxt)

        @pl.when(flag[0] != 1)
        def _():
            stage_scores_safe()
            stage_ln1(nxt)

        stage_pv()
        stage_out(s)
        stage_mem_update()
        out_copy(s).start()
        return carry

    jax.lax.fori_loop(0, NSEG, segment, 0)

    idx = jnp.sum(besti[0:1, 0:1])
    r_sel = bestv[0:1, 0:1]
    blk = idx >> 7
    hb = h_all[blk]
    hn = _layernorm_t(hb)
    onehot = jax.lax.broadcasted_iota(I32, (16, 128), 1) == idx - blk * 128
    xs = _dot(onehot.astype(BF16), hn.astype(BF16), NT).astype(BF16)
    cp_wg.wait()
    cp_wu.wait()
    cp_wd.wait()
    ga = _dot(xs, wg_v[...])
    up = _dot(xs, wu_v[...])
    act = (ga * _sigmoid(ga) * up).astype(BF16)
    y = _dot(act, wdt_v[...], NT) * _sigmoid(r_sel)
    y_hi = y.astype(BF16)
    y_lo = (y - y_hi.astype(F32)).astype(BF16)
    row = jax.lax.broadcasted_iota(I32, (16, D), 0)
    y2 = jnp.where(row == 0, y_hi, jnp.where(row == 1, y_lo, jnp.zeros_like(y_hi)))
    upd = _dot(y2, onehot.astype(BF16), TN)
    stage[...] = (hb + hn + upd).astype(BF16)
    for s in range(NSEG):
        out_copy(s).wait()
    fix = pltpu.make_async_copy(
        stage, out_hbm.at[:, pl.ds(pl.multiple_of(blk * 128, 128), 128)], sem_w.at[7])
    fix.start()
    fix.wait()


@jax.jit
def pallas_sequential_preLN__memory_aug_infini_attn__moe_arch_mod__prompt_kernel(
    A_x: jax.Array,
    A_wq: jax.Array,
    A_wk: jax.Array,
    A_wv: jax.Array,
    A_wo: jax.Array,
    A_beta: jax.Array,
    B_x: jax.Array,
    B_w_r: jax.Array,
    B_w_gate: jax.Array,
    B_w_up: jax.Array,
    B_w_down: jax.Array,
):
    del B_x
    hbm = pl.BlockSpec(memory_space=pltpu.HBM)
    vmem = pl.BlockSpec(memory_space=pltpu.VMEM)
    scratch = [
        pltpu.VMEM((D, S), BF16),
        pltpu.VMEM((D, D), BF16),
        pltpu.VMEM((D, D), BF16),
        pltpu.VMEM((D, D), BF16),
        pltpu.VMEM((D, D), BF16),
        pltpu.VMEM((D, D), BF16),
        pltpu.VMEM((D, D), BF16),
        pltpu.VMEM((D, D), BF16),
        pltpu.VMEM((D, D), BF16),
        pltpu.VMEM((D, L), BF16),
        pltpu.VMEM((NG, L, 128), BF16),
        pltpu.VMEM((D, L), BF16),
        pltpu.VMEM((D, L), BF16),
        pltpu.VMEM((D, L), BF16),
        pltpu.VMEM((H * 32, L), BF16),
        pltpu.VMEM((H, NTILE * 64, 128), U32),
        pltpu.VMEM((NG, 32 * GH_MAX, 128), F32),
        pltpu.VMEM((NG, 32 * GH_MAX, 128), BF16),
        pltpu.VMEM((NQB, D + 24, 128), F32),
        pltpu.VMEM((NSEG * NQB, D, 128), F32),
        pltpu.VMEM((D, S), BF16),
        pltpu.VMEM((D, FF), BF16),
        pltpu.VMEM((D, FF), BF16),
        pltpu.VMEM((D, FF), BF16),
        pltpu.VMEM((128, 128), F32),
        pltpu.VMEM((D, 128), F32),
        pltpu.VMEM((64, 128), U32),
        pltpu.VMEM((8, 128), F32),
        pltpu.VMEM((8, 128), I32),
        pltpu.VMEM((D, 128), BF16),
        pltpu.SMEM((1,), I32),
        pltpu.SemaphoreType.DMA((NSEG,)),
        pltpu.SemaphoreType.DMA((8,)),
        pltpu.SemaphoreType.DMA((NSEG,)),
    ]
    out_t = pl.pallas_call(
        _kernel,
        out_shape=jax.ShapeDtypeStruct((D, S), BF16),
        in_specs=[hbm, hbm, hbm, hbm, hbm, vmem, vmem, hbm, hbm, hbm],
        out_specs=hbm,
        scratch_shapes=scratch,
        compiler_params=pltpu.CompilerParams(vmem_limit_bytes=100 * 1024 * 1024),
        name="infini_moe",
    )(A_x.reshape(S, D).T, A_wq, A_wk, A_wv, A_wo, A_beta, B_w_r, B_w_gate, B_w_up, B_w_down.T)
    return out_t.T.reshape(1, S, D)
```

```python
import functools

import jax
import jax.numpy as jnp
import jax.experimental.pallas as pl
import jax.experimental.pallas.tpu as pltpu

F32 = jnp.float32
BF16 = jnp.bfloat16
U32 = jnp.uint32
I32 = jnp.int32

S = 2048
D = 576
H = 32
DH = 18
NSEG = 4
L = S // NSEG
FF = 4608
NQB = L // 128
TOFF = (0, 1, 3, 6)
NTILE = 10
NG = 5
WIN = 112
GROUP_HEADS = tuple(tuple(h for h in range(H)
                          if min(max(0, -(-(DH * h + DH - 128) // WIN)), NG - 1) == g)
                    for g in range(NG))
GROUP_OF = {h: g for g in range(NG) for h in GROUP_HEADS[g]}
MROWS = 144
CH = 144
NCH = D // CH
RS = 64
LN1_STEPS = NQB * 3 * (D // RS)
OUT_STEPS = NQB * (2 * (D // RS) + 1)
LN_EPS = 1e-5
LOG2E = 1.4426950408889634
QSCALE = (DH ** -0.5) * LOG2E
SAFE_LOGIT = 60.0
SAFE_V = 2.0 ** 50

NN = (((1,), (0,)), ((), ()))
NT = (((1,), (1,)), ((), ()))
TN = (((0,), (0,)), ((), ()))

for _g, _hs in enumerate(GROUP_HEADS):
    for _h in _hs:
        assert WIN * _g <= DH * _h and DH * _h + DH <= WIN * _g + 128


def _dot(a, b, dims=NN):
    return jax.lax.dot_general(a, b, dims, preferred_element_type=F32)


class _Filler:
    def __init__(self, gens, counts):
        self.gens, self.counts, self.done = gens, counts, [0] * len(gens)

    def upto(self, frac):
        for k, gen in enumerate(self.gens):
            while self.done[k] < min(frac, 1.0) * self.counts[k]:
                next(gen, None)
                self.done[k] += 1
            if frac >= 1.0:
                for _ in gen:
                    pass


def _phi(t):
    return jnp.where(t > 0, t + 1.0, jnp.exp(t))


def _sigmoid(t):
    return 1.0 / (1.0 + jnp.exp(-t))


def _max_col_norm(w):
    wf = w.astype(F32)
    ss = jnp.sum(wf * wf, axis=0, keepdims=True)
    return jnp.sqrt(jnp.max(ss, axis=1, keepdims=True))


def _kernel(xt_hbm, wq_hbm, wk_hbm, wv_hbm, wo_hbm, beta_ref, wr_ref, wg_hbm, wu_hbm, wdt_hbm,
            out_hbm,
            xbuf, wq_raw, wk_raw, wv_raw, wo_raw, wqt, wkt, wvt, wot, xn, ktn, kb, qt, pkt, pqt,
            vtn, vt32, pbuf, m_f32, m_bf, keep, amem, ot, at, hn_all, obuf, wg_v, wu_v, wdt_v,
            gcol, wrcol, stat1, stat2, r_all, stage, flag, sem_x, sem_w, sem_o):
    def x_copy(s):
        cols = pl.ds(pl.multiple_of(s * L, L), L)
        return pltpu.make_async_copy(xt_hbm.at[:, cols], xbuf.at[:, cols], sem_x.at[s])

    def out_copy(s):
        cols = pl.ds(pl.multiple_of(s * L, L), L)
        return pltpu.make_async_copy(obuf.at[:, cols], out_hbm.at[:, cols], sem_o.at[s])

    cp_wk = pltpu.make_async_copy(wk_hbm, wk_raw, sem_w.at[0])
    cp_wq = pltpu.make_async_copy(wq_hbm, wq_raw, sem_w.at[1])
    cp_wv = pltpu.make_async_copy(wv_hbm, wv_raw, sem_w.at[2])
    cp_wo = pltpu.make_async_copy(wo_hbm, wo_raw, sem_w.at[3])
    cp_wg = pltpu.make_async_copy(wg_hbm, wg_v, sem_w.at[4])
    cp_wu = pltpu.make_async_copy(wu_hbm, wu_v, sem_w.at[5])
    cp_wd = pltpu.make_async_copy(wdt_hbm, wdt_v, sem_w.at[6])

    def fold8(v):
        return jnp.sum(v.reshape(v.shape[0] // 8, 8, 128), axis=0)

    def col_total(acc):
        return jnp.sum(acc, axis=0, keepdims=True) * (1.0 / D)

    def ln1_steps(s):
        seg = jnp.minimum(s, NSEG - 1)
        for c in range(NQB):
            cols = pl.ds(pl.multiple_of(seg * L + 128 * c, 128), 128)
            xs = lambda r: xbuf[RS * r:RS * (r + 1), cols].astype(F32)
            acc = None
            for r in range(D // RS):
                part = fold8(xs(r))
                acc = part if acc is None else acc + part
                yield
            m = col_total(acc)
            stat1[c, 0:1, :] = m
            acc = None
            for r in range(D // RS):
                xc = xs(r) - m
                part = fold8(xc * xc)
                acc = part if acc is None else acc + part
                yield
            rstd = jax.lax.rsqrt(col_total(acc) + LN_EPS)
            stat1[c, 1:2, :] = rstd
            for r in range(D // RS):
                xn[RS * r:RS * (r + 1), 128 * c:128 * (c + 1)] = (
                    (xs(r) - m) * rstd).astype(BF16)
                yield

    def rows_of(c):
        return slice(CH * c, CH * (c + 1))

    def proj_k(c):
        kt = _dot(wkt[rows_of(c), :], xn[...])
        pkt[rows_of(c), :] = _phi(kt).astype(BF16)
        ktn[rows_of(c), :] = kt.astype(BF16)
        for g in range(NG):
            if (WIN * g + 127) // CH == c:
                kb[g] = ktn[WIN * g:WIN * g + 128, :].T

    def proj_q(c):
        qf = _dot(wqt[rows_of(c), :], xn[...])
        qt[rows_of(c), :] = (qf * QSCALE).astype(BF16)
        pqt[rows_of(c), :] = _phi(qf).astype(BF16)

    def proj_v(c):
        tail = jnp.concatenate([jnp.ones((1, L), F32), jnp.zeros((13, L), F32)], axis=0)
        vt = _dot(wvt[rows_of(c), :], xn[...])
        vtn[rows_of(c), :] = vt.astype(BF16)
        for j in range(CH // DH):
            h = (CH // DH) * c + j
            vt32[32 * h:32 * h + 16, :] = vt[DH * j:DH * j + 16].astype(BF16)
            vt32[32 * h + 16:32 * h + 32, :] = jnp.concatenate(
                [vt[DH * j + 16:DH * j + 18], tail], axis=0).astype(BF16)

    def masked_q(w0, i, word_mask):
        qu = pltpu.bitcast(qt[pl.ds(w0, 128), 128 * i:128 * (i + 1)], U32)
        return pltpu.bitcast(jnp.where(word_mask, qu, jnp.uint32(0)), BF16)

    def head_word_mask(lo):
        word = jax.lax.broadcasted_iota(I32, (64, 128), 0)
        return (2 * word >= lo) & (2 * word < lo + DH)

    def causal_mask():
        return (jax.lax.broadcasted_iota(I32, (128, 128), 0)
                <= jax.lax.broadcasted_iota(I32, (128, 128), 1))

    def stage_scores_fast(filler):
        causal = causal_mask()
        for h in range(H):
            g = GROUP_OF[h]
            word_mask = head_word_mask(DH * h - WIN * g)
            for i in range(NQB):
                n = 128 * (i + 1)
                filler.upto((NTILE * h + TOFF[i] + i + 1) / (NTILE * (H - 1)))
                st = _dot(kb[g, 0:n, :], masked_q(WIN * g, i, word_mask))
                p = jnp.exp2(st)
                r0 = TOFF[i] * 128
                if i > 0:
                    pbuf[h, r0:r0 + 128 * i, :] = p[:n - 128].astype(BF16)
                pbuf[h, r0 + 128 * i:r0 + n, :] = jnp.where(causal, p[n - 128:n], 0.0).astype(BF16)

    def stage_scores_safe():
        causal = causal_mask()

        def head(h, carry):
            g = jnp.clip((DH * h + DH - 128 + WIN - 1) // WIN, 0, NG - 1)
            g = jnp.where(DH * h + DH <= 128, 0, g)
            w0 = pl.multiple_of(WIN * g, 16)
            word_mask = head_word_mask(DH * h - WIN * g)
            for i in range(NQB):
                n = 128 * (i + 1)
                st = _dot(kb[g, 0:n, :], masked_q(w0, i, word_mask))
                sd = jnp.where(causal, st[n - 128:n], -jnp.inf)
                m = jnp.max(sd, axis=0, keepdims=True)
                if i > 0:
                    m = jnp.maximum(m, jnp.max(st[:n - 128], axis=0, keepdims=True))
                r0 = TOFF[i] * 128
                if i > 0:
                    pbuf[h, r0:r0 + 128 * i, :] = jnp.exp2(st[:n - 128] - m).astype(BF16)
                pbuf[h, r0 + 128 * i:r0 + n, :] = jnp.exp2(sd - m).astype(BF16)
            return carry

        jax.lax.fori_loop(0, H, head, 0)

    def pv_block(i):
        n = 128 * (i + 1)
        r0 = TOFF[i] * 128
        for h in range(H):
            o = _dot(vt32[32 * h:32 * h + 32, 0:n], pbuf[h, r0:r0 + n, :])
            a = (1.0 - gcol[h:h + 1, :]) / o[DH:DH + 1, :]
            ot[i, DH * h:DH * h + 24, :] = o[0:24] * a + amem[i, DH * h:DH * h + 24, :]

    def attn_block(s, i):
        cols = pl.ds(pl.multiple_of(s * L + 128 * i, 128), 128)
        otb = ot[i, 0:D, :].astype(BF16)
        tot = None
        for c in range(NCH):
            hh = _dot(wot[rows_of(c), :], otb) + xbuf[rows_of(c), cols].astype(F32)
            at[i, rows_of(c), :] = hh
            part = jnp.sum(hh, axis=0, keepdims=True)
            tot = part if tot is None else tot + part
        stat2[i, 0:1, :] = tot * (1.0 / D)

    def stage_pv_attn(s):
        pv_block(0)
        pv_block(1)
        attn_block(s, 0)
        pv_block(2)
        attn_block(s, 1)
        pv_block(3)
        attn_block(s, 2)
        attn_block(s, 3)

    def mem_update(g):
        lhs = jnp.concatenate([vtn[WIN * g:WIN * g + 128, :], jnp.ones((16, L), BF16)], axis=0)
        upd = _dot(lhs, pkt[WIN * g:WIN * g + 128, :], NT)
        m_new = m_f32[g] + upd * keep[g]
        m_f32[g] = m_new
        m_bf[g] = m_new.astype(BF16)

    def mem_read(g):
        for i in range(NQB):
            nm = _dot(m_bf[g], pqt[WIN * g:WIN * g + 128, 128 * i:128 * (i + 1)])
            for j, h in enumerate(GROUP_HEADS[g]):
                lo = DH * h - WIN * g
                b = gcol[h:h + 1, :] / (nm[128 + j:129 + j, :] + 1e-6)
                amem[i, DH * h:DH * h + 24, :] = nm[lo:lo + 24] * b

    def out_steps(s):
        seg = jnp.maximum(s, 0)
        for i in range(NQB):
            cols = pl.ds(pl.multiple_of(seg * L + 128 * i, 128), 128)
            m = stat2[i, 0:1, :]
            acc = None
            for r in range(D // RS):
                hc = at[i, RS * r:RS * (r + 1), :] - m
                part = fold8(hc * hc)
                acc = part if acc is None else acc + part
                yield
            rstd = jax.lax.rsqrt(col_total(acc) + LN_EPS)
            stat2[i, 1:2, :] = rstd
            acc = None
            for r in range(D // RS):
                rows = slice(RS * r, RS * (r + 1))
                hh = at[i, rows, :]
                hn = (hh - m) * rstd
                hn_all[seg * NQB + i, rows, :] = hn.astype(BF16)
                obuf[rows, cols] = (hh + hn).astype(BF16)
                part = fold8(hn * wrcol[rows, :])
                acc = part if acc is None else acc + part
                yield
            r_all[pl.ds(seg * NQB + i, 1), :] = jnp.sum(acc, axis=0, keepdims=True)
            yield

    x_copy(0).start()
    cp_wk.start()

    beta = beta_ref[...].astype(F32).reshape(1, H)
    gpad = jnp.concatenate([_sigmoid(beta), jnp.zeros((1, 128 - H), F32)], axis=1)
    gcol[...] = jnp.transpose(jnp.broadcast_to(gpad, (128, 128)))
    wr = jnp.concatenate([wr_ref[...].astype(F32).reshape(1, D), jnp.zeros((1, 64), F32)], axis=1)
    wrcol[...] = jnp.transpose(jnp.broadcast_to(wr, (128, D + 64)))[0:D]
    row = jax.lax.broadcasted_iota(I32, (MROWS, 128), 0)
    lane = jax.lax.broadcasted_iota(I32, (MROWS, 128), 1)
    for g in range(NG):
        first, nh = GROUP_HEADS[g][0], len(GROUP_HEADS[g])
        lane_head = ((lane + WIN * g) * 3641) >> 16
        row_head = jnp.where(row < 128, ((row + WIN * g) * 3641) >> 16, row - 128 + first)
        ok = (lane_head == row_head) & (row_head >= first) & (row_head < first + nh)
        keep[g] = jnp.where(ok, 1.0, 0.0)
    m_f32[...] = jnp.zeros_like(m_f32)
    amem[...] = jnp.zeros_like(amem)

    at[...] = jnp.zeros_like(at)
    stat2[...] = jnp.zeros_like(stat2)

    x_copy(0).wait()
    cp_wq.start()
    for _ in ln1_steps(0):
        pass
    cp_wk.wait()
    cp_wv.start()
    wk = wk_raw[...]
    wkt[...] = wk.T
    cp_wq.wait()
    wq = wq_raw[...]
    wqt[...] = wq.T
    proj_k(0)
    nk = _max_col_norm(wk)
    proj_k(1)
    nq = _max_col_norm(wq)
    proj_k(2)
    proj_k(3)
    cp_wv.wait()
    cp_wo.start()
    x_copy(1).start()
    wv = wv_raw[...]
    wvt[...] = wv.T
    proj_q(0)
    nv = _max_col_norm(wv)
    proj_q(1)
    proj_q(2)
    proj_q(3)
    cp_wo.wait()
    for s in range(2, NSEG):
        x_copy(s).start()
    cp_wg.start()
    cp_wu.start()
    cp_wd.start()
    wot[...] = wo_raw[...].T
    for c in range(NCH):
        proj_v(c)

    bound = (QSCALE * DH * D) * nq * nk
    safe = (bound <= SAFE_LOGIT) & (nv * (D ** 0.5) <= SAFE_V)
    flag[0] = jnp.sum(jnp.where(safe, 1, 0).astype(I32))

    def segment(s, carry):
        @pl.when(s + 1 < NSEG)
        def _():
            x_copy(s + 1).wait()

        def side_work():
            return _Filler([out_steps(s - 1), ln1_steps(s + 1)], [OUT_STEPS, LN1_STEPS])

        @pl.when(flag[0] == 1)
        def _():
            stage_scores_fast(side_work())

        @pl.when(flag[0] != 1)
        def _():
            stage_scores_safe()
            side_work().upto(1.0)

        @pl.when(s > 0)
        def _():
            out_copy(s - 1).start()

        stage_pv_attn(s)

        @pl.when(s + 1 < NSEG)
        def _():
            for g in range(NG):
                mem_update(g)
            for c in range(NCH):
                proj_q(c)
            for c in range(NCH):
                proj_k(c)
            for g in range(NG):
                mem_read(g)
            for c in range(NCH):
                proj_v(c)

        return carry

    jax.lax.fori_loop(0, NSEG, segment, 0)

    for _ in out_steps(NSEG - 1):
        pass
    out_copy(NSEG - 1).start()

    r = r_all[...]
    r_sel = jnp.max(jnp.max(r, axis=0, keepdims=True), axis=1, keepdims=True)
    ids = (128 * jax.lax.broadcasted_iota(I32, r.shape, 0)
           + jax.lax.broadcasted_iota(I32, r.shape, 1))
    cand = jnp.min(jnp.where(r == r_sel, ids, S), axis=0, keepdims=True)
    idx = jnp.sum(jnp.min(cand, axis=1, keepdims=True))
    blk = idx >> 7
    cols = pl.ds(pl.multiple_of(blk * 128, 128), 128)
    onehot = (jax.lax.broadcasted_iota(I32, (16, 128), 1) == idx - blk * 128).astype(BF16)
    xs = _dot(onehot, hn_all[blk], NT).astype(BF16)
    cp_wg.wait()
    cp_wu.wait()
    cp_wd.wait()
    ga = _dot(xs, wg_v[...])
    up = _dot(xs, wu_v[...])
    act = (ga * _sigmoid(ga) * up).astype(BF16)
    y = _dot(act, wdt_v[...], NT) * _sigmoid(r_sel)
    y_hi = y.astype(BF16)
    y_lo = (y - y_hi.astype(F32)).astype(BF16)
    row16 = jax.lax.broadcasted_iota(I32, (16, D), 0)
    y2 = jnp.where(row16 == 0, y_hi, jnp.where(row16 == 1, y_lo, jnp.zeros_like(y_hi)))
    upd = _dot(y2, onehot, TN)
    stage[...] = (obuf[:, cols].astype(F32) + upd).astype(BF16)
    for s in range(NSEG):
        out_copy(s).wait()
    fix = pltpu.make_async_copy(stage, out_hbm.at[:, cols], sem_w.at[7])
    fix.start()
    fix.wait()


@jax.jit
def pallas_sequential_preLN__memory_aug_infini_attn__moe_arch_mod__prompt_kernel(
    A_x: jax.Array,
    A_wq: jax.Array,
    A_wk: jax.Array,
    A_wv: jax.Array,
    A_wo: jax.Array,
    A_beta: jax.Array,
    B_x: jax.Array,
    B_w_r: jax.Array,
    B_w_gate: jax.Array,
    B_w_up: jax.Array,
    B_w_down: jax.Array,
):
    del B_x
    hbm = pl.BlockSpec(memory_space=pltpu.HBM)
    vmem = pl.BlockSpec(memory_space=pltpu.VMEM)
    scratch = [
        pltpu.VMEM((D, S), BF16),
        pltpu.VMEM((D, D), BF16),
        pltpu.VMEM((D, D), BF16),
        pltpu.VMEM((D, D), BF16),
        pltpu.VMEM((D, D), BF16),
        pltpu.VMEM((D, D), BF16),
        pltpu.VMEM((D, D), BF16),
        pltpu.VMEM((D, D), BF16),
        pltpu.VMEM((D, D), BF16),
        pltpu.VMEM((D, L), BF16),
        pltpu.VMEM((D, L), BF16),
        pltpu.VMEM((NG, L, 128), BF16),
        pltpu.VMEM((D, L), BF16),
        pltpu.VMEM((D, L), BF16),
        pltpu.VMEM((D, L), BF16),
        pltpu.VMEM((D, L), BF16),
        pltpu.VMEM((H * 32, L), BF16),
        pltpu.VMEM((H, NTILE * 128, 128), BF16),
        pltpu.VMEM((NG, MROWS, 128), F32),
        pltpu.VMEM((NG, MROWS, 128), BF16),
        pltpu.VMEM((NG, MROWS, 128), F32),
        pltpu.VMEM((NQB, D + 24, 128), F32),
        pltpu.VMEM((NQB, D + 24, 128), F32),
        pltpu.VMEM((NQB, D, 128), F32),
        pltpu.VMEM((NSEG * NQB, D, 128), BF16),
        pltpu.VMEM((D, S), BF16),
        pltpu.VMEM((D, FF), BF16),
        pltpu.VMEM((D, FF), BF16),
        pltpu.VMEM((D, FF), BF16),
        pltpu.VMEM((128, 128), F32),
        pltpu.VMEM((D, 128), F32),
        pltpu.VMEM((NQB, 8, 128), F32),
        pltpu.VMEM((NQB, 8, 128), F32),
        pltpu.VMEM((NSEG * NQB, 128), F32),
        pltpu.VMEM((D, 128), BF16),
        pltpu.SMEM((1,), I32),
        pltpu.SemaphoreType.DMA((NSEG,)),
        pltpu.SemaphoreType.DMA((8,)),
        pltpu.SemaphoreType.DMA((NSEG,)),
    ]
    out_t = pl.pallas_call(
        _kernel,
        out_shape=jax.ShapeDtypeStruct((D, S), BF16),
        in_specs=[hbm, hbm, hbm, hbm, hbm, vmem, vmem, hbm, hbm, hbm],
        out_specs=hbm,
        scratch_shapes=scratch,
        compiler_params=pltpu.CompilerParams(vmem_limit_bytes=100 * 1024 * 1024),
        name="infini_moe",
    )(A_x.reshape(S, D).T, A_wq, A_wk, A_wv, A_wo, A_beta, B_w_r, B_w_gate, B_w_up, B_w_down.T)
    return out_t.T.reshape(1, S, D)
```

```python
import functools

import jax
import jax.numpy as jnp
import jax.experimental.pallas as pl
import jax.experimental.pallas.tpu as pltpu

F32 = jnp.float32
BF16 = jnp.bfloat16
U32 = jnp.uint32
I32 = jnp.int32

S = 2048
D = 576
H = 32
DH = 18
NSEG = 4
L = S // NSEG
FF = 4608
NQB = L // 128
TOFF = (0, 1, 3, 6)
NTILE = 10
NG = 5
WIN = 112
GROUP_HEADS = tuple(tuple(h for h in range(H)
                          if min(max(0, -(-(DH * h + DH - 128) // WIN)), NG - 1) == g)
                    for g in range(NG))
GROUP_OF = {h: g for g in range(NG) for h in GROUP_HEADS[g]}
MROWS = 144
CH = 144
NCH = D // CH
RS = 64
LN1_STEPS = NQB * 3 * (D // RS)
OUT_STEPS = NQB * (2 * (D // RS) + 1)
LN_EPS = 1e-5
LOG2E = 1.4426950408889634
QSCALE = (DH ** -0.5) * LOG2E
SAFE_LOGIT = 60.0
SAFE_V = 2.0 ** 50

NN = (((1,), (0,)), ((), ()))
NT = (((1,), (1,)), ((), ()))
TN = (((0,), (0,)), ((), ()))

for _g, _hs in enumerate(GROUP_HEADS):
    for _h in _hs:
        assert WIN * _g <= DH * _h and DH * _h + DH <= WIN * _g + 128


def _dot(a, b, dims=NN):
    return jax.lax.dot_general(a, b, dims, preferred_element_type=F32)


class _Filler:
    def __init__(self, gens, counts):
        self.gens, self.counts, self.done = gens, counts, [0] * len(gens)

    def upto(self, frac):
        for k, gen in enumerate(self.gens):
            while self.done[k] < min(frac, 1.0) * self.counts[k]:
                next(gen, None)
                self.done[k] += 1
            if frac >= 1.0:
                for _ in gen:
                    pass


def _phi(t):
    return jnp.where(t > 0, t + 1.0, jnp.exp(t))


def _sigmoid(t):
    return 1.0 / (1.0 + jnp.exp(-t))


def _recip(x):
    r = pl.reciprocal(x, approx=True)
    return r * (2.0 - x * r)


def _kernel(xt_hbm, wq_hbm, wk_hbm, wv_hbm, wo_hbm, beta_ref, wr_ref, wg_hbm, wu_hbm, wdt_hbm,
            out_hbm,
            xbuf, wq_raw, wk_raw, wv_raw, wo_raw, wqt, wkt, wvt, wot, xn, ktn, kb, qt, pkt, pqt,
            vtn, vt32, pbuf, m_f32, m_bf, keep, amem, ot, at, hn_all, obuf, wg_v, wu_v, wdt_v,
            gcol, wrcol, stat1, stat2, wnorm, r_all, stage, flag, sem_x, sem_w, sem_o):
    def x_copy(s):
        cols = pl.ds(pl.multiple_of(s * L, L), L)
        return pltpu.make_async_copy(xt_hbm.at[:, cols], xbuf.at[:, cols], sem_x.at[s])

    def out_copy(s):
        cols = pl.ds(pl.multiple_of(s * L, L), L)
        return pltpu.make_async_copy(obuf.at[:, cols], out_hbm.at[:, cols], sem_o.at[s])

    cp_wk = pltpu.make_async_copy(wk_hbm, wk_raw, sem_w.at[0])
    cp_wq = pltpu.make_async_copy(wq_hbm, wq_raw, sem_w.at[1])
    cp_wv = pltpu.make_async_copy(wv_hbm, wv_raw, sem_w.at[2])
    cp_wo = pltpu.make_async_copy(wo_hbm, wo_raw, sem_w.at[3])
    cp_wg = pltpu.make_async_copy(wg_hbm, wg_v, sem_w.at[4])
    cp_wu = pltpu.make_async_copy(wu_hbm, wu_v, sem_w.at[5])
    cp_wd = pltpu.make_async_copy(wdt_hbm, wdt_v, sem_w.at[6])

    def fold8(v):
        return jnp.sum(v.reshape(v.shape[0] // 8, 8, 128), axis=0)

    def col_total(acc):
        return jnp.sum(acc, axis=0, keepdims=True) * (1.0 / D)

    def ln1_steps(s):
        seg = jnp.minimum(s, NSEG - 1)
        for c in range(NQB):
            cols = pl.ds(pl.multiple_of(seg * L + 128 * c, 128), 128)
            xs = lambda r: xbuf[RS * r:RS * (r + 1), cols].astype(F32)
            acc = None
            for r in range(D // RS):
                part = fold8(xs(r))
                acc = part if acc is None else acc + part
                yield
            m = col_total(acc)
            stat1[c, 0:1, :] = m
            acc = None
            for r in range(D // RS):
                xc = xs(r) - m
                part = fold8(xc * xc)
                acc = part if acc is None else acc + part
                yield
            rstd = jax.lax.rsqrt(col_total(acc) + LN_EPS)
            stat1[c, 1:2, :] = rstd
            for r in range(D // RS):
                xn[RS * r:RS * (r + 1), 128 * c:128 * (c + 1)] = (
                    (xs(r) - m) * rstd).astype(BF16)
                yield

    def rows_of(c):
        return slice(CH * c, CH * (c + 1))

    def proj_k(c):
        kt = _dot(wkt[rows_of(c), :], xn[...])
        pkt[rows_of(c), :] = _phi(kt).astype(BF16)
        ktn[rows_of(c), :] = kt.astype(BF16)
        for g in range(NG):
            if (WIN * g + 127) // CH == c:
                kb[g] = ktn[WIN * g:WIN * g + 128, :].T

    def proj_q(c):
        qf = _dot(wqt[rows_of(c), :], xn[...])
        qt[rows_of(c), :] = (qf * QSCALE).astype(BF16)
        pqt[rows_of(c), :] = _phi(qf).astype(BF16)

    def proj_v(c):
        tail = jnp.concatenate([jnp.ones((1, L), F32), jnp.zeros((13, L), F32)], axis=0)
        vt = _dot(wvt[rows_of(c), :], xn[...])
        vtn[rows_of(c), :] = vt.astype(BF16)
        for j in range(CH // DH):
            h = (CH // DH) * c + j
            vt32[32 * h:32 * h + 16, :] = vt[DH * j:DH * j + 16].astype(BF16)
            vt32[32 * h + 16:32 * h + 32, :] = jnp.concatenate(
                [vt[DH * j + 16:DH * j + 18], tail], axis=0).astype(BF16)

    def masked_q(w0, i, word_mask):
        qu = pltpu.bitcast(qt[pl.ds(w0, 128), 128 * i:128 * (i + 1)], U32)
        return pltpu.bitcast(jnp.where(word_mask, qu, jnp.uint32(0)), BF16)

    def head_word_mask(lo):
        word = jax.lax.broadcasted_iota(I32, (64, 128), 0)
        return (2 * word >= lo) & (2 * word < lo + DH)

    def causal_mask():
        return (jax.lax.broadcasted_iota(I32, (128, 128), 0)
                <= jax.lax.broadcasted_iota(I32, (128, 128), 1))

    def stage_scores_fast(filler):
        causal = causal_mask()
        for h in range(H):
            g = GROUP_OF[h]
            word_mask = head_word_mask(DH * h - WIN * g)
            for i in range(NQB):
                n = 128 * (i + 1)
                filler.upto((NTILE * h + TOFF[i] + i + 1) / (NTILE * (H - 1)))
                st = _dot(kb[g, 0:n, :], masked_q(WIN * g, i, word_mask))
                p = jnp.exp2(st)
                r0 = TOFF[i] * 128
                if i > 0:
                    pbuf[h, r0:r0 + 128 * i, :] = p[:n - 128].astype(BF16)
                pbuf[h, r0 + 128 * i:r0 + n, :] = jnp.where(causal, p[n - 128:n], 0.0).astype(BF16)

    def stage_scores_safe():
        causal = causal_mask()

        def head(h, carry):
            g = jnp.clip((DH * h + DH - 128 + WIN - 1) // WIN, 0, NG - 1)
            g = jnp.where(DH * h + DH <= 128, 0, g)
            w0 = pl.multiple_of(WIN * g, 16)
            word_mask = head_word_mask(DH * h - WIN * g)
            for i in range(NQB):
                n = 128 * (i + 1)
                st = _dot(kb[g, 0:n, :], masked_q(w0, i, word_mask))
                sd = jnp.where(causal, st[n - 128:n], -jnp.inf)
                m = jnp.max(sd, axis=0, keepdims=True)
                if i > 0:
                    m = jnp.maximum(m, jnp.max(st[:n - 128], axis=0, keepdims=True))
                r0 = TOFF[i] * 128
                if i > 0:
                    pbuf[h, r0:r0 + 128 * i, :] = jnp.exp2(st[:n - 128] - m).astype(BF16)
                pbuf[h, r0 + 128 * i:r0 + n, :] = jnp.exp2(sd - m).astype(BF16)
            return carry

        jax.lax.fori_loop(0, H, head, 0)

    def pv_block(i):
        n = 128 * (i + 1)
        r0 = TOFF[i] * 128
        for h in range(H):
            o = _dot(vt32[32 * h:32 * h + 32, 0:n], pbuf[h, r0:r0 + n, :])
            a = (1.0 - gcol[h:h + 1, :]) * _recip(o[DH:DH + 1, :])
            ot[i, DH * h:DH * h + 24, :] = o[0:24] * a + amem[i, DH * h:DH * h + 24, :]

    def attn_block(s, i):
        cols = pl.ds(pl.multiple_of(s * L + 128 * i, 128), 128)
        otb = ot[i, 0:D, :].astype(BF16)
        tot = None
        for c in range(NCH):
            hh = _dot(wot[rows_of(c), :], otb) + xbuf[rows_of(c), cols].astype(F32)
            at[i, rows_of(c), :] = hh
            part = jnp.sum(hh, axis=0, keepdims=True)
            tot = part if tot is None else tot + part
        stat2[i, 0:1, :] = tot * (1.0 / D)

    def stage_pv_attn(s):
        pv_block(0)
        pv_block(1)
        attn_block(s, 0)
        pv_block(2)
        attn_block(s, 1)
        pv_block(3)
        attn_block(s, 2)
        attn_block(s, 3)

    def mem_update(g):
        lhs = jnp.concatenate([vtn[WIN * g:WIN * g + 128, :], jnp.ones((16, L), BF16)], axis=0)
        upd = _dot(lhs, pkt[WIN * g:WIN * g + 128, :], NT)
        m_new = m_f32[g] + upd * keep[g]
        m_f32[g] = m_new
        m_bf[g] = m_new.astype(BF16)

    def mem_read(g):
        for i in range(NQB):
            nm = _dot(m_bf[g], pqt[WIN * g:WIN * g + 128, 128 * i:128 * (i + 1)])
            first = GROUP_HEADS[g][0]
            b = gcol[first:first + 8, :] / (nm[128:136, :] + 1e-6)
            for j, h in enumerate(GROUP_HEADS[g]):
                lo = DH * h - WIN * g
                amem[i, DH * h:DH * h + 24, :] = nm[lo:lo + 24] * b[j:j + 1, :]

    def out_steps(s):
        seg = jnp.maximum(s, 0)
        for i in range(NQB):
            cols = pl.ds(pl.multiple_of(seg * L + 128 * i, 128), 128)
            m = stat2[i, 0:1, :]
            acc = None
            for r in range(D // RS):
                hc = at[i, RS * r:RS * (r + 1), :] - m
                part = fold8(hc * hc)
                acc = part if acc is None else acc + part
                yield
            rstd = jax.lax.rsqrt(col_total(acc) + LN_EPS)
            stat2[i, 1:2, :] = rstd
            acc = None
            for r in range(D // RS):
                rows = slice(RS * r, RS * (r + 1))
                hh = at[i, rows, :]
                hn = (hh - m) * rstd
                hn_all[seg * NQB + i, rows, :] = hn.astype(BF16)
                obuf[rows, cols] = (hh + hn).astype(BF16)
                part = fold8(hn * wrcol[rows, :])
                acc = part if acc is None else acc + part
                yield
            r_all[pl.ds(seg * NQB + i, 1), :] = jnp.sum(acc, axis=0, keepdims=True)
            yield

    x_copy(0).start()
    cp_wk.start()

    beta = beta_ref[...].astype(F32).reshape(1, H)
    gpad = jnp.concatenate([_sigmoid(beta), jnp.zeros((1, 128 - H), F32)], axis=1)
    gcol[...] = jnp.transpose(jnp.broadcast_to(gpad, (128, 128)))
    wr = jnp.concatenate([wr_ref[...].astype(F32).reshape(1, D), jnp.zeros((1, 64), F32)], axis=1)
    wrcol[...] = jnp.transpose(jnp.broadcast_to(wr, (128, D + 64)))[0:D]
    row = jax.lax.broadcasted_iota(I32, (MROWS, 128), 0)
    lane = jax.lax.broadcasted_iota(I32, (MROWS, 128), 1)
    for g in range(NG):
        first, nh = GROUP_HEADS[g][0], len(GROUP_HEADS[g])
        lane_head = ((lane + WIN * g) * 3641) >> 16
        row_head = jnp.where(row < 128, ((row + WIN * g) * 3641) >> 16, row - 128 + first)
        ok = (lane_head == row_head) & (row_head >= first) & (row_head < first + nh)
        keep[g] = jnp.where(ok, 1.0, 0.0)
    m_f32[...] = jnp.zeros_like(m_f32)
    amem[...] = jnp.zeros_like(amem)

    at[...] = jnp.zeros_like(at)
    stat2[...] = jnp.zeros_like(stat2)

    def transpose_tile(dst, raw, t):
        hi = min(128 * (t + 1), D)
        dst[128 * t:hi, :] = raw[:, 128 * t:hi].T

    def col_norm_steps(raw, slot):
        for t in range(5):
            hi = min(128 * (t + 1), D)
            for k in range(3):
                w = raw[192 * k:192 * (k + 1), 128 * t:hi].astype(F32)
                wnorm[slot, 8 * k:8 * (k + 1), 128 * t:hi] = jnp.sum(
                    (w * w).reshape(24, 8, hi - 128 * t), axis=0)
                yield

    x_copy(0).wait()
    cp_wq.start()
    for _ in ln1_steps(0):
        pass
    cp_wk.wait()
    cp_wv.start()
    side = _Filler([col_norm_steps(wk_raw, 0)], [15])
    transpose_tile(wkt, wk_raw, 0)
    transpose_tile(wkt, wk_raw, 1)
    proj_k(0)
    transpose_tile(wkt, wk_raw, 2)
    side.upto(0.5)
    proj_k(1)
    transpose_tile(wkt, wk_raw, 3)
    side.upto(1.0)
    proj_k(2)
    transpose_tile(wkt, wk_raw, 4)
    cp_wq.wait()
    cp_wv.wait()
    cp_wo.start()
    x_copy(1).start()
    transpose_tile(wqt, wq_raw, 0)
    transpose_tile(wqt, wq_raw, 1)
    proj_k(3)
    side = _Filler([col_norm_steps(wq_raw, 1), col_norm_steps(wv_raw, 2)], [15, 15])
    for c in range(NCH):
        proj_q(c)
        if c + 2 < 5:
            transpose_tile(wqt, wq_raw, c + 2)
        if c >= 2:
            transpose_tile(wvt, wv_raw, c - 2)
        if c < NCH - 1:
            side.upto((c + 1) / (NCH - 1))
    cp_wo.wait()
    for s in range(2, NSEG):
        x_copy(s).start()
    cp_wg.start()
    cp_wu.start()
    cp_wd.start()
    for c in range(NCH):
        proj_v(c)
        if c + 2 < 5:
            transpose_tile(wvt, wv_raw, c + 2)
        transpose_tile(wot, wo_raw, c)
    transpose_tile(wot, wo_raw, 4)

    x_copy(1).wait()

    def max_norm(slot):
        ss = jnp.sum(wnorm[slot], axis=0, keepdims=True)
        return jnp.sqrt(jnp.max(ss, axis=1, keepdims=True))

    nk, nq, nv = max_norm(0), max_norm(1), max_norm(2)

    bound = (QSCALE * DH * D) * nq * nk
    safe = (bound <= SAFE_LOGIT) & (nv * (D ** 0.5) <= SAFE_V)
    flag[0] = jnp.sum(jnp.where(safe, 1, 0).astype(I32))

    def segment(s, carry):
        @pl.when(jnp.logical_and(s > 0, s + 1 < NSEG))
        def _():
            x_copy(s + 1).wait()

        def side_work():
            return _Filler([out_steps(s - 1), ln1_steps(s + 1)], [OUT_STEPS, LN1_STEPS])

        @pl.when(flag[0] == 1)
        def _():
            stage_scores_fast(side_work())

        @pl.when(flag[0] != 1)
        def _():
            stage_scores_safe()
            side_work().upto(1.0)

        @pl.when(s > 0)
        def _():
            out_copy(s - 1).start()

        stage_pv_attn(s)

        @pl.when(s + 1 < NSEG)
        def _():
            for g in range(NG):
                mem_update(g)
            for c in range(NCH):
                proj_q(c)
            for c in range(NCH):
                proj_k(c)
            for g in range(NG):
                mem_read(g)
            for c in range(NCH):
                proj_v(c)

        return carry

    jax.lax.fori_loop(0, NSEG, segment, 0)

    for _ in out_steps(NSEG - 1):
        pass
    out_copy(NSEG - 1).start()

    r = r_all[...]
    r_sel = jnp.max(jnp.max(r, axis=0, keepdims=True), axis=1, keepdims=True)
    ids = (128 * jax.lax.broadcasted_iota(I32, r.shape, 0)
           + jax.lax.broadcasted_iota(I32, r.shape, 1))
    cand = jnp.min(jnp.where(r == r_sel, ids, S), axis=0, keepdims=True)
    idx = jnp.sum(jnp.min(cand, axis=1, keepdims=True))
    blk = idx >> 7
    cols = pl.ds(pl.multiple_of(blk * 128, 128), 128)
    onehot = (jax.lax.broadcasted_iota(I32, (16, 128), 1) == idx - blk * 128).astype(BF16)
    xs = _dot(onehot, hn_all[blk], NT).astype(BF16)
    cp_wg.wait()
    cp_wu.wait()
    cp_wd.wait()
    ga = _dot(xs, wg_v[...])
    up = _dot(xs, wu_v[...])
    act = (ga * _sigmoid(ga) * up).astype(BF16)
    y = _dot(act, wdt_v[...], NT) * _sigmoid(r_sel)
    y_hi = y.astype(BF16)
    y_lo = (y - y_hi.astype(F32)).astype(BF16)
    row16 = jax.lax.broadcasted_iota(I32, (16, D), 0)
    y2 = jnp.where(row16 == 0, y_hi, jnp.where(row16 == 1, y_lo, jnp.zeros_like(y_hi)))
    upd = _dot(y2, onehot, TN)
    stage[...] = (obuf[:, cols].astype(F32) + upd).astype(BF16)
    for s in range(NSEG):
        out_copy(s).wait()
    fix = pltpu.make_async_copy(stage, out_hbm.at[:, cols], sem_w.at[7])
    fix.start()
    fix.wait()


@jax.jit
def pallas_sequential_preLN__memory_aug_infini_attn__moe_arch_mod__prompt_kernel(
    A_x: jax.Array,
    A_wq: jax.Array,
    A_wk: jax.Array,
    A_wv: jax.Array,
    A_wo: jax.Array,
    A_beta: jax.Array,
    B_x: jax.Array,
    B_w_r: jax.Array,
    B_w_gate: jax.Array,
    B_w_up: jax.Array,
    B_w_down: jax.Array,
):
    del B_x
    hbm = pl.BlockSpec(memory_space=pltpu.HBM)
    vmem = pl.BlockSpec(memory_space=pltpu.VMEM)
    scratch = [
        pltpu.VMEM((D, S), BF16),
        pltpu.VMEM((D, D), BF16),
        pltpu.VMEM((D, D), BF16),
        pltpu.VMEM((D, D), BF16),
        pltpu.VMEM((D, D), BF16),
        pltpu.VMEM((D, D), BF16),
        pltpu.VMEM((D, D), BF16),
        pltpu.VMEM((D, D), BF16),
        pltpu.VMEM((D, D), BF16),
        pltpu.VMEM((D, L), BF16),
        pltpu.VMEM((D, L), BF16),
        pltpu.VMEM((NG, L, 128), BF16),
        pltpu.VMEM((D, L), BF16),
        pltpu.VMEM((D, L), BF16),
        pltpu.VMEM((D, L), BF16),
        pltpu.VMEM((D, L), BF16),
        pltpu.VMEM((H * 32, L), BF16),
        pltpu.VMEM((H, NTILE * 128, 128), BF16),
        pltpu.VMEM((NG, MROWS, 128), F32),
        pltpu.VMEM((NG, MROWS, 128), BF16),
        pltpu.VMEM((NG, MROWS, 128), F32),
        pltpu.VMEM((NQB, D + 24, 128), F32),
        pltpu.VMEM((NQB, D + 24, 128), F32),
        pltpu.VMEM((NQB, D, 128), F32),
        pltpu.VMEM((NSEG * NQB, D, 128), BF16),
        pltpu.VMEM((D, S), BF16),
        pltpu.VMEM((D, FF), BF16),
        pltpu.VMEM((D, FF), BF16),
        pltpu.VMEM((D, FF), BF16),
        pltpu.VMEM((128, 128), F32),
        pltpu.VMEM((D, 128), F32),
        pltpu.VMEM((NQB, 8, 128), F32),
        pltpu.VMEM((NQB, 8, 128), F32),
        pltpu.VMEM((3, 24, D), F32),
        pltpu.VMEM((NSEG * NQB, 128), F32),
        pltpu.VMEM((D, 128), BF16),
        pltpu.SMEM((1,), I32),
        pltpu.SemaphoreType.DMA((NSEG,)),
        pltpu.SemaphoreType.DMA((8,)),
        pltpu.SemaphoreType.DMA((NSEG,)),
    ]
    out_t = pl.pallas_call(
        _kernel,
        out_shape=jax.ShapeDtypeStruct((D, S), BF16),
        in_specs=[hbm, hbm, hbm, hbm, hbm, vmem, vmem, hbm, hbm, hbm],
        out_specs=hbm,
        scratch_shapes=scratch,
        compiler_params=pltpu.CompilerParams(vmem_limit_bytes=100 * 1024 * 1024),
        name="infini_moe",
    )(A_x.reshape(S, D).T, A_wq, A_wk, A_wv, A_wo, A_beta, B_w_r, B_w_gate, B_w_up, B_w_down.T)
    return out_t.T.reshape(1, S, D)
```

```python
import functools

import jax
import jax.numpy as jnp
import jax.experimental.pallas as pl
import jax.experimental.pallas.tpu as pltpu

F32 = jnp.float32
BF16 = jnp.bfloat16
U32 = jnp.uint32
I32 = jnp.int32

S = 2048
D = 576
H = 32
DH = 18
NSEG = 4
L = S // NSEG
FF = 4608
NQB = L // 128
TOFF = (0, 1, 3, 6)
NTILE = 10
NG = 5
WIN = 112
GROUP_HEADS = tuple(tuple(h for h in range(H)
                          if min(max(0, -(-(DH * h + DH - 128) // WIN)), NG - 1) == g)
                    for g in range(NG))
GROUP_OF = {h: g for g in range(NG) for h in GROUP_HEADS[g]}
MROWS = 144
CH = 144
NCH = D // CH
RS = 64
PASS_STEPS = NQB * (D // RS)
FC = 512
LN_EPS = 1e-5
LOG2E = 1.4426950408889634
QSCALE = (DH ** -0.5) * LOG2E
SAFE_LOGIT = 60.0
SAFE_V = 2.0 ** 50

NN = (((1,), (0,)), ((), ()))
NT = (((1,), (1,)), ((), ()))
TN = (((0,), (0,)), ((), ()))

for _g, _hs in enumerate(GROUP_HEADS):
    for _h in _hs:
        assert WIN * _g <= DH * _h and DH * _h + DH <= WIN * _g + 128


def _dot(a, b, dims=NN):
    return jax.lax.dot_general(a, b, dims, preferred_element_type=F32)


class _Filler:
    def __init__(self, gens, counts):
        self.gens, self.counts, self.done = gens, counts, [0] * len(gens)

    def upto(self, frac):
        for k, gen in enumerate(self.gens):
            while self.done[k] < min(frac, 1.0) * self.counts[k]:
                next(gen, None)
                self.done[k] += 1
            if frac >= 1.0:
                for _ in gen:
                    pass


def _chain(*gens):
    for gen in gens:
        yield from gen


def _phi(t):
    return jnp.where(t > 0, t + 1.0, jnp.exp(t))


def _sigmoid(t):
    return 1.0 / (1.0 + jnp.exp(-t))


def _recip(x):
    r = pl.reciprocal(x, approx=True)
    return r * (2.0 - x * r)


def _kernel(xt_hbm, wq_hbm, wk_hbm, wv_hbm, wo_hbm, beta_ref, wr_ref, wg_hbm, wu_hbm, wdt_hbm,
            out_hbm,
            xbuf, wq_raw, wk_raw, wv_raw, wo_raw, wqt, wkt, wvt, wot, xn, ktn, kb, qt, pkt, pqt,
            vtn, vt32, pbuf, m_f32, m_bf, keep, amem, ot, h_all, hn_sel, yacc, obuf, wg_v, wu_v, wdt_v,
            gcol, wrcol, stat1, stat2, wnorm, r_all, stage, flag, sem_x, sem_w, sem_o):
    def x_copy(s):
        cols = pl.ds(pl.multiple_of(s * L, L), L)
        return pltpu.make_async_copy(xt_hbm.at[:, cols], xbuf.at[:, cols], sem_x.at[s])

    def out_copy(s):
        cols = pl.ds(pl.multiple_of(s * L, L), L)
        return pltpu.make_async_copy(obuf.at[:, cols], out_hbm.at[:, cols], sem_o.at[s])

    cp_wk = pltpu.make_async_copy(wk_hbm, wk_raw, sem_w.at[0])
    cp_wq = pltpu.make_async_copy(wq_hbm, wq_raw, sem_w.at[1])
    cp_wv = pltpu.make_async_copy(wv_hbm, wv_raw, sem_w.at[2])
    cp_wo = pltpu.make_async_copy(wo_hbm, wo_raw, sem_w.at[3])
    cp_wg = pltpu.make_async_copy(wg_hbm, wg_v, sem_w.at[4])
    cp_wu = pltpu.make_async_copy(wu_hbm, wu_v, sem_w.at[5])
    cp_wd = pltpu.make_async_copy(wdt_hbm, wdt_v, sem_w.at[6])

    def fold8(v):
        return jnp.sum(v.reshape(v.shape[0] // 8, 8, 128), axis=0)

    def col_total(acc):
        return jnp.sum(acc, axis=0, keepdims=True) * (1.0 / D)

    def ln1_steps(s):
        seg = jnp.minimum(s, NSEG - 1)
        for c in range(NQB):
            cols = pl.ds(pl.multiple_of(seg * L + 128 * c, 128), 128)
            xs = lambda r: xbuf[RS * r:RS * (r + 1), cols].astype(F32)
            acc = None
            for r in range(D // RS):
                part = fold8(xs(r))
                acc = part if acc is None else acc + part
                yield
            m = col_total(acc)
            stat1[c, 0:1, :] = m
            acc = None
            for r in range(D // RS):
                xc = xs(r) - m
                part = fold8(xc * xc)
                acc = part if acc is None else acc + part
                yield
            rstd = jax.lax.rsqrt(col_total(acc) + LN_EPS)
            stat1[c, 1:2, :] = rstd
            for r in range(D // RS):
                xn[RS * r:RS * (r + 1), 128 * c:128 * (c + 1)] = (
                    (xs(r) - m) * rstd).astype(BF16)
                yield

    def rows_of(c):
        return slice(CH * c, CH * (c + 1))

    def proj_k(c):
        kt = _dot(wkt[rows_of(c), :], xn[...])
        pkt[rows_of(c), :] = _phi(kt).astype(BF16)
        ktn[rows_of(c), :] = kt.astype(BF16)
        for g in range(NG):
            if (WIN * g + 127) // CH == c:
                kb[g] = ktn[WIN * g:WIN * g + 128, :].T

    def proj_q(c):
        qf = _dot(wqt[rows_of(c), :], xn[...])
        qt[rows_of(c), :] = (qf * QSCALE).astype(BF16)
        pqt[rows_of(c), :] = _phi(qf).astype(BF16)

    def proj_v(c):
        tail = jnp.concatenate([jnp.ones((1, L), F32), jnp.zeros((13, L), F32)], axis=0)
        vt = _dot(wvt[rows_of(c), :], xn[...])
        vtn[rows_of(c), :] = vt.astype(BF16)
        for j in range(CH // DH):
            h = (CH // DH) * c + j
            vt32[32 * h:32 * h + 16, :] = vt[DH * j:DH * j + 16].astype(BF16)
            vt32[32 * h + 16:32 * h + 32, :] = jnp.concatenate(
                [vt[DH * j + 16:DH * j + 18], tail], axis=0).astype(BF16)

    def masked_q(w0, i, word_mask):
        qu = pltpu.bitcast(qt[pl.ds(w0, 128), 128 * i:128 * (i + 1)], U32)
        return pltpu.bitcast(jnp.where(word_mask, qu, jnp.uint32(0)), BF16)

    def head_word_mask(lo):
        word = jax.lax.broadcasted_iota(I32, (64, 128), 0)
        return (2 * word >= lo) & (2 * word < lo + DH)

    def causal_mask():
        return (jax.lax.broadcasted_iota(I32, (128, 128), 0)
                <= jax.lax.broadcasted_iota(I32, (128, 128), 1))

    def stage_scores_fast(filler):
        causal = causal_mask()
        for h in range(H):
            g = GROUP_OF[h]
            word_mask = head_word_mask(DH * h - WIN * g)
            for i in range(NQB):
                n = 128 * (i + 1)
                filler.upto((NTILE * h + TOFF[i] + i + 1) / (NTILE * (H - 1)))
                st = _dot(kb[g, 0:n, :], masked_q(WIN * g, i, word_mask))
                p = jnp.exp2(st)
                r0 = TOFF[i] * 128
                if i > 0:
                    pbuf[h, r0:r0 + 128 * i, :] = p[:n - 128].astype(BF16)
                pbuf[h, r0 + 128 * i:r0 + n, :] = jnp.where(causal, p[n - 128:n], 0.0).astype(BF16)

    def stage_scores_safe():
        causal = causal_mask()

        def head(h, carry):
            g = jnp.clip((DH * h + DH - 128 + WIN - 1) // WIN, 0, NG - 1)
            g = jnp.where(DH * h + DH <= 128, 0, g)
            w0 = pl.multiple_of(WIN * g, 16)
            word_mask = head_word_mask(DH * h - WIN * g)
            for i in range(NQB):
                n = 128 * (i + 1)
                st = _dot(kb[g, 0:n, :], masked_q(w0, i, word_mask))
                sd = jnp.where(causal, st[n - 128:n], -jnp.inf)
                m = jnp.max(sd, axis=0, keepdims=True)
                if i > 0:
                    m = jnp.maximum(m, jnp.max(st[:n - 128], axis=0, keepdims=True))
                r0 = TOFF[i] * 128
                if i > 0:
                    pbuf[h, r0:r0 + 128 * i, :] = jnp.exp2(st[:n - 128] - m).astype(BF16)
                pbuf[h, r0 + 128 * i:r0 + n, :] = jnp.exp2(sd - m).astype(BF16)
            return carry

        jax.lax.fori_loop(0, H, head, 0)

    def pv_block(i):
        n = 128 * (i + 1)
        r0 = TOFF[i] * 128
        for h in range(H):
            o = _dot(vt32[32 * h:32 * h + 32, 0:n], pbuf[h, r0:r0 + n, :])
            a = (1.0 - gcol[h:h + 1, :]) * _recip(o[DH:DH + 1, :])
            ot[i, DH * h:DH * h + 24, :] = o[0:24] * a + amem[i, DH * h:DH * h + 24, :]

    def attn_block(s, i):
        cols = pl.ds(pl.multiple_of(s * L + 128 * i, 128), 128)
        blk = s * NQB + i
        otb = ot[i, 0:D, :].astype(BF16)
        tot = None
        for c in range(NCH):
            hh = _dot(wot[rows_of(c), :], otb) + xbuf[rows_of(c), cols].astype(F32)
            h_all[blk, rows_of(c), :] = hh
            part = jnp.sum(hh, axis=0, keepdims=True)
            tot = part if tot is None else tot + part
        stat2[blk, 0:1, :] = tot * (1.0 / D)

    def stage_pv_attn(s):
        pv_block(0)
        pv_block(1)
        attn_block(s, 0)
        pv_block(2)
        attn_block(s, 1)
        pv_block(3)
        attn_block(s, 2)
        attn_block(s, 3)

    def mem_update(g):
        lhs = jnp.concatenate([vtn[WIN * g:WIN * g + 128, :], jnp.ones((16, L), BF16)], axis=0)
        upd = _dot(lhs, pkt[WIN * g:WIN * g + 128, :], NT)
        m_new = m_f32[g] + upd * keep[g]
        m_f32[g] = m_new
        m_bf[g] = m_new.astype(BF16)

    def mem_read(g):
        for i in range(NQB):
            nm = _dot(m_bf[g], pqt[WIN * g:WIN * g + 128, 128 * i:128 * (i + 1)])
            first = GROUP_HEADS[g][0]
            b = gcol[first:first + 8, :] / (nm[128:136, :] + 1e-6)
            for j, h in enumerate(GROUP_HEADS[g]):
                lo = DH * h - WIN * g
                amem[i, DH * h:DH * h + 24, :] = nm[lo:lo + 24] * b[j:j + 1, :]

    def stat_steps(s):
        seg = jnp.maximum(s, 0)
        for i in range(NQB):
            blk = seg * NQB + i
            m = stat2[blk, 0:1, :]
            acc_v = acc_r = None
            for r in range(D // RS):
                rows = slice(RS * r, RS * (r + 1))
                hc = h_all[blk, rows, :] - m
                pv = fold8(hc * hc)
                pr = fold8(hc * wrcol[rows, :])
                acc_v = pv if acc_v is None else acc_v + pv
                acc_r = pr if acc_r is None else acc_r + pr
                yield
            rstd = jax.lax.rsqrt(col_total(acc_v) + LN_EPS)
            stat2[blk, 1:2, :] = rstd
            r_all[pl.ds(blk, 1), :] = jnp.sum(acc_r, axis=0, keepdims=True) * rstd

    def out_steps(s):
        seg = jnp.maximum(s, 0)
        for i in range(NQB):
            cols = pl.ds(pl.multiple_of(seg * L + 128 * i, 128), 128)
            blk = seg * NQB + i
            m = stat2[blk, 0:1, :]
            rstd = stat2[blk, 1:2, :]
            for r in range(D // RS):
                rows = slice(RS * r, RS * (r + 1))
                hh = h_all[blk, rows, :]
                obuf[rows, cols] = (hh + (hh - m) * rstd).astype(BF16)
                yield

    x_copy(0).start()
    cp_wk.start()

    beta = beta_ref[...].astype(F32).reshape(1, H)
    gpad = jnp.concatenate([_sigmoid(beta), jnp.zeros((1, 128 - H), F32)], axis=1)
    gcol[...] = jnp.transpose(jnp.broadcast_to(gpad, (128, 128)))
    wr = jnp.concatenate([wr_ref[...].astype(F32).reshape(1, D), jnp.zeros((1, 64), F32)], axis=1)
    wrcol[...] = jnp.transpose(jnp.broadcast_to(wr, (128, D + 64)))[0:D]
    row = jax.lax.broadcasted_iota(I32, (MROWS, 128), 0)
    lane = jax.lax.broadcasted_iota(I32, (MROWS, 128), 1)
    for g in range(NG):
        first, nh = GROUP_HEADS[g][0], len(GROUP_HEADS[g])
        lane_head = ((lane + WIN * g) * 3641) >> 16
        row_head = jnp.where(row < 128, ((row + WIN * g) * 3641) >> 16, row - 128 + first)
        ok = (lane_head == row_head) & (row_head >= first) & (row_head < first + nh)
        keep[g] = jnp.where(ok, 1.0, 0.0)
    m_f32[...] = jnp.zeros_like(m_f32)
    amem[...] = jnp.zeros_like(amem)

    h_all[0:NQB] = jnp.zeros((NQB, D, 128), F32)
    stat2[0:NQB] = jnp.zeros((NQB, 8, 128), F32)

    def transpose_tile(dst, raw, t):
        hi = min(128 * (t + 1), D)
        dst[128 * t:hi, :] = raw[:, 128 * t:hi].T

    def col_norm_steps(raw, slot):
        for t in range(5):
            hi = min(128 * (t + 1), D)
            for k in range(3):
                w = raw[192 * k:192 * (k + 1), 128 * t:hi].astype(F32)
                wnorm[slot, 8 * k:8 * (k + 1), 128 * t:hi] = jnp.sum(
                    (w * w).reshape(24, 8, hi - 128 * t), axis=0)
                yield

    x_copy(0).wait()
    cp_wq.start()
    for _ in ln1_steps(0):
        pass
    cp_wk.wait()
    cp_wv.start()
    side = _Filler([col_norm_steps(wk_raw, 0)], [15])
    transpose_tile(wkt, wk_raw, 0)
    transpose_tile(wkt, wk_raw, 1)
    proj_k(0)
    transpose_tile(wkt, wk_raw, 2)
    side.upto(0.5)
    proj_k(1)
    transpose_tile(wkt, wk_raw, 3)
    side.upto(1.0)
    proj_k(2)
    transpose_tile(wkt, wk_raw, 4)
    cp_wq.wait()
    cp_wv.wait()
    cp_wo.start()
    x_copy(1).start()
    transpose_tile(wqt, wq_raw, 0)
    transpose_tile(wqt, wq_raw, 1)
    proj_k(3)
    side = _Filler([col_norm_steps(wq_raw, 1), col_norm_steps(wv_raw, 2)], [15, 15])
    for c in range(NCH):
        proj_q(c)
        if c + 2 < 5:
            transpose_tile(wqt, wq_raw, c + 2)
        if c >= 2:
            transpose_tile(wvt, wv_raw, c - 2)
        if c < NCH - 1:
            side.upto((c + 1) / (NCH - 1))
    cp_wo.wait()
    for s in range(2, NSEG):
        x_copy(s).start()
    cp_wg.start()
    cp_wu.start()
    cp_wd.start()
    for c in range(NCH):
        proj_v(c)
        if c + 2 < 5:
            transpose_tile(wvt, wv_raw, c + 2)
        transpose_tile(wot, wo_raw, c)
    transpose_tile(wot, wo_raw, 4)

    x_copy(1).wait()

    def max_norm(slot):
        ss = jnp.sum(wnorm[slot], axis=0, keepdims=True)
        return jnp.sqrt(jnp.max(ss, axis=1, keepdims=True))

    nk, nq, nv = max_norm(0), max_norm(1), max_norm(2)

    bound = (QSCALE * DH * D) * nq * nk
    safe = (bound <= SAFE_LOGIT) & (nv * (D ** 0.5) <= SAFE_V)
    flag[0] = jnp.sum(jnp.where(safe, 1, 0).astype(I32))

    def segment(s, carry):
        @pl.when(jnp.logical_and(s > 0, s + 1 < NSEG))
        def _():
            x_copy(s + 1).wait()

        def side_work():
            return _Filler([_chain(stat_steps(s - 1), out_steps(s - 1)), ln1_steps(s + 1)],
                           [2 * PASS_STEPS, 3 * PASS_STEPS])

        @pl.when(flag[0] == 1)
        def _():
            stage_scores_fast(side_work())

        @pl.when(flag[0] != 1)
        def _():
            stage_scores_safe()
            side_work().upto(1.0)

        @pl.when(s > 0)
        def _():
            out_copy(s - 1).start()

        stage_pv_attn(s)

        @pl.when(s + 1 < NSEG)
        def _():
            for g in range(NG):
                mem_update(g)
            for c in range(NCH):
                proj_q(c)
            for c in range(NCH):
                proj_k(c)
            for g in range(NG):
                mem_read(g)
            for c in range(NCH):
                proj_v(c)

        return carry

    jax.lax.fori_loop(0, NSEG, segment, 0)

    for _ in stat_steps(NSEG - 1):
        pass
    r = r_all[...]
    r_sel = jnp.max(jnp.max(r, axis=0, keepdims=True), axis=1, keepdims=True)
    ids = (128 * jax.lax.broadcasted_iota(I32, r.shape, 0)
           + jax.lax.broadcasted_iota(I32, r.shape, 1))
    cand = jnp.min(jnp.where(r == r_sel, ids, S), axis=0, keepdims=True)
    idx = jnp.minimum(jnp.sum(jnp.min(cand, axis=1, keepdims=True)), S - 1)
    for _ in out_steps(NSEG - 1):
        pass
    out_copy(NSEG - 1).start()
    blk = idx >> 7
    cols = pl.ds(pl.multiple_of(blk * 128, 128), 128)
    m_sel = stat2[blk, 0:1, :]
    rstd_sel = stat2[blk, 1:2, :]
    for r in range(D // RS):
        rows = slice(RS * r, RS * (r + 1))
        hn_sel[rows, :] = ((h_all[blk, rows, :] - m_sel) * rstd_sel).astype(BF16)
    onehot = (jax.lax.broadcasted_iota(I32, (16, 128), 1) == idx - blk * 128).astype(BF16)
    xs = _dot(onehot, hn_sel[...], NT).astype(BF16)
    cp_wg.wait()
    cp_wu.wait()
    cp_wd.wait()

    def down_steps(c, act):
        for r in range(D // RS):
            rows = slice(RS * r, RS * (r + 1))
            part = None if c == 0 else yacc[rows, :]
            for t in range(FC // 128):
                w = wdt_v[rows, FC * c + 128 * t:FC * c + 128 * (t + 1)].astype(F32)
                part = w * act[t] if part is None else part + w * act[t]
            yacc[rows, :] = part
            yield

    nch = FF // FC
    pending = None
    for c in range(nch):
        ga, up = [], []
        for t in range(FC // 128):
            tile = slice(FC * c + 128 * t, FC * c + 128 * (t + 1))
            ga.append(_dot(xs, wg_v[:, tile])[0:1])
            up.append(_dot(xs, wu_v[:, tile])[0:1])
            if pending is not None:
                pending.upto((t + 1) / (FC // 128))
        act = [g * _sigmoid(g) * u for g, u in zip(ga, up)]
        pending = _Filler([down_steps(c, act)], [D // RS])
    pending.upto(1.0)
    y = jnp.sum(yacc[...], axis=1, keepdims=True) * _sigmoid(r_sel)
    sel = jax.lax.broadcasted_iota(I32, (RS, 128), 1) == idx - blk * 128
    for r in range(D // RS):
        rows = slice(RS * r, RS * (r + 1))
        hh = h_all[blk, rows, :]
        stage[rows, :] = (hh + (hh - m_sel) * rstd_sel
                          + jnp.where(sel, y[rows], 0.0)).astype(BF16)
    for s in range(NSEG):
        out_copy(s).wait()
    fix = pltpu.make_async_copy(stage, out_hbm.at[:, cols], sem_w.at[7])
    fix.start()
    fix.wait()


@jax.jit
def pallas_sequential_preLN__memory_aug_infini_attn__moe_arch_mod__prompt_kernel(
    A_x: jax.Array,
    A_wq: jax.Array,
    A_wk: jax.Array,
    A_wv: jax.Array,
    A_wo: jax.Array,
    A_beta: jax.Array,
    B_x: jax.Array,
    B_w_r: jax.Array,
    B_w_gate: jax.Array,
    B_w_up: jax.Array,
    B_w_down: jax.Array,
):
    del B_x
    hbm = pl.BlockSpec(memory_space=pltpu.HBM)
    vmem = pl.BlockSpec(memory_space=pltpu.VMEM)
    scratch = [
        pltpu.VMEM((D, S), BF16),
        pltpu.VMEM((D, D), BF16),
        pltpu.VMEM((D, D), BF16),
        pltpu.VMEM((D, D), BF16),
        pltpu.VMEM((D, D), BF16),
        pltpu.VMEM((D, D), BF16),
        pltpu.VMEM((D, D), BF16),
        pltpu.VMEM((D, D), BF16),
        pltpu.VMEM((D, D), BF16),
        pltpu.VMEM((D, L), BF16),
        pltpu.VMEM((D, L), BF16),
        pltpu.VMEM((NG, L, 128), BF16),
        pltpu.VMEM((D, L), BF16),
        pltpu.VMEM((D, L), BF16),
        pltpu.VMEM((D, L), BF16),
        pltpu.VMEM((D, L), BF16),
        pltpu.VMEM((H * 32, L), BF16),
        pltpu.VMEM((H, NTILE * 128, 128), BF16),
        pltpu.VMEM((NG, MROWS, 128), F32),
        pltpu.VMEM((NG, MROWS, 128), BF16),
        pltpu.VMEM((NG, MROWS, 128), F32),
        pltpu.VMEM((NQB, D + 24, 128), F32),
        pltpu.VMEM((NQB, D + 24, 128), F32),
        pltpu.VMEM((NSEG * NQB, D, 128), F32),
        pltpu.VMEM((D, 128), BF16),
        pltpu.VMEM((D, 128), F32),
        pltpu.VMEM((D, S), BF16),
        pltpu.VMEM((D, FF), BF16),
        pltpu.VMEM((D, FF), BF16),
        pltpu.VMEM((D, FF), BF16),
        pltpu.VMEM((128, 128), F32),
        pltpu.VMEM((D, 128), F32),
        pltpu.VMEM((NQB, 8, 128), F32),
        pltpu.VMEM((NSEG * NQB, 8, 128), F32),
        pltpu.VMEM((3, 24, D), F32),
        pltpu.VMEM((NSEG * NQB, 128), F32),
        pltpu.VMEM((D, 128), BF16),
        pltpu.SMEM((1,), I32),
        pltpu.SemaphoreType.DMA((NSEG,)),
        pltpu.SemaphoreType.DMA((8,)),
        pltpu.SemaphoreType.DMA((NSEG,)),
    ]
    out_t = pl.pallas_call(
        _kernel,
        out_shape=jax.ShapeDtypeStruct((D, S), BF16),
        in_specs=[hbm, hbm, hbm, hbm, hbm, vmem, vmem, hbm, hbm, hbm],
        out_specs=hbm,
        scratch_shapes=scratch,
        compiler_params=pltpu.CompilerParams(vmem_limit_bytes=100 * 1024 * 1024),
        name="infini_moe",
    )(A_x.reshape(S, D).T, A_wq, A_wk, A_wv, A_wo, A_beta, B_w_r, B_w_gate, B_w_up, B_w_down.T)
    return out_t.T.reshape(1, S, D)
```

```python
import functools

import jax
import jax.numpy as jnp
import jax.experimental.pallas as pl
import jax.experimental.pallas.tpu as pltpu

F32 = jnp.float32
BF16 = jnp.bfloat16
U32 = jnp.uint32
I32 = jnp.int32

S = 2048
D = 576
H = 32
DH = 18
NSEG = 4
L = S // NSEG
FF = 4608
NQB = L // 128
TOFF = (0, 1, 3, 6)
NTILE = 10
NG = 5
WIN = 112
GROUP_HEADS = tuple(tuple(h for h in range(H)
                          if min(max(0, -(-(DH * h + DH - 128) // WIN)), NG - 1) == g)
                    for g in range(NG))
GROUP_OF = {h: g for g in range(NG) for h in GROUP_HEADS[g]}
MROWS = 144
CH = 144
NCH = D // CH
RS = 64
PASS_STEPS = NQB * (D // RS)
FC = 512
LAG = 4
LN_EPS = 1e-5
LOG2E = 1.4426950408889634
QSCALE = (DH ** -0.5) * LOG2E
SAFE_LOGIT = 60.0
SAFE_V = 2.0 ** 50

NN = (((1,), (0,)), ((), ()))
NT = (((1,), (1,)), ((), ()))
TN = (((0,), (0,)), ((), ()))

for _g, _hs in enumerate(GROUP_HEADS):
    for _h in _hs:
        assert WIN * _g <= DH * _h and DH * _h + DH <= WIN * _g + 128


def _dot(a, b, dims=NN):
    return jax.lax.dot_general(a, b, dims, preferred_element_type=F32)


class _Filler:
    def __init__(self, gens, counts):
        self.gens, self.counts, self.done = gens, counts, [0] * len(gens)

    def upto(self, frac):
        for k, gen in enumerate(self.gens):
            while self.done[k] < min(frac, 1.0) * self.counts[k]:
                next(gen, None)
                self.done[k] += 1
            if frac >= 1.0:
                for _ in gen:
                    pass


def _chain(*gens):
    for gen in gens:
        yield from gen


def _phi(t):
    return jnp.where(t > 0, t + 1.0, jnp.exp(t))


def _sigmoid(t):
    return 1.0 / (1.0 + jnp.exp(-t))


def _recip(x):
    r = pl.reciprocal(x, approx=True)
    return r * (2.0 - x * r)


def _kernel(xt_hbm, wq_hbm, wk_hbm, wv_hbm, wo_hbm, beta_ref, wr_ref, wg_hbm, wu_hbm, wdt_hbm,
            out_hbm,
            xbuf, wq_raw, wk_raw, wv_raw, wo_raw, wqt, wkt, wvt, wot, xn, ktn, kb, qt, pkt, pqt,
            vtn, vt32, pbuf, m_f32, m_bf, keep, amem, ot, h_all, hn_sel, yacc, obuf, wg_v, wu_v, wdt_v,
            gcol, wrcol, stat1, stat2, wnorm, r_all, stage, flag, sem_x, sem_w, sem_o):
    def x_copy(s):
        cols = pl.ds(pl.multiple_of(s * L, L), L)
        return pltpu.make_async_copy(xt_hbm.at[:, cols], xbuf.at[:, cols], sem_x.at[s])

    def out_copy(s):
        cols = pl.ds(pl.multiple_of(s * L, L), L)
        return pltpu.make_async_copy(obuf.at[:, cols], out_hbm.at[:, cols], sem_o.at[s])

    cp_wk = pltpu.make_async_copy(wk_hbm, wk_raw, sem_w.at[0])
    cp_wq = pltpu.make_async_copy(wq_hbm, wq_raw, sem_w.at[1])
    cp_wv = pltpu.make_async_copy(wv_hbm, wv_raw, sem_w.at[2])
    cp_wo = pltpu.make_async_copy(wo_hbm, wo_raw, sem_w.at[3])
    cp_wg = pltpu.make_async_copy(wg_hbm, wg_v, sem_w.at[4])
    cp_wu = pltpu.make_async_copy(wu_hbm, wu_v, sem_w.at[5])
    cp_wd = pltpu.make_async_copy(wdt_hbm, wdt_v, sem_w.at[6])

    def fold8(v):
        return jnp.sum(v.reshape(v.shape[0] // 8, 8, 128), axis=0)

    def col_total(acc):
        return jnp.sum(acc, axis=0, keepdims=True) * (1.0 / D)

    def ln1_steps(s):
        seg = jnp.minimum(s, NSEG - 1)
        for c in range(NQB):
            cols = pl.ds(pl.multiple_of(seg * L + 128 * c, 128), 128)
            xs = lambda r: xbuf[RS * r:RS * (r + 1), cols].astype(F32)
            acc = None
            for r in range(D // RS):
                part = fold8(xs(r))
                acc = part if acc is None else acc + part
                yield
            m = col_total(acc)
            stat1[c, 0:1, :] = m
            acc = None
            for r in range(D // RS):
                xc = xs(r) - m
                part = fold8(xc * xc)
                acc = part if acc is None else acc + part
                yield
            rstd = jax.lax.rsqrt(col_total(acc) + LN_EPS)
            stat1[c, 1:2, :] = rstd
            for r in range(D // RS):
                xn[RS * r:RS * (r + 1), 128 * c:128 * (c + 1)] = (
                    (xs(r) - m) * rstd).astype(BF16)
                yield

    def rows_of(c):
        return slice(CH * c, CH * (c + 1))

    def proj_k(c):
        kt = _dot(wkt[rows_of(c), :], xn[...])
        pkt[rows_of(c), :] = _phi(kt).astype(BF16)
        ktn[rows_of(c), :] = kt.astype(BF16)
        for g in range(NG):
            if (WIN * g + 127) // CH == c:
                kb[g] = ktn[WIN * g:WIN * g + 128, :].T

    def proj_q(c):
        qf = _dot(wqt[rows_of(c), :], xn[...])
        qt[rows_of(c), :] = (qf * QSCALE).astype(BF16)
        pqt[rows_of(c), :] = _phi(qf).astype(BF16)

    def proj_v(c):
        tail = jnp.concatenate([jnp.ones((1, L), F32), jnp.zeros((13, L), F32)], axis=0)
        vt = _dot(wvt[rows_of(c), :], xn[...])
        vtn[rows_of(c), :] = vt.astype(BF16)
        for j in range(CH // DH):
            h = (CH // DH) * c + j
            vt32[32 * h:32 * h + 16, :] = vt[DH * j:DH * j + 16].astype(BF16)
            vt32[32 * h + 16:32 * h + 32, :] = jnp.concatenate(
                [vt[DH * j + 16:DH * j + 18], tail], axis=0).astype(BF16)

    def masked_q(w0, i, word_mask):
        qu = pltpu.bitcast(qt[pl.ds(w0, 128), 128 * i:128 * (i + 1)], U32)
        return pltpu.bitcast(jnp.where(word_mask, qu, jnp.uint32(0)), BF16)

    def head_word_mask(lo):
        word = jax.lax.broadcasted_iota(I32, (64, 128), 0)
        return (2 * word >= lo) & (2 * word < lo + DH)

    def causal_mask():
        return (jax.lax.broadcasted_iota(I32, (128, 128), 0)
                <= jax.lax.broadcasted_iota(I32, (128, 128), 1))

    def pv_head(h, i):
        n = 128 * (i + 1)
        r0 = TOFF[i] * 128
        o = _dot(vt32[32 * h:32 * h + 32, 0:n], pbuf[h, r0:r0 + n, :])
        a = (1.0 - gcol[h:h + 1, :]) * _recip(o[DH:DH + 1, :])
        ot[i, DH * h:DH * h + 24, :] = o[0:24] * a + amem[i, DH * h:DH * h + 24, :]

    def stage_attention_fast(filler):
        causal = causal_mask()
        for h in range(H + LAG):
            if h < H:
                g = GROUP_OF[h]
                word_mask = head_word_mask(DH * h - WIN * g)
            for i in range(NQB):
                n = 128 * (i + 1)
                if h < H:
                    filler.upto((NTILE * h + TOFF[i] + i + 1) / (NTILE * (H - 1)))
                    st = _dot(kb[g, 0:n, :], masked_q(WIN * g, i, word_mask))
                    p = jnp.exp2(st)
                    r0 = TOFF[i] * 128
                    if i > 0:
                        pbuf[h, r0:r0 + 128 * i, :] = p[:n - 128].astype(BF16)
                    pbuf[h, r0 + 128 * i:r0 + n, :] = jnp.where(
                        causal, p[n - 128:n], 0.0).astype(BF16)
                if h >= LAG:
                    pv_head(h - LAG, i)

    def stage_scores_safe():
        causal = causal_mask()

        def head(h, carry):
            g = jnp.clip((DH * h + DH - 128 + WIN - 1) // WIN, 0, NG - 1)
            g = jnp.where(DH * h + DH <= 128, 0, g)
            w0 = pl.multiple_of(WIN * g, 16)
            word_mask = head_word_mask(DH * h - WIN * g)
            for i in range(NQB):
                n = 128 * (i + 1)
                st = _dot(kb[g, 0:n, :], masked_q(w0, i, word_mask))
                sd = jnp.where(causal, st[n - 128:n], -jnp.inf)
                m = jnp.max(sd, axis=0, keepdims=True)
                if i > 0:
                    m = jnp.maximum(m, jnp.max(st[:n - 128], axis=0, keepdims=True))
                r0 = TOFF[i] * 128
                if i > 0:
                    pbuf[h, r0:r0 + 128 * i, :] = jnp.exp2(st[:n - 128] - m).astype(BF16)
                pbuf[h, r0 + 128 * i:r0 + n, :] = jnp.exp2(sd - m).astype(BF16)
            return carry

        jax.lax.fori_loop(0, H, head, 0)

    def attn_block(s, i):
        cols = pl.ds(pl.multiple_of(s * L + 128 * i, 128), 128)
        blk = s * NQB + i
        otb = ot[i, 0:D, :].astype(BF16)
        tot = None
        for c in range(NCH):
            hh = _dot(wot[rows_of(c), :], otb) + xbuf[rows_of(c), cols].astype(F32)
            h_all[blk, rows_of(c), :] = hh
            part = jnp.sum(hh, axis=0, keepdims=True)
            tot = part if tot is None else tot + part
        stat2[blk, 0:1, :] = tot * (1.0 / D)

    def mem_update(g):
        lhs = jnp.concatenate([vtn[WIN * g:WIN * g + 128, :], jnp.ones((16, L), BF16)], axis=0)
        upd = _dot(lhs, pkt[WIN * g:WIN * g + 128, :], NT)
        m_new = m_f32[g] + upd * keep[g]
        m_f32[g] = m_new
        m_bf[g] = m_new.astype(BF16)

    def mem_read(g):
        for i in range(NQB):
            nm = _dot(m_bf[g], pqt[WIN * g:WIN * g + 128, 128 * i:128 * (i + 1)])
            first = GROUP_HEADS[g][0]
            b = gcol[first:first + 8, :] / (nm[128:136, :] + 1e-6)
            for j, h in enumerate(GROUP_HEADS[g]):
                lo = DH * h - WIN * g
                amem[i, DH * h:DH * h + 24, :] = nm[lo:lo + 24] * b[j:j + 1, :]

    def stat_steps(s):
        seg = jnp.maximum(s, 0)
        for i in range(NQB):
            blk = seg * NQB + i
            m = stat2[blk, 0:1, :]
            acc_v = acc_r = None
            for r in range(D // RS):
                rows = slice(RS * r, RS * (r + 1))
                hc = h_all[blk, rows, :] - m
                pv = fold8(hc * hc)
                pr = fold8(hc * wrcol[rows, :])
                acc_v = pv if acc_v is None else acc_v + pv
                acc_r = pr if acc_r is None else acc_r + pr
                yield
            rstd = jax.lax.rsqrt(col_total(acc_v) + LN_EPS)
            stat2[blk, 1:2, :] = rstd
            r_all[pl.ds(blk, 1), :] = jnp.sum(acc_r, axis=0, keepdims=True) * rstd

    def out_steps(s):
        seg = jnp.maximum(s, 0)
        for i in range(NQB):
            cols = pl.ds(pl.multiple_of(seg * L + 128 * i, 128), 128)
            blk = seg * NQB + i
            m = stat2[blk, 0:1, :]
            rstd = stat2[blk, 1:2, :]
            for r in range(D // RS):
                rows = slice(RS * r, RS * (r + 1))
                hh = h_all[blk, rows, :]
                obuf[rows, cols] = (hh + (hh - m) * rstd).astype(BF16)
                yield

    x_copy(0).start()
    cp_wk.start()

    beta = beta_ref[...].astype(F32).reshape(1, H)
    gpad = jnp.concatenate([_sigmoid(beta), jnp.zeros((1, 128 - H), F32)], axis=1)
    gcol[...] = jnp.transpose(jnp.broadcast_to(gpad, (128, 128)))
    wr = jnp.concatenate([wr_ref[...].astype(F32).reshape(1, D), jnp.zeros((1, 64), F32)], axis=1)
    wrcol[...] = jnp.transpose(jnp.broadcast_to(wr, (128, D + 64)))[0:D]
    row = jax.lax.broadcasted_iota(I32, (MROWS, 128), 0)
    lane = jax.lax.broadcasted_iota(I32, (MROWS, 128), 1)
    for g in range(NG):
        first, nh = GROUP_HEADS[g][0], len(GROUP_HEADS[g])
        lane_head = ((lane + WIN * g) * 3641) >> 16
        row_head = jnp.where(row < 128, ((row + WIN * g) * 3641) >> 16, row - 128 + first)
        ok = (lane_head == row_head) & (row_head >= first) & (row_head < first + nh)
        keep[g] = jnp.where(ok, 1.0, 0.0)
    m_f32[...] = jnp.zeros_like(m_f32)
    amem[...] = jnp.zeros_like(amem)

    h_all[0:NQB] = jnp.zeros((NQB, D, 128), F32)
    stat2[0:NQB] = jnp.zeros((NQB, 8, 128), F32)

    def transpose_tile(dst, raw, t):
        hi = min(128 * (t + 1), D)
        dst[128 * t:hi, :] = raw[:, 128 * t:hi].T

    def col_norm_steps(raw, slot):
        for t in range(5):
            hi = min(128 * (t + 1), D)
            for k in range(3):
                w = raw[192 * k:192 * (k + 1), 128 * t:hi].astype(F32)
                wnorm[slot, 8 * k:8 * (k + 1), 128 * t:hi] = jnp.sum(
                    (w * w).reshape(24, 8, hi - 128 * t), axis=0)
                yield

    x_copy(0).wait()
    cp_wq.start()
    for _ in ln1_steps(0):
        pass
    cp_wk.wait()
    cp_wv.start()
    side = _Filler([col_norm_steps(wk_raw, 0)], [15])
    transpose_tile(wkt, wk_raw, 0)
    transpose_tile(wkt, wk_raw, 1)
    proj_k(0)
    transpose_tile(wkt, wk_raw, 2)
    side.upto(0.5)
    proj_k(1)
    transpose_tile(wkt, wk_raw, 3)
    side.upto(1.0)
    proj_k(2)
    transpose_tile(wkt, wk_raw, 4)
    cp_wq.wait()
    cp_wv.wait()
    cp_wo.start()
    x_copy(1).start()
    transpose_tile(wqt, wq_raw, 0)
    transpose_tile(wqt, wq_raw, 1)
    proj_k(3)
    side = _Filler([col_norm_steps(wq_raw, 1), col_norm_steps(wv_raw, 2)], [15, 15])
    for c in range(NCH):
        proj_q(c)
        if c + 2 < 5:
            transpose_tile(wqt, wq_raw, c + 2)
        if c >= 2:
            transpose_tile(wvt, wv_raw, c - 2)
        if c < NCH - 1:
            side.upto((c + 1) / (NCH - 1))
    cp_wo.wait()
    for s in range(2, NSEG):
        x_copy(s).start()
    cp_wg.start()
    cp_wu.start()
    cp_wd.start()
    for c in range(NCH):
        proj_v(c)
        if c + 2 < 5:
            transpose_tile(wvt, wv_raw, c + 2)
        transpose_tile(wot, wo_raw, c)
    transpose_tile(wot, wo_raw, 4)

    x_copy(1).wait()

    def max_norm(slot):
        ss = jnp.sum(wnorm[slot], axis=0, keepdims=True)
        return jnp.sqrt(jnp.max(ss, axis=1, keepdims=True))

    nk, nq, nv = max_norm(0), max_norm(1), max_norm(2)

    bound = (QSCALE * DH * D) * nq * nk
    safe = (bound <= SAFE_LOGIT) & (nv * (D ** 0.5) <= SAFE_V)
    flag[0] = jnp.sum(jnp.where(safe, 1, 0).astype(I32))

    def segment(s, carry):
        @pl.when(jnp.logical_and(s > 0, s + 1 < NSEG))
        def _():
            x_copy(s + 1).wait()

        def side_work():
            return _Filler([_chain(stat_steps(s - 1), out_steps(s - 1)), ln1_steps(s + 1)],
                           [2 * PASS_STEPS, 3 * PASS_STEPS])

        @pl.when(flag[0] == 1)
        def _():
            stage_attention_fast(side_work())

        @pl.when(flag[0] != 1)
        def _():
            stage_scores_safe()
            side_work().upto(1.0)
            for h in range(H):
                for i in range(NQB):
                    pv_head(h, i)

        @pl.when(s > 0)
        def _():
            out_copy(s - 1).start()

        @pl.when(s + 1 < NSEG)
        def _():
            for i in range(NQB):
                attn_block(s, i)
            for g in range(NG):
                mem_update(g)
            for c in range(NCH):
                proj_q(c)
            for c in range(NCH):
                proj_k(c)
            for g in range(NG):
                mem_read(g)
            for c in range(NCH):
                proj_v(c)

        @pl.when(s + 1 == NSEG)
        def _():
            for i in range(NQB):
                attn_block(s, i)

        return carry

    jax.lax.fori_loop(0, NSEG, segment, 0)

    for _ in stat_steps(NSEG - 1):
        pass
    r = r_all[...]
    r_sel = jnp.max(jnp.max(r, axis=0, keepdims=True), axis=1, keepdims=True)
    ids = (128 * jax.lax.broadcasted_iota(I32, r.shape, 0)
           + jax.lax.broadcasted_iota(I32, r.shape, 1))
    cand = jnp.min(jnp.where(r == r_sel, ids, S), axis=0, keepdims=True)
    idx = jnp.minimum(jnp.sum(jnp.min(cand, axis=1, keepdims=True)), S - 1)
    for _ in out_steps(NSEG - 1):
        pass
    out_copy(NSEG - 1).start()
    blk = idx >> 7
    cols = pl.ds(pl.multiple_of(blk * 128, 128), 128)
    m_sel = stat2[blk, 0:1, :]
    rstd_sel = stat2[blk, 1:2, :]
    for r in range(D // RS):
        rows = slice(RS * r, RS * (r + 1))
        hn_sel[rows, :] = ((h_all[blk, rows, :] - m_sel) * rstd_sel).astype(BF16)
    onehot = (jax.lax.broadcasted_iota(I32, (16, 128), 1) == idx - blk * 128).astype(BF16)
    xs = _dot(onehot, hn_sel[...], NT).astype(BF16)
    cp_wg.wait()
    cp_wu.wait()
    cp_wd.wait()

    def down_steps(c, act):
        for r in range(D // RS):
            rows = slice(RS * r, RS * (r + 1))
            part = None if c == 0 else yacc[rows, :]
            for t in range(FC // 128):
                w = wdt_v[rows, FC * c + 128 * t:FC * c + 128 * (t + 1)].astype(F32)
                part = w * act[t] if part is None else part + w * act[t]
            yacc[rows, :] = part
            yield

    nch = FF // FC
    pending = None
    for c in range(nch):
        ga, up = [], []
        for t in range(FC // 128):
            tile = slice(FC * c + 128 * t, FC * c + 128 * (t + 1))
            ga.append(_dot(xs, wg_v[:, tile])[0:1])
            up.append(_dot(xs, wu_v[:, tile])[0:1])
            if pending is not None:
                pending.upto((t + 1) / (FC // 128))
        act = [g * _sigmoid(g) * u for g, u in zip(ga, up)]
        pending = _Filler([down_steps(c, act)], [D // RS])
    pending.upto(1.0)
    y = jnp.sum(yacc[...], axis=1, keepdims=True) * _sigmoid(r_sel)
    sel = jax.lax.broadcasted_iota(I32, (RS, 128), 1) == idx - blk * 128
    for r in range(D // RS):
        rows = slice(RS * r, RS * (r + 1))
        hh = h_all[blk, rows, :]
        stage[rows, :] = (hh + (hh - m_sel) * rstd_sel
                          + jnp.where(sel, y[rows], 0.0)).astype(BF16)
    for s in range(NSEG):
        out_copy(s).wait()
    fix = pltpu.make_async_copy(stage, out_hbm.at[:, cols], sem_w.at[7])
    fix.start()
    fix.wait()


@jax.jit
def pallas_sequential_preLN__memory_aug_infini_attn__moe_arch_mod__prompt_kernel(
    A_x: jax.Array,
    A_wq: jax.Array,
    A_wk: jax.Array,
    A_wv: jax.Array,
    A_wo: jax.Array,
    A_beta: jax.Array,
    B_x: jax.Array,
    B_w_r: jax.Array,
    B_w_gate: jax.Array,
    B_w_up: jax.Array,
    B_w_down: jax.Array,
):
    del B_x
    hbm = pl.BlockSpec(memory_space=pltpu.HBM)
    vmem = pl.BlockSpec(memory_space=pltpu.VMEM)
    scratch = [
        pltpu.VMEM((D, S), BF16),
        pltpu.VMEM((D, D), BF16),
        pltpu.VMEM((D, D), BF16),
        pltpu.VMEM((D, D), BF16),
        pltpu.VMEM((D, D), BF16),
        pltpu.VMEM((D, D), BF16),
        pltpu.VMEM((D, D), BF16),
        pltpu.VMEM((D, D), BF16),
        pltpu.VMEM((D, D), BF16),
        pltpu.VMEM((D, L), BF16),
        pltpu.VMEM((D, L), BF16),
        pltpu.VMEM((NG, L, 128), BF16),
        pltpu.VMEM((D, L), BF16),
        pltpu.VMEM((D, L), BF16),
        pltpu.VMEM((D, L), BF16),
        pltpu.VMEM((D, L), BF16),
        pltpu.VMEM((H * 32, L), BF16),
        pltpu.VMEM((H, NTILE * 128, 128), BF16),
        pltpu.VMEM((NG, MROWS, 128), F32),
        pltpu.VMEM((NG, MROWS, 128), BF16),
        pltpu.VMEM((NG, MROWS, 128), F32),
        pltpu.VMEM((NQB, D + 24, 128), F32),
        pltpu.VMEM((NQB, D + 24, 128), F32),
        pltpu.VMEM((NSEG * NQB, D, 128), F32),
        pltpu.VMEM((D, 128), BF16),
        pltpu.VMEM((D, 128), F32),
        pltpu.VMEM((D, S), BF16),
        pltpu.VMEM((D, FF), BF16),
        pltpu.VMEM((D, FF), BF16),
        pltpu.VMEM((D, FF), BF16),
        pltpu.VMEM((128, 128), F32),
        pltpu.VMEM((D, 128), F32),
        pltpu.VMEM((NQB, 8, 128), F32),
        pltpu.VMEM((NSEG * NQB, 8, 128), F32),
        pltpu.VMEM((3, 24, D), F32),
        pltpu.VMEM((NSEG * NQB, 128), F32),
        pltpu.VMEM((D, 128), BF16),
        pltpu.SMEM((1,), I32),
        pltpu.SemaphoreType.DMA((NSEG,)),
        pltpu.SemaphoreType.DMA((8,)),
        pltpu.SemaphoreType.DMA((NSEG,)),
    ]
    out_t = pl.pallas_call(
        _kernel,
        out_shape=jax.ShapeDtypeStruct((D, S), BF16),
        in_specs=[hbm, hbm, hbm, hbm, hbm, vmem, vmem, hbm, hbm, hbm],
        out_specs=hbm,
        scratch_shapes=scratch,
        compiler_params=pltpu.CompilerParams(vmem_limit_bytes=100 * 1024 * 1024),
        name="infini_moe",
    )(A_x.reshape(S, D).T, A_wq, A_wk, A_wv, A_wo, A_beta, B_w_r, B_w_gate, B_w_up, B_w_down.T)
    return out_t.T.reshape(1, S, D)
```

```python
import functools

import jax
import jax.numpy as jnp
import jax.experimental.pallas as pl
import jax.experimental.pallas.tpu as pltpu

F32 = jnp.float32
BF16 = jnp.bfloat16
U32 = jnp.uint32
I32 = jnp.int32

S = 2048
D = 576
H = 32
DH = 18
NSEG = 4
L = S // NSEG
FF = 4608
NQB = L // 128
TOFF = (0, 1, 3, 6)
NTILE = 10
NG = 5
WIN = 112
GROUP_HEADS = tuple(tuple(h for h in range(H)
                          if min(max(0, -(-(DH * h + DH - 128) // WIN)), NG - 1) == g)
                    for g in range(NG))
GROUP_OF = {h: g for g in range(NG) for h in GROUP_HEADS[g]}
MROWS = 144
CH = 144
NCH = D // CH
RS = 64
PASS_STEPS = NQB * (D // RS)
FC = 512
LAG = 20
LN_EPS = 1e-5
LOG2E = 1.4426950408889634
QSCALE = (DH ** -0.5) * LOG2E
SAFE_LOGIT = 60.0
SAFE_V = 2.0 ** 50

NN = (((1,), (0,)), ((), ()))
NT = (((1,), (1,)), ((), ()))
TN = (((0,), (0,)), ((), ()))

for _g, _hs in enumerate(GROUP_HEADS):
    for _h in _hs:
        assert WIN * _g <= DH * _h and DH * _h + DH <= WIN * _g + 128


def _dot(a, b, dims=NN):
    return jax.lax.dot_general(a, b, dims, preferred_element_type=F32)


class _Filler:
    def __init__(self, gens, counts):
        self.gens, self.counts, self.done = gens, counts, [0] * len(gens)

    def upto(self, frac):
        for k, gen in enumerate(self.gens):
            while self.done[k] < min(frac, 1.0) * self.counts[k]:
                next(gen, None)
                self.done[k] += 1
            if frac >= 1.0:
                for _ in gen:
                    pass


def _chain(*gens):
    for gen in gens:
        yield from gen


def _phi(t):
    return jnp.where(t > 0, t + 1.0, jnp.exp(t))


def _sigmoid(t):
    return 1.0 / (1.0 + jnp.exp(-t))


def _recip(x):
    r = pl.reciprocal(x, approx=True)
    return r * (2.0 - x * r)


def _kernel(xt_hbm, wq_hbm, wk_hbm, wv_hbm, wo_hbm, beta_ref, wr_ref, wg_hbm, wu_hbm, wdt_hbm,
            out_hbm,
            xbuf, wq_raw, wk_raw, wv_raw, wo_raw, wqt, wkt, wvt, wot, xn, ktn, kb, qt, pkt, pqt,
            vtn, vt32, pbuf, m_f32, m_bf, keep, amem, ot, h_all, hn_sel, yacc, obuf, wg_v, wu_v, wdt_v,
            gcol, wrcol, stat1, stat2, wnorm, r_all, stage, flag, sem_x, sem_w, sem_o):
    class _Group:
        def __init__(self, copies):
            self.copies = copies

        def start(self):
            for cp in self.copies:
                cp.start()

        def wait(self):
            for cp in self.copies:
                cp.wait()

    def hbm_cols(blk):
        return pl.ds(pl.multiple_of(blk * 128, 128), 128)

    def x_copy(s):
        return _Group([pltpu.make_async_copy(xt_hbm.at[:, hbm_cols(s * NQB + i)],
                                             xbuf.at[s * NQB + i], sem_x.at[s])
                       for i in range(NQB)])

    def out_copy(s):
        return _Group([pltpu.make_async_copy(obuf.at[s * NQB + i],
                                             out_hbm.at[:, hbm_cols(s * NQB + i)], sem_o.at[s])
                       for i in range(NQB)])

    cp_wk = pltpu.make_async_copy(wk_hbm, wk_raw, sem_w.at[0])
    cp_wq = pltpu.make_async_copy(wq_hbm, wq_raw, sem_w.at[1])
    cp_wv = pltpu.make_async_copy(wv_hbm, wv_raw, sem_w.at[2])
    cp_wo = pltpu.make_async_copy(wo_hbm, wo_raw, sem_w.at[3])
    cp_wg = pltpu.make_async_copy(wg_hbm, wg_v, sem_w.at[4])
    cp_wu = pltpu.make_async_copy(wu_hbm, wu_v, sem_w.at[5])
    cp_wd = pltpu.make_async_copy(wdt_hbm, wdt_v, sem_w.at[6])

    def fold8(v):
        return jnp.sum(v.reshape(v.shape[0] // 8, 8, 128), axis=0)

    def col_total(acc):
        return jnp.sum(acc, axis=0, keepdims=True) * (1.0 / D)

    def ln1_steps(s):
        seg = jnp.minimum(s, NSEG - 1)
        for c in range(NQB):
            xs = lambda r: xbuf[seg * NQB + c, RS * r:RS * (r + 1), :].astype(F32)
            acc = None
            for r in range(D // RS):
                part = fold8(xs(r))
                acc = part if acc is None else acc + part
                yield
            m = col_total(acc)
            stat1[c, 0:1, :] = m
            acc = None
            for r in range(D // RS):
                xc = xs(r) - m
                part = fold8(xc * xc)
                acc = part if acc is None else acc + part
                yield
            rstd = jax.lax.rsqrt(col_total(acc) + LN_EPS)
            stat1[c, 1:2, :] = rstd
            for r in range(D // RS):
                xn[c, RS * r:RS * (r + 1), :] = (
                    (xs(r) - m) * rstd).astype(BF16)
                yield

    def xn_all():
        return jnp.concatenate([xn[c] for c in range(NQB)], axis=1)

    def rows_of(c):
        return slice(CH * c, CH * (c + 1))

    def transpose_keys(g):
        kb[g] = ktn[WIN * g:WIN * g + 128, :].T

    def proj_k(c):
        kt = _dot(wkt[rows_of(c), :], xn_all())
        pkt[rows_of(c), :] = _phi(kt).astype(BF16)
        ktn[rows_of(c), :] = kt.astype(BF16)
        if c == 0:
            transpose_keys(0)

    def proj_q(c):
        qf = _dot(wqt[rows_of(c), :], xn_all())
        qt[rows_of(c), :] = (qf * QSCALE).astype(BF16)
        pqt[rows_of(c), :] = _phi(qf).astype(BF16)

    def proj_v(c):
        tail = jnp.concatenate([jnp.ones((1, L), F32), jnp.zeros((13, L), F32)], axis=0)
        vt = _dot(wvt[rows_of(c), :], xn_all())
        vtn[rows_of(c), :] = vt.astype(BF16)
        for j in range(CH // DH):
            h = (CH // DH) * c + j
            vt32[32 * h:32 * h + 16, :] = vt[DH * j:DH * j + 16].astype(BF16)
            vt32[32 * h + 16:32 * h + 32, :] = jnp.concatenate(
                [vt[DH * j + 16:DH * j + 18], tail], axis=0).astype(BF16)

    def masked_q(w0, i, word_mask):
        qu = pltpu.bitcast(qt[pl.ds(w0, 128), 128 * i:128 * (i + 1)], U32)
        return pltpu.bitcast(jnp.where(word_mask, qu, jnp.uint32(0)), BF16)

    def head_word_mask(lo):
        word = jax.lax.broadcasted_iota(I32, (64, 128), 0)
        return (2 * word >= lo) & (2 * word < lo + DH)

    def causal_mask():
        return (jax.lax.broadcasted_iota(I32, (128, 128), 0)
                <= jax.lax.broadcasted_iota(I32, (128, 128), 1))

    def pv_head(h, i):
        n = 128 * (i + 1)
        r0 = TOFF[i] * 128
        o = _dot(vt32[32 * h:32 * h + 32, 0:n], pbuf[h, r0:r0 + n, :])
        a = (1.0 - gcol[h:h + 1, :]) * _recip(o[DH:DH + 1, :])
        ot[i, DH * h:DH * h + 24, :] = o[0:24] * a + amem[i, DH * h:DH * h + 24, :]

    def stage_attention_fast(filler):
        causal = causal_mask()
        for h in range(H + LAG):
            if h < H:
                g = GROUP_OF[h]
                word_mask = head_word_mask(DH * h - WIN * g)
                if h == GROUP_HEADS[g][0] and g + 1 < NG:
                    transpose_keys(g + 1)
            for i in range(NQB):
                n = 128 * (i + 1)
                if h < H:
                    filler.upto((NTILE * h + TOFF[i] + i + 1) / (NTILE * (H - 1)))
                    st = _dot(kb[g, 0:n, :], masked_q(WIN * g, i, word_mask))
                    p = jnp.exp2(st)
                    r0 = TOFF[i] * 128
                    if i > 0:
                        pbuf[h, r0:r0 + 128 * i, :] = p[:n - 128].astype(BF16)
                    pbuf[h, r0 + 128 * i:r0 + n, :] = jnp.where(
                        causal, p[n - 128:n], 0.0).astype(BF16)
                if h >= LAG:
                    pv_head(h - LAG, i)

    def stage_scores_safe():
        causal = causal_mask()
        for g in range(1, NG):
            transpose_keys(g)

        def head(h, carry):
            g = jnp.clip((DH * h + DH - 128 + WIN - 1) // WIN, 0, NG - 1)
            g = jnp.where(DH * h + DH <= 128, 0, g)
            w0 = pl.multiple_of(WIN * g, 16)
            word_mask = head_word_mask(DH * h - WIN * g)
            for i in range(NQB):
                n = 128 * (i + 1)
                st = _dot(kb[g, 0:n, :], masked_q(w0, i, word_mask))
                sd = jnp.where(causal, st[n - 128:n], -jnp.inf)
                m = jnp.max(sd, axis=0, keepdims=True)
                if i > 0:
                    m = jnp.maximum(m, jnp.max(st[:n - 128], axis=0, keepdims=True))
                r0 = TOFF[i] * 128
                if i > 0:
                    pbuf[h, r0:r0 + 128 * i, :] = jnp.exp2(st[:n - 128] - m).astype(BF16)
                pbuf[h, r0 + 128 * i:r0 + n, :] = jnp.exp2(sd - m).astype(BF16)
            return carry

        jax.lax.fori_loop(0, H, head, 0)

    def attn_block(s, i):
        blk = s * NQB + i
        otb = ot[i, 0:D, :].astype(BF16)
        tot = None
        for c in range(NCH):
            hh = _dot(wot[rows_of(c), :], otb) + xbuf[blk, rows_of(c), :].astype(F32)
            h_all[blk, rows_of(c), :] = hh
            part = jnp.sum(hh, axis=0, keepdims=True)
            tot = part if tot is None else tot + part
        stat2[blk, 0:1, :] = tot * (1.0 / D)

    def mem_update(g):
        lhs = jnp.concatenate([vtn[WIN * g:WIN * g + 128, :], jnp.ones((16, L), BF16)], axis=0)
        upd = _dot(lhs, pkt[WIN * g:WIN * g + 128, :], NT)
        m_new = m_f32[g] + upd * keep[g]
        m_f32[g] = m_new
        m_bf[g] = m_new.astype(BF16)

    def mem_read(g):
        for i in range(NQB):
            nm = _dot(m_bf[g], pqt[WIN * g:WIN * g + 128, 128 * i:128 * (i + 1)])
            first = GROUP_HEADS[g][0]
            b = gcol[first:first + 8, :] / (nm[128:136, :] + 1e-6)
            for j, h in enumerate(GROUP_HEADS[g]):
                lo = DH * h - WIN * g
                amem[i, DH * h:DH * h + 24, :] = nm[lo:lo + 24] * b[j:j + 1, :]

    def stat_steps(s, blocks=range(NQB)):
        seg = jnp.maximum(s, 0)
        for i in blocks:
            blk = seg * NQB + i
            m = stat2[blk, 0:1, :]
            acc_v = acc_r = None
            for r in range(D // RS):
                rows = slice(RS * r, RS * (r + 1))
                hc = h_all[blk, rows, :] - m
                pv = fold8(hc * hc)
                pr = fold8(hc * wrcol[rows, :])
                acc_v = pv if acc_v is None else acc_v + pv
                acc_r = pr if acc_r is None else acc_r + pr
                yield
            rstd = jax.lax.rsqrt(col_total(acc_v) + LN_EPS)
            stat2[blk, 1:2, :] = rstd
            r_all[pl.ds(blk, 1), :] = jnp.sum(acc_r, axis=0, keepdims=True) * rstd

    def out_steps(s):
        seg = jnp.maximum(s, 0)
        for i in range(NQB):
            blk = seg * NQB + i
            m = stat2[blk, 0:1, :]
            rstd = stat2[blk, 1:2, :]
            for r in range(D // RS):
                rows = slice(RS * r, RS * (r + 1))
                hh = h_all[blk, rows, :]
                obuf[blk, rows, :] = (hh + (hh - m) * rstd).astype(BF16)
                yield

    x_copy(0).start()
    cp_wk.start()

    beta = beta_ref[...].astype(F32).reshape(1, H)
    gpad = jnp.concatenate([_sigmoid(beta), jnp.zeros((1, 128 - H), F32)], axis=1)
    gcol[...] = jnp.transpose(jnp.broadcast_to(gpad, (128, 128)))
    wr = jnp.concatenate([wr_ref[...].astype(F32).reshape(1, D), jnp.zeros((1, 64), F32)], axis=1)
    wrcol[...] = jnp.transpose(jnp.broadcast_to(wr, (128, D + 64)))[0:D]
    row = jax.lax.broadcasted_iota(I32, (MROWS, 128), 0)
    lane = jax.lax.broadcasted_iota(I32, (MROWS, 128), 1)
    for g in range(NG):
        first, nh = GROUP_HEADS[g][0], len(GROUP_HEADS[g])
        lane_head = ((lane + WIN * g) * 3641) >> 16
        row_head = jnp.where(row < 128, ((row + WIN * g) * 3641) >> 16, row - 128 + first)
        ok = (lane_head == row_head) & (row_head >= first) & (row_head < first + nh)
        keep[g] = jnp.where(ok, 1.0, 0.0)
    m_f32[...] = jnp.zeros_like(m_f32)
    amem[...] = jnp.zeros_like(amem)

    h_all[0:NQB] = jnp.zeros((NQB, D, 128), F32)
    stat2[0:NQB] = jnp.zeros((NQB, 8, 128), F32)

    def transpose_tile(dst, raw, t):
        hi = min(128 * (t + 1), D)
        dst[128 * t:hi, :] = raw[:, 128 * t:hi].T

    def col_norm_steps(raw, slot):
        for t in range(5):
            hi = min(128 * (t + 1), D)
            for k in range(3):
                w = raw[192 * k:192 * (k + 1), 128 * t:hi].astype(F32)
                wnorm[slot, 8 * k:8 * (k + 1), 128 * t:hi] = jnp.sum(
                    (w * w).reshape(24, 8, hi - 128 * t), axis=0)
                yield

    x_copy(0).wait()
    cp_wq.start()
    for _ in ln1_steps(0):
        pass
    cp_wk.wait()
    cp_wv.start()
    side = _Filler([col_norm_steps(wk_raw, 0)], [15])
    transpose_tile(wkt, wk_raw, 0)
    transpose_tile(wkt, wk_raw, 1)
    proj_k(0)
    transpose_tile(wkt, wk_raw, 2)
    side.upto(0.5)
    proj_k(1)
    transpose_tile(wkt, wk_raw, 3)
    side.upto(1.0)
    proj_k(2)
    transpose_tile(wkt, wk_raw, 4)
    cp_wq.wait()
    cp_wv.wait()
    cp_wo.start()
    x_copy(1).start()
    transpose_tile(wqt, wq_raw, 0)
    transpose_tile(wqt, wq_raw, 1)
    proj_k(3)
    side = _Filler([col_norm_steps(wq_raw, 1), col_norm_steps(wv_raw, 2)], [15, 15])
    for c in range(NCH):
        proj_q(c)
        if c + 2 < 5:
            transpose_tile(wqt, wq_raw, c + 2)
        if c >= 2:
            transpose_tile(wvt, wv_raw, c - 2)
        if c < NCH - 1:
            side.upto((c + 1) / (NCH - 1))
    cp_wo.wait()
    for s in range(2, NSEG):
        x_copy(s).start()
    cp_wg.start()
    cp_wu.start()
    cp_wd.start()
    for c in range(NCH):
        proj_v(c)
        if c + 2 < 5:
            transpose_tile(wvt, wv_raw, c + 2)
        transpose_tile(wot, wo_raw, c)
    transpose_tile(wot, wo_raw, 4)

    x_copy(1).wait()

    def max_norm(slot):
        ss = jnp.sum(wnorm[slot], axis=0, keepdims=True)
        return jnp.sqrt(jnp.max(ss, axis=1, keepdims=True))

    nk, nq, nv = max_norm(0), max_norm(1), max_norm(2)

    bound = (QSCALE * DH * D) * nq * nk
    safe = (bound <= SAFE_LOGIT) & (nv * (D ** 0.5) <= SAFE_V)
    flag[0] = jnp.sum(jnp.where(safe, 1, 0).astype(I32))

    def segment(s, carry):
        @pl.when(jnp.logical_and(s > 0, s + 1 < NSEG))
        def _():
            x_copy(s + 1).wait()

        def side_work():
            return _Filler([_chain(stat_steps(s - 1), out_steps(s - 1)), ln1_steps(s + 1)],
                           [2 * PASS_STEPS, 3 * PASS_STEPS])

        @pl.when(flag[0] == 1)
        def _():
            stage_attention_fast(side_work())

        @pl.when(flag[0] != 1)
        def _():
            stage_scores_safe()
            side_work().upto(1.0)
            for h in range(H):
                for i in range(NQB):
                    pv_head(h, i)

        @pl.when(s > 0)
        def _():
            out_copy(s - 1).start()

        @pl.when(s + 1 < NSEG)
        def _():
            for i in range(NQB):
                attn_block(s, i)
            for g in range(NG):
                mem_update(g)
            for c in range(NCH):
                proj_q(c)
            for c in range(NCH):
                proj_k(c)
            for g in range(NG):
                mem_read(g)
            for c in range(NCH):
                proj_v(c)

        @pl.when(s + 1 == NSEG)
        def _():
            for i in range(NQB):
                attn_block(s, i)
                if i > 0:
                    for _ in stat_steps(s, [i - 1]):
                        pass
            for _ in stat_steps(s, [NQB - 1]):
                pass

        return carry

    jax.lax.fori_loop(0, NSEG, segment, 0)

    r = r_all[...]
    r_sel = jnp.max(jnp.max(r, axis=0, keepdims=True), axis=1, keepdims=True)
    ids = (128 * jax.lax.broadcasted_iota(I32, r.shape, 0)
           + jax.lax.broadcasted_iota(I32, r.shape, 1))
    cand = jnp.min(jnp.where(r == r_sel, ids, S), axis=0, keepdims=True)
    idx = jnp.minimum(jnp.sum(jnp.min(cand, axis=1, keepdims=True)), S - 1)
    for _ in out_steps(NSEG - 1):
        pass
    out_copy(NSEG - 1).start()
    blk = idx >> 7
    m_sel = stat2[blk, 0:1, :]
    rstd_sel = stat2[blk, 1:2, :]
    for r in range(D // RS):
        rows = slice(RS * r, RS * (r + 1))
        hn_sel[rows, :] = ((h_all[blk, rows, :] - m_sel) * rstd_sel).astype(BF16)
    onehot = (jax.lax.broadcasted_iota(I32, (16, 128), 1) == idx - blk * 128).astype(BF16)
    xs = _dot(onehot, hn_sel[...], NT).astype(BF16)
    cp_wg.wait()
    cp_wu.wait()
    cp_wd.wait()

    def down_steps(c, act):
        for r in range(D // RS):
            rows = slice(RS * r, RS * (r + 1))
            part = None if c == 0 else yacc[rows, :]
            for t in range(FC // 128):
                w = wdt_v[rows, FC * c + 128 * t:FC * c + 128 * (t + 1)].astype(F32)
                part = w * act[t] if part is None else part + w * act[t]
            yacc[rows, :] = part
            yield

    nch = FF // FC
    pending = None
    for c in range(nch):
        ga, up = [], []
        for t in range(FC // 128):
            tile = slice(FC * c + 128 * t, FC * c + 128 * (t + 1))
            ga.append(_dot(xs, wg_v[:, tile])[0:1])
            up.append(_dot(xs, wu_v[:, tile])[0:1])
            if pending is not None:
                pending.upto((t + 1) / (FC // 128))
        act = [g * _sigmoid(g) * u for g, u in zip(ga, up)]
        pending = _Filler([down_steps(c, act)], [D // RS])
    pending.upto(1.0)
    y = jnp.sum(yacc[...], axis=1, keepdims=True) * _sigmoid(r_sel)
    sel = jax.lax.broadcasted_iota(I32, (RS, 128), 1) == idx - blk * 128
    for r in range(D // RS):
        rows = slice(RS * r, RS * (r + 1))
        hh = h_all[blk, rows, :]
        stage[rows, :] = (hh + (hh - m_sel) * rstd_sel
                          + jnp.where(sel, y[rows], 0.0)).astype(BF16)
    for s in range(NSEG):
        out_copy(s).wait()
    fix = pltpu.make_async_copy(stage, out_hbm.at[:, hbm_cols(blk)], sem_w.at[7])
    fix.start()
    fix.wait()


@jax.jit
def pallas_sequential_preLN__memory_aug_infini_attn__moe_arch_mod__prompt_kernel(
    A_x: jax.Array,
    A_wq: jax.Array,
    A_wk: jax.Array,
    A_wv: jax.Array,
    A_wo: jax.Array,
    A_beta: jax.Array,
    B_x: jax.Array,
    B_w_r: jax.Array,
    B_w_gate: jax.Array,
    B_w_up: jax.Array,
    B_w_down: jax.Array,
):
    del B_x
    hbm = pl.BlockSpec(memory_space=pltpu.HBM)
    vmem = pl.BlockSpec(memory_space=pltpu.VMEM)
    scratch = [
        pltpu.VMEM((NSEG * NQB, D, 128), BF16),
        pltpu.VMEM((D, D), BF16),
        pltpu.VMEM((D, D), BF16),
        pltpu.VMEM((D, D), BF16),
        pltpu.VMEM((D, D), BF16),
        pltpu.VMEM((D, D), BF16),
        pltpu.VMEM((D, D), BF16),
        pltpu.VMEM((D, D), BF16),
        pltpu.VMEM((D, D), BF16),
        pltpu.VMEM((NQB, D, 128), BF16),
        pltpu.VMEM((D, L), BF16),
        pltpu.VMEM((NG, L, 128), BF16),
        pltpu.VMEM((D, L), BF16),
        pltpu.VMEM((D, L), BF16),
        pltpu.VMEM((D, L), BF16),
        pltpu.VMEM((D, L), BF16),
        pltpu.VMEM((H * 32, L), BF16),
        pltpu.VMEM((H, NTILE * 128, 128), BF16),
        pltpu.VMEM((NG, MROWS, 128), F32),
        pltpu.VMEM((NG, MROWS, 128), BF16),
        pltpu.VMEM((NG, MROWS, 128), F32),
        pltpu.VMEM((NQB, D + 24, 128), F32),
        pltpu.VMEM((NQB, D + 24, 128), F32),
        pltpu.VMEM((NSEG * NQB, D, 128), F32),
        pltpu.VMEM((D, 128), BF16),
        pltpu.VMEM((D, 128), F32),
        pltpu.VMEM((NSEG * NQB, D, 128), BF16),
        pltpu.VMEM((D, FF), BF16),
        pltpu.VMEM((D, FF), BF16),
        pltpu.VMEM((D, FF), BF16),
        pltpu.VMEM((128, 128), F32),
        pltpu.VMEM((D, 128), F32),
        pltpu.VMEM((NQB, 8, 128), F32),
        pltpu.VMEM((NSEG * NQB, 8, 128), F32),
        pltpu.VMEM((3, 24, D), F32),
        pltpu.VMEM((NSEG * NQB, 128), F32),
        pltpu.VMEM((D, 128), BF16),
        pltpu.SMEM((1,), I32),
        pltpu.SemaphoreType.DMA((NSEG,)),
        pltpu.SemaphoreType.DMA((8,)),
        pltpu.SemaphoreType.DMA((NSEG,)),
    ]
    out_t = pl.pallas_call(
        _kernel,
        out_shape=jax.ShapeDtypeStruct((D, S), BF16),
        in_specs=[hbm, hbm, hbm, hbm, hbm, vmem, vmem, hbm, hbm, hbm],
        out_specs=hbm,
        scratch_shapes=scratch,
        compiler_params=pltpu.CompilerParams(vmem_limit_bytes=100 * 1024 * 1024),
        name="infini_moe",
    )(A_x.reshape(S, D).T, A_wq, A_wk, A_wv, A_wo, A_beta, B_w_r, B_w_gate, B_w_up, B_w_down.T)
    return out_t.T.reshape(1, S, D)
```

```python
import functools

import jax
import jax.numpy as jnp
import jax.experimental.pallas as pl
import jax.experimental.pallas.tpu as pltpu

F32 = jnp.float32
BF16 = jnp.bfloat16
U32 = jnp.uint32
I32 = jnp.int32

S = 2048
D = 576
H = 32
DH = 18
NSEG = 4
L = S // NSEG
FF = 4608
NQB = L // 128
TOFF = (0, 1, 3, 6)
NTILE = 10
NG = 5
WIN = 112
GROUP_HEADS = tuple(tuple(h for h in range(H)
                          if min(max(0, -(-(DH * h + DH - 128) // WIN)), NG - 1) == g)
                    for g in range(NG))
GROUP_OF = {h: g for g in range(NG) for h in GROUP_HEADS[g]}
MROWS = 144
CH = 144
NCH = D // CH
RS = 64
PASS_STEPS = NQB * (D // RS)
FC = 512
LAG = 20
LN_EPS = 1e-5
LOG2E = 1.4426950408889634
QSCALE = (DH ** -0.5) * LOG2E
SAFE_LOGIT = 60.0
SAFE_V = 2.0 ** 50

NN = (((1,), (0,)), ((), ()))
NT = (((1,), (1,)), ((), ()))
TN = (((0,), (0,)), ((), ()))

for _g, _hs in enumerate(GROUP_HEADS):
    for _h in _hs:
        assert WIN * _g <= DH * _h and DH * _h + DH <= WIN * _g + 128


def _dot(a, b, dims=NN):
    return jax.lax.dot_general(a, b, dims, preferred_element_type=F32)


class _Filler:
    def __init__(self, gens, counts):
        self.gens, self.counts, self.done = gens, counts, [0] * len(gens)

    def upto(self, frac):
        for k, gen in enumerate(self.gens):
            while self.done[k] < min(frac, 1.0) * self.counts[k]:
                next(gen, None)
                self.done[k] += 1
            if frac >= 1.0:
                for _ in gen:
                    pass


def _chain(*gens):
    for gen in gens:
        yield from gen


def _phi(t):
    return jnp.where(t > 0, t + 1.0, jnp.exp(t))


def _sigmoid(t):
    return 1.0 / (1.0 + jnp.exp(-t))


def _recip(x):
    r = pl.reciprocal(x, approx=True)
    return r * (2.0 - x * r)


def _kernel(xt_hbm, wq_hbm, wk_hbm, wv_hbm, wo_hbm, beta_ref, wr_ref, wg_hbm, wu_hbm, wdt_hbm,
            out_hbm,
            xbuf, wq_raw, wk_raw, wv_raw, wo_raw, wqt, wkt, wvt, wot, xn, ktn, kb, qt, pkt, pqt,
            vtn, vt32, pbuf, m_f32, m_bf, keep, amem, ot, h_all, hn_sel, yacc, obuf, wg_v, wu_v, wdt_v,
            gcol, wrcol, stat1, stat2, wnorm, r_all, stage, flag, sem_x, sem_w, sem_o):
    class _Group:
        def __init__(self, copies):
            self.copies = copies

        def start(self):
            for cp in self.copies:
                cp.start()

        def wait(self):
            for cp in self.copies:
                cp.wait()

    def hbm_cols(blk):
        return pl.ds(pl.multiple_of(blk * 128, 128), 128)

    def x_copy(s):
        return _Group([pltpu.make_async_copy(xt_hbm.at[:, hbm_cols(s * NQB + i)],
                                             xbuf.at[s * NQB + i], sem_x.at[s])
                       for i in range(NQB)])

    def out_copy(s):
        return _Group([pltpu.make_async_copy(obuf.at[s * NQB + i],
                                             out_hbm.at[:, hbm_cols(s * NQB + i)], sem_o.at[s])
                       for i in range(NQB)])

    cp_wk = pltpu.make_async_copy(wk_hbm, wk_raw, sem_w.at[0])
    cp_wq = pltpu.make_async_copy(wq_hbm, wq_raw, sem_w.at[1])
    cp_wv = pltpu.make_async_copy(wv_hbm, wv_raw, sem_w.at[2])
    cp_wo = pltpu.make_async_copy(wo_hbm, wo_raw, sem_w.at[3])
    cp_wg = pltpu.make_async_copy(wg_hbm, wg_v, sem_w.at[4])
    cp_wu = pltpu.make_async_copy(wu_hbm, wu_v, sem_w.at[5])
    cp_wd = pltpu.make_async_copy(wdt_hbm, wdt_v, sem_w.at[6])

    def fold8(v):
        return jnp.sum(v.reshape(v.shape[0] // 8, 8, 128), axis=0)

    def col_total(acc):
        return jnp.sum(acc, axis=0, keepdims=True) * (1.0 / D)

    def ln1_steps(s):
        seg = jnp.minimum(s, NSEG - 1)
        for c in range(NQB):
            xs = lambda r: xbuf[seg * NQB + c, RS * r:RS * (r + 1), :].astype(F32)
            acc = None
            for r in range(D // RS):
                part = fold8(xs(r))
                acc = part if acc is None else acc + part
                yield
            m = col_total(acc)
            stat1[c, 0:1, :] = m
            acc = None
            for r in range(D // RS):
                xc = xs(r) - m
                part = fold8(xc * xc)
                acc = part if acc is None else acc + part
                yield
            rstd = jax.lax.rsqrt(col_total(acc) + LN_EPS)
            stat1[c, 1:2, :] = rstd
            for r in range(D // RS):
                xn[c, RS * r:RS * (r + 1), :] = (
                    (xs(r) - m) * rstd).astype(BF16)
                yield

    def xn_all():
        return jnp.concatenate([xn[c] for c in range(NQB)], axis=1)

    def rows_of(c):
        return slice(CH * c, CH * (c + 1))

    def transpose_keys(g):
        kb[g] = ktn[WIN * g:WIN * g + 128, :].T

    def proj_k(c):
        kt = _dot(wkt[rows_of(c), :], xn_all())
        pkt[rows_of(c), :] = _phi(kt).astype(BF16)
        ktn[rows_of(c), :] = kt.astype(BF16)
        if c == 0:
            transpose_keys(0)

    def proj_q(c):
        qf = _dot(wqt[rows_of(c), :], xn_all())
        qt[rows_of(c), :] = (qf * QSCALE).astype(BF16)
        pqt[rows_of(c), :] = _phi(qf).astype(BF16)

    def proj_v(c):
        tail = jnp.concatenate([jnp.ones((1, L), F32), jnp.zeros((13, L), F32)], axis=0)
        vt = _dot(wvt[rows_of(c), :], xn_all())
        vtn[rows_of(c), :] = vt.astype(BF16)
        for j in range(CH // DH):
            h = (CH // DH) * c + j
            vt32[32 * h:32 * h + 16, :] = vt[DH * j:DH * j + 16].astype(BF16)
            vt32[32 * h + 16:32 * h + 32, :] = jnp.concatenate(
                [vt[DH * j + 16:DH * j + 18], tail], axis=0).astype(BF16)

    def masked_q(w0, i, word_mask):
        qu = pltpu.bitcast(qt[pl.ds(w0, 128), 128 * i:128 * (i + 1)], U32)
        return pltpu.bitcast(jnp.where(word_mask, qu, jnp.uint32(0)), BF16)

    def head_word_mask(lo):
        word = jax.lax.broadcasted_iota(I32, (64, 128), 0)
        return (2 * word >= lo) & (2 * word < lo + DH)

    def causal_mask():
        return (jax.lax.broadcasted_iota(I32, (128, 128), 0)
                <= jax.lax.broadcasted_iota(I32, (128, 128), 1))

    def pv_head(h, i):
        n = 128 * (i + 1)
        r0 = TOFF[i] * 128
        o = _dot(vt32[32 * h:32 * h + 32, 0:n], pbuf[h, r0:r0 + n, :])
        a = (1.0 - gcol[h:h + 1, :]) * _recip(o[DH:DH + 1, :])
        ot[i, DH * h:DH * h + 24, :] = o[0:24] * a + amem[i, DH * h:DH * h + 24, :]

    def stage_attention_fast(filler):
        causal = causal_mask()
        for h in range(H + LAG):
            if h < H:
                g = GROUP_OF[h]
                word_mask = head_word_mask(DH * h - WIN * g)
                if h == GROUP_HEADS[g][0] and g + 1 < NG:
                    transpose_keys(g + 1)
            for i in range(NQB):
                n = 128 * (i + 1)
                if h < H:
                    filler.upto((NTILE * h + TOFF[i] + i + 1) / (NTILE * (H - 1)))
                    st = _dot(kb[g, 0:n, :], masked_q(WIN * g, i, word_mask))
                    p = jnp.exp2(st)
                    r0 = TOFF[i] * 128
                    if i > 0:
                        pbuf[h, r0:r0 + 128 * i, :] = p[:n - 128].astype(BF16)
                    pbuf[h, r0 + 128 * i:r0 + n, :] = jnp.where(
                        causal, p[n - 128:n], 0.0).astype(BF16)
                if h >= LAG:
                    pv_head(h - LAG, i)

    def stage_scores_safe():
        causal = causal_mask()
        for g in range(1, NG):
            transpose_keys(g)

        def head(h, carry):
            g = jnp.clip((DH * h + DH - 128 + WIN - 1) // WIN, 0, NG - 1)
            g = jnp.where(DH * h + DH <= 128, 0, g)
            w0 = pl.multiple_of(WIN * g, 16)
            word_mask = head_word_mask(DH * h - WIN * g)
            for i in range(NQB):
                n = 128 * (i + 1)
                st = _dot(kb[g, 0:n, :], masked_q(w0, i, word_mask))
                sd = jnp.where(causal, st[n - 128:n], -jnp.inf)
                m = jnp.max(sd, axis=0, keepdims=True)
                if i > 0:
                    m = jnp.maximum(m, jnp.max(st[:n - 128], axis=0, keepdims=True))
                r0 = TOFF[i] * 128
                if i > 0:
                    pbuf[h, r0:r0 + 128 * i, :] = jnp.exp2(st[:n - 128] - m).astype(BF16)
                pbuf[h, r0 + 128 * i:r0 + n, :] = jnp.exp2(sd - m).astype(BF16)
            return carry

        jax.lax.fori_loop(0, H, head, 0)

    def attn_block(s, i):
        blk = s * NQB + i
        otb = ot[i, 0:D, :].astype(BF16)
        tot = None
        for c in range(NCH):
            hh = _dot(wot[rows_of(c), :], otb) + xbuf[blk, rows_of(c), :].astype(F32)
            h_all[blk, rows_of(c), :] = hh
            part = jnp.sum(hh, axis=0, keepdims=True)
            tot = part if tot is None else tot + part
        stat2[blk, 0:1, :] = tot * (1.0 / D)

    def mem_update(g):
        lhs = jnp.concatenate([jnp.ones((16, L), BF16), vtn[WIN * g:WIN * g + 128, :]], axis=0)
        upd = _dot(lhs, pkt[WIN * g:WIN * g + 128, :], NT)
        m_new = m_f32[g] + upd * keep[g]
        m_f32[g] = m_new
        m_bf[g] = m_new.astype(BF16)

    def mem_read(g):
        for i in range(NQB):
            nm = _dot(m_bf[g], pqt[WIN * g:WIN * g + 128, 128 * i:128 * (i + 1)])
            first = GROUP_HEADS[g][0]
            b = gcol[first:first + 8, :] * _recip(nm[0:8, :] + 1e-6)
            for j, h in enumerate(GROUP_HEADS[g]):
                lo = 16 + DH * h - WIN * g
                n = min(24, MROWS - lo)
                amem[i, DH * h:DH * h + n, :] = nm[lo:lo + n] * b[j:j + 1, :]

    def stat_steps(s, blocks=range(NQB)):
        seg = jnp.maximum(s, 0)
        for i in blocks:
            blk = seg * NQB + i
            m = stat2[blk, 0:1, :]
            acc_v = acc_r = None
            for r in range(D // RS):
                rows = slice(RS * r, RS * (r + 1))
                hc = h_all[blk, rows, :] - m
                pv = fold8(hc * hc)
                pr = fold8(hc * wrcol[rows, :])
                acc_v = pv if acc_v is None else acc_v + pv
                acc_r = pr if acc_r is None else acc_r + pr
                yield
            rstd = jax.lax.rsqrt(col_total(acc_v) + LN_EPS)
            stat2[blk, 1:2, :] = rstd
            r_all[pl.ds(blk, 1), :] = jnp.sum(acc_r, axis=0, keepdims=True) * rstd

    def out_steps(s):
        seg = jnp.maximum(s, 0)
        for i in range(NQB):
            blk = seg * NQB + i
            m = stat2[blk, 0:1, :]
            rstd = stat2[blk, 1:2, :]
            for r in range(D // RS):
                rows = slice(RS * r, RS * (r + 1))
                hh = h_all[blk, rows, :]
                obuf[blk, rows, :] = (hh + (hh - m) * rstd).astype(BF16)
                yield

    x_copy(0).start()
    cp_wk.start()

    beta = beta_ref[...].astype(F32).reshape(1, H)
    gpad = jnp.concatenate([_sigmoid(beta), jnp.zeros((1, 128 - H), F32)], axis=1)
    gcol[...] = jnp.transpose(jnp.broadcast_to(gpad, (128, 128)))
    wr = jnp.concatenate([wr_ref[...].astype(F32).reshape(1, D), jnp.zeros((1, 64), F32)], axis=1)
    wrcol[...] = jnp.transpose(jnp.broadcast_to(wr, (128, D + 64)))[0:D]
    row = jax.lax.broadcasted_iota(I32, (MROWS, 128), 0)
    lane = jax.lax.broadcasted_iota(I32, (MROWS, 128), 1)
    for g in range(NG):
        first, nh = GROUP_HEADS[g][0], len(GROUP_HEADS[g])
        lane_head = ((lane + WIN * g) * 3641) >> 16
        row_head = jnp.where(row < 16, row + first, ((row - 16 + WIN * g) * 3641) >> 16)
        ok = (lane_head == row_head) & (row_head >= first) & (row_head < first + nh)
        keep[g] = jnp.where(ok, 1.0, 0.0)
    m_f32[...] = jnp.zeros_like(m_f32)
    amem[...] = jnp.zeros_like(amem)

    h_all[0:NQB] = jnp.zeros((NQB, D, 128), F32)
    stat2[0:NQB] = jnp.zeros((NQB, 8, 128), F32)

    def transpose_tile(dst, raw, t):
        hi = min(128 * (t + 1), D)
        dst[128 * t:hi, :] = raw[:, 128 * t:hi].T

    def col_norm_steps(raw, slot):
        for t in range(5):
            hi = min(128 * (t + 1), D)
            for k in range(3):
                w = raw[192 * k:192 * (k + 1), 128 * t:hi].astype(F32)
                wnorm[slot, 8 * k:8 * (k + 1), 128 * t:hi] = jnp.sum(
                    (w * w).reshape(24, 8, hi - 128 * t), axis=0)
                yield

    x_copy(0).wait()
    cp_wq.start()
    for _ in ln1_steps(0):
        pass
    cp_wk.wait()
    cp_wv.start()
    side = _Filler([col_norm_steps(wk_raw, 0)], [15])
    transpose_tile(wkt, wk_raw, 0)
    transpose_tile(wkt, wk_raw, 1)
    proj_k(0)
    transpose_tile(wkt, wk_raw, 2)
    side.upto(0.5)
    proj_k(1)
    transpose_tile(wkt, wk_raw, 3)
    side.upto(1.0)
    proj_k(2)
    transpose_tile(wkt, wk_raw, 4)
    cp_wq.wait()
    cp_wv.wait()
    cp_wo.start()
    x_copy(1).start()
    transpose_tile(wqt, wq_raw, 0)
    transpose_tile(wqt, wq_raw, 1)
    proj_k(3)
    side = _Filler([col_norm_steps(wq_raw, 1), col_norm_steps(wv_raw, 2)], [15, 15])
    for c in range(NCH):
        proj_q(c)
        if c + 2 < 5:
            transpose_tile(wqt, wq_raw, c + 2)
        if c >= 2:
            transpose_tile(wvt, wv_raw, c - 2)
        if c < NCH - 1:
            side.upto((c + 1) / (NCH - 1))
    cp_wo.wait()
    for s in range(2, NSEG):
        x_copy(s).start()
    cp_wg.start()
    cp_wu.start()
    cp_wd.start()
    for c in range(NCH):
        proj_v(c)
        if c + 2 < 5:
            transpose_tile(wvt, wv_raw, c + 2)
        transpose_tile(wot, wo_raw, c)
    transpose_tile(wot, wo_raw, 4)

    x_copy(1).wait()

    def max_norm(slot):
        ss = jnp.sum(wnorm[slot], axis=0, keepdims=True)
        return jnp.sqrt(jnp.max(ss, axis=1, keepdims=True))

    nk, nq, nv = max_norm(0), max_norm(1), max_norm(2)

    bound = (QSCALE * DH * D) * nq * nk
    safe = (bound <= SAFE_LOGIT) & (nv * (D ** 0.5) <= SAFE_V)
    flag[0] = jnp.sum(jnp.where(safe, 1, 0).astype(I32))

    def segment(s, carry):
        @pl.when(jnp.logical_and(s > 0, s + 1 < NSEG))
        def _():
            x_copy(s + 1).wait()

        def side_work():
            return _Filler([_chain(stat_steps(s - 1), out_steps(s - 1)), ln1_steps(s + 1)],
                           [2 * PASS_STEPS, 3 * PASS_STEPS])

        @pl.when(flag[0] == 1)
        def _():
            stage_attention_fast(side_work())

        @pl.when(flag[0] != 1)
        def _():
            stage_scores_safe()
            side_work().upto(1.0)
            for h in range(H):
                for i in range(NQB):
                    pv_head(h, i)

        @pl.when(s > 0)
        def _():
            out_copy(s - 1).start()

        @pl.when(s + 1 < NSEG)
        def _():
            for i in range(NQB):
                attn_block(s, i)
            for g in range(NG):
                mem_update(g)
            for c in range(NCH):
                proj_q(c)
            for c in range(NCH):
                proj_k(c)
            for g in range(NG):
                mem_read(g)
            for c in range(NCH):
                proj_v(c)

        @pl.when(s + 1 == NSEG)
        def _():
            for i in range(NQB):
                attn_block(s, i)
                if i > 0:
                    for _ in stat_steps(s, [i - 1]):
                        pass
            for _ in stat_steps(s, [NQB - 1]):
                pass

        return carry

    jax.lax.fori_loop(0, NSEG, segment, 0)

    r = r_all[...]
    r_sel = jnp.max(jnp.max(r, axis=0, keepdims=True), axis=1, keepdims=True)
    ids = (128 * jax.lax.broadcasted_iota(I32, r.shape, 0)
           + jax.lax.broadcasted_iota(I32, r.shape, 1))
    cand = jnp.min(jnp.where(r == r_sel, ids, S), axis=0, keepdims=True)
    idx = jnp.minimum(jnp.sum(jnp.min(cand, axis=1, keepdims=True)), S - 1)
    for _ in out_steps(NSEG - 1):
        pass
    out_copy(NSEG - 1).start()
    blk = idx >> 7
    m_sel = stat2[blk, 0:1, :]
    rstd_sel = stat2[blk, 1:2, :]
    for r in range(D // RS):
        rows = slice(RS * r, RS * (r + 1))
        hn_sel[rows, :] = ((h_all[blk, rows, :] - m_sel) * rstd_sel).astype(BF16)
    onehot = (jax.lax.broadcasted_iota(I32, (16, 128), 1) == idx - blk * 128).astype(BF16)
    xs = _dot(onehot, hn_sel[...], NT).astype(BF16)
    cp_wg.wait()
    cp_wu.wait()
    cp_wd.wait()

    def down_steps(c, act):
        for r in range(D // RS):
            rows = slice(RS * r, RS * (r + 1))
            part = None if c == 0 else yacc[rows, :]
            for t in range(FC // 128):
                w = wdt_v[rows, FC * c + 128 * t:FC * c + 128 * (t + 1)].astype(F32)
                part = w * act[t] if part is None else part + w * act[t]
            yacc[rows, :] = part
            yield

    nch = FF // FC
    pending = None
    for c in range(nch):
        ga, up = [], []
        for t in range(FC // 128):
            tile = slice(FC * c + 128 * t, FC * c + 128 * (t + 1))
            ga.append(_dot(xs, wg_v[:, tile])[0:1])
            up.append(_dot(xs, wu_v[:, tile])[0:1])
            if pending is not None:
                pending.upto((t + 1) / (FC // 128))
        act = [g * _sigmoid(g) * u for g, u in zip(ga, up)]
        pending = _Filler([down_steps(c, act)], [D // RS])
    pending.upto(1.0)
    y = jnp.sum(yacc[...], axis=1, keepdims=True) * _sigmoid(r_sel)
    sel = jax.lax.broadcasted_iota(I32, (RS, 128), 1) == idx - blk * 128
    for r in range(D // RS):
        rows = slice(RS * r, RS * (r + 1))
        hh = h_all[blk, rows, :]
        stage[rows, :] = (hh + (hh - m_sel) * rstd_sel
                          + jnp.where(sel, y[rows], 0.0)).astype(BF16)
    for s in range(NSEG):
        out_copy(s).wait()
    fix = pltpu.make_async_copy(stage, out_hbm.at[:, hbm_cols(blk)], sem_w.at[7])
    fix.start()
    fix.wait()


@jax.jit
def pallas_sequential_preLN__memory_aug_infini_attn__moe_arch_mod__prompt_kernel(
    A_x: jax.Array,
    A_wq: jax.Array,
    A_wk: jax.Array,
    A_wv: jax.Array,
    A_wo: jax.Array,
    A_beta: jax.Array,
    B_x: jax.Array,
    B_w_r: jax.Array,
    B_w_gate: jax.Array,
    B_w_up: jax.Array,
    B_w_down: jax.Array,
):
    del B_x
    hbm = pl.BlockSpec(memory_space=pltpu.HBM)
    vmem = pl.BlockSpec(memory_space=pltpu.VMEM)
    scratch = [
        pltpu.VMEM((NSEG * NQB, D, 128), BF16),
        pltpu.VMEM((D, D), BF16),
        pltpu.VMEM((D, D), BF16),
        pltpu.VMEM((D, D), BF16),
        pltpu.VMEM((D, D), BF16),
        pltpu.VMEM((D, D), BF16),
        pltpu.VMEM((D, D), BF16),
        pltpu.VMEM((D, D), BF16),
        pltpu.VMEM((D, D), BF16),
        pltpu.VMEM((NQB, D, 128), BF16),
        pltpu.VMEM((D, L), BF16),
        pltpu.VMEM((NG, L, 128), BF16),
        pltpu.VMEM((D, L), BF16),
        pltpu.VMEM((D, L), BF16),
        pltpu.VMEM((D, L), BF16),
        pltpu.VMEM((D, L), BF16),
        pltpu.VMEM((H * 32, L), BF16),
        pltpu.VMEM((H, NTILE * 128, 128), BF16),
        pltpu.VMEM((NG, MROWS, 128), F32),
        pltpu.VMEM((NG, MROWS, 128), BF16),
        pltpu.VMEM((NG, MROWS, 128), F32),
        pltpu.VMEM((NQB, D + 24, 128), F32),
        pltpu.VMEM((NQB, D + 24, 128), F32),
        pltpu.VMEM((NSEG * NQB, D, 128), F32),
        pltpu.VMEM((D, 128), BF16),
        pltpu.VMEM((D, 128), F32),
        pltpu.VMEM((NSEG * NQB, D, 128), BF16),
        pltpu.VMEM((D, FF), BF16),
        pltpu.VMEM((D, FF), BF16),
        pltpu.VMEM((D, FF), BF16),
        pltpu.VMEM((128, 128), F32),
        pltpu.VMEM((D, 128), F32),
        pltpu.VMEM((NQB, 8, 128), F32),
        pltpu.VMEM((NSEG * NQB, 8, 128), F32),
        pltpu.VMEM((3, 24, D), F32),
        pltpu.VMEM((NSEG * NQB, 128), F32),
        pltpu.VMEM((D, 128), BF16),
        pltpu.SMEM((1,), I32),
        pltpu.SemaphoreType.DMA((NSEG,)),
        pltpu.SemaphoreType.DMA((8,)),
        pltpu.SemaphoreType.DMA((NSEG,)),
    ]
    out_t = pl.pallas_call(
        _kernel,
        out_shape=jax.ShapeDtypeStruct((D, S), BF16),
        in_specs=[hbm, hbm, hbm, hbm, hbm, vmem, vmem, hbm, hbm, hbm],
        out_specs=hbm,
        scratch_shapes=scratch,
        compiler_params=pltpu.CompilerParams(vmem_limit_bytes=100 * 1024 * 1024),
        name="infini_moe",
    )(A_x.reshape(S, D).T, A_wq, A_wk, A_wv, A_wo, A_beta, B_w_r, B_w_gate, B_w_up, B_w_down.T)
    return out_t.T.reshape(1, S, D)
```

```python
import functools

import jax
import jax.numpy as jnp
import jax.experimental.pallas as pl
import jax.experimental.pallas.tpu as pltpu

F32 = jnp.float32
BF16 = jnp.bfloat16
U32 = jnp.uint32
I32 = jnp.int32

S = 2048
D = 576
H = 32
DH = 18
NSEG = 4
L = S // NSEG
FF = 4608
NQB = L // 128
TOFF = (0, 1, 3, 6)
NTILE = 10
NG = 5
WIN = 112
GROUP_HEADS = tuple(tuple(h for h in range(H)
                          if min(max(0, -(-(DH * h + DH - 128) // WIN)), NG - 1) == g)
                    for g in range(NG))
GROUP_OF = {h: g for g in range(NG) for h in GROUP_HEADS[g]}
MROWS = 144
CH = 144
NCH = D // CH
RS = 64
PASS_STEPS = NQB * (D // RS)
FC = 512
LAG = 20
LN_EPS = 1e-5
LOG2E = 1.4426950408889634
QSCALE = (DH ** -0.5) * LOG2E
SAFE_LOGIT = 60.0
SAFE_V = 2.0 ** 50

NN = (((1,), (0,)), ((), ()))
NT = (((1,), (1,)), ((), ()))
TN = (((0,), (0,)), ((), ()))

for _g, _hs in enumerate(GROUP_HEADS):
    for _h in _hs:
        assert WIN * _g <= DH * _h and DH * _h + DH <= WIN * _g + 128


def _dot(a, b, dims=NN):
    return jax.lax.dot_general(a, b, dims, preferred_element_type=F32)


class _Filler:
    def __init__(self, gens, counts):
        self.gens, self.counts, self.done = gens, counts, [0] * len(gens)

    def upto(self, frac):
        for k, gen in enumerate(self.gens):
            while self.done[k] < min(frac, 1.0) * self.counts[k]:
                next(gen, None)
                self.done[k] += 1
            if frac >= 1.0:
                for _ in gen:
                    pass


def _chain(*gens):
    for gen in gens:
        yield from gen


def _phi(t):
    return jnp.where(t > 0, t + 1.0, jnp.exp(t))


def _sigmoid(t):
    return 1.0 / (1.0 + jnp.exp(-t))


def _recip(x):
    r = pl.reciprocal(x, approx=True)
    return r * (2.0 - x * r)


def _kernel(xt_hbm, wq_hbm, wk_hbm, wv_hbm, wo_hbm, beta_ref, wr_ref, wg_hbm, wu_hbm, wdt_hbm,
            out_hbm,
            xbuf, wq_raw, wk_raw, wv_raw, wo_raw, wqt, wkt, wvt, wot, xn, ktn, kb, qt, pkt, pqt,
            vtn, vt32, pbuf, m_f32, m_bf, keep, amem, ot, h_all, hn_sel, yacc, obuf, wg_v, wu_v, wdt_v,
            gcol, omg, wrcol, stat1, stat2, wnorm, r_all, stage, flag, sem_x, sem_w, sem_o):
    class _Group:
        def __init__(self, copies):
            self.copies = copies

        def start(self):
            for cp in self.copies:
                cp.start()

        def wait(self):
            for cp in self.copies:
                cp.wait()

    def hbm_cols(blk):
        return pl.ds(pl.multiple_of(blk * 128, 128), 128)

    def x_copy(s):
        return _Group([pltpu.make_async_copy(xt_hbm.at[:, hbm_cols(s * NQB + i)],
                                             xbuf.at[s * NQB + i], sem_x.at[s])
                       for i in range(NQB)])

    def out_copy(s):
        return _Group([pltpu.make_async_copy(obuf.at[s * NQB + i],
                                             out_hbm.at[:, hbm_cols(s * NQB + i)], sem_o.at[s])
                       for i in range(NQB)])

    cp_wk = pltpu.make_async_copy(wk_hbm, wk_raw, sem_w.at[0])
    cp_wq = pltpu.make_async_copy(wq_hbm, wq_raw, sem_w.at[1])
    cp_wv = pltpu.make_async_copy(wv_hbm, wv_raw, sem_w.at[2])
    cp_wo = pltpu.make_async_copy(wo_hbm, wo_raw, sem_w.at[3])
    cp_wg = pltpu.make_async_copy(wg_hbm, wg_v, sem_w.at[4])
    cp_wu = pltpu.make_async_copy(wu_hbm, wu_v, sem_w.at[5])
    cp_wd = pltpu.make_async_copy(wdt_hbm, wdt_v, sem_w.at[6])

    def fold8(v):
        return jnp.sum(v.reshape(v.shape[0] // 8, 8, 128), axis=0)

    def col_total(acc):
        return jnp.sum(acc, axis=0, keepdims=True) * (1.0 / D)

    def ln1_steps(s):
        seg = jnp.minimum(s, NSEG - 1)
        for c in range(NQB):
            xs = lambda r: xbuf[seg * NQB + c, RS * r:RS * (r + 1), :].astype(F32)
            acc = None
            for r in range(D // RS):
                part = fold8(xs(r))
                acc = part if acc is None else acc + part
                yield
            m = col_total(acc)
            stat1[c, 0:1, :] = m
            acc = None
            for r in range(D // RS):
                xc = xs(r) - m
                part = fold8(xc * xc)
                acc = part if acc is None else acc + part
                yield
            rstd = jax.lax.rsqrt(col_total(acc) + LN_EPS)
            stat1[c, 1:2, :] = rstd
            for r in range(D // RS):
                xn[c, RS * r:RS * (r + 1), :] = (
                    (xs(r) - m) * rstd).astype(BF16)
                yield

    def xn_all():
        return jnp.concatenate([xn[c] for c in range(NQB)], axis=1)

    def rows_of(c):
        return slice(CH * c, CH * (c + 1))

    def transpose_keys(g):
        kb[g] = ktn[WIN * g:WIN * g + 128, :].T

    def proj_k(c):
        kt = _dot(wkt[rows_of(c), :], xn_all())
        pkt[rows_of(c), :] = _phi(kt).astype(BF16)
        ktn[rows_of(c), :] = kt.astype(BF16)
        if c == 0:
            transpose_keys(0)

    def proj_q(c):
        qf = _dot(wqt[rows_of(c), :], xn_all())
        qt[rows_of(c), :] = (qf * QSCALE).astype(BF16)
        pqt[rows_of(c), :] = _phi(qf).astype(BF16)

    def proj_v(c):
        tail = jnp.concatenate([jnp.zeros((6, L), F32), jnp.ones((8, L), F32)], axis=0)
        vt = _dot(wvt[rows_of(c), :], xn_all())
        vtn[rows_of(c), :] = vt.astype(BF16)
        for j in range(CH // DH):
            h = (CH // DH) * c + j
            vt32[32 * h:32 * h + 16, :] = vt[DH * j:DH * j + 16].astype(BF16)
            vt32[32 * h + 16:32 * h + 32, :] = jnp.concatenate(
                [vt[DH * j + 16:DH * j + 18], tail], axis=0).astype(BF16)

    def masked_q(w0, i, word_mask):
        qu = pltpu.bitcast(qt[pl.ds(w0, 128), 128 * i:128 * (i + 1)], U32)
        return pltpu.bitcast(jnp.where(word_mask, qu, jnp.uint32(0)), BF16)

    def head_word_mask(lo):
        word = jax.lax.broadcasted_iota(I32, (64, 128), 0)
        return (2 * word >= lo) & (2 * word < lo + DH)

    def causal_mask():
        return (jax.lax.broadcasted_iota(I32, (128, 128), 0)
                <= jax.lax.broadcasted_iota(I32, (128, 128), 1))

    def pv_head(h, i):
        n = 128 * (i + 1)
        r0 = TOFF[i] * 128
        o = _dot(vt32[32 * h:32 * h + 32, 0:n], pbuf[h, r0:r0 + n, :])
        a = omg[h] * _recip(o[24:32, :])
        on = (o[0:24].reshape(3, 8, 128) * a).reshape(24, 128)
        ot[i, DH * h:DH * h + 24, :] = on + amem[i, DH * h:DH * h + 24, :]

    def stage_attention_fast(filler):
        causal = causal_mask()
        for h in range(H + LAG):
            if h < H:
                g = GROUP_OF[h]
                word_mask = head_word_mask(DH * h - WIN * g)
                if h == GROUP_HEADS[g][0] and g + 1 < NG:
                    transpose_keys(g + 1)
            for i in range(NQB):
                n = 128 * (i + 1)
                if h < H:
                    filler.upto((NTILE * h + TOFF[i] + i + 1) / (NTILE * (H - 1)))
                    st = _dot(kb[g, 0:n, :], masked_q(WIN * g, i, word_mask))
                    p = jnp.exp2(st)
                    r0 = TOFF[i] * 128
                    if i > 0:
                        pbuf[h, r0:r0 + 128 * i, :] = p[:n - 128].astype(BF16)
                    pbuf[h, r0 + 128 * i:r0 + n, :] = jnp.where(
                        causal, p[n - 128:n], 0.0).astype(BF16)
                if h >= LAG:
                    pv_head(h - LAG, i)

    def stage_scores_safe():
        causal = causal_mask()
        for g in range(1, NG):
            transpose_keys(g)

        def head(h, carry):
            g = jnp.clip((DH * h + DH - 128 + WIN - 1) // WIN, 0, NG - 1)
            g = jnp.where(DH * h + DH <= 128, 0, g)
            w0 = pl.multiple_of(WIN * g, 16)
            word_mask = head_word_mask(DH * h - WIN * g)
            for i in range(NQB):
                n = 128 * (i + 1)
                st = _dot(kb[g, 0:n, :], masked_q(w0, i, word_mask))
                sd = jnp.where(causal, st[n - 128:n], -jnp.inf)
                m = jnp.max(sd, axis=0, keepdims=True)
                if i > 0:
                    m = jnp.maximum(m, jnp.max(st[:n - 128], axis=0, keepdims=True))
                r0 = TOFF[i] * 128
                if i > 0:
                    pbuf[h, r0:r0 + 128 * i, :] = jnp.exp2(st[:n - 128] - m).astype(BF16)
                pbuf[h, r0 + 128 * i:r0 + n, :] = jnp.exp2(sd - m).astype(BF16)
            return carry

        jax.lax.fori_loop(0, H, head, 0)

    def attn_block(s, i):
        blk = s * NQB + i
        otb = ot[i, 0:D, :].astype(BF16)
        tot = None
        for c in range(NCH):
            hh = _dot(wot[rows_of(c), :], otb) + xbuf[blk, rows_of(c), :].astype(F32)
            h_all[blk, rows_of(c), :] = hh
            part = jnp.sum(hh, axis=0, keepdims=True)
            tot = part if tot is None else tot + part
        stat2[blk, 0:1, :] = tot * (1.0 / D)

    def mem_update(g):
        lhs = jnp.concatenate([jnp.ones((16, L), BF16), vtn[WIN * g:WIN * g + 128, :]], axis=0)
        upd = _dot(lhs, pkt[WIN * g:WIN * g + 128, :], NT)
        m_new = m_f32[g] + upd * keep[g]
        m_f32[g] = m_new
        m_bf[g] = m_new.astype(BF16)

    def mem_read(g):
        for i in range(NQB):
            nm = _dot(m_bf[g], pqt[WIN * g:WIN * g + 128, 128 * i:128 * (i + 1)])
            first = GROUP_HEADS[g][0]
            b = gcol[first:first + 8, :] * _recip(nm[0:8, :] + 1e-6)
            for j, h in enumerate(GROUP_HEADS[g]):
                lo = 16 + DH * h - WIN * g
                n = min(24, MROWS - lo)
                amem[i, DH * h:DH * h + n, :] = nm[lo:lo + n] * b[j:j + 1, :]

    def stat_steps(s, blocks=range(NQB)):
        seg = jnp.maximum(s, 0)
        for i in blocks:
            blk = seg * NQB + i
            m = stat2[blk, 0:1, :]
            acc_v = acc_r = None
            for r in range(D // RS):
                rows = slice(RS * r, RS * (r + 1))
                hc = h_all[blk, rows, :] - m
                pv = fold8(hc * hc)
                pr = fold8(hc * wrcol[rows, :])
                acc_v = pv if acc_v is None else acc_v + pv
                acc_r = pr if acc_r is None else acc_r + pr
                yield
            rstd = jax.lax.rsqrt(col_total(acc_v) + LN_EPS)
            stat2[blk, 1:2, :] = rstd
            r_all[pl.ds(blk, 1), :] = jnp.sum(acc_r, axis=0, keepdims=True) * rstd

    def out_steps(s):
        seg = jnp.maximum(s, 0)
        for i in range(NQB):
            blk = seg * NQB + i
            m = stat2[blk, 0:1, :]
            rstd = stat2[blk, 1:2, :]
            for r in range(D // RS):
                rows = slice(RS * r, RS * (r + 1))
                hh = h_all[blk, rows, :]
                obuf[blk, rows, :] = (hh + (hh - m) * rstd).astype(BF16)
                yield

    x_copy(0).start()
    cp_wk.start()

    beta = beta_ref[...].astype(F32).reshape(1, H)
    gpad = jnp.concatenate([_sigmoid(beta), jnp.zeros((1, 128 - H), F32)], axis=1)
    gcol[...] = jnp.transpose(jnp.broadcast_to(gpad, (128, 128)))
    for h in range(H):
        omg[h] = jnp.broadcast_to(1.0 - gcol[h:h + 1, :], (8, 128))
    wr = jnp.concatenate([wr_ref[...].astype(F32).reshape(1, D), jnp.zeros((1, 64), F32)], axis=1)
    wrcol[...] = jnp.transpose(jnp.broadcast_to(wr, (128, D + 64)))[0:D]
    row = jax.lax.broadcasted_iota(I32, (MROWS, 128), 0)
    lane = jax.lax.broadcasted_iota(I32, (MROWS, 128), 1)
    for g in range(NG):
        first, nh = GROUP_HEADS[g][0], len(GROUP_HEADS[g])
        lane_head = ((lane + WIN * g) * 3641) >> 16
        row_head = jnp.where(row < 16, row + first, ((row - 16 + WIN * g) * 3641) >> 16)
        ok = (lane_head == row_head) & (row_head >= first) & (row_head < first + nh)
        keep[g] = jnp.where(ok, 1.0, 0.0)
    m_f32[...] = jnp.zeros_like(m_f32)
    amem[...] = jnp.zeros_like(amem)

    h_all[0:NQB] = jnp.zeros((NQB, D, 128), F32)
    stat2[0:NQB] = jnp.zeros((NQB, 8, 128), F32)

    def transpose_tile(dst, raw, t):
        hi = min(128 * (t + 1), D)
        dst[128 * t:hi, :] = raw[:, 128 * t:hi].T

    def col_norm_steps(raw, slot):
        for t in range(5):
            hi = min(128 * (t + 1), D)
            for k in range(3):
                w = raw[192 * k:192 * (k + 1), 128 * t:hi].astype(F32)
                wnorm[slot, 8 * k:8 * (k + 1), 128 * t:hi] = jnp.sum(
                    (w * w).reshape(24, 8, hi - 128 * t), axis=0)
                yield

    x_copy(0).wait()
    cp_wq.start()
    for _ in ln1_steps(0):
        pass
    cp_wk.wait()
    cp_wv.start()
    side = _Filler([col_norm_steps(wk_raw, 0)], [15])
    transpose_tile(wkt, wk_raw, 0)
    transpose_tile(wkt, wk_raw, 1)
    proj_k(0)
    transpose_tile(wkt, wk_raw, 2)
    side.upto(0.5)
    proj_k(1)
    transpose_tile(wkt, wk_raw, 3)
    side.upto(1.0)
    proj_k(2)
    transpose_tile(wkt, wk_raw, 4)
    cp_wq.wait()
    cp_wv.wait()
    cp_wo.start()
    x_copy(1).start()
    transpose_tile(wqt, wq_raw, 0)
    transpose_tile(wqt, wq_raw, 1)
    proj_k(3)
    side = _Filler([col_norm_steps(wq_raw, 1), col_norm_steps(wv_raw, 2)], [15, 15])
    for c in range(NCH):
        proj_q(c)
        if c + 2 < 5:
            transpose_tile(wqt, wq_raw, c + 2)
        if c >= 2:
            transpose_tile(wvt, wv_raw, c - 2)
        if c < NCH - 1:
            side.upto((c + 1) / (NCH - 1))
    cp_wo.wait()
    for s in range(2, NSEG):
        x_copy(s).start()
    cp_wg.start()
    cp_wu.start()
    cp_wd.start()
    for c in range(NCH):
        proj_v(c)
        if c + 2 < 5:
            transpose_tile(wvt, wv_raw, c + 2)
        transpose_tile(wot, wo_raw, c)
    transpose_tile(wot, wo_raw, 4)

    x_copy(1).wait()

    def max_norm(slot):
        ss = jnp.sum(wnorm[slot], axis=0, keepdims=True)
        return jnp.sqrt(jnp.max(ss, axis=1, keepdims=True))

    nk, nq, nv = max_norm(0), max_norm(1), max_norm(2)

    bound = (QSCALE * DH * D) * nq * nk
    safe = (bound <= SAFE_LOGIT) & (nv * (D ** 0.5) <= SAFE_V)
    flag[0] = jnp.sum(jnp.where(safe, 1, 0).astype(I32))

    def segment(s, carry):
        @pl.when(jnp.logical_and(s > 0, s + 1 < NSEG))
        def _():
            x_copy(s + 1).wait()

        def side_work():
            return _Filler([_chain(stat_steps(s - 1), out_steps(s - 1)), ln1_steps(s + 1)],
                           [2 * PASS_STEPS, 3 * PASS_STEPS])

        @pl.when(flag[0] == 1)
        def _():
            stage_attention_fast(side_work())

        @pl.when(flag[0] != 1)
        def _():
            stage_scores_safe()
            side_work().upto(1.0)
            for h in range(H):
                for i in range(NQB):
                    pv_head(h, i)

        @pl.when(s > 0)
        def _():
            out_copy(s - 1).start()

        @pl.when(s + 1 < NSEG)
        def _():
            for i in range(NQB):
                attn_block(s, i)
            for g in range(NG):
                mem_update(g)
            for c in range(NCH):
                proj_q(c)
            for c in range(NCH):
                proj_k(c)
            for g in range(NG):
                mem_read(g)
            for c in range(NCH):
                proj_v(c)

        @pl.when(s + 1 == NSEG)
        def _():
            for i in range(NQB):
                attn_block(s, i)
                if i > 0:
                    for _ in stat_steps(s, [i - 1]):
                        pass
            for _ in stat_steps(s, [NQB - 1]):
                pass

        return carry

    jax.lax.fori_loop(0, NSEG, segment, 0)

    r = r_all[...]
    r_sel = jnp.max(jnp.max(r, axis=0, keepdims=True), axis=1, keepdims=True)
    ids = (128 * jax.lax.broadcasted_iota(I32, r.shape, 0)
           + jax.lax.broadcasted_iota(I32, r.shape, 1))
    cand = jnp.min(jnp.where(r == r_sel, ids, S), axis=0, keepdims=True)
    idx = jnp.minimum(jnp.sum(jnp.min(cand, axis=1, keepdims=True)), S - 1)
    for _ in out_steps(NSEG - 1):
        pass
    out_copy(NSEG - 1).start()
    blk = idx >> 7
    m_sel = stat2[blk, 0:1, :]
    rstd_sel = stat2[blk, 1:2, :]
    for r in range(D // RS):
        rows = slice(RS * r, RS * (r + 1))
        hn_sel[rows, :] = ((h_all[blk, rows, :] - m_sel) * rstd_sel).astype(BF16)
    onehot = (jax.lax.broadcasted_iota(I32, (16, 128), 1) == idx - blk * 128).astype(BF16)
    xs = _dot(onehot, hn_sel[...], NT).astype(BF16)
    cp_wg.wait()
    cp_wu.wait()
    cp_wd.wait()

    def down_steps(c, act):
        for r in range(D // RS):
            rows = slice(RS * r, RS * (r + 1))
            part = None if c == 0 else yacc[rows, :]
            for t in range(FC // 128):
                w = wdt_v[rows, FC * c + 128 * t:FC * c + 128 * (t + 1)].astype(F32)
                part = w * act[t] if part is None else part + w * act[t]
            yacc[rows, :] = part
            yield

    nch = FF // FC
    pending = None
    for c in range(nch):
        ga, up = [], []
        for t in range(FC // 128):
            tile = slice(FC * c + 128 * t, FC * c + 128 * (t + 1))
            ga.append(_dot(xs, wg_v[:, tile])[0:1])
            up.append(_dot(xs, wu_v[:, tile])[0:1])
            if pending is not None:
                pending.upto((t + 1) / (FC // 128))
        act = [g * _sigmoid(g) * u for g, u in zip(ga, up)]
        pending = _Filler([down_steps(c, act)], [D // RS])
    pending.upto(1.0)
    y = jnp.sum(yacc[...], axis=1, keepdims=True) * _sigmoid(r_sel)
    sel = jax.lax.broadcasted_iota(I32, (RS, 128), 1) == idx - blk * 128
    for r in range(D // RS):
        rows = slice(RS * r, RS * (r + 1))
        hh = h_all[blk, rows, :]
        stage[rows, :] = (hh + (hh - m_sel) * rstd_sel
                          + jnp.where(sel, y[rows], 0.0)).astype(BF16)
    for s in range(NSEG):
        out_copy(s).wait()
    fix = pltpu.make_async_copy(stage, out_hbm.at[:, hbm_cols(blk)], sem_w.at[7])
    fix.start()
    fix.wait()


@jax.jit
def pallas_sequential_preLN__memory_aug_infini_attn__moe_arch_mod__prompt_kernel(
    A_x: jax.Array,
    A_wq: jax.Array,
    A_wk: jax.Array,
    A_wv: jax.Array,
    A_wo: jax.Array,
    A_beta: jax.Array,
    B_x: jax.Array,
    B_w_r: jax.Array,
    B_w_gate: jax.Array,
    B_w_up: jax.Array,
    B_w_down: jax.Array,
):
    del B_x
    hbm = pl.BlockSpec(memory_space=pltpu.HBM)
    vmem = pl.BlockSpec(memory_space=pltpu.VMEM)
    scratch = [
        pltpu.VMEM((NSEG * NQB, D, 128), BF16),
        pltpu.VMEM((D, D), BF16),
        pltpu.VMEM((D, D), BF16),
        pltpu.VMEM((D, D), BF16),
        pltpu.VMEM((D, D), BF16),
        pltpu.VMEM((D, D), BF16),
        pltpu.VMEM((D, D), BF16),
        pltpu.VMEM((D, D), BF16),
        pltpu.VMEM((D, D), BF16),
        pltpu.VMEM((NQB, D, 128), BF16),
        pltpu.VMEM((D, L), BF16),
        pltpu.VMEM((NG, L, 128), BF16),
        pltpu.VMEM((D, L), BF16),
        pltpu.VMEM((D, L), BF16),
        pltpu.VMEM((D, L), BF16),
        pltpu.VMEM((D, L), BF16),
        pltpu.VMEM((H * 32, L), BF16),
        pltpu.VMEM((H, NTILE * 128, 128), BF16),
        pltpu.VMEM((NG, MROWS, 128), F32),
        pltpu.VMEM((NG, MROWS, 128), BF16),
        pltpu.VMEM((NG, MROWS, 128), F32),
        pltpu.VMEM((NQB, D + 24, 128), F32),
        pltpu.VMEM((NQB, D + 24, 128), F32),
        pltpu.VMEM((NSEG * NQB, D, 128), F32),
        pltpu.VMEM((D, 128), BF16),
        pltpu.VMEM((D, 128), F32),
        pltpu.VMEM((NSEG * NQB, D, 128), BF16),
        pltpu.VMEM((D, FF), BF16),
        pltpu.VMEM((D, FF), BF16),
        pltpu.VMEM((D, FF), BF16),
        pltpu.VMEM((128, 128), F32),
        pltpu.VMEM((H, 8, 128), F32),
        pltpu.VMEM((D, 128), F32),
        pltpu.VMEM((NQB, 8, 128), F32),
        pltpu.VMEM((NSEG * NQB, 8, 128), F32),
        pltpu.VMEM((3, 24, D), F32),
        pltpu.VMEM((NSEG * NQB, 128), F32),
        pltpu.VMEM((D, 128), BF16),
        pltpu.SMEM((1,), I32),
        pltpu.SemaphoreType.DMA((NSEG,)),
        pltpu.SemaphoreType.DMA((8,)),
        pltpu.SemaphoreType.DMA((NSEG,)),
    ]
    out_t = pl.pallas_call(
        _kernel,
        out_shape=jax.ShapeDtypeStruct((D, S), BF16),
        in_specs=[hbm, hbm, hbm, hbm, hbm, vmem, vmem, hbm, hbm, hbm],
        out_specs=hbm,
        scratch_shapes=scratch,
        compiler_params=pltpu.CompilerParams(vmem_limit_bytes=100 * 1024 * 1024),
        name="infini_moe",
    )(A_x.reshape(S, D).T, A_wq, A_wk, A_wv, A_wo, A_beta, B_w_r, B_w_gate, B_w_up, B_w_down.T)
    return out_t.T.reshape(1, S, D)
```

```python
import functools

import jax
import jax.numpy as jnp
import jax.experimental.pallas as pl
import jax.experimental.pallas.tpu as pltpu

F32 = jnp.float32
BF16 = jnp.bfloat16
U32 = jnp.uint32
I32 = jnp.int32

S = 2048
D = 576
H = 32
DH = 18
NSEG = 4
L = S // NSEG
FF = 4608
NQB = L // 128
TOFF = (0, 1, 3, 6)
NTILE = 10
NG = 5
WIN = 112
GROUP_HEADS = tuple(tuple(h for h in range(H)
                          if min(max(0, -(-(DH * h + DH - 128) // WIN)), NG - 1) == g)
                    for g in range(NG))
GROUP_OF = {h: g for g in range(NG) for h in GROUP_HEADS[g]}
MROWS = 144
CH = 144
NCH = D // CH
RS = 64
PASS_STEPS = NQB * (D // RS)
FC = 512
LAG = 20
LN_EPS = 1e-5
LOG2E = 1.4426950408889634
QSCALE = (DH ** -0.5) * LOG2E
SAFE_LOGIT = 60.0
SAFE_V = 2.0 ** 50

NN = (((1,), (0,)), ((), ()))
NT = (((1,), (1,)), ((), ()))
TN = (((0,), (0,)), ((), ()))

for _g, _hs in enumerate(GROUP_HEADS):
    for _h in _hs:
        assert WIN * _g <= DH * _h and DH * _h + DH <= WIN * _g + 128


def _dot(a, b, dims=NN):
    return jax.lax.dot_general(a, b, dims, preferred_element_type=F32)


class _Filler:
    def __init__(self, gens, counts):
        self.gens, self.counts, self.done = gens, counts, [0] * len(gens)

    def upto(self, frac):
        for k, gen in enumerate(self.gens):
            while self.done[k] < min(frac, 1.0) * self.counts[k]:
                next(gen, None)
                self.done[k] += 1
            if frac >= 1.0:
                for _ in gen:
                    pass


def _chain(*gens):
    for gen in gens:
        yield from gen


def _phi(t):
    return jnp.where(t > 0, t + 1.0, jnp.exp(t))


def _sigmoid(t):
    return 1.0 / (1.0 + jnp.exp(-t))


def _recip(x):
    r = pl.reciprocal(x, approx=True)
    return r * (2.0 - x * r)


def _kernel(xt_hbm, wq_hbm, wk_hbm, wv_hbm, wo_hbm, beta_ref, wr_ref, wg_hbm, wu_hbm, wdt_hbm,
            out_hbm,
            xbuf, wq_raw, wk_raw, wv_raw, wo_raw, wqt, wkt, wvt, wot, xn, ktn, kb, qt, pkt, pqt,
            vtn, vt32, pbuf, m_f32, m_bf, keep, amem, ot, h_all, hn_sel, yacc, obuf, wg_v, wu_v, wdt_v,
            gcol, omg, wrcol, stat1, stat2, wnorm, r_all, stage, flag, sem_x, sem_w, sem_o):
    class _Group:
        def __init__(self, copies):
            self.copies = copies

        def start(self):
            for cp in self.copies:
                cp.start()

        def wait(self):
            for cp in self.copies:
                cp.wait()

    def hbm_cols(blk):
        return pl.ds(pl.multiple_of(blk * 128, 128), 128)

    def x_copy(s):
        return _Group([pltpu.make_async_copy(xt_hbm.at[:, hbm_cols(s * NQB + i)],
                                             xbuf.at[s * NQB + i], sem_x.at[s])
                       for i in range(NQB)])

    def out_copy(s):
        return _Group([pltpu.make_async_copy(obuf.at[s * NQB + i],
                                             out_hbm.at[:, hbm_cols(s * NQB + i)], sem_o.at[s])
                       for i in range(NQB)])

    cp_wk = pltpu.make_async_copy(wk_hbm, wk_raw, sem_w.at[0])
    cp_wq = pltpu.make_async_copy(wq_hbm, wq_raw, sem_w.at[1])
    cp_wv = pltpu.make_async_copy(wv_hbm, wv_raw, sem_w.at[2])
    cp_wo = pltpu.make_async_copy(wo_hbm, wo_raw, sem_w.at[3])
    cp_wg = pltpu.make_async_copy(wg_hbm, wg_v, sem_w.at[4])
    cp_wu = pltpu.make_async_copy(wu_hbm, wu_v, sem_w.at[5])
    cp_wd = pltpu.make_async_copy(wdt_hbm, wdt_v, sem_w.at[6])

    def fold8(v):
        return jnp.sum(v.reshape(v.shape[0] // 8, 8, 128), axis=0)

    def col_total(acc):
        return jnp.sum(acc, axis=0, keepdims=True) * (1.0 / D)

    def ln1_steps(s):
        seg = jnp.minimum(s, NSEG - 1)
        for c in range(NQB):
            xs = lambda r: xbuf[seg * NQB + c, RS * r:RS * (r + 1), :].astype(F32)
            acc = None
            for r in range(D // RS):
                part = fold8(xs(r))
                acc = part if acc is None else acc + part
                yield
            m = col_total(acc)
            stat1[c, 0:1, :] = m
            acc = None
            for r in range(D // RS):
                xc = xs(r) - m
                part = fold8(xc * xc)
                acc = part if acc is None else acc + part
                yield
            rstd = jax.lax.rsqrt(col_total(acc) + LN_EPS)
            stat1[c, 1:2, :] = rstd
            for r in range(D // RS):
                xn[c, RS * r:RS * (r + 1), :] = (
                    (xs(r) - m) * rstd).astype(BF16)
                yield

    def xn_all():
        return jnp.concatenate([xn[c] for c in range(NQB)], axis=1)

    def rows_of(c):
        return slice(CH * c, CH * (c + 1))

    def packed(words):
        return pltpu.bitcast(words, BF16)

    def wt_rows(wt, c):
        return packed(wt[CH // 2 * c:CH // 2 * (c + 1), :])

    def transpose_keys(g):
        kb[g] = pltpu.bitcast(ktn[WIN * g:WIN * g + 128, :].T, U32)

    def proj_k(c):
        kt = _dot(wt_rows(wkt, c), xn_all())
        pkt[rows_of(c), :] = _phi(kt).astype(BF16)
        ktn[rows_of(c), :] = kt.astype(BF16)
        if c == 0:
            transpose_keys(0)

    def proj_q(c):
        qf = _dot(wt_rows(wqt, c), xn_all())
        qt[rows_of(c), :] = (qf * QSCALE).astype(BF16)
        pqt[rows_of(c), :] = _phi(qf).astype(BF16)

    def proj_v(c):
        tail = jnp.concatenate([jnp.zeros((6, L), F32), jnp.ones((8, L), F32)], axis=0)
        vt = _dot(wt_rows(wvt, c), xn_all())
        vtn[rows_of(c), :] = vt.astype(BF16)
        for j in range(CH // DH):
            h = (CH // DH) * c + j
            vt32[32 * h:32 * h + 16, :] = vt[DH * j:DH * j + 16].astype(BF16)
            vt32[32 * h + 16:32 * h + 32, :] = jnp.concatenate(
                [vt[DH * j + 16:DH * j + 18], tail], axis=0).astype(BF16)

    def masked_q(w0, i, word_mask):
        qu = pltpu.bitcast(qt[pl.ds(w0, 128), 128 * i:128 * (i + 1)], U32)
        return pltpu.bitcast(jnp.where(word_mask, qu, jnp.uint32(0)), BF16)

    def head_word_mask(lo):
        word = jax.lax.broadcasted_iota(I32, (64, 128), 0)
        return (2 * word >= lo) & (2 * word < lo + DH)

    def causal_mask():
        return (jax.lax.broadcasted_iota(I32, (128, 128), 0)
                <= jax.lax.broadcasted_iota(I32, (128, 128), 1))

    def pv_head(h, i):
        n = 128 * (i + 1)
        r0 = TOFF[i] * 128
        o = _dot(vt32[32 * h:32 * h + 32, 0:n], pbuf[h, r0:r0 + n, :])
        a = omg[h] * _recip(o[24:32, :])
        on = (o[0:24].reshape(3, 8, 128) * a).reshape(24, 128)
        ot[i, DH * h:DH * h + 24, :] = on + amem[i, DH * h:DH * h + 24, :]

    def stage_attention_fast(filler):
        causal = causal_mask()
        for h in range(H + LAG):
            if h < H:
                g = GROUP_OF[h]
                word_mask = head_word_mask(DH * h - WIN * g)
                if h == GROUP_HEADS[g][0] and g + 1 < NG:
                    transpose_keys(g + 1)
            for i in range(NQB):
                n = 128 * (i + 1)
                if h < H:
                    filler.upto((NTILE * h + TOFF[i] + i + 1) / (NTILE * (H - 1)))
                    st = _dot(packed(kb[g, 0:n // 2, :]), masked_q(WIN * g, i, word_mask))
                    p = jnp.exp2(st)
                    r0 = TOFF[i] * 128
                    if i > 0:
                        pbuf[h, r0:r0 + 128 * i, :] = p[:n - 128].astype(BF16)
                    pbuf[h, r0 + 128 * i:r0 + n, :] = jnp.where(
                        causal, p[n - 128:n], 0.0).astype(BF16)
                if h >= LAG:
                    pv_head(h - LAG, i)

    def stage_scores_safe():
        causal = causal_mask()
        for g in range(1, NG):
            transpose_keys(g)

        def head(h, carry):
            g = jnp.clip((DH * h + DH - 128 + WIN - 1) // WIN, 0, NG - 1)
            g = jnp.where(DH * h + DH <= 128, 0, g)
            w0 = pl.multiple_of(WIN * g, 16)
            word_mask = head_word_mask(DH * h - WIN * g)
            for i in range(NQB):
                n = 128 * (i + 1)
                st = _dot(packed(kb[g, 0:n // 2, :]), masked_q(w0, i, word_mask))
                sd = jnp.where(causal, st[n - 128:n], -jnp.inf)
                m = jnp.max(sd, axis=0, keepdims=True)
                if i > 0:
                    m = jnp.maximum(m, jnp.max(st[:n - 128], axis=0, keepdims=True))
                r0 = TOFF[i] * 128
                if i > 0:
                    pbuf[h, r0:r0 + 128 * i, :] = jnp.exp2(st[:n - 128] - m).astype(BF16)
                pbuf[h, r0 + 128 * i:r0 + n, :] = jnp.exp2(sd - m).astype(BF16)
            return carry

        jax.lax.fori_loop(0, H, head, 0)

    def attn_block(s, i):
        blk = s * NQB + i
        otb = ot[i, 0:D, :].astype(BF16)
        tot = None
        for c in range(NCH):
            hh = _dot(wt_rows(wot, c), otb) + xbuf[blk, rows_of(c), :].astype(F32)
            h_all[blk, rows_of(c), :] = hh
            part = jnp.sum(hh, axis=0, keepdims=True)
            tot = part if tot is None else tot + part
        stat2[blk, 0:1, :] = tot * (1.0 / D)

    def mem_update(g):
        lhs = jnp.concatenate([jnp.ones((16, L), BF16), vtn[WIN * g:WIN * g + 128, :]], axis=0)
        upd = _dot(lhs, pkt[WIN * g:WIN * g + 128, :], NT)
        m_new = m_f32[g] + upd * keep[g]
        m_f32[g] = m_new
        m_bf[g] = m_new.astype(BF16)

    def mem_read(g):
        for i in range(NQB):
            nm = _dot(m_bf[g], pqt[WIN * g:WIN * g + 128, 128 * i:128 * (i + 1)])
            first = GROUP_HEADS[g][0]
            b = gcol[first:first + 8, :] * _recip(nm[0:8, :] + 1e-6)
            for j, h in enumerate(GROUP_HEADS[g]):
                lo = 16 + DH * h - WIN * g
                n = min(24, MROWS - lo)
                amem[i, DH * h:DH * h + n, :] = nm[lo:lo + n] * b[j:j + 1, :]

    def stat_steps(s, blocks=range(NQB)):
        seg = jnp.maximum(s, 0)
        for i in blocks:
            blk = seg * NQB + i
            m = stat2[blk, 0:1, :]
            acc_v = acc_r = None
            for r in range(D // RS):
                rows = slice(RS * r, RS * (r + 1))
                hc = h_all[blk, rows, :] - m
                pv = fold8(hc * hc)
                pr = fold8(hc * wrcol[rows, :])
                acc_v = pv if acc_v is None else acc_v + pv
                acc_r = pr if acc_r is None else acc_r + pr
                yield
            rstd = jax.lax.rsqrt(col_total(acc_v) + LN_EPS)
            stat2[blk, 1:2, :] = rstd
            r_all[pl.ds(blk, 1), :] = jnp.sum(acc_r, axis=0, keepdims=True) * rstd

    def out_steps(s):
        seg = jnp.maximum(s, 0)
        for i in range(NQB):
            blk = seg * NQB + i
            m = stat2[blk, 0:1, :]
            rstd = stat2[blk, 1:2, :]
            for r in range(D // RS):
                rows = slice(RS * r, RS * (r + 1))
                hh = h_all[blk, rows, :]
                obuf[blk, rows, :] = (hh + (hh - m) * rstd).astype(BF16)
                yield

    x_copy(0).start()
    cp_wk.start()

    beta = beta_ref[...].astype(F32).reshape(1, H)
    gpad = jnp.concatenate([_sigmoid(beta), jnp.zeros((1, 128 - H), F32)], axis=1)
    gcol[...] = jnp.transpose(jnp.broadcast_to(gpad, (128, 128)))
    for h in range(H):
        omg[h] = jnp.broadcast_to(1.0 - gcol[h:h + 1, :], (8, 128))
    wr = jnp.concatenate([wr_ref[...].astype(F32).reshape(1, D), jnp.zeros((1, 64), F32)], axis=1)
    wrcol[...] = jnp.transpose(jnp.broadcast_to(wr, (128, D + 64)))[0:D]
    row = jax.lax.broadcasted_iota(I32, (MROWS, 128), 0)
    lane = jax.lax.broadcasted_iota(I32, (MROWS, 128), 1)
    for g in range(NG):
        first, nh = GROUP_HEADS[g][0], len(GROUP_HEADS[g])
        lane_head = ((lane + WIN * g) * 3641) >> 16
        row_head = jnp.where(row < 16, row + first, ((row - 16 + WIN * g) * 3641) >> 16)
        ok = (lane_head == row_head) & (row_head >= first) & (row_head < first + nh)
        keep[g] = jnp.where(ok, 1.0, 0.0)
    m_f32[...] = jnp.zeros_like(m_f32)
    amem[...] = jnp.zeros_like(amem)

    h_all[0:NQB] = jnp.zeros((NQB, D, 128), F32)
    stat2[0:NQB] = jnp.zeros((NQB, 8, 128), F32)

    def transpose_tile(dst, raw, t):
        hi = min(128 * (t + 1), D)
        dst[64 * t:hi // 2, :] = pltpu.bitcast(raw[:, 128 * t:hi].T, U32)

    def col_norm_steps(raw, slot):
        for t in range(5):
            hi = min(128 * (t + 1), D)
            for k in range(3):
                w = raw[192 * k:192 * (k + 1), 128 * t:hi].astype(F32)
                wnorm[slot, 8 * k:8 * (k + 1), 128 * t:hi] = jnp.sum(
                    (w * w).reshape(24, 8, hi - 128 * t), axis=0)
                yield

    x_copy(0).wait()
    cp_wq.start()
    for _ in ln1_steps(0):
        pass
    cp_wk.wait()
    cp_wv.start()
    side = _Filler([col_norm_steps(wk_raw, 0)], [15])
    transpose_tile(wkt, wk_raw, 0)
    transpose_tile(wkt, wk_raw, 1)
    proj_k(0)
    transpose_tile(wkt, wk_raw, 2)
    side.upto(0.5)
    proj_k(1)
    transpose_tile(wkt, wk_raw, 3)
    side.upto(1.0)
    proj_k(2)
    transpose_tile(wkt, wk_raw, 4)
    cp_wq.wait()
    cp_wv.wait()
    cp_wo.start()
    x_copy(1).start()
    transpose_tile(wqt, wq_raw, 0)
    transpose_tile(wqt, wq_raw, 1)
    proj_k(3)
    side = _Filler([col_norm_steps(wq_raw, 1), col_norm_steps(wv_raw, 2)], [15, 15])
    for c in range(NCH):
        proj_q(c)
        if c + 2 < 5:
            transpose_tile(wqt, wq_raw, c + 2)
        if c >= 2:
            transpose_tile(wvt, wv_raw, c - 2)
        if c < NCH - 1:
            side.upto((c + 1) / (NCH - 1))
    cp_wo.wait()
    for s in range(2, NSEG):
        x_copy(s).start()
    cp_wg.start()
    cp_wu.start()
    cp_wd.start()
    for c in range(NCH):
        proj_v(c)
        if c + 2 < 5:
            transpose_tile(wvt, wv_raw, c + 2)
        transpose_tile(wot, wo_raw, c)
    transpose_tile(wot, wo_raw, 4)

    x_copy(1).wait()

    def max_norm(slot):
        ss = jnp.sum(wnorm[slot], axis=0, keepdims=True)
        return jnp.sqrt(jnp.max(ss, axis=1, keepdims=True))

    nk, nq, nv = max_norm(0), max_norm(1), max_norm(2)

    bound = (QSCALE * DH * D) * nq * nk
    safe = (bound <= SAFE_LOGIT) & (nv * (D ** 0.5) <= SAFE_V)
    flag[0] = jnp.sum(jnp.where(safe, 1, 0).astype(I32))

    def segment(s, carry):
        @pl.when(jnp.logical_and(s > 0, s + 1 < NSEG))
        def _():
            x_copy(s + 1).wait()

        def side_work():
            return _Filler([_chain(stat_steps(s - 1), out_steps(s - 1)), ln1_steps(s + 1)],
                           [2 * PASS_STEPS, 3 * PASS_STEPS])

        @pl.when(flag[0] == 1)
        def _():
            stage_attention_fast(side_work())

        @pl.when(flag[0] != 1)
        def _():
            stage_scores_safe()
            side_work().upto(1.0)
            for h in range(H):
                for i in range(NQB):
                    pv_head(h, i)

        @pl.when(s > 0)
        def _():
            out_copy(s - 1).start()

        @pl.when(s + 1 < NSEG)
        def _():
            for i in range(NQB):
                attn_block(s, i)
            for g in range(NG):
                mem_update(g)
            for c in range(NCH):
                proj_q(c)
            for c in range(NCH):
                proj_k(c)
            for g in range(NG):
                mem_read(g)
            for c in range(NCH):
                proj_v(c)

        @pl.when(s + 1 == NSEG)
        def _():
            for i in range(NQB):
                attn_block(s, i)
                if i > 0:
                    for _ in stat_steps(s, [i - 1]):
                        pass
            for _ in stat_steps(s, [NQB - 1]):
                pass

        return carry

    jax.lax.fori_loop(0, NSEG, segment, 0)

    r = r_all[...]
    r_sel = jnp.max(jnp.max(r, axis=0, keepdims=True), axis=1, keepdims=True)
    ids = (128 * jax.lax.broadcasted_iota(I32, r.shape, 0)
           + jax.lax.broadcasted_iota(I32, r.shape, 1))
    cand = jnp.min(jnp.where(r == r_sel, ids, S), axis=0, keepdims=True)
    idx = jnp.minimum(jnp.sum(jnp.min(cand, axis=1, keepdims=True)), S - 1)
    for _ in out_steps(NSEG - 1):
        pass
    out_copy(NSEG - 1).start()
    blk = idx >> 7
    m_sel = stat2[blk, 0:1, :]
    rstd_sel = stat2[blk, 1:2, :]
    for r in range(D // RS):
        rows = slice(RS * r, RS * (r + 1))
        hn_sel[rows, :] = ((h_all[blk, rows, :] - m_sel) * rstd_sel).astype(BF16)
    onehot = (jax.lax.broadcasted_iota(I32, (16, 128), 1) == idx - blk * 128).astype(BF16)
    xs = _dot(onehot, hn_sel[...], NT).astype(BF16)
    cp_wg.wait()
    cp_wu.wait()
    cp_wd.wait()

    def down_steps(c, act):
        for r in range(D // RS):
            rows = slice(RS * r, RS * (r + 1))
            part = None if c == 0 else yacc[rows, :]
            for t in range(FC // 128):
                w = wdt_v[rows, FC * c + 128 * t:FC * c + 128 * (t + 1)].astype(F32)
                part = w * act[t] if part is None else part + w * act[t]
            yacc[rows, :] = part
            yield

    nch = FF // FC
    pending = None
    for c in range(nch):
        ga, up = [], []
        for t in range(FC // 128):
            tile = slice(FC * c + 128 * t, FC * c + 128 * (t + 1))
            ga.append(_dot(xs, wg_v[:, tile])[0:1])
            up.append(_dot(xs, wu_v[:, tile])[0:1])
            if pending is not None:
                pending.upto((t + 1) / (FC // 128))
        act = [g * _sigmoid(g) * u for g, u in zip(ga, up)]
        pending = _Filler([down_steps(c, act)], [D // RS])
    pending.upto(1.0)
    y = jnp.sum(yacc[...], axis=1, keepdims=True) * _sigmoid(r_sel)
    sel = jax.lax.broadcasted_iota(I32, (RS, 128), 1) == idx - blk * 128
    for r in range(D // RS):
        rows = slice(RS * r, RS * (r + 1))
        hh = h_all[blk, rows, :]
        stage[rows, :] = (hh + (hh - m_sel) * rstd_sel
                          + jnp.where(sel, y[rows], 0.0)).astype(BF16)
    for s in range(NSEG):
        out_copy(s).wait()
    fix = pltpu.make_async_copy(stage, out_hbm.at[:, hbm_cols(blk)], sem_w.at[7])
    fix.start()
    fix.wait()


@jax.jit
def pallas_sequential_preLN__memory_aug_infini_attn__moe_arch_mod__prompt_kernel(
    A_x: jax.Array,
    A_wq: jax.Array,
    A_wk: jax.Array,
    A_wv: jax.Array,
    A_wo: jax.Array,
    A_beta: jax.Array,
    B_x: jax.Array,
    B_w_r: jax.Array,
    B_w_gate: jax.Array,
    B_w_up: jax.Array,
    B_w_down: jax.Array,
):
    del B_x
    hbm = pl.BlockSpec(memory_space=pltpu.HBM)
    vmem = pl.BlockSpec(memory_space=pltpu.VMEM)
    scratch = [
        pltpu.VMEM((NSEG * NQB, D, 128), BF16),
        pltpu.VMEM((D, D), BF16),
        pltpu.VMEM((D, D), BF16),
        pltpu.VMEM((D, D), BF16),
        pltpu.VMEM((D, D), BF16),
        pltpu.VMEM((D // 2, D), U32),
        pltpu.VMEM((D // 2, D), U32),
        pltpu.VMEM((D // 2, D), U32),
        pltpu.VMEM((D // 2, D), U32),
        pltpu.VMEM((NQB, D, 128), BF16),
        pltpu.VMEM((D, L), BF16),
        pltpu.VMEM((NG, L // 2, 128), U32),
        pltpu.VMEM((D, L), BF16),
        pltpu.VMEM((D, L), BF16),
        pltpu.VMEM((D, L), BF16),
        pltpu.VMEM((D, L), BF16),
        pltpu.VMEM((H * 32, L), BF16),
        pltpu.VMEM((H, NTILE * 128, 128), BF16),
        pltpu.VMEM((NG, MROWS, 128), F32),
        pltpu.VMEM((NG, MROWS, 128), BF16),
        pltpu.VMEM((NG, MROWS, 128), F32),
        pltpu.VMEM((NQB, D + 24, 128), F32),
        pltpu.VMEM((NQB, D + 24, 128), F32),
        pltpu.VMEM((NSEG * NQB, D, 128), F32),
        pltpu.VMEM((D, 128), BF16),
        pltpu.VMEM((D, 128), F32),
        pltpu.VMEM((NSEG * NQB, D, 128), BF16),
        pltpu.VMEM((D, FF), BF16),
        pltpu.VMEM((D, FF), BF16),
        pltpu.VMEM((D, FF), BF16),
        pltpu.VMEM((128, 128), F32),
        pltpu.VMEM((H, 8, 128), F32),
        pltpu.VMEM((D, 128), F32),
        pltpu.VMEM((NQB, 8, 128), F32),
        pltpu.VMEM((NSEG * NQB, 8, 128), F32),
        pltpu.VMEM((3, 24, D), F32),
        pltpu.VMEM((NSEG * NQB, 128), F32),
        pltpu.VMEM((D, 128), BF16),
        pltpu.SMEM((1,), I32),
        pltpu.SemaphoreType.DMA((NSEG,)),
        pltpu.SemaphoreType.DMA((8,)),
        pltpu.SemaphoreType.DMA((NSEG,)),
    ]
    out_t = pl.pallas_call(
        _kernel,
        out_shape=jax.ShapeDtypeStruct((D, S), BF16),
        in_specs=[hbm, hbm, hbm, hbm, hbm, vmem, vmem, hbm, hbm, hbm],
        out_specs=hbm,
        scratch_shapes=scratch,
        compiler_params=pltpu.CompilerParams(vmem_limit_bytes=100 * 1024 * 1024),
        name="infini_moe",
    )(A_x.reshape(S, D).T, A_wq, A_wk, A_wv, A_wo, A_beta, B_w_r, B_w_gate, B_w_up, B_w_down.T)
    return out_t.T.reshape(1, S, D)
```

```python
import functools

import jax
import jax.numpy as jnp
import jax.experimental.pallas as pl
import jax.experimental.pallas.tpu as pltpu

F32 = jnp.float32
BF16 = jnp.bfloat16
U32 = jnp.uint32
I32 = jnp.int32

S = 2048
D = 576
H = 32
DH = 18
NSEG = 4
L = S // NSEG
FF = 4608
NQB = L // 128
TOFF = (0, 1, 3, 6)
NTILE = 10
NG = 5
WIN = 112
GROUP_HEADS = tuple(tuple(h for h in range(H)
                          if min(max(0, -(-(DH * h + DH - 128) // WIN)), NG - 1) == g)
                    for g in range(NG))
GROUP_OF = {h: g for g in range(NG) for h in GROUP_HEADS[g]}
MROWS = 144
CH = 144
NCH = D // CH
RS = 64
PASS_STEPS = NQB * (D // RS)
FC = 512
LAG = 20
LN_EPS = 1e-5
LOG2E = 1.4426950408889634
QSCALE = (DH ** -0.5) * LOG2E
SAFE_LOGIT = 60.0
SAFE_V = 2.0 ** 50

NN = (((1,), (0,)), ((), ()))
NT = (((1,), (1,)), ((), ()))
TN = (((0,), (0,)), ((), ()))

for _g, _hs in enumerate(GROUP_HEADS):
    for _h in _hs:
        assert WIN * _g <= DH * _h and DH * _h + DH <= WIN * _g + 128


def _dot(a, b, dims=NN):
    return jax.lax.dot_general(a, b, dims, preferred_element_type=F32)


class _Filler:
    def __init__(self, gens, counts):
        self.gens, self.counts, self.done = gens, counts, [0] * len(gens)

    def upto(self, frac):
        for k, gen in enumerate(self.gens):
            while self.done[k] < min(frac, 1.0) * self.counts[k]:
                next(gen, None)
                self.done[k] += 1
            if frac >= 1.0:
                for _ in gen:
                    pass


def _chain(*gens):
    for gen in gens:
        yield from gen


def _phi(t):
    return jnp.where(t > 0, t + 1.0, jnp.exp(t))


def _sigmoid(t):
    return 1.0 / (1.0 + jnp.exp(-t))


def _recip(x):
    r = pl.reciprocal(x, approx=True)
    return r * (2.0 - x * r)


def _kernel(xt_hbm, wq_hbm, wk_hbm, wv_hbm, wo_hbm, beta_ref, wr_ref, wg_hbm, wu_hbm, wdt_hbm,
            out_hbm,
            xbuf, wq_raw, wk_raw, wv_raw, wo_raw, wqt, wkt, wvt, wot, xn, ktn, kb, qt, pkt, pqt,
            vtn, vt32, pbuf, m_f32, m_bf, keep, amem, ot, h_all, hn_sel, yacc, obuf, wg_v, wu_v, wdt_v,
            gcol, omg, wrcol, stat1, stat2, wnorm, r_all, stage, flag, sem_x, sem_w, sem_o):
    class _Group:
        def __init__(self, copies):
            self.copies = copies

        def start(self):
            for cp in self.copies:
                cp.start()

        def wait(self):
            for cp in self.copies:
                cp.wait()

    def hbm_cols(blk):
        return pl.ds(pl.multiple_of(blk * 128, 128), 128)

    def x_copy(s):
        return _Group([pltpu.make_async_copy(xt_hbm.at[:, hbm_cols(s * NQB + i)],
                                             xbuf.at[s * NQB + i], sem_x.at[s])
                       for i in range(NQB)])

    def out_copy(s):
        return _Group([pltpu.make_async_copy(obuf.at[s * NQB + i],
                                             out_hbm.at[:, hbm_cols(s * NQB + i)], sem_o.at[s])
                       for i in range(NQB)])

    cp_wk = pltpu.make_async_copy(wk_hbm, wk_raw, sem_w.at[0])
    cp_wq = pltpu.make_async_copy(wq_hbm, wq_raw, sem_w.at[1])
    cp_wv = pltpu.make_async_copy(wv_hbm, wv_raw, sem_w.at[2])
    cp_wo = pltpu.make_async_copy(wo_hbm, wo_raw, sem_w.at[3])
    cp_wg = pltpu.make_async_copy(wg_hbm, wg_v, sem_w.at[4])
    cp_wu = pltpu.make_async_copy(wu_hbm, wu_v, sem_w.at[5])
    cp_wd = pltpu.make_async_copy(wdt_hbm, wdt_v, sem_w.at[6])

    def fold8(v):
        return jnp.sum(v.reshape(v.shape[0] // 8, 8, 128), axis=0)

    def col_total(acc):
        return jnp.sum(acc, axis=0, keepdims=True) * (1.0 / D)

    def ln1_steps(s):
        seg = jnp.minimum(s, NSEG - 1)
        for c in range(NQB):
            xs = lambda r: xbuf[seg * NQB + c, RS * r:RS * (r + 1), :].astype(F32)
            acc = None
            for r in range(D // RS):
                part = fold8(xs(r))
                acc = part if acc is None else acc + part
                yield
            m = col_total(acc)
            stat1[c, 0:1, :] = m
            acc = None
            for r in range(D // RS):
                xc = xs(r) - m
                part = fold8(xc * xc)
                acc = part if acc is None else acc + part
                yield
            rstd = jax.lax.rsqrt(col_total(acc) + LN_EPS)
            stat1[c, 1:2, :] = rstd
            for r in range(D // RS):
                xn[c, RS * r:RS * (r + 1), :] = (
                    (xs(r) - m) * rstd).astype(BF16)
                yield

    def xn_all():
        return jnp.concatenate([xn[c] for c in range(NQB)], axis=1)

    def rows_of(c):
        return slice(CH * c, CH * (c + 1))

    def packed(words):
        return pltpu.bitcast(words, BF16)

    def wt_rows(wt, c):
        return packed(wt[CH // 2 * c:CH // 2 * (c + 1), :])

    def transpose_keys(g):
        kb[g] = pltpu.bitcast(ktn[WIN * g:WIN * g + 128, :].T, U32)

    def proj_k(c):
        kt = _dot(wt_rows(wkt, c), xn_all())
        pkt[rows_of(c), :] = _phi(kt).astype(BF16)
        ktn[rows_of(c), :] = kt.astype(BF16)
        if c == 0:
            transpose_keys(0)

    def proj_q(c):
        qf = _dot(wt_rows(wqt, c), xn_all())
        qt[rows_of(c), :] = (qf * QSCALE).astype(BF16)
        pqt[rows_of(c), :] = _phi(qf).astype(BF16)

    def proj_v(c):
        tail = jnp.concatenate([jnp.zeros((6, L), F32), jnp.ones((8, L), F32)], axis=0)
        vt = _dot(wt_rows(wvt, c), xn_all())
        vtn[rows_of(c), :] = vt.astype(BF16)
        for j in range(CH // DH):
            h = (CH // DH) * c + j
            vt32[32 * h:32 * h + 16, :] = vt[DH * j:DH * j + 16].astype(BF16)
            vt32[32 * h + 16:32 * h + 32, :] = jnp.concatenate(
                [vt[DH * j + 16:DH * j + 18], tail], axis=0).astype(BF16)

    def masked_q(w0, i, word_mask):
        qu = pltpu.bitcast(qt[pl.ds(w0, 128), 128 * i:128 * (i + 1)], U32)
        return pltpu.bitcast(jnp.where(word_mask, qu, jnp.uint32(0)), BF16)

    def head_word_mask(lo):
        word = jax.lax.broadcasted_iota(I32, (64, 128), 0)
        return (2 * word >= lo) & (2 * word < lo + DH)

    def causal_mask():
        return (jax.lax.broadcasted_iota(I32, (128, 128), 0)
                <= jax.lax.broadcasted_iota(I32, (128, 128), 1))

    def pv_head(h, i):
        n = 128 * (i + 1)
        r0 = TOFF[i] * 128
        o = _dot(vt32[32 * h:32 * h + 32, 0:n], pbuf[h, r0:r0 + n, :])
        a = omg[h] * _recip(o[24:32, :])
        on = (o[0:24].reshape(3, 8, 128) * a).reshape(24, 128)
        ot[i, DH * h:DH * h + 24, :] = on + amem[i, DH * h:DH * h + 24, :]

    def stage_attention_fast(filler):
        causal = causal_mask()
        for h in range(H + LAG):
            if h < H:
                g = GROUP_OF[h]
                word_mask = head_word_mask(DH * h - WIN * g)
                if h == GROUP_HEADS[g][0] and g + 1 < NG:
                    transpose_keys(g + 1)
            for i in range(NQB):
                n = 128 * (i + 1)
                if h < H:
                    filler.upto((NTILE * h + TOFF[i] + i + 1) / (NTILE * (H - 1)))
                    st = _dot(packed(kb[g, 0:n // 2, :]), masked_q(WIN * g, i, word_mask))
                    p = jnp.exp2(st)
                    r0 = TOFF[i] * 128
                    if i > 0:
                        pbuf[h, r0:r0 + 128 * i, :] = p[:n - 128].astype(BF16)
                    pbuf[h, r0 + 128 * i:r0 + n, :] = jnp.where(
                        causal, p[n - 128:n], 0.0).astype(BF16)
                if h >= LAG:
                    pv_head(h - LAG, i)

    def stage_scores_safe():
        causal = causal_mask()
        for g in range(1, NG):
            transpose_keys(g)

        def head(h, carry):
            g = jnp.clip((DH * h + DH - 128 + WIN - 1) // WIN, 0, NG - 1)
            g = jnp.where(DH * h + DH <= 128, 0, g)
            w0 = pl.multiple_of(WIN * g, 16)
            word_mask = head_word_mask(DH * h - WIN * g)
            for i in range(NQB):
                n = 128 * (i + 1)
                st = _dot(packed(kb[g, 0:n // 2, :]), masked_q(w0, i, word_mask))
                sd = jnp.where(causal, st[n - 128:n], -jnp.inf)
                m = jnp.max(sd, axis=0, keepdims=True)
                if i > 0:
                    m = jnp.maximum(m, jnp.max(st[:n - 128], axis=0, keepdims=True))
                r0 = TOFF[i] * 128
                if i > 0:
                    pbuf[h, r0:r0 + 128 * i, :] = jnp.exp2(st[:n - 128] - m).astype(BF16)
                pbuf[h, r0 + 128 * i:r0 + n, :] = jnp.exp2(sd - m).astype(BF16)
            return carry

        jax.lax.fori_loop(0, H, head, 0)

    def attn_block(s, i):
        blk = s * NQB + i
        otb = ot[i, 0:D, :].astype(BF16)
        tot = None
        for c in range(NCH):
            hh = _dot(wt_rows(wot, c), otb) + xbuf[blk, rows_of(c), :].astype(F32)
            h_all[blk, rows_of(c), :] = hh
            part = jnp.sum(hh, axis=0, keepdims=True)
            tot = part if tot is None else tot + part
        stat2[blk, 0:1, :] = tot * (1.0 / D)

    def mem_update(g):
        lhs = jnp.concatenate([jnp.ones((16, L), BF16), vtn[WIN * g:WIN * g + 128, :]], axis=0)
        upd = _dot(lhs, pkt[WIN * g:WIN * g + 128, :], NT)
        m_new = m_f32[g] + upd * keep[g]
        m_f32[g] = m_new
        m_bf[g] = m_new.astype(BF16)

    def mem_read(g):
        for i in range(NQB):
            nm = _dot(m_bf[g], pqt[WIN * g:WIN * g + 128, 128 * i:128 * (i + 1)])
            first = GROUP_HEADS[g][0]
            b = gcol[first:first + 8, :] * _recip(nm[0:8, :] + 1e-6)
            for j, h in enumerate(GROUP_HEADS[g]):
                lo = 16 + DH * h - WIN * g
                n = min(24, MROWS - lo)
                amem[i, DH * h:DH * h + n, :] = nm[lo:lo + n] * b[j:j + 1, :]

    def stat_steps(s, blocks=range(NQB)):
        seg = jnp.maximum(s, 0)
        for i in blocks:
            blk = seg * NQB + i
            m = stat2[blk, 0:1, :]
            acc_v = acc_r = None
            for r in range(D // RS):
                rows = slice(RS * r, RS * (r + 1))
                hc = h_all[blk, rows, :] - m
                pv = fold8(hc * hc)
                pr = fold8(hc * wrcol[rows, :])
                acc_v = pv if acc_v is None else acc_v + pv
                acc_r = pr if acc_r is None else acc_r + pr
                yield
            rstd = jax.lax.rsqrt(col_total(acc_v) + LN_EPS)
            stat2[blk, 1:2, :] = rstd
            r_all[pl.ds(blk, 1), :] = jnp.sum(acc_r, axis=0, keepdims=True) * rstd

    def out_steps(s):
        seg = jnp.maximum(s, 0)
        for i in range(NQB):
            blk = seg * NQB + i
            m = stat2[blk, 0:1, :]
            rstd = stat2[blk, 1:2, :]
            for r in range(D // RS):
                rows = slice(RS * r, RS * (r + 1))
                hh = h_all[blk, rows, :]
                obuf[blk, rows, :] = (hh + (hh - m) * rstd).astype(BF16)
                yield

    x_copy(0).start()
    cp_wk.start()

    beta = beta_ref[...].astype(F32).reshape(1, H)
    gpad = jnp.concatenate([_sigmoid(beta), jnp.zeros((1, 128 - H), F32)], axis=1)
    gcol[...] = jnp.transpose(jnp.broadcast_to(gpad, (128, 128)))
    for h in range(H):
        omg[h] = jnp.broadcast_to(1.0 - gcol[h:h + 1, :], (8, 128))
    wr = jnp.concatenate([wr_ref[...].astype(F32).reshape(1, D), jnp.zeros((1, 64), F32)], axis=1)
    wrcol[...] = jnp.transpose(jnp.broadcast_to(wr, (128, D + 64)))[0:D]
    row = jax.lax.broadcasted_iota(I32, (MROWS, 128), 0)
    lane = jax.lax.broadcasted_iota(I32, (MROWS, 128), 1)
    for g in range(NG):
        first, nh = GROUP_HEADS[g][0], len(GROUP_HEADS[g])
        lane_head = ((lane + WIN * g) * 3641) >> 16
        row_head = jnp.where(row < 16, row + first, ((row - 16 + WIN * g) * 3641) >> 16)
        ok = (lane_head == row_head) & (row_head >= first) & (row_head < first + nh)
        keep[g] = jnp.where(ok, 1.0, 0.0)
    m_f32[...] = jnp.zeros_like(m_f32)
    amem[...] = jnp.zeros_like(amem)

    h_all[0:NQB] = jnp.zeros((NQB, D, 128), F32)
    stat2[0:NQB] = jnp.zeros((NQB, 8, 128), F32)

    def transpose_tile(dst, raw, t):
        hi = min(128 * (t + 1), D)
        dst[64 * t:hi // 2, :] = pltpu.bitcast(raw[:, 128 * t:hi].T, U32)

    def col_norm_steps(raw, slot):
        for t in range(5):
            hi = min(128 * (t + 1), D)
            for k in range(3):
                w = raw[192 * k:192 * (k + 1), 128 * t:hi].astype(F32)
                wnorm[slot, 8 * k:8 * (k + 1), 128 * t:hi] = jnp.sum(
                    (w * w).reshape(24, 8, hi - 128 * t), axis=0)
                yield

    x_copy(0).wait()
    cp_wq.start()
    for _ in ln1_steps(0):
        pass
    cp_wk.wait()
    cp_wv.start()
    side = _Filler([col_norm_steps(wk_raw, 0)], [15])
    transpose_tile(wkt, wk_raw, 0)
    transpose_tile(wkt, wk_raw, 1)
    proj_k(0)
    transpose_tile(wkt, wk_raw, 2)
    side.upto(0.5)
    proj_k(1)
    transpose_tile(wkt, wk_raw, 3)
    side.upto(1.0)
    proj_k(2)
    transpose_tile(wkt, wk_raw, 4)
    cp_wq.wait()
    cp_wv.wait()
    cp_wo.start()
    x_copy(1).start()
    transpose_tile(wqt, wq_raw, 0)
    transpose_tile(wqt, wq_raw, 1)
    proj_k(3)
    side = _Filler([col_norm_steps(wq_raw, 1), col_norm_steps(wv_raw, 2)], [15, 15])
    for c in range(NCH):
        proj_q(c)
        if c + 2 < 5:
            transpose_tile(wqt, wq_raw, c + 2)
        if c >= 2:
            transpose_tile(wvt, wv_raw, c - 2)
        if c < NCH - 1:
            side.upto((c + 1) / (NCH - 1))
    cp_wo.wait()
    x_copy(1).wait()
    for s in range(2, NSEG):
        x_copy(s).start()
    cp_wg.start()
    cp_wu.start()
    cp_wd.start()
    for c in range(NCH):
        proj_v(c)
        if c + 2 < 5:
            transpose_tile(wvt, wv_raw, c + 2)
        transpose_tile(wot, wo_raw, c)
    transpose_tile(wot, wo_raw, 4)

    def max_norm(slot):
        ss = jnp.sum(wnorm[slot], axis=0, keepdims=True)
        return jnp.sqrt(jnp.max(ss, axis=1, keepdims=True))

    nk, nq, nv = max_norm(0), max_norm(1), max_norm(2)

    bound = (QSCALE * DH * D) * nq * nk
    safe = (bound <= SAFE_LOGIT) & (nv * (D ** 0.5) <= SAFE_V)
    flag[0] = jnp.sum(jnp.where(safe, 1, 0).astype(I32))

    def segment(s, carry):
        @pl.when(jnp.logical_and(s > 0, s + 1 < NSEG))
        def _():
            x_copy(s + 1).wait()

        def side_work():
            return _Filler([_chain(stat_steps(s - 1), out_steps(s - 1)), ln1_steps(s + 1)],
                           [2 * PASS_STEPS, 3 * PASS_STEPS])

        @pl.when(flag[0] == 1)
        def _():
            stage_attention_fast(side_work())

        @pl.when(flag[0] != 1)
        def _():
            stage_scores_safe()
            side_work().upto(1.0)
            for h in range(H):
                for i in range(NQB):
                    pv_head(h, i)

        @pl.when(s > 0)
        def _():
            out_copy(s - 1).start()

        @pl.when(s + 1 < NSEG)
        def _():
            for i in range(NQB):
                attn_block(s, i)
            for g in range(NG):
                mem_update(g)
            for c in range(NCH):
                proj_q(c)
            for c in range(NCH):
                proj_k(c)
            for g in range(NG):
                mem_read(g)
            for c in range(NCH):
                proj_v(c)

        return carry

    jax.lax.fori_loop(0, NSEG, segment, 0)

    for i in range(NQB):
        attn_block(NSEG - 1, i)
        if i > 0:
            for _ in stat_steps(NSEG - 1, [i - 1]):
                pass
    for _ in stat_steps(NSEG - 1, [NQB - 1]):
        pass

    r = r_all[...]
    r_sel = jnp.max(jnp.max(r, axis=0, keepdims=True), axis=1, keepdims=True)
    ids = (128 * jax.lax.broadcasted_iota(I32, r.shape, 0)
           + jax.lax.broadcasted_iota(I32, r.shape, 1))
    cand = jnp.min(jnp.where(r == r_sel, ids, S), axis=0, keepdims=True)
    idx = jnp.minimum(jnp.sum(jnp.min(cand, axis=1, keepdims=True)), S - 1)
    for _ in out_steps(NSEG - 1):
        pass
    out_copy(NSEG - 1).start()
    blk = idx >> 7
    m_sel = stat2[blk, 0:1, :]
    rstd_sel = stat2[blk, 1:2, :]
    for r in range(D // RS):
        rows = slice(RS * r, RS * (r + 1))
        hn_sel[rows, :] = ((h_all[blk, rows, :] - m_sel) * rstd_sel).astype(BF16)
    onehot = (jax.lax.broadcasted_iota(I32, (16, 128), 1) == idx - blk * 128).astype(BF16)
    xs = _dot(onehot, hn_sel[...], NT).astype(BF16)
    cp_wg.wait()
    cp_wu.wait()
    cp_wd.wait()

    def down_steps(c, act):
        for r in range(D // RS):
            rows = slice(RS * r, RS * (r + 1))
            part = None if c == 0 else yacc[rows, :]
            for t in range(FC // 128):
                w = wdt_v[rows, FC * c + 128 * t:FC * c + 128 * (t + 1)].astype(F32)
                part = w * act[t] if part is None else part + w * act[t]
            yacc[rows, :] = part
            yield

    nch = FF // FC
    pending = None
    for c in range(nch):
        ga, up = [], []
        for t in range(FC // 128):
            tile = slice(FC * c + 128 * t, FC * c + 128 * (t + 1))
            ga.append(_dot(xs, wg_v[:, tile])[0:1])
            up.append(_dot(xs, wu_v[:, tile])[0:1])
            if pending is not None:
                pending.upto((t + 1) / (FC // 128))
        act = [g * _sigmoid(g) * u for g, u in zip(ga, up)]
        pending = _Filler([down_steps(c, act)], [D // RS])
    pending.upto(1.0)
    y = jnp.sum(yacc[...], axis=1, keepdims=True) * _sigmoid(r_sel)
    sel = jax.lax.broadcasted_iota(I32, (RS, 128), 1) == idx - blk * 128
    for r in range(D // RS):
        rows = slice(RS * r, RS * (r + 1))
        hh = h_all[blk, rows, :]
        stage[rows, :] = (hh + (hh - m_sel) * rstd_sel
                          + jnp.where(sel, y[rows], 0.0)).astype(BF16)
    for s in range(NSEG):
        out_copy(s).wait()
    fix = pltpu.make_async_copy(stage, out_hbm.at[:, hbm_cols(blk)], sem_w.at[7])
    fix.start()
    fix.wait()


@jax.jit
def pallas_sequential_preLN__memory_aug_infini_attn__moe_arch_mod__prompt_kernel(
    A_x: jax.Array,
    A_wq: jax.Array,
    A_wk: jax.Array,
    A_wv: jax.Array,
    A_wo: jax.Array,
    A_beta: jax.Array,
    B_x: jax.Array,
    B_w_r: jax.Array,
    B_w_gate: jax.Array,
    B_w_up: jax.Array,
    B_w_down: jax.Array,
):
    del B_x
    hbm = pl.BlockSpec(memory_space=pltpu.HBM)
    vmem = pl.BlockSpec(memory_space=pltpu.VMEM)
    scratch = [
        pltpu.VMEM((NSEG * NQB, D, 128), BF16),
        pltpu.VMEM((D, D), BF16),
        pltpu.VMEM((D, D), BF16),
        pltpu.VMEM((D, D), BF16),
        pltpu.VMEM((D, D), BF16),
        pltpu.VMEM((D // 2, D), U32),
        pltpu.VMEM((D // 2, D), U32),
        pltpu.VMEM((D // 2, D), U32),
        pltpu.VMEM((D // 2, D), U32),
        pltpu.VMEM((NQB, D, 128), BF16),
        pltpu.VMEM((D, L), BF16),
        pltpu.VMEM((NG, L // 2, 128), U32),
        pltpu.VMEM((D, L), BF16),
        pltpu.VMEM((D, L), BF16),
        pltpu.VMEM((D, L), BF16),
        pltpu.VMEM((D, L), BF16),
        pltpu.VMEM((H * 32, L), BF16),
        pltpu.VMEM((H, NTILE * 128, 128), BF16),
        pltpu.VMEM((NG, MROWS, 128), F32),
        pltpu.VMEM((NG, MROWS, 128), BF16),
        pltpu.VMEM((NG, MROWS, 128), F32),
        pltpu.VMEM((NQB, D + 24, 128), F32),
        pltpu.VMEM((NQB, D + 24, 128), F32),
        pltpu.VMEM((NSEG * NQB, D, 128), F32),
        pltpu.VMEM((D, 128), BF16),
        pltpu.VMEM((D, 128), F32),
        pltpu.VMEM((NSEG * NQB, D, 128), BF16),
        pltpu.VMEM((D, FF), BF16),
        pltpu.VMEM((D, FF), BF16),
        pltpu.VMEM((D, FF), BF16),
        pltpu.VMEM((128, 128), F32),
        pltpu.VMEM((H, 8, 128), F32),
        pltpu.VMEM((D, 128), F32),
        pltpu.VMEM((NQB, 8, 128), F32),
        pltpu.VMEM((NSEG * NQB, 8, 128), F32),
        pltpu.VMEM((3, 24, D), F32),
        pltpu.VMEM((NSEG * NQB, 128), F32),
        pltpu.VMEM((D, 128), BF16),
        pltpu.SMEM((1,), I32),
        pltpu.SemaphoreType.DMA((NSEG,)),
        pltpu.SemaphoreType.DMA((8,)),
        pltpu.SemaphoreType.DMA((NSEG,)),
    ]
    out_t = pl.pallas_call(
        _kernel,
        out_shape=jax.ShapeDtypeStruct((D, S), BF16),
        in_specs=[hbm, hbm, hbm, hbm, hbm, vmem, vmem, hbm, hbm, hbm],
        out_specs=hbm,
        scratch_shapes=scratch,
        compiler_params=pltpu.CompilerParams(vmem_limit_bytes=100 * 1024 * 1024),
        name="infini_moe",
    )(A_x.reshape(S, D).T, A_wq, A_wk, A_wv, A_wo, A_beta, B_w_r, B_w_gate, B_w_up, B_w_down.T)
    return out_t.T.reshape(1, S, D)
```

```python
import functools

import jax
import jax.numpy as jnp
import jax.experimental.pallas as pl
import jax.experimental.pallas.tpu as pltpu

F32 = jnp.float32
BF16 = jnp.bfloat16
U32 = jnp.uint32
I32 = jnp.int32

S = 2048
D = 576
H = 32
DH = 18
NSEG = 4
L = S // NSEG
FF = 4608
NQB = L // 128
TOFF = (0, 1, 3, 6)
NTILE = 10
NG = 5
WIN = 112
GROUP_HEADS = tuple(tuple(h for h in range(H)
                          if min(max(0, -(-(DH * h + DH - 128) // WIN)), NG - 1) == g)
                    for g in range(NG))
GROUP_OF = {h: g for g in range(NG) for h in GROUP_HEADS[g]}
MROWS = 144
CH = 144
NCH = D // CH
RS = 64
PASS_STEPS = NQB * (D // RS)
FC = 512
LAG = 20
LN_EPS = 1e-5
LOG2E = 1.4426950408889634
QSCALE = (DH ** -0.5) * LOG2E
SAFE_LOGIT = 60.0
SAFE_V = 2.0 ** 50

NN = (((1,), (0,)), ((), ()))
NT = (((1,), (1,)), ((), ()))
TN = (((0,), (0,)), ((), ()))

for _g, _hs in enumerate(GROUP_HEADS):
    for _h in _hs:
        assert WIN * _g <= DH * _h and DH * _h + DH <= WIN * _g + 128


def _dot(a, b, dims=NN):
    return jax.lax.dot_general(a, b, dims, preferred_element_type=F32)


class _Filler:
    def __init__(self, gens, counts):
        self.gens, self.counts, self.done = gens, counts, [0] * len(gens)

    def upto(self, frac):
        for k, gen in enumerate(self.gens):
            while self.done[k] < min(frac, 1.0) * self.counts[k]:
                next(gen, None)
                self.done[k] += 1
            if frac >= 1.0:
                for _ in gen:
                    pass


def _chain(*gens):
    for gen in gens:
        yield from gen


def _phi(t):
    return jnp.where(t > 0, t + 1.0, jnp.exp(t))


def _sigmoid(t):
    return 1.0 / (1.0 + jnp.exp(-t))


def _recip(x):
    r = pl.reciprocal(x, approx=True)
    return r * (2.0 - x * r)


def _kernel(xt_hbm, wq_hbm, wk_hbm, wv_hbm, wo_hbm, beta_ref, wr_ref, wg_hbm, wu_hbm, wdt_hbm,
            out_hbm,
            xbuf, wq_raw, wk_raw, wv_raw, wo_raw, wqt, wkt, wvt, wot, xn, ktn, kb, qt, pkt, pqt,
            vtn, vt32, pbuf, m_f32, m_bf, keep, amem, ot, h_all, hn_sel, yacc, obuf, wg_v, wu_v, wdt_v,
            gcol, omg, wrcol, stat1, stat2, wnorm, r_all, stage, flag, sem_x, sem_w, sem_o):
    class _Group:
        def __init__(self, copies):
            self.copies = copies

        def start(self):
            for cp in self.copies:
                cp.start()

        def wait(self):
            for cp in self.copies:
                cp.wait()

    def hbm_cols(blk):
        return pl.ds(pl.multiple_of(blk * 128, 128), 128)

    def x_copy(s):
        return _Group([pltpu.make_async_copy(xt_hbm.at[:, hbm_cols(s * NQB + i)],
                                             xbuf.at[s * NQB + i], sem_x.at[s])
                       for i in range(NQB)])

    def out_copy(s):
        return _Group([pltpu.make_async_copy(obuf.at[s * NQB + i],
                                             out_hbm.at[:, hbm_cols(s * NQB + i)], sem_o.at[s])
                       for i in range(NQB)])

    def prev_out_copy(s):
        src = jnp.where(s > 0, s - 1, NSEG) * NQB
        dst = jnp.where(s > 0, s - 1, NSEG - 1) * NQB
        sem = jnp.where(s > 0, s - 1, NSEG)
        return _Group([pltpu.make_async_copy(obuf.at[src + i], out_hbm.at[:, hbm_cols(dst + i)],
                                             sem_o.at[sem]) for i in range(NQB)])

    cp_wk = pltpu.make_async_copy(wk_hbm, wk_raw, sem_w.at[0])
    cp_wq = pltpu.make_async_copy(wq_hbm, wq_raw, sem_w.at[1])
    cp_wv = pltpu.make_async_copy(wv_hbm, wv_raw, sem_w.at[2])
    cp_wo = pltpu.make_async_copy(wo_hbm, wo_raw, sem_w.at[3])
    cp_wg = pltpu.make_async_copy(wg_hbm, wg_v, sem_w.at[4])
    cp_wu = pltpu.make_async_copy(wu_hbm, wu_v, sem_w.at[5])
    cp_wd = pltpu.make_async_copy(wdt_hbm, wdt_v, sem_w.at[6])

    def fold8(v):
        return jnp.sum(v.reshape(v.shape[0] // 8, 8, 128), axis=0)

    def col_total(acc):
        return jnp.sum(acc, axis=0, keepdims=True) * (1.0 / D)

    def ln1_steps(s):
        seg = jnp.minimum(s, NSEG - 1)
        for c in range(NQB):
            xs = lambda r: xbuf[seg * NQB + c, RS * r:RS * (r + 1), :].astype(F32)
            acc = None
            for r in range(D // RS):
                part = fold8(xs(r))
                acc = part if acc is None else acc + part
                yield
            m = col_total(acc)
            stat1[c, 0:1, :] = m
            acc = None
            for r in range(D // RS):
                xc = xs(r) - m
                part = fold8(xc * xc)
                acc = part if acc is None else acc + part
                yield
            rstd = jax.lax.rsqrt(col_total(acc) + LN_EPS)
            stat1[c, 1:2, :] = rstd
            for r in range(D // RS):
                xn[c, RS * r:RS * (r + 1), :] = (
                    (xs(r) - m) * rstd).astype(BF16)
                yield

    def xn_all():
        return jnp.concatenate([xn[c] for c in range(NQB)], axis=1)

    def rows_of(c):
        return slice(CH * c, CH * (c + 1))

    def packed(words):
        return pltpu.bitcast(words, BF16)

    def wt_rows(wt, c):
        return packed(wt[CH // 2 * c:CH // 2 * (c + 1), :])

    def transpose_keys(g):
        kb[g] = pltpu.bitcast(ktn[WIN * g:WIN * g + 128, :].T, U32)

    def proj_k(c):
        kt = _dot(wt_rows(wkt, c), xn_all())
        pkt[rows_of(c), :] = _phi(kt).astype(BF16)
        ktn[rows_of(c), :] = kt.astype(BF16)
        if c == 0:
            transpose_keys(0)

    def proj_q(c):
        qf = _dot(wt_rows(wqt, c), xn_all())
        qt[rows_of(c), :] = (qf * QSCALE).astype(BF16)
        pqt[rows_of(c), :] = _phi(qf).astype(BF16)

    def proj_v(c):
        tail = jnp.concatenate([jnp.zeros((6, L), F32), jnp.ones((8, L), F32)], axis=0)
        vt = _dot(wt_rows(wvt, c), xn_all())
        vtn[rows_of(c), :] = vt.astype(BF16)
        for j in range(CH // DH):
            h = (CH // DH) * c + j
            vt32[32 * h:32 * h + 16, :] = vt[DH * j:DH * j + 16].astype(BF16)
            vt32[32 * h + 16:32 * h + 32, :] = jnp.concatenate(
                [vt[DH * j + 16:DH * j + 18], tail], axis=0).astype(BF16)

    def masked_q(w0, i, word_mask):
        qu = pltpu.bitcast(qt[pl.ds(w0, 128), 128 * i:128 * (i + 1)], U32)
        return pltpu.bitcast(jnp.where(word_mask, qu, jnp.uint32(0)), BF16)

    def head_word_mask(lo):
        word = jax.lax.broadcasted_iota(I32, (64, 128), 0)
        return (2 * word >= lo) & (2 * word < lo + DH)

    def causal_mask():
        return (jax.lax.broadcasted_iota(I32, (128, 128), 0)
                <= jax.lax.broadcasted_iota(I32, (128, 128), 1))

    def pv_head(h, i):
        n = 128 * (i + 1)
        r0 = TOFF[i] * 128
        o = _dot(vt32[32 * h:32 * h + 32, 0:n], pbuf[h, r0:r0 + n, :])
        a = omg[h] * _recip(o[24:32, :])
        on = (o[0:24].reshape(3, 8, 128) * a).reshape(24, 128)
        ot[i, DH * h:DH * h + 24, :] = on + amem[i, DH * h:DH * h + 24, :]

    def stage_attention_fast(filler):
        causal = causal_mask()
        for h in range(H + LAG):
            if h < H:
                g = GROUP_OF[h]
                word_mask = head_word_mask(DH * h - WIN * g)
                if h == GROUP_HEADS[g][0] and g + 1 < NG:
                    transpose_keys(g + 1)
            for i in range(NQB):
                n = 128 * (i + 1)
                if h < H:
                    filler.upto((NTILE * h + TOFF[i] + i + 1) / (NTILE * (H - 1)))
                    st = _dot(packed(kb[g, 0:n // 2, :]), masked_q(WIN * g, i, word_mask))
                    p = jnp.exp2(st)
                    r0 = TOFF[i] * 128
                    if i > 0:
                        pbuf[h, r0:r0 + 128 * i, :] = p[:n - 128].astype(BF16)
                    pbuf[h, r0 + 128 * i:r0 + n, :] = jnp.where(
                        causal, p[n - 128:n], 0.0).astype(BF16)
                if h >= LAG:
                    pv_head(h - LAG, i)

    def stage_scores_safe():
        causal = causal_mask()
        for g in range(1, NG):
            transpose_keys(g)

        def head(h, carry):
            g = jnp.clip((DH * h + DH - 128 + WIN - 1) // WIN, 0, NG - 1)
            g = jnp.where(DH * h + DH <= 128, 0, g)
            w0 = pl.multiple_of(WIN * g, 16)
            word_mask = head_word_mask(DH * h - WIN * g)
            for i in range(NQB):
                n = 128 * (i + 1)
                st = _dot(packed(kb[g, 0:n // 2, :]), masked_q(w0, i, word_mask))
                sd = jnp.where(causal, st[n - 128:n], -jnp.inf)
                m = jnp.max(sd, axis=0, keepdims=True)
                if i > 0:
                    m = jnp.maximum(m, jnp.max(st[:n - 128], axis=0, keepdims=True))
                r0 = TOFF[i] * 128
                if i > 0:
                    pbuf[h, r0:r0 + 128 * i, :] = jnp.exp2(st[:n - 128] - m).astype(BF16)
                pbuf[h, r0 + 128 * i:r0 + n, :] = jnp.exp2(sd - m).astype(BF16)
            return carry

        jax.lax.fori_loop(0, H, head, 0)

    def attn_block(s, i):
        blk = s * NQB + i
        otb = ot[i, 0:D, :].astype(BF16)
        tot = None
        for c in range(NCH):
            hh = _dot(wt_rows(wot, c), otb) + xbuf[blk, rows_of(c), :].astype(F32)
            h_all[blk, rows_of(c), :] = hh
            part = jnp.sum(hh, axis=0, keepdims=True)
            tot = part if tot is None else tot + part
        stat2[blk, 0:1, :] = tot * (1.0 / D)

    def mem_update(g):
        lhs = jnp.concatenate([jnp.ones((16, L), BF16), vtn[WIN * g:WIN * g + 128, :]], axis=0)
        upd = _dot(lhs, pkt[WIN * g:WIN * g + 128, :], NT)
        m_new = m_f32[g] + upd * keep[g]
        m_f32[g] = m_new
        m_bf[g] = m_new.astype(BF16)

    def mem_read(g):
        for i in range(NQB):
            nm = _dot(m_bf[g], pqt[WIN * g:WIN * g + 128, 128 * i:128 * (i + 1)])
            first = GROUP_HEADS[g][0]
            b = gcol[first:first + 8, :] * _recip(nm[0:8, :] + 1e-6)
            for j, h in enumerate(GROUP_HEADS[g]):
                lo = 16 + DH * h - WIN * g
                n = min(24, MROWS - lo)
                amem[i, DH * h:DH * h + n, :] = nm[lo:lo + n] * b[j:j + 1, :]

    def stat_steps(s, blocks=range(NQB)):
        seg = jnp.maximum(s, 0)
        for i in blocks:
            blk = seg * NQB + i
            m = stat2[blk, 0:1, :]
            acc_v = acc_r = None
            for r in range(D // RS):
                rows = slice(RS * r, RS * (r + 1))
                hc = h_all[blk, rows, :] - m
                pv = fold8(hc * hc)
                pr = fold8(hc * wrcol[rows, :])
                acc_v = pv if acc_v is None else acc_v + pv
                acc_r = pr if acc_r is None else acc_r + pr
                yield
            rstd = jax.lax.rsqrt(col_total(acc_v) + LN_EPS)
            stat2[blk, 1:2, :] = rstd
            r_all[pl.ds(blk, 1), :] = jnp.sum(acc_r, axis=0, keepdims=True) * rstd

    def out_steps(s):
        seg = jnp.maximum(s, 0)
        for i in range(NQB):
            blk = seg * NQB + i
            m = stat2[blk, 0:1, :]
            rstd = stat2[blk, 1:2, :]
            for r in range(D // RS):
                rows = slice(RS * r, RS * (r + 1))
                hh = h_all[blk, rows, :]
                obuf[blk, rows, :] = (hh + (hh - m) * rstd).astype(BF16)
                yield

    x_copy(0).start()
    cp_wk.start()

    beta = beta_ref[...].astype(F32).reshape(1, H)
    gpad = jnp.concatenate([_sigmoid(beta), jnp.zeros((1, 128 - H), F32)], axis=1)
    gcol[...] = jnp.transpose(jnp.broadcast_to(gpad, (128, 128)))
    for h in range(H):
        omg[h] = jnp.broadcast_to(1.0 - gcol[h:h + 1, :], (8, 128))
    wr = jnp.concatenate([wr_ref[...].astype(F32).reshape(1, D), jnp.zeros((1, 64), F32)], axis=1)
    wrcol[...] = jnp.transpose(jnp.broadcast_to(wr, (128, D + 64)))[0:D]
    row = jax.lax.broadcasted_iota(I32, (MROWS, 128), 0)
    lane = jax.lax.broadcasted_iota(I32, (MROWS, 128), 1)
    for g in range(NG):
        first, nh = GROUP_HEADS[g][0], len(GROUP_HEADS[g])
        lane_head = ((lane + WIN * g) * 3641) >> 16
        row_head = jnp.where(row < 16, row + first, ((row - 16 + WIN * g) * 3641) >> 16)
        ok = (lane_head == row_head) & (row_head >= first) & (row_head < first + nh)
        keep[g] = jnp.where(ok, 1.0, 0.0)
    m_f32[...] = jnp.zeros_like(m_f32)
    amem[...] = jnp.zeros_like(amem)

    h_all[0:NQB] = jnp.zeros((NQB, D, 128), F32)
    obuf[NSEG * NQB:(NSEG + 1) * NQB] = jnp.zeros((NQB, D, 128), BF16)
    stat2[0:NQB] = jnp.zeros((NQB, 8, 128), F32)

    def transpose_tile(dst, raw, t):
        hi = min(128 * (t + 1), D)
        dst[64 * t:hi // 2, :] = pltpu.bitcast(raw[:, 128 * t:hi].T, U32)

    def col_norm_steps(raw, slot):
        for t in range(5):
            hi = min(128 * (t + 1), D)
            for k in range(3):
                w = raw[192 * k:192 * (k + 1), 128 * t:hi].astype(F32)
                wnorm[slot, 8 * k:8 * (k + 1), 128 * t:hi] = jnp.sum(
                    (w * w).reshape(24, 8, hi - 128 * t), axis=0)
                yield

    x_copy(0).wait()
    cp_wq.start()
    for _ in ln1_steps(0):
        pass
    cp_wk.wait()
    cp_wv.start()
    side = _Filler([col_norm_steps(wk_raw, 0)], [15])
    transpose_tile(wkt, wk_raw, 0)
    transpose_tile(wkt, wk_raw, 1)
    proj_k(0)
    transpose_tile(wkt, wk_raw, 2)
    side.upto(0.5)
    proj_k(1)
    transpose_tile(wkt, wk_raw, 3)
    side.upto(1.0)
    proj_k(2)
    transpose_tile(wkt, wk_raw, 4)
    cp_wq.wait()
    cp_wv.wait()
    cp_wo.start()
    x_copy(1).start()
    transpose_tile(wqt, wq_raw, 0)
    transpose_tile(wqt, wq_raw, 1)
    proj_k(3)
    side = _Filler([col_norm_steps(wq_raw, 1), col_norm_steps(wv_raw, 2)], [15, 15])
    for c in range(NCH):
        proj_q(c)
        if c + 2 < 5:
            transpose_tile(wqt, wq_raw, c + 2)
        if c >= 2:
            transpose_tile(wvt, wv_raw, c - 2)
        if c < NCH - 1:
            side.upto((c + 1) / (NCH - 1))
    cp_wo.wait()
    x_copy(1).wait()
    for s in range(2, NSEG):
        x_copy(s).start()
    cp_wg.start()
    cp_wu.start()
    cp_wd.start()
    for c in range(NCH):
        proj_v(c)
        if c + 2 < 5:
            transpose_tile(wvt, wv_raw, c + 2)
        transpose_tile(wot, wo_raw, c)
    transpose_tile(wot, wo_raw, 4)

    def max_norm(slot):
        ss = jnp.sum(wnorm[slot], axis=0, keepdims=True)
        return jnp.sqrt(jnp.max(ss, axis=1, keepdims=True))

    nk, nq, nv = max_norm(0), max_norm(1), max_norm(2)

    bound = (QSCALE * DH * D) * nq * nk
    safe = (bound <= SAFE_LOGIT) & (nv * (D ** 0.5) <= SAFE_V)
    flag[0] = jnp.sum(jnp.where(safe, 1, 0).astype(I32))

    def segment(s, carry):
        @pl.when(jnp.logical_and(s > 0, s + 1 < NSEG))
        def _():
            x_copy(s + 1).wait()

        def side_work():
            return _Filler([_chain(stat_steps(s - 1), out_steps(s - 1)), ln1_steps(s + 1)],
                           [2 * PASS_STEPS, 3 * PASS_STEPS])

        def fast():
            stage_attention_fast(side_work())

        def safe():
            stage_scores_safe()
            side_work().upto(1.0)
            for h in range(H):
                for i in range(NQB):
                    pv_head(h, i)

        jax.lax.cond(flag[0] == 1, fast, safe)

        @pl.when(s + 1 < NSEG)
        def _():
            prev_out_copy(s).start()
            for i in range(NQB):
                attn_block(s, i)
            for g in range(NG):
                mem_update(g)
            for c in range(NCH):
                proj_q(c)
            for c in range(NCH):
                proj_k(c)
            for g in range(NG):
                mem_read(g)
            for c in range(NCH):
                proj_v(c)

        return carry

    jax.lax.fori_loop(0, NSEG, segment, 0)

    out_copy(NSEG - 2).start()
    prev_out_copy(0).wait()
    for i in range(NQB):
        attn_block(NSEG - 1, i)
        if i > 0:
            for _ in stat_steps(NSEG - 1, [i - 1]):
                pass
    for _ in stat_steps(NSEG - 1, [NQB - 1]):
        pass

    r = r_all[...]
    r_sel = jnp.max(jnp.max(r, axis=0, keepdims=True), axis=1, keepdims=True)
    ids = (128 * jax.lax.broadcasted_iota(I32, r.shape, 0)
           + jax.lax.broadcasted_iota(I32, r.shape, 1))
    cand = jnp.min(jnp.where(r == r_sel, ids, S), axis=0, keepdims=True)
    idx = jnp.minimum(jnp.sum(jnp.min(cand, axis=1, keepdims=True)), S - 1)
    for _ in out_steps(NSEG - 1):
        pass
    out_copy(NSEG - 1).start()
    blk = idx >> 7
    m_sel = stat2[blk, 0:1, :]
    rstd_sel = stat2[blk, 1:2, :]
    for r in range(D // RS):
        rows = slice(RS * r, RS * (r + 1))
        hn_sel[rows, :] = ((h_all[blk, rows, :] - m_sel) * rstd_sel).astype(BF16)
    onehot = (jax.lax.broadcasted_iota(I32, (16, 128), 1) == idx - blk * 128).astype(BF16)
    xs = _dot(onehot, hn_sel[...], NT).astype(BF16)
    cp_wg.wait()
    cp_wu.wait()
    cp_wd.wait()

    def down_steps(c, act):
        for r in range(D // RS):
            rows = slice(RS * r, RS * (r + 1))
            part = None if c == 0 else yacc[rows, :]
            for t in range(FC // 128):
                w = wdt_v[rows, FC * c + 128 * t:FC * c + 128 * (t + 1)].astype(F32)
                part = w * act[t] if part is None else part + w * act[t]
            yacc[rows, :] = part
            yield

    nch = FF // FC
    pending = None
    for c in range(nch):
        ga, up = [], []
        for t in range(FC // 128):
            tile = slice(FC * c + 128 * t, FC * c + 128 * (t + 1))
            ga.append(_dot(xs, wg_v[:, tile])[0:1])
            up.append(_dot(xs, wu_v[:, tile])[0:1])
            if pending is not None:
                pending.upto((t + 1) / (FC // 128))
        act = [g * _sigmoid(g) * u for g, u in zip(ga, up)]
        pending = _Filler([down_steps(c, act)], [D // RS])
    pending.upto(1.0)
    y = jnp.sum(yacc[...], axis=1, keepdims=True) * _sigmoid(r_sel)
    sel = jax.lax.broadcasted_iota(I32, (RS, 128), 1) == idx - blk * 128
    for r in range(D // RS):
        rows = slice(RS * r, RS * (r + 1))
        hh = h_all[blk, rows, :]
        stage[rows, :] = (hh + (hh - m_sel) * rstd_sel
                          + jnp.where(sel, y[rows], 0.0)).astype(BF16)
    for s in range(NSEG):
        out_copy(s).wait()
    fix = pltpu.make_async_copy(stage, out_hbm.at[:, hbm_cols(blk)], sem_w.at[7])
    fix.start()
    fix.wait()


@jax.jit
def pallas_sequential_preLN__memory_aug_infini_attn__moe_arch_mod__prompt_kernel(
    A_x: jax.Array,
    A_wq: jax.Array,
    A_wk: jax.Array,
    A_wv: jax.Array,
    A_wo: jax.Array,
    A_beta: jax.Array,
    B_x: jax.Array,
    B_w_r: jax.Array,
    B_w_gate: jax.Array,
    B_w_up: jax.Array,
    B_w_down: jax.Array,
):
    del B_x
    hbm = pl.BlockSpec(memory_space=pltpu.HBM)
    vmem = pl.BlockSpec(memory_space=pltpu.VMEM)
    scratch = [
        pltpu.VMEM((NSEG * NQB, D, 128), BF16),
        pltpu.VMEM((D, D), BF16),
        pltpu.VMEM((D, D), BF16),
        pltpu.VMEM((D, D), BF16),
        pltpu.VMEM((D, D), BF16),
        pltpu.VMEM((D // 2, D), U32),
        pltpu.VMEM((D // 2, D), U32),
        pltpu.VMEM((D // 2, D), U32),
        pltpu.VMEM((D // 2, D), U32),
        pltpu.VMEM((NQB, D, 128), BF16),
        pltpu.VMEM((D, L), BF16),
        pltpu.VMEM((NG, L // 2, 128), U32),
        pltpu.VMEM((D, L), BF16),
        pltpu.VMEM((D, L), BF16),
        pltpu.VMEM((D, L), BF16),
        pltpu.VMEM((D, L), BF16),
        pltpu.VMEM((H * 32, L), BF16),
        pltpu.VMEM((H, NTILE * 128, 128), BF16),
        pltpu.VMEM((NG, MROWS, 128), F32),
        pltpu.VMEM((NG, MROWS, 128), BF16),
        pltpu.VMEM((NG, MROWS, 128), F32),
        pltpu.VMEM((NQB, D + 24, 128), F32),
        pltpu.VMEM((NQB, D + 24, 128), F32),
        pltpu.VMEM((NSEG * NQB, D, 128), F32),
        pltpu.VMEM((D, 128), BF16),
        pltpu.VMEM((D, 128), F32),
        pltpu.VMEM(((NSEG + 1) * NQB, D, 128), BF16),
        pltpu.VMEM((D, FF), BF16),
        pltpu.VMEM((D, FF), BF16),
        pltpu.VMEM((D, FF), BF16),
        pltpu.VMEM((128, 128), F32),
        pltpu.VMEM((H, 8, 128), F32),
        pltpu.VMEM((D, 128), F32),
        pltpu.VMEM((NQB, 8, 128), F32),
        pltpu.VMEM((NSEG * NQB, 8, 128), F32),
        pltpu.VMEM((3, 24, D), F32),
        pltpu.VMEM((NSEG * NQB, 128), F32),
        pltpu.VMEM((D, 128), BF16),
        pltpu.SMEM((1,), I32),
        pltpu.SemaphoreType.DMA((NSEG,)),
        pltpu.SemaphoreType.DMA((8,)),
        pltpu.SemaphoreType.DMA((NSEG + 1,)),
    ]
    out_t = pl.pallas_call(
        _kernel,
        out_shape=jax.ShapeDtypeStruct((D, S), BF16),
        in_specs=[hbm, hbm, hbm, hbm, hbm, vmem, vmem, hbm, hbm, hbm],
        out_specs=hbm,
        scratch_shapes=scratch,
        compiler_params=pltpu.CompilerParams(vmem_limit_bytes=100 * 1024 * 1024),
        name="infini_moe",
    )(A_x.reshape(S, D).T, A_wq, A_wk, A_wv, A_wo, A_beta, B_w_r, B_w_gate, B_w_up, B_w_down.T)
    return out_t.T.reshape(1, S, D)
```

```python
import functools

import jax
import jax.numpy as jnp
import jax.experimental.pallas as pl
import jax.experimental.pallas.tpu as pltpu

F32 = jnp.float32
BF16 = jnp.bfloat16
U32 = jnp.uint32
I32 = jnp.int32

S = 2048
D = 576
H = 32
DH = 18
NSEG = 4
L = S // NSEG
FF = 4608
NQB = L // 128
TOFF = (0, 1, 3, 6)
NTILE = 10
NG = 5
WIN = 112
GROUP_HEADS = tuple(tuple(h for h in range(H)
                          if min(max(0, -(-(DH * h + DH - 128) // WIN)), NG - 1) == g)
                    for g in range(NG))
GROUP_OF = {h: g for g in range(NG) for h in GROUP_HEADS[g]}
MROWS = 144
CH = 144
NCH = D // CH
RS = 64
PASS_STEPS = NQB * (D // RS)
FC = 512
LAG = 20
LN_EPS = 1e-5
LOG2E = 1.4426950408889634
QSCALE = (DH ** -0.5) * LOG2E
SAFE_LOGIT = 60.0
SAFE_V = 2.0 ** 50

NN = (((1,), (0,)), ((), ()))
NT = (((1,), (1,)), ((), ()))

for _g, _hs in enumerate(GROUP_HEADS):
    for _h in _hs:
        assert WIN * _g <= DH * _h and DH * _h + DH <= WIN * _g + 128


def _dot(a, b, dims=NN):
    return jax.lax.dot_general(a, b, dims, preferred_element_type=F32)


class _Filler:
    def __init__(self, gens, counts):
        self.gens, self.counts, self.done = gens, counts, [0] * len(gens)

    def upto(self, frac):
        for k, gen in enumerate(self.gens):
            while self.done[k] < min(frac, 1.0) * self.counts[k]:
                next(gen, None)
                self.done[k] += 1
            if frac >= 1.0:
                for _ in gen:
                    pass


def _chain(*gens):
    for gen in gens:
        yield from gen


def _phi(t):
    return jnp.where(t > 0, t + 1.0, jnp.exp(t))


def _sigmoid(t):
    return 1.0 / (1.0 + jnp.exp(-t))


def _recip(x):
    r = pl.reciprocal(x, approx=True)
    return r * (2.0 - x * r)


def _kernel(xt_hbm, wq_hbm, wk_hbm, wv_hbm, wo_hbm, beta_ref, wr_ref, wg_hbm, wu_hbm, wdt_hbm,
            out_hbm,
            xbuf, wq_raw, wk_raw, wv_raw, wo_raw, wqt, wkt, wvt, wot, xn, ktn, kb, qt, pkt, pqt,
            vtn, vt32, pbuf, m_f32, m_bf, keep, amem, ot, h_all, hn_sel, yacc, obuf, wg_v, wu_v, wdt_v,
            gcol, omg, wrcol, stat2, wnorm, r_all, stage, flag, sem_x, sem_w, sem_o):
    class _Group:
        def __init__(self, copies):
            self.copies = copies

        def start(self):
            for cp in self.copies:
                cp.start()

        def wait(self):
            for cp in self.copies:
                cp.wait()

    def hbm_cols(blk):
        return pl.ds(pl.multiple_of(blk * 128, 128), 128)

    def x_copy(s):
        return _Group([pltpu.make_async_copy(xt_hbm.at[:, hbm_cols(s * NQB + i)],
                                             xbuf.at[s * NQB + i], sem_x.at[s])
                       for i in range(NQB)])

    def out_copy(s):
        return _Group([pltpu.make_async_copy(obuf.at[s * NQB + i],
                                             out_hbm.at[:, hbm_cols(s * NQB + i)], sem_o.at[s])
                       for i in range(NQB)])

    def prev_out_copy(s):
        src = jnp.where(s > 0, s - 1, NSEG) * NQB
        dst = jnp.where(s > 0, s - 1, NSEG - 1) * NQB
        sem = jnp.where(s > 0, s - 1, NSEG)
        return _Group([pltpu.make_async_copy(obuf.at[src + i], out_hbm.at[:, hbm_cols(dst + i)],
                                             sem_o.at[sem]) for i in range(NQB)])

    cp_wk = pltpu.make_async_copy(wk_hbm, wk_raw, sem_w.at[0])
    cp_wq = pltpu.make_async_copy(wq_hbm, wq_raw, sem_w.at[1])
    cp_wv = pltpu.make_async_copy(wv_hbm, wv_raw, sem_w.at[2])
    cp_wo = pltpu.make_async_copy(wo_hbm, wo_raw, sem_w.at[3])
    cp_wg = pltpu.make_async_copy(wg_hbm, wg_v, sem_w.at[4])
    cp_wu = pltpu.make_async_copy(wu_hbm, wu_v, sem_w.at[5])
    cp_wd = pltpu.make_async_copy(wdt_hbm, wdt_v, sem_w.at[6])

    def fold8(v):
        return jnp.sum(v.reshape(v.shape[0] // 8, 8, 128), axis=0)

    def col_total(acc):
        return jnp.sum(acc, axis=0, keepdims=True) * (1.0 / D)

    def ln1_steps(s):
        seg = jnp.minimum(s, NSEG - 1)
        for c in range(NQB):
            xs = lambda r: xbuf[seg * NQB + c, RS * r:RS * (r + 1), :].astype(F32)
            acc = None
            for r in range(D // RS):
                part = fold8(xs(r))
                acc = part if acc is None else acc + part
                yield
            m = col_total(acc)
            acc = None
            for r in range(D // RS):
                xc = xs(r) - m
                part = fold8(xc * xc)
                acc = part if acc is None else acc + part
                yield
            rstd = jax.lax.rsqrt(col_total(acc) + LN_EPS)
            for r in range(D // RS):
                xn[c, RS * r:RS * (r + 1), :] = (
                    (xs(r) - m) * rstd).astype(BF16)
                yield

    def xn_all():
        return jnp.concatenate([xn[c] for c in range(NQB)], axis=1)

    def rows_of(c):
        return slice(CH * c, CH * (c + 1))

    def packed(words):
        return pltpu.bitcast(words, BF16)

    def wt_rows(wt, c):
        return packed(wt[CH // 2 * c:CH // 2 * (c + 1), :])

    def transpose_keys(g):
        kb[g] = pltpu.bitcast(ktn[WIN * g:WIN * g + 128, :].T, U32)

    def proj_k(c):
        kt = _dot(wt_rows(wkt, c), xn_all())
        pkt[rows_of(c), :] = _phi(kt).astype(BF16)
        ktn[rows_of(c), :] = kt.astype(BF16)
        if c == 0:
            transpose_keys(0)

    def proj_q(c):
        qf = _dot(wt_rows(wqt, c), xn_all())
        qt[rows_of(c), :] = (qf * QSCALE).astype(BF16)
        pqt[rows_of(c), :] = _phi(qf).astype(BF16)

    def proj_v(c):
        tail = jnp.concatenate([jnp.zeros((6, L), F32), jnp.ones((8, L), F32)], axis=0)
        vt = _dot(wt_rows(wvt, c), xn_all())
        vtn[rows_of(c), :] = vt.astype(BF16)
        for j in range(CH // DH):
            h = (CH // DH) * c + j
            vt32[32 * h:32 * h + 16, :] = vt[DH * j:DH * j + 16].astype(BF16)
            vt32[32 * h + 16:32 * h + 32, :] = jnp.concatenate(
                [vt[DH * j + 16:DH * j + 18], tail], axis=0).astype(BF16)

    def masked_q(w0, i, word_mask):
        qu = pltpu.bitcast(qt[pl.ds(w0, 128), 128 * i:128 * (i + 1)], U32)
        return pltpu.bitcast(jnp.where(word_mask, qu, jnp.uint32(0)), BF16)

    def head_word_mask(lo):
        word = jax.lax.broadcasted_iota(I32, (64, 128), 0)
        return (2 * word >= lo) & (2 * word < lo + DH)

    def causal_mask():
        return (jax.lax.broadcasted_iota(I32, (128, 128), 0)
                <= jax.lax.broadcasted_iota(I32, (128, 128), 1))

    def pv_head(h, i):
        n = 128 * (i + 1)
        r0 = TOFF[i] * 128
        o = _dot(vt32[32 * h:32 * h + 32, 0:n], pbuf[h, r0:r0 + n, :])
        a = omg[h] * _recip(o[24:32, :])
        on = (o[0:24].reshape(3, 8, 128) * a).reshape(24, 128)
        ot[i, DH * h:DH * h + 24, :] = on + amem[i, DH * h:DH * h + 24, :]

    def stage_attention_fast(filler):
        causal = causal_mask()
        for h in range(H + LAG):
            if h < H:
                g = GROUP_OF[h]
                word_mask = head_word_mask(DH * h - WIN * g)
                if h == GROUP_HEADS[g][0] and g + 1 < NG:
                    transpose_keys(g + 1)
            for i in range(NQB):
                n = 128 * (i + 1)
                if h < H:
                    filler.upto((NTILE * h + TOFF[i] + i + 1) / (NTILE * (H - 1)))
                    st = _dot(packed(kb[g, 0:n // 2, :]), masked_q(WIN * g, i, word_mask))
                    p = jnp.exp2(st)
                    r0 = TOFF[i] * 128
                    if i > 0:
                        pbuf[h, r0:r0 + 128 * i, :] = p[:n - 128].astype(BF16)
                    pbuf[h, r0 + 128 * i:r0 + n, :] = jnp.where(
                        causal, p[n - 128:n], 0.0).astype(BF16)
                if h >= LAG:
                    pv_head(h - LAG, i)

    def stage_scores_safe():
        causal = causal_mask()
        for g in range(1, NG):
            transpose_keys(g)

        def head(h, carry):
            g = jnp.clip((DH * h + DH - 128 + WIN - 1) // WIN, 0, NG - 1)
            g = jnp.where(DH * h + DH <= 128, 0, g)
            w0 = pl.multiple_of(WIN * g, 16)
            word_mask = head_word_mask(DH * h - WIN * g)
            for i in range(NQB):
                n = 128 * (i + 1)
                st = _dot(packed(kb[g, 0:n // 2, :]), masked_q(w0, i, word_mask))
                sd = jnp.where(causal, st[n - 128:n], -jnp.inf)
                m = jnp.max(sd, axis=0, keepdims=True)
                if i > 0:
                    m = jnp.maximum(m, jnp.max(st[:n - 128], axis=0, keepdims=True))
                r0 = TOFF[i] * 128
                if i > 0:
                    pbuf[h, r0:r0 + 128 * i, :] = jnp.exp2(st[:n - 128] - m).astype(BF16)
                pbuf[h, r0 + 128 * i:r0 + n, :] = jnp.exp2(sd - m).astype(BF16)
            return carry

        jax.lax.fori_loop(0, H, head, 0)

    def attn_block(s, i):
        blk = s * NQB + i
        otb = ot[i, 0:D, :].astype(BF16)
        tot = None
        for c in range(NCH):
            hh = _dot(wt_rows(wot, c), otb) + xbuf[blk, rows_of(c), :].astype(F32)
            h_all[blk, rows_of(c), :] = hh
            part = jnp.sum(hh, axis=0, keepdims=True)
            tot = part if tot is None else tot + part
        stat2[blk, 0:1, :] = tot * (1.0 / D)

    def mem_update(g):
        lhs = jnp.concatenate([jnp.ones((16, L), BF16), vtn[WIN * g:WIN * g + 128, :]], axis=0)
        upd = _dot(lhs, pkt[WIN * g:WIN * g + 128, :], NT)
        m_new = m_f32[g] + upd * keep[g]
        m_f32[g] = m_new
        m_bf[g] = m_new.astype(BF16)

    def mem_read(g):
        for i in range(NQB):
            nm = _dot(m_bf[g], pqt[WIN * g:WIN * g + 128, 128 * i:128 * (i + 1)])
            first = GROUP_HEADS[g][0]
            b = gcol[first:first + 8, :] * _recip(nm[0:8, :] + 1e-6)
            for j, h in enumerate(GROUP_HEADS[g]):
                lo = 16 + DH * h - WIN * g
                n = min(24, MROWS - lo)
                amem[i, DH * h:DH * h + n, :] = nm[lo:lo + n] * b[j:j + 1, :]

    def stat_steps(s, blocks=range(NQB)):
        seg = jnp.maximum(s, 0)
        for i in blocks:
            blk = seg * NQB + i
            m = stat2[blk, 0:1, :]
            acc_v = acc_r = None
            for r in range(D // RS):
                rows = slice(RS * r, RS * (r + 1))
                hc = h_all[blk, rows, :] - m
                pv = fold8(hc * hc)
                pr = fold8(hc * wrcol[rows, :])
                acc_v = pv if acc_v is None else acc_v + pv
                acc_r = pr if acc_r is None else acc_r + pr
                yield
            rstd = jax.lax.rsqrt(col_total(acc_v) + LN_EPS)
            stat2[blk, 1:2, :] = rstd
            r_all[pl.ds(blk, 1), :] = jnp.sum(acc_r, axis=0, keepdims=True) * rstd

    def out_steps(s):
        seg = jnp.maximum(s, 0)
        for i in range(NQB):
            blk = seg * NQB + i
            m = stat2[blk, 0:1, :]
            rstd = stat2[blk, 1:2, :]
            for r in range(D // RS):
                rows = slice(RS * r, RS * (r + 1))
                hh = h_all[blk, rows, :]
                obuf[blk, rows, :] = (hh + (hh - m) * rstd).astype(BF16)
                yield

    x_copy(0).start()
    cp_wk.start()

    beta = beta_ref[...].astype(F32).reshape(1, H)
    gpad = jnp.concatenate([_sigmoid(beta), jnp.zeros((1, 128 - H), F32)], axis=1)
    gcol[...] = jnp.transpose(jnp.broadcast_to(gpad, (128, 128)))
    for h in range(H):
        omg[h] = jnp.broadcast_to(1.0 - gcol[h:h + 1, :], (8, 128))
    wr = jnp.concatenate([wr_ref[...].astype(F32).reshape(1, D), jnp.zeros((1, 64), F32)], axis=1)
    wrcol[...] = jnp.transpose(jnp.broadcast_to(wr, (128, D + 64)))[0:D]
    row = jax.lax.broadcasted_iota(I32, (MROWS, 128), 0)
    lane = jax.lax.broadcasted_iota(I32, (MROWS, 128), 1)
    for g in range(NG):
        first, nh = GROUP_HEADS[g][0], len(GROUP_HEADS[g])
        lane_head = ((lane + WIN * g) * 3641) >> 16
        row_head = jnp.where(row < 16, row + first, ((row - 16 + WIN * g) * 3641) >> 16)
        ok = (lane_head == row_head) & (row_head >= first) & (row_head < first + nh)
        keep[g] = jnp.where(ok, 1.0, 0.0)
    m_f32[...] = jnp.zeros_like(m_f32)
    amem[...] = jnp.zeros_like(amem)

    h_all[0:NQB] = jnp.zeros((NQB, D, 128), F32)
    obuf[NSEG * NQB:(NSEG + 1) * NQB] = jnp.zeros((NQB, D, 128), BF16)
    stat2[0:NQB] = jnp.zeros((NQB, 8, 128), F32)

    def transpose_tile(dst, raw, t):
        hi = min(128 * (t + 1), D)
        dst[64 * t:hi // 2, :] = pltpu.bitcast(raw[:, 128 * t:hi].T, U32)

    def col_norm_steps(raw, slot):
        for t in range(5):
            hi = min(128 * (t + 1), D)
            for k in range(3):
                w = raw[192 * k:192 * (k + 1), 128 * t:hi].astype(F32)
                wnorm[slot, 8 * k:8 * (k + 1), 128 * t:hi] = jnp.sum(
                    (w * w).reshape(24, 8, hi - 128 * t), axis=0)
                yield

    x_copy(0).wait()
    cp_wq.start()
    for _ in ln1_steps(0):
        pass
    cp_wk.wait()
    cp_wv.start()
    side = _Filler([col_norm_steps(wk_raw, 0)], [15])
    transpose_tile(wkt, wk_raw, 0)
    transpose_tile(wkt, wk_raw, 1)
    proj_k(0)
    transpose_tile(wkt, wk_raw, 2)
    side.upto(0.5)
    proj_k(1)
    transpose_tile(wkt, wk_raw, 3)
    side.upto(1.0)
    proj_k(2)
    transpose_tile(wkt, wk_raw, 4)
    cp_wq.wait()
    cp_wv.wait()
    cp_wo.start()
    x_copy(1).start()
    transpose_tile(wqt, wq_raw, 0)
    transpose_tile(wqt, wq_raw, 1)
    proj_k(3)
    side = _Filler([col_norm_steps(wq_raw, 1), col_norm_steps(wv_raw, 2)], [15, 15])
    for c in range(NCH):
        proj_q(c)
        if c + 2 < 5:
            transpose_tile(wqt, wq_raw, c + 2)
        if c >= 2:
            transpose_tile(wvt, wv_raw, c - 2)
        if c < NCH - 1:
            side.upto((c + 1) / (NCH - 1))
    cp_wo.wait()
    x_copy(1).wait()
    for s in range(2, NSEG):
        x_copy(s).start()
    cp_wg.start()
    cp_wu.start()
    cp_wd.start()
    for c in range(NCH):
        proj_v(c)
        if c + 2 < 5:
            transpose_tile(wvt, wv_raw, c + 2)
        transpose_tile(wot, wo_raw, c)
    transpose_tile(wot, wo_raw, 4)

    def max_norm(slot):
        ss = jnp.sum(wnorm[slot], axis=0, keepdims=True)
        return jnp.sqrt(jnp.max(ss, axis=1, keepdims=True))

    nk, nq, nv = max_norm(0), max_norm(1), max_norm(2)

    bound = (QSCALE * DH * D) * nq * nk
    safe = (bound <= SAFE_LOGIT) & (nv * (D ** 0.5) <= SAFE_V)
    flag[0] = jnp.sum(jnp.where(safe, 1, 0).astype(I32))

    def segment(s, carry):
        @pl.when(jnp.logical_and(s > 0, s + 1 < NSEG))
        def _():
            x_copy(s + 1).wait()

        def side_work():
            return _Filler([_chain(stat_steps(s - 1), out_steps(s - 1)), ln1_steps(s + 1)],
                           [2 * PASS_STEPS, 3 * PASS_STEPS])

        def fast():
            stage_attention_fast(side_work())

        def safe():
            stage_scores_safe()
            side_work().upto(1.0)
            for h in range(H):
                for i in range(NQB):
                    pv_head(h, i)

        jax.lax.cond(flag[0] == 1, fast, safe)

        @pl.when(s + 1 < NSEG)
        def _():
            prev_out_copy(s).start()
            for i in range(NQB):
                attn_block(s, i)
            for g in range(NG):
                mem_update(g)
            for c in range(NCH):
                proj_q(c)
            for c in range(NCH):
                proj_k(c)
            for g in range(NG):
                mem_read(g)
            for c in range(NCH):
                proj_v(c)

        return carry

    jax.lax.fori_loop(0, NSEG, segment, 0)

    out_copy(NSEG - 2).start()
    prev_out_copy(0).wait()
    for i in range(NQB):
        attn_block(NSEG - 1, i)
        if i > 0:
            for _ in stat_steps(NSEG - 1, [i - 1]):
                pass
    for _ in stat_steps(NSEG - 1, [NQB - 1]):
        pass

    r = r_all[...]
    r_sel = jnp.max(jnp.max(r, axis=0, keepdims=True), axis=1, keepdims=True)
    ids = (128 * jax.lax.broadcasted_iota(I32, r.shape, 0)
           + jax.lax.broadcasted_iota(I32, r.shape, 1))
    cand = jnp.min(jnp.where(r == r_sel, ids, S), axis=0, keepdims=True)
    idx = jnp.minimum(jnp.sum(jnp.min(cand, axis=1, keepdims=True)), S - 1)
    for _ in out_steps(NSEG - 1):
        pass
    out_copy(NSEG - 1).start()
    blk = idx >> 7
    m_sel = stat2[blk, 0:1, :]
    rstd_sel = stat2[blk, 1:2, :]
    for r in range(D // RS):
        rows = slice(RS * r, RS * (r + 1))
        hn_sel[rows, :] = ((h_all[blk, rows, :] - m_sel) * rstd_sel).astype(BF16)
    onehot = (jax.lax.broadcasted_iota(I32, (16, 128), 1) == idx - blk * 128).astype(BF16)
    xs = _dot(onehot, hn_sel[...], NT).astype(BF16)
    cp_wg.wait()
    cp_wu.wait()
    cp_wd.wait()

    def down_steps(c, act):
        for r in range(D // RS):
            rows = slice(RS * r, RS * (r + 1))
            part = None if c == 0 else yacc[rows, :]
            for t in range(FC // 128):
                w = wdt_v[rows, FC * c + 128 * t:FC * c + 128 * (t + 1)].astype(F32)
                part = w * act[t] if part is None else part + w * act[t]
            yacc[rows, :] = part
            yield

    nch = FF // FC
    pending = None
    for c in range(nch):
        ga, up = [], []
        for t in range(FC // 128):
            tile = slice(FC * c + 128 * t, FC * c + 128 * (t + 1))
            ga.append(_dot(xs, wg_v[:, tile])[0:1])
            up.append(_dot(xs, wu_v[:, tile])[0:1])
            if pending is not None:
                pending.upto((t + 1) / (FC // 128))
        act = [g * _sigmoid(g) * u for g, u in zip(ga, up)]
        pending = _Filler([down_steps(c, act)], [D // RS])
    pending.upto(1.0)
    y = jnp.sum(yacc[...], axis=1, keepdims=True) * _sigmoid(r_sel)
    sel = jax.lax.broadcasted_iota(I32, (RS, 128), 1) == idx - blk * 128
    for r in range(D // RS):
        rows = slice(RS * r, RS * (r + 1))
        hh = h_all[blk, rows, :]
        stage[rows, :] = (hh + (hh - m_sel) * rstd_sel
                          + jnp.where(sel, y[rows], 0.0)).astype(BF16)
    for s in range(NSEG):
        out_copy(s).wait()
    fix = pltpu.make_async_copy(stage, out_hbm.at[:, hbm_cols(blk)], sem_w.at[7])
    fix.start()
    fix.wait()


@jax.jit
def pallas_sequential_preLN__memory_aug_infini_attn__moe_arch_mod__prompt_kernel(
    A_x: jax.Array,
    A_wq: jax.Array,
    A_wk: jax.Array,
    A_wv: jax.Array,
    A_wo: jax.Array,
    A_beta: jax.Array,
    B_x: jax.Array,
    B_w_r: jax.Array,
    B_w_gate: jax.Array,
    B_w_up: jax.Array,
    B_w_down: jax.Array,
):
    del B_x
    hbm = pl.BlockSpec(memory_space=pltpu.HBM)
    vmem = pl.BlockSpec(memory_space=pltpu.VMEM)
    scratch = [
        pltpu.VMEM((NSEG * NQB, D, 128), BF16),
        pltpu.VMEM((D, D), BF16),
        pltpu.VMEM((D, D), BF16),
        pltpu.VMEM((D, D), BF16),
        pltpu.VMEM((D, D), BF16),
        pltpu.VMEM((D // 2, D), U32),
        pltpu.VMEM((D // 2, D), U32),
        pltpu.VMEM((D // 2, D), U32),
        pltpu.VMEM((D // 2, D), U32),
        pltpu.VMEM((NQB, D, 128), BF16),
        pltpu.VMEM((D, L), BF16),
        pltpu.VMEM((NG, L // 2, 128), U32),
        pltpu.VMEM((D, L), BF16),
        pltpu.VMEM((D, L), BF16),
        pltpu.VMEM((D, L), BF16),
        pltpu.VMEM((D, L), BF16),
        pltpu.VMEM((H * 32, L), BF16),
        pltpu.VMEM((H, NTILE * 128, 128), BF16),
        pltpu.VMEM((NG, MROWS, 128), F32),
        pltpu.VMEM((NG, MROWS, 128), BF16),
        pltpu.VMEM((NG, MROWS, 128), F32),
        pltpu.VMEM((NQB, D + 24, 128), F32),
        pltpu.VMEM((NQB, D + 24, 128), F32),
        pltpu.VMEM((NSEG * NQB, D, 128), F32),
        pltpu.VMEM((D, 128), BF16),
        pltpu.VMEM((D, 128), F32),
        pltpu.VMEM(((NSEG + 1) * NQB, D, 128), BF16),
        pltpu.VMEM((D, FF), BF16),
        pltpu.VMEM((D, FF), BF16),
        pltpu.VMEM((D, FF), BF16),
        pltpu.VMEM((128, 128), F32),
        pltpu.VMEM((H, 8, 128), F32),
        pltpu.VMEM((D, 128), F32),
        pltpu.VMEM((NSEG * NQB, 8, 128), F32),
        pltpu.VMEM((3, 24, D), F32),
        pltpu.VMEM((NSEG * NQB, 128), F32),
        pltpu.VMEM((D, 128), BF16),
        pltpu.SMEM((1,), I32),
        pltpu.SemaphoreType.DMA((NSEG,)),
        pltpu.SemaphoreType.DMA((8,)),
        pltpu.SemaphoreType.DMA((NSEG + 1,)),
    ]
    out_t = pl.pallas_call(
        _kernel,
        out_shape=jax.ShapeDtypeStruct((D, S), BF16),
        in_specs=[hbm, hbm, hbm, hbm, hbm, vmem, vmem, hbm, hbm, hbm],
        out_specs=hbm,
        scratch_shapes=scratch,
        compiler_params=pltpu.CompilerParams(vmem_limit_bytes=100 * 1024 * 1024),
        name="infini_moe",
    )(A_x.reshape(S, D).T, A_wq, A_wk, A_wv, A_wo, A_beta, B_w_r, B_w_gate, B_w_up, B_w_down.T)
    return out_t.T.reshape(1, S, D)
```

```python
import functools

import jax
import jax.numpy as jnp
import jax.experimental.pallas as pl
import jax.experimental.pallas.tpu as pltpu

F32 = jnp.float32
BF16 = jnp.bfloat16
U32 = jnp.uint32
I32 = jnp.int32

S = 2048
D = 576
H = 32
DH = 18
NSEG = 4
L = S // NSEG
FF = 4608
NQB = L // 128
TOFF = (0, 1, 3, 6)
NTILE = 10
NG = 5
WIN = 112
GROUP_HEADS = tuple(tuple(h for h in range(H)
                          if min(max(0, -(-(DH * h + DH - 128) // WIN)), NG - 1) == g)
                    for g in range(NG))
GROUP_OF = {h: g for g in range(NG) for h in GROUP_HEADS[g]}
MROWS = 144
CH = 144
NCH = D // CH
RS = 64
PASS_STEPS = NQB * (D // RS)
FC = 512
LAG = 20
LN_EPS = 1e-5
LOG2E = 1.4426950408889634
QSCALE = (DH ** -0.5) * LOG2E
SAFE_LOGIT = 60.0
SAFE_V = 2.0 ** 50

NN = (((1,), (0,)), ((), ()))
NT = (((1,), (1,)), ((), ()))

for _g, _hs in enumerate(GROUP_HEADS):
    for _h in _hs:
        assert WIN * _g <= DH * _h and DH * _h + DH <= WIN * _g + 128


def _dot(a, b, dims=NN):
    return jax.lax.dot_general(a, b, dims, preferred_element_type=F32)


class _Filler:
    def __init__(self, gens, counts):
        self.gens, self.counts, self.done = gens, counts, [0] * len(gens)

    def upto(self, frac):
        for k, gen in enumerate(self.gens):
            while self.done[k] < min(frac, 1.0) * self.counts[k]:
                next(gen, None)
                self.done[k] += 1
            if frac >= 1.0:
                for _ in gen:
                    pass


def _chain(*gens):
    for gen in gens:
        yield from gen


def _phi(t):
    return jnp.where(t > 0, t + 1.0, jnp.exp(t))


def _sigmoid(t):
    return 1.0 / (1.0 + jnp.exp(-t))


def _recip(x):
    r = pl.reciprocal(x, approx=True)
    return r * (2.0 - x * r)


def _kernel(xt_hbm, wq_hbm, wk_hbm, wv_hbm, wo_hbm, beta_hbm, wr_hbm, wg_hbm, wu_hbm, wdt_hbm,
            out_hbm,
            beta_ref, wr_ref, xbuf, wq_raw, wk_raw, wv_raw, wo_raw, wqt, wkt, wvt, wot, xn, ktn, kb, qt, pkt, pqt,
            vtn, vt32, pbuf, m_f32, m_bf, keep, amem, ot, h_all, hn_sel, yacc, obuf, wg_v, wu_v, wdt_v,
            gcol, omg, wrcol, stat2, wnorm, r_all, stage, flag, sem_x, sem_w, sem_o):
    class _Group:
        def __init__(self, copies):
            self.copies = copies

        def start(self):
            for cp in self.copies:
                cp.start()

        def wait(self):
            for cp in self.copies:
                cp.wait()

    def hbm_cols(blk):
        return pl.ds(pl.multiple_of(blk * 128, 128), 128)

    def x_copy(s):
        return _Group([pltpu.make_async_copy(xt_hbm.at[:, hbm_cols(s * NQB + i)],
                                             xbuf.at[s * NQB + i], sem_x.at[s])
                       for i in range(NQB)])

    def out_copy(s):
        return _Group([pltpu.make_async_copy(obuf.at[s * NQB + i],
                                             out_hbm.at[:, hbm_cols(s * NQB + i)], sem_o.at[s])
                       for i in range(NQB)])

    def prev_out_copy(s):
        src = jnp.where(s > 0, s - 1, NSEG) * NQB
        dst = jnp.where(s > 0, s - 1, NSEG - 1) * NQB
        sem = jnp.where(s > 0, s - 1, NSEG)
        return _Group([pltpu.make_async_copy(obuf.at[src + i], out_hbm.at[:, hbm_cols(dst + i)],
                                             sem_o.at[sem]) for i in range(NQB)])

    cp_beta = pltpu.make_async_copy(beta_hbm, beta_ref, sem_w.at[8])
    cp_wr = pltpu.make_async_copy(wr_hbm, wr_ref, sem_w.at[9])
    cp_wk = pltpu.make_async_copy(wk_hbm, wk_raw, sem_w.at[0])
    cp_wq = pltpu.make_async_copy(wq_hbm, wq_raw, sem_w.at[1])
    cp_wv = pltpu.make_async_copy(wv_hbm, wv_raw, sem_w.at[2])
    cp_wo = pltpu.make_async_copy(wo_hbm, wo_raw, sem_w.at[3])
    cp_wg = pltpu.make_async_copy(wg_hbm, wg_v, sem_w.at[4])
    cp_wu = pltpu.make_async_copy(wu_hbm, wu_v, sem_w.at[5])
    cp_wd = pltpu.make_async_copy(wdt_hbm, wdt_v, sem_w.at[6])

    def fold8(v):
        return jnp.sum(v.reshape(v.shape[0] // 8, 8, 128), axis=0)

    def col_total(acc):
        return jnp.sum(acc, axis=0, keepdims=True) * (1.0 / D)

    def ln1_steps(s):
        seg = jnp.minimum(s, NSEG - 1)
        for c in range(NQB):
            xs = lambda r: xbuf[seg * NQB + c, RS * r:RS * (r + 1), :].astype(F32)
            acc = None
            for r in range(D // RS):
                part = fold8(xs(r))
                acc = part if acc is None else acc + part
                yield
            m = col_total(acc)
            acc = None
            for r in range(D // RS):
                xc = xs(r) - m
                part = fold8(xc * xc)
                acc = part if acc is None else acc + part
                yield
            rstd = jax.lax.rsqrt(col_total(acc) + LN_EPS)
            for r in range(D // RS):
                xn[c, RS * r:RS * (r + 1), :] = (
                    (xs(r) - m) * rstd).astype(BF16)
                yield

    def xn_all():
        return jnp.concatenate([xn[c] for c in range(NQB)], axis=1)

    def rows_of(c):
        return slice(CH * c, CH * (c + 1))

    def packed(words):
        return pltpu.bitcast(words, BF16)

    def wt_rows(wt, c):
        return packed(wt[CH // 2 * c:CH // 2 * (c + 1), :])

    def transpose_keys(g):
        kb[g] = pltpu.bitcast(ktn[WIN * g:WIN * g + 128, :].T, U32)

    def proj_k(c):
        kt = _dot(wt_rows(wkt, c), xn_all())
        pkt[rows_of(c), :] = _phi(kt).astype(BF16)
        ktn[rows_of(c), :] = kt.astype(BF16)
        if c == 0:
            transpose_keys(0)

    def proj_q(c):
        qf = _dot(wt_rows(wqt, c), xn_all())
        qt[rows_of(c), :] = (qf * QSCALE).astype(BF16)
        pqt[rows_of(c), :] = _phi(qf).astype(BF16)

    def proj_v(c):
        tail = jnp.concatenate([jnp.zeros((6, L), F32), jnp.ones((8, L), F32)], axis=0)
        vt = _dot(wt_rows(wvt, c), xn_all())
        vtn[rows_of(c), :] = vt.astype(BF16)
        for j in range(CH // DH):
            h = (CH // DH) * c + j
            vt32[32 * h:32 * h + 16, :] = vt[DH * j:DH * j + 16].astype(BF16)
            vt32[32 * h + 16:32 * h + 32, :] = jnp.concatenate(
                [vt[DH * j + 16:DH * j + 18], tail], axis=0).astype(BF16)

    def masked_q(w0, i, word_mask):
        qu = pltpu.bitcast(qt[pl.ds(w0, 128), 128 * i:128 * (i + 1)], U32)
        return pltpu.bitcast(jnp.where(word_mask, qu, jnp.uint32(0)), BF16)

    def head_word_mask(lo):
        word = jax.lax.broadcasted_iota(I32, (64, 128), 0)
        return (2 * word >= lo) & (2 * word < lo + DH)

    def causal_mask():
        return (jax.lax.broadcasted_iota(I32, (128, 128), 0)
                <= jax.lax.broadcasted_iota(I32, (128, 128), 1))

    def pv_head(h, i):
        n = 128 * (i + 1)
        r0 = TOFF[i] * 128
        o = _dot(vt32[32 * h:32 * h + 32, 0:n], pbuf[h, r0:r0 + n, :])
        a = omg[h] * _recip(o[24:32, :])
        on = (o[0:24].reshape(3, 8, 128) * a).reshape(24, 128)
        ot[i, DH * h:DH * h + 24, :] = on + amem[i, DH * h:DH * h + 24, :]

    def stage_attention_fast(filler):
        causal = causal_mask()
        for h in range(H + LAG):
            if h < H:
                g = GROUP_OF[h]
                word_mask = head_word_mask(DH * h - WIN * g)
                if h == GROUP_HEADS[g][0] and g + 1 < NG:
                    transpose_keys(g + 1)
            for i in range(NQB):
                n = 128 * (i + 1)
                if h < H:
                    filler.upto((NTILE * h + TOFF[i] + i + 1) / (NTILE * (H - 1)))
                    st = _dot(packed(kb[g, 0:n // 2, :]), masked_q(WIN * g, i, word_mask))
                    p = jnp.exp2(st)
                    r0 = TOFF[i] * 128
                    if i > 0:
                        pbuf[h, r0:r0 + 128 * i, :] = p[:n - 128].astype(BF16)
                    pbuf[h, r0 + 128 * i:r0 + n, :] = jnp.where(
                        causal, p[n - 128:n], 0.0).astype(BF16)
                if h >= LAG:
                    pv_head(h - LAG, i)

    def stage_scores_safe():
        causal = causal_mask()
        for g in range(1, NG):
            transpose_keys(g)

        def head(h, carry):
            g = jnp.clip((DH * h + DH - 128 + WIN - 1) // WIN, 0, NG - 1)
            g = jnp.where(DH * h + DH <= 128, 0, g)
            w0 = pl.multiple_of(WIN * g, 16)
            word_mask = head_word_mask(DH * h - WIN * g)
            for i in range(NQB):
                n = 128 * (i + 1)
                st = _dot(packed(kb[g, 0:n // 2, :]), masked_q(w0, i, word_mask))
                sd = jnp.where(causal, st[n - 128:n], -jnp.inf)
                m = jnp.max(sd, axis=0, keepdims=True)
                if i > 0:
                    m = jnp.maximum(m, jnp.max(st[:n - 128], axis=0, keepdims=True))
                r0 = TOFF[i] * 128
                if i > 0:
                    pbuf[h, r0:r0 + 128 * i, :] = jnp.exp2(st[:n - 128] - m).astype(BF16)
                pbuf[h, r0 + 128 * i:r0 + n, :] = jnp.exp2(sd - m).astype(BF16)
            return carry

        jax.lax.fori_loop(0, H, head, 0)

    def attn_block(s, i):
        blk = s * NQB + i
        otb = ot[i, 0:D, :].astype(BF16)
        tot = None
        for c in range(NCH):
            hh = _dot(wt_rows(wot, c), otb) + xbuf[blk, rows_of(c), :].astype(F32)
            h_all[blk, rows_of(c), :] = hh
            part = jnp.sum(hh, axis=0, keepdims=True)
            tot = part if tot is None else tot + part
        stat2[blk, 0:1, :] = tot * (1.0 / D)

    def mem_update(g):
        lhs = jnp.concatenate([jnp.ones((16, L), BF16), vtn[WIN * g:WIN * g + 128, :]], axis=0)
        upd = _dot(lhs, pkt[WIN * g:WIN * g + 128, :], NT)
        m_new = m_f32[g] + upd * keep[g]
        m_f32[g] = m_new
        m_bf[g] = m_new.astype(BF16)

    def mem_read(g):
        for i in range(NQB):
            nm = _dot(m_bf[g], pqt[WIN * g:WIN * g + 128, 128 * i:128 * (i + 1)])
            first = GROUP_HEADS[g][0]
            b = gcol[first:first + 8, :] * _recip(nm[0:8, :] + 1e-6)
            for j, h in enumerate(GROUP_HEADS[g]):
                lo = 16 + DH * h - WIN * g
                n = min(24, MROWS - lo)
                amem[i, DH * h:DH * h + n, :] = nm[lo:lo + n] * b[j:j + 1, :]

    def stat_steps(s, blocks=range(NQB)):
        seg = jnp.maximum(s, 0)
        for i in blocks:
            blk = seg * NQB + i
            m = stat2[blk, 0:1, :]
            acc_v = acc_r = None
            for r in range(D // RS):
                rows = slice(RS * r, RS * (r + 1))
                hc = h_all[blk, rows, :] - m
                pv = fold8(hc * hc)
                pr = fold8(hc * wrcol[rows, :])
                acc_v = pv if acc_v is None else acc_v + pv
                acc_r = pr if acc_r is None else acc_r + pr
                yield
            rstd = jax.lax.rsqrt(col_total(acc_v) + LN_EPS)
            stat2[blk, 1:2, :] = rstd
            r_all[pl.ds(blk, 1), :] = jnp.sum(acc_r, axis=0, keepdims=True) * rstd

    def out_steps(s):
        seg = jnp.maximum(s, 0)
        for i in range(NQB):
            blk = seg * NQB + i
            m = stat2[blk, 0:1, :]
            rstd = stat2[blk, 1:2, :]
            for r in range(D // RS):
                rows = slice(RS * r, RS * (r + 1))
                hh = h_all[blk, rows, :]
                obuf[blk, rows, :] = (hh + (hh - m) * rstd).astype(BF16)
                yield

    cp_beta.start()
    cp_wr.start()
    x_copy(0).start()
    cp_wk.start()

    row = jax.lax.broadcasted_iota(I32, (MROWS, 128), 0)
    lane = jax.lax.broadcasted_iota(I32, (MROWS, 128), 1)
    for g in range(NG):
        first, nh = GROUP_HEADS[g][0], len(GROUP_HEADS[g])
        lane_head = ((lane + WIN * g) * 3641) >> 16
        row_head = jnp.where(row < 16, row + first, ((row - 16 + WIN * g) * 3641) >> 16)
        ok = (lane_head == row_head) & (row_head >= first) & (row_head < first + nh)
        keep[g] = jnp.where(ok, 1.0, 0.0)
    m_f32[...] = jnp.zeros_like(m_f32)
    amem[...] = jnp.zeros_like(amem)
    h_all[0:NQB] = jnp.zeros((NQB, D, 128), F32)
    obuf[NSEG * NQB:(NSEG + 1) * NQB] = jnp.zeros((NQB, D, 128), BF16)
    stat2[0:NQB] = jnp.zeros((NQB, 8, 128), F32)

    cp_beta.wait()
    cp_wr.wait()
    beta = beta_ref[...].astype(F32).reshape(1, H)
    gpad = jnp.concatenate([_sigmoid(beta), jnp.zeros((1, 128 - H), F32)], axis=1)
    gcol[...] = jnp.transpose(jnp.broadcast_to(gpad, (128, 128)))
    for h in range(H):
        omg[h] = jnp.broadcast_to(1.0 - gcol[h:h + 1, :], (8, 128))
    wr = jnp.concatenate([wr_ref[...].astype(F32).reshape(1, D), jnp.zeros((1, 64), F32)], axis=1)
    wrcol[...] = jnp.transpose(jnp.broadcast_to(wr, (128, D + 64)))[0:D]

    def transpose_tile(dst, raw, t):
        hi = min(128 * (t + 1), D)
        dst[64 * t:hi // 2, :] = pltpu.bitcast(raw[:, 128 * t:hi].T, U32)

    def col_norm_steps(raw, slot):
        for t in range(5):
            hi = min(128 * (t + 1), D)
            for k in range(3):
                w = raw[192 * k:192 * (k + 1), 128 * t:hi].astype(F32)
                wnorm[slot, 8 * k:8 * (k + 1), 128 * t:hi] = jnp.sum(
                    (w * w).reshape(24, 8, hi - 128 * t), axis=0)
                yield

    x_copy(0).wait()
    cp_wq.start()
    for _ in ln1_steps(0):
        pass
    cp_wk.wait()
    cp_wv.start()
    side = _Filler([col_norm_steps(wk_raw, 0)], [15])
    transpose_tile(wkt, wk_raw, 0)
    transpose_tile(wkt, wk_raw, 1)
    proj_k(0)
    transpose_tile(wkt, wk_raw, 2)
    side.upto(0.5)
    proj_k(1)
    transpose_tile(wkt, wk_raw, 3)
    side.upto(1.0)
    proj_k(2)
    transpose_tile(wkt, wk_raw, 4)
    cp_wq.wait()
    cp_wv.wait()
    cp_wo.start()
    x_copy(1).start()
    transpose_tile(wqt, wq_raw, 0)
    transpose_tile(wqt, wq_raw, 1)
    proj_k(3)
    side = _Filler([col_norm_steps(wq_raw, 1), col_norm_steps(wv_raw, 2)], [15, 15])
    for c in range(NCH):
        proj_q(c)
        if c + 2 < 5:
            transpose_tile(wqt, wq_raw, c + 2)
        if c >= 2:
            transpose_tile(wvt, wv_raw, c - 2)
        if c < NCH - 1:
            side.upto((c + 1) / (NCH - 1))
    cp_wo.wait()
    x_copy(1).wait()
    for s in range(2, NSEG):
        x_copy(s).start()
    cp_wg.start()
    cp_wu.start()
    cp_wd.start()
    for c in range(NCH):
        proj_v(c)
        if c + 2 < 5:
            transpose_tile(wvt, wv_raw, c + 2)
        transpose_tile(wot, wo_raw, c)
    transpose_tile(wot, wo_raw, 4)

    def max_norm(slot):
        ss = jnp.sum(wnorm[slot], axis=0, keepdims=True)
        return jnp.sqrt(jnp.max(ss, axis=1, keepdims=True))

    nk, nq, nv = max_norm(0), max_norm(1), max_norm(2)

    bound = (QSCALE * DH * D) * nq * nk
    safe = (bound <= SAFE_LOGIT) & (nv * (D ** 0.5) <= SAFE_V)
    flag[0] = jnp.sum(jnp.where(safe, 1, 0).astype(I32))

    def segment(s, carry):
        @pl.when(jnp.logical_and(s > 0, s + 1 < NSEG))
        def _():
            x_copy(s + 1).wait()

        def side_work():
            return _Filler([_chain(stat_steps(s - 1), out_steps(s - 1)), ln1_steps(s + 1)],
                           [2 * PASS_STEPS, 3 * PASS_STEPS])

        def fast():
            stage_attention_fast(side_work())

        def safe():
            stage_scores_safe()
            side_work().upto(1.0)
            for h in range(H):
                for i in range(NQB):
                    pv_head(h, i)

        jax.lax.cond(flag[0] == 1, fast, safe)

        @pl.when(s + 1 < NSEG)
        def _():
            prev_out_copy(s).start()
            for i in range(NQB):
                attn_block(s, i)
            for g in range(NG):
                mem_update(g)
            for c in range(NCH):
                proj_q(c)
            for c in range(NCH):
                proj_k(c)
            for g in range(NG):
                mem_read(g)
            for c in range(NCH):
                proj_v(c)

        return carry

    jax.lax.fori_loop(0, NSEG, segment, 0)

    out_copy(NSEG - 2).start()
    prev_out_copy(0).wait()
    for i in range(NQB):
        attn_block(NSEG - 1, i)
        if i > 0:
            for _ in stat_steps(NSEG - 1, [i - 1]):
                pass
    for _ in stat_steps(NSEG - 1, [NQB - 1]):
        pass

    r = r_all[...]
    r_sel = jnp.max(jnp.max(r, axis=0, keepdims=True), axis=1, keepdims=True)
    ids = (128 * jax.lax.broadcasted_iota(I32, r.shape, 0)
           + jax.lax.broadcasted_iota(I32, r.shape, 1))
    cand = jnp.min(jnp.where(r == r_sel, ids, S), axis=0, keepdims=True)
    idx = jnp.minimum(jnp.sum(jnp.min(cand, axis=1, keepdims=True)), S - 1)
    for _ in out_steps(NSEG - 1):
        pass
    out_copy(NSEG - 1).start()
    blk = idx >> 7
    m_sel = stat2[blk, 0:1, :]
    rstd_sel = stat2[blk, 1:2, :]
    for r in range(D // RS):
        rows = slice(RS * r, RS * (r + 1))
        hn_sel[rows, :] = ((h_all[blk, rows, :] - m_sel) * rstd_sel).astype(BF16)
    onehot = (jax.lax.broadcasted_iota(I32, (16, 128), 1) == idx - blk * 128).astype(BF16)
    xs = _dot(onehot, hn_sel[...], NT).astype(BF16)
    cp_wg.wait()
    cp_wu.wait()
    cp_wd.wait()

    def down_steps(c, act):
        for r in range(D // RS):
            rows = slice(RS * r, RS * (r + 1))
            part = None if c == 0 else yacc[rows, :]
            for t in range(FC // 128):
                w = wdt_v[rows, FC * c + 128 * t:FC * c + 128 * (t + 1)].astype(F32)
                part = w * act[t] if part is None else part + w * act[t]
            yacc[rows, :] = part
            yield

    nch = FF // FC
    pending = None
    for c in range(nch):
        ga, up = [], []
        for t in range(FC // 128):
            tile = slice(FC * c + 128 * t, FC * c + 128 * (t + 1))
            ga.append(_dot(xs, wg_v[:, tile])[0:1])
            up.append(_dot(xs, wu_v[:, tile])[0:1])
            if pending is not None:
                pending.upto((t + 1) / (FC // 128))
        act = [g * _sigmoid(g) * u for g, u in zip(ga, up)]
        pending = _Filler([down_steps(c, act)], [D // RS])
    pending.upto(1.0)
    y = jnp.sum(yacc[...], axis=1, keepdims=True) * _sigmoid(r_sel)
    sel = jax.lax.broadcasted_iota(I32, (RS, 128), 1) == idx - blk * 128
    for r in range(D // RS):
        rows = slice(RS * r, RS * (r + 1))
        hh = h_all[blk, rows, :]
        stage[rows, :] = (hh + (hh - m_sel) * rstd_sel
                          + jnp.where(sel, y[rows], 0.0)).astype(BF16)
    for s in range(NSEG):
        out_copy(s).wait()
    fix = pltpu.make_async_copy(stage, out_hbm.at[:, hbm_cols(blk)], sem_w.at[7])
    fix.start()
    fix.wait()


@jax.jit
def pallas_sequential_preLN__memory_aug_infini_attn__moe_arch_mod__prompt_kernel(
    A_x: jax.Array,
    A_wq: jax.Array,
    A_wk: jax.Array,
    A_wv: jax.Array,
    A_wo: jax.Array,
    A_beta: jax.Array,
    B_x: jax.Array,
    B_w_r: jax.Array,
    B_w_gate: jax.Array,
    B_w_up: jax.Array,
    B_w_down: jax.Array,
):
    del B_x
    hbm = pl.BlockSpec(memory_space=pltpu.HBM)
    scratch = [
        pltpu.VMEM((H,), BF16),
        pltpu.VMEM((D,), BF16),
        pltpu.VMEM((NSEG * NQB, D, 128), BF16),
        pltpu.VMEM((D, D), BF16),
        pltpu.VMEM((D, D), BF16),
        pltpu.VMEM((D, D), BF16),
        pltpu.VMEM((D, D), BF16),
        pltpu.VMEM((D // 2, D), U32),
        pltpu.VMEM((D // 2, D), U32),
        pltpu.VMEM((D // 2, D), U32),
        pltpu.VMEM((D // 2, D), U32),
        pltpu.VMEM((NQB, D, 128), BF16),
        pltpu.VMEM((D, L), BF16),
        pltpu.VMEM((NG, L // 2, 128), U32),
        pltpu.VMEM((D, L), BF16),
        pltpu.VMEM((D, L), BF16),
        pltpu.VMEM((D, L), BF16),
        pltpu.VMEM((D, L), BF16),
        pltpu.VMEM((H * 32, L), BF16),
        pltpu.VMEM((H, NTILE * 128, 128), BF16),
        pltpu.VMEM((NG, MROWS, 128), F32),
        pltpu.VMEM((NG, MROWS, 128), BF16),
        pltpu.VMEM((NG, MROWS, 128), F32),
        pltpu.VMEM((NQB, D + 24, 128), F32),
        pltpu.VMEM((NQB, D + 24, 128), F32),
        pltpu.VMEM((NSEG * NQB, D, 128), F32),
        pltpu.VMEM((D, 128), BF16),
        pltpu.VMEM((D, 128), F32),
        pltpu.VMEM(((NSEG + 1) * NQB, D, 128), BF16),
        pltpu.VMEM((D, FF), BF16),
        pltpu.VMEM((D, FF), BF16),
        pltpu.VMEM((D, FF), BF16),
        pltpu.VMEM((128, 128), F32),
        pltpu.VMEM((H, 8, 128), F32),
        pltpu.VMEM((D, 128), F32),
        pltpu.VMEM((NSEG * NQB, 8, 128), F32),
        pltpu.VMEM((3, 24, D), F32),
        pltpu.VMEM((NSEG * NQB, 128), F32),
        pltpu.VMEM((D, 128), BF16),
        pltpu.SMEM((1,), I32),
        pltpu.SemaphoreType.DMA((NSEG,)),
        pltpu.SemaphoreType.DMA((10,)),
        pltpu.SemaphoreType.DMA((NSEG + 1,)),
    ]
    out_t = pl.pallas_call(
        _kernel,
        out_shape=jax.ShapeDtypeStruct((D, S), BF16),
        in_specs=[hbm] * 10,
        out_specs=hbm,
        scratch_shapes=scratch,
        compiler_params=pltpu.CompilerParams(vmem_limit_bytes=100 * 1024 * 1024),
        name="infini_moe",
    )(A_x.reshape(S, D).T, A_wq, A_wk, A_wv, A_wo, A_beta, B_w_r, B_w_gate, B_w_up, B_w_down.T)
    return out_t.T.reshape(1, S, D)
```

```python
import functools

import jax
import jax.numpy as jnp
import jax.experimental.pallas as pl
import jax.experimental.pallas.tpu as pltpu

F32 = jnp.float32
BF16 = jnp.bfloat16
U32 = jnp.uint32
I32 = jnp.int32

S = 2048
D = 576
H = 32
DH = 18
NSEG = 4
L = S // NSEG
FF = 4608
NQB = L // 128
TOFF = (0, 1, 3, 6)
NTILE = 10
NG = 5
WIN = 112
GROUP_HEADS = tuple(tuple(h for h in range(H)
                          if min(max(0, -(-(DH * h + DH - 128) // WIN)), NG - 1) == g)
                    for g in range(NG))
GROUP_OF = {h: g for g in range(NG) for h in GROUP_HEADS[g]}
MROWS = 144
CH = 144
NCH = D // CH
RS = 64
PASS_STEPS = NQB * (D // RS)
FC = 512
LAG = 20
LN_EPS = 1e-5
LOG2E = 1.4426950408889634
QSCALE = (DH ** -0.5) * LOG2E
SAFE_LOGIT = 60.0
SAFE_V = 2.0 ** 50

NN = (((1,), (0,)), ((), ()))
NT = (((1,), (1,)), ((), ()))

for _g, _hs in enumerate(GROUP_HEADS):
    for _h in _hs:
        assert WIN * _g <= DH * _h and DH * _h + DH <= WIN * _g + 128


def _dot(a, b, dims=NN):
    return jax.lax.dot_general(a, b, dims, preferred_element_type=F32)


class _Filler:
    def __init__(self, gens, counts):
        self.gens, self.counts, self.done = gens, counts, [0] * len(gens)

    def upto(self, frac):
        for k, gen in enumerate(self.gens):
            while self.done[k] < min(frac, 1.0) * self.counts[k]:
                next(gen, None)
                self.done[k] += 1
            if frac >= 1.0:
                for _ in gen:
                    pass


def _chain(*gens):
    for gen in gens:
        yield from gen


def _phi(t):
    return jnp.where(t > 0, t + 1.0, jnp.exp(t))


def _sigmoid(t):
    return 1.0 / (1.0 + jnp.exp(-t))


def _recip(x):
    r = pl.reciprocal(x, approx=True)
    return r * (2.0 - x * r)


def _kernel(xt_hbm, wq_hbm, wk_hbm, wv_hbm, wo_hbm, beta_hbm, wr_hbm, wg_hbm, wu_hbm, wdt_hbm,
            out_hbm,
            beta_ref, wr_ref, xbuf, wq_raw, wk_raw, wv_raw, wo_raw, wqt, wkt, wvt, wot, xn, ktn, kb, qt, pkt, pqt,
            vtn, vt32, pbuf, m_f32, m_bf, keep, amem, ot, h_all, hn_sel, yacc, obuf, wg_v, wu_v, wdt_v,
            gcol, omg, wrcol, stat2, wnorm, r_all, stage, flag, sem_x, sem_x0, sem_w, sem_o):
    class _Group:
        def __init__(self, copies):
            self.copies = copies

        def start(self):
            for cp in self.copies:
                cp.start()

        def wait(self):
            for cp in self.copies:
                cp.wait()

    def hbm_cols(blk):
        return pl.ds(pl.multiple_of(blk * 128, 128), 128)

    def x_copy(s):
        return _Group([pltpu.make_async_copy(xt_hbm.at[:, hbm_cols(s * NQB + i)],
                                             xbuf.at[s * NQB + i], sem_x.at[s])
                       for i in range(NQB)])

    def out_copy(s):
        return _Group([pltpu.make_async_copy(obuf.at[s * NQB + i],
                                             out_hbm.at[:, hbm_cols(s * NQB + i)], sem_o.at[s])
                       for i in range(NQB)])

    def prev_out_copy(s):
        src = jnp.where(s > 0, s - 1, NSEG) * NQB
        dst = jnp.where(s > 0, s - 1, NSEG - 1) * NQB
        sem = jnp.where(s > 0, s - 1, NSEG)
        return _Group([pltpu.make_async_copy(obuf.at[src + i], out_hbm.at[:, hbm_cols(dst + i)],
                                             sem_o.at[sem]) for i in range(NQB)])

    cp_beta = pltpu.make_async_copy(beta_hbm, beta_ref, sem_w.at[8])
    cp_wr = pltpu.make_async_copy(wr_hbm, wr_ref, sem_w.at[9])
    ksplit = 384
    cp_wk = pltpu.make_async_copy(wk_hbm.at[:, 0:ksplit], wk_raw.at[:, 0:ksplit], sem_w.at[0])
    cp_wk2 = pltpu.make_async_copy(wk_hbm.at[:, ksplit:D], wk_raw.at[:, ksplit:D], sem_w.at[10])
    x0_copies = [pltpu.make_async_copy(xt_hbm.at[:, 128 * i:128 * (i + 1)], xbuf.at[i],
                                       sem_x0.at[i]) for i in range(NQB)]
    cp_wq = pltpu.make_async_copy(wq_hbm, wq_raw, sem_w.at[1])
    cp_wv = pltpu.make_async_copy(wv_hbm, wv_raw, sem_w.at[2])
    cp_wo = pltpu.make_async_copy(wo_hbm, wo_raw, sem_w.at[3])
    cp_wg = pltpu.make_async_copy(wg_hbm, wg_v, sem_w.at[4])
    cp_wu = pltpu.make_async_copy(wu_hbm, wu_v, sem_w.at[5])
    cp_wd = pltpu.make_async_copy(wdt_hbm, wdt_v, sem_w.at[6])

    def fold8(v):
        return jnp.sum(v.reshape(v.shape[0] // 8, 8, 128), axis=0)

    def col_total(acc):
        return jnp.sum(acc, axis=0, keepdims=True) * (1.0 / D)

    def ln1_steps(s, arrivals=None):
        seg = jnp.minimum(s, NSEG - 1)
        for c in range(NQB):
            if arrivals is not None:
                arrivals[c].wait()
            xs = lambda r: xbuf[seg * NQB + c, RS * r:RS * (r + 1), :].astype(F32)
            acc = None
            for r in range(D // RS):
                part = fold8(xs(r))
                acc = part if acc is None else acc + part
                yield
            m = col_total(acc)
            acc = None
            for r in range(D // RS):
                xc = xs(r) - m
                part = fold8(xc * xc)
                acc = part if acc is None else acc + part
                yield
            rstd = jax.lax.rsqrt(col_total(acc) + LN_EPS)
            for r in range(D // RS):
                xn[c, RS * r:RS * (r + 1), :] = (
                    (xs(r) - m) * rstd).astype(BF16)
                yield

    def xn_all():
        return jnp.concatenate([xn[c] for c in range(NQB)], axis=1)

    def rows_of(c):
        return slice(CH * c, CH * (c + 1))

    def packed(words):
        return pltpu.bitcast(words, BF16)

    def wt_rows(wt, c):
        return packed(wt[CH // 2 * c:CH // 2 * (c + 1), :])

    def transpose_keys(g):
        kb[g] = pltpu.bitcast(ktn[WIN * g:WIN * g + 128, :].T, U32)

    def proj_k(c):
        kt = _dot(wt_rows(wkt, c), xn_all())
        pkt[rows_of(c), :] = _phi(kt).astype(BF16)
        ktn[rows_of(c), :] = kt.astype(BF16)
        if c == 0:
            transpose_keys(0)

    def proj_q(c):
        qf = _dot(wt_rows(wqt, c), xn_all())
        qt[rows_of(c), :] = (qf * QSCALE).astype(BF16)
        pqt[rows_of(c), :] = _phi(qf).astype(BF16)

    def proj_v(c):
        tail = jnp.concatenate([jnp.zeros((6, L), F32), jnp.ones((8, L), F32)], axis=0)
        vt = _dot(wt_rows(wvt, c), xn_all())
        vtn[rows_of(c), :] = vt.astype(BF16)
        for j in range(CH // DH):
            h = (CH // DH) * c + j
            vt32[32 * h:32 * h + 16, :] = vt[DH * j:DH * j + 16].astype(BF16)
            vt32[32 * h + 16:32 * h + 32, :] = jnp.concatenate(
                [vt[DH * j + 16:DH * j + 18], tail], axis=0).astype(BF16)

    def masked_q(w0, i, word_mask):
        qu = pltpu.bitcast(qt[pl.ds(w0, 128), 128 * i:128 * (i + 1)], U32)
        return pltpu.bitcast(jnp.where(word_mask, qu, jnp.uint32(0)), BF16)

    def head_word_mask(lo):
        word = jax.lax.broadcasted_iota(I32, (64, 128), 0)
        return (2 * word >= lo) & (2 * word < lo + DH)

    def causal_mask():
        return (jax.lax.broadcasted_iota(I32, (128, 128), 0)
                <= jax.lax.broadcasted_iota(I32, (128, 128), 1))

    def pv_head(h, i):
        n = 128 * (i + 1)
        r0 = TOFF[i] * 128
        o = _dot(vt32[32 * h:32 * h + 32, 0:n], pbuf[h, r0:r0 + n, :])
        a = omg[h] * _recip(o[24:32, :])
        on = (o[0:24].reshape(3, 8, 128) * a).reshape(24, 128)
        ot[i, DH * h:DH * h + 24, :] = on + amem[i, DH * h:DH * h + 24, :]

    def stage_attention_fast(filler):
        causal = causal_mask()
        for h in range(H + LAG):
            if h < H:
                g = GROUP_OF[h]
                word_mask = head_word_mask(DH * h - WIN * g)
                if h == GROUP_HEADS[g][0] and g + 1 < NG:
                    transpose_keys(g + 1)
            for i in range(NQB):
                n = 128 * (i + 1)
                if h < H:
                    filler.upto((NTILE * h + TOFF[i] + i + 1) / (NTILE * (H - 1)))
                    st = _dot(packed(kb[g, 0:n // 2, :]), masked_q(WIN * g, i, word_mask))
                    p = jnp.exp2(st)
                    r0 = TOFF[i] * 128
                    if i > 0:
                        pbuf[h, r0:r0 + 128 * i, :] = p[:n - 128].astype(BF16)
                    pbuf[h, r0 + 128 * i:r0 + n, :] = jnp.where(
                        causal, p[n - 128:n], 0.0).astype(BF16)
                if h >= LAG:
                    pv_head(h - LAG, i)

    def stage_scores_safe():
        causal = causal_mask()
        for g in range(1, NG):
            transpose_keys(g)

        def head(h, carry):
            g = jnp.clip((DH * h + DH - 128 + WIN - 1) // WIN, 0, NG - 1)
            g = jnp.where(DH * h + DH <= 128, 0, g)
            w0 = pl.multiple_of(WIN * g, 16)
            word_mask = head_word_mask(DH * h - WIN * g)
            for i in range(NQB):
                n = 128 * (i + 1)
                st = _dot(packed(kb[g, 0:n // 2, :]), masked_q(w0, i, word_mask))
                sd = jnp.where(causal, st[n - 128:n], -jnp.inf)
                m = jnp.max(sd, axis=0, keepdims=True)
                if i > 0:
                    m = jnp.maximum(m, jnp.max(st[:n - 128], axis=0, keepdims=True))
                r0 = TOFF[i] * 128
                if i > 0:
                    pbuf[h, r0:r0 + 128 * i, :] = jnp.exp2(st[:n - 128] - m).astype(BF16)
                pbuf[h, r0 + 128 * i:r0 + n, :] = jnp.exp2(sd - m).astype(BF16)
            return carry

        jax.lax.fori_loop(0, H, head, 0)

    def attn_block(s, i):
        blk = s * NQB + i
        otb = ot[i, 0:D, :].astype(BF16)
        tot = None
        for c in range(NCH):
            hh = _dot(wt_rows(wot, c), otb) + xbuf[blk, rows_of(c), :].astype(F32)
            h_all[blk, rows_of(c), :] = hh
            part = jnp.sum(hh, axis=0, keepdims=True)
            tot = part if tot is None else tot + part
        stat2[blk, 0:1, :] = tot * (1.0 / D)

    def mem_update(g):
        lhs = jnp.concatenate([jnp.ones((16, L), BF16), vtn[WIN * g:WIN * g + 128, :]], axis=0)
        upd = _dot(lhs, pkt[WIN * g:WIN * g + 128, :], NT)
        m_new = m_f32[g] + upd * keep[g]
        m_f32[g] = m_new
        m_bf[g] = m_new.astype(BF16)

    def mem_read(g):
        for i in range(NQB):
            nm = _dot(m_bf[g], pqt[WIN * g:WIN * g + 128, 128 * i:128 * (i + 1)])
            first = GROUP_HEADS[g][0]
            b = gcol[first:first + 8, :] * _recip(nm[0:8, :] + 1e-6)
            for j, h in enumerate(GROUP_HEADS[g]):
                lo = 16 + DH * h - WIN * g
                n = min(24, MROWS - lo)
                amem[i, DH * h:DH * h + n, :] = nm[lo:lo + n] * b[j:j + 1, :]

    def stat_steps(s, blocks=range(NQB)):
        seg = jnp.maximum(s, 0)
        for i in blocks:
            blk = seg * NQB + i
            m = stat2[blk, 0:1, :]
            acc_v = acc_r = None
            for r in range(D // RS):
                rows = slice(RS * r, RS * (r + 1))
                hc = h_all[blk, rows, :] - m
                pv = fold8(hc * hc)
                pr = fold8(hc * wrcol[rows, :])
                acc_v = pv if acc_v is None else acc_v + pv
                acc_r = pr if acc_r is None else acc_r + pr
                yield
            rstd = jax.lax.rsqrt(col_total(acc_v) + LN_EPS)
            stat2[blk, 1:2, :] = rstd
            r_all[pl.ds(blk, 1), :] = jnp.sum(acc_r, axis=0, keepdims=True) * rstd

    def out_steps(s):
        seg = jnp.maximum(s, 0)
        for i in range(NQB):
            blk = seg * NQB + i
            m = stat2[blk, 0:1, :]
            rstd = stat2[blk, 1:2, :]
            for r in range(D // RS):
                rows = slice(RS * r, RS * (r + 1))
                hh = h_all[blk, rows, :]
                obuf[blk, rows, :] = (hh + (hh - m) * rstd).astype(BF16)
                yield

    for cp in [cp_beta, cp_wr] + x0_copies + [cp_wk]:
        cp.start()

    row = jax.lax.broadcasted_iota(I32, (MROWS, 128), 0)
    lane = jax.lax.broadcasted_iota(I32, (MROWS, 128), 1)
    for g in range(NG):
        first, nh = GROUP_HEADS[g][0], len(GROUP_HEADS[g])
        lane_head = ((lane + WIN * g) * 3641) >> 16
        row_head = jnp.where(row < 16, row + first, ((row - 16 + WIN * g) * 3641) >> 16)
        ok = (lane_head == row_head) & (row_head >= first) & (row_head < first + nh)
        keep[g] = jnp.where(ok, 1.0, 0.0)
    m_f32[...] = jnp.zeros_like(m_f32)
    amem[...] = jnp.zeros_like(amem)
    h_all[0:NQB] = jnp.zeros((NQB, D, 128), F32)
    obuf[NSEG * NQB:(NSEG + 1) * NQB] = jnp.zeros((NQB, D, 128), BF16)
    stat2[0:NQB] = jnp.zeros((NQB, 8, 128), F32)

    cp_beta.wait()
    cp_wr.wait()
    cp_wk2.start()
    cp_wq.start()
    beta = beta_ref[...].astype(F32).reshape(1, H)
    gpad = jnp.concatenate([_sigmoid(beta), jnp.zeros((1, 128 - H), F32)], axis=1)
    gcol[...] = jnp.transpose(jnp.broadcast_to(gpad, (128, 128)))
    for h in range(H):
        omg[h] = jnp.broadcast_to(1.0 - gcol[h:h + 1, :], (8, 128))
    wr = jnp.concatenate([wr_ref[...].astype(F32).reshape(1, D), jnp.zeros((1, 64), F32)], axis=1)
    wrcol[...] = jnp.transpose(jnp.broadcast_to(wr, (128, D + 64)))[0:D]

    def transpose_tile(dst, raw, t):
        hi = min(128 * (t + 1), D)
        dst[64 * t:hi // 2, :] = pltpu.bitcast(raw[:, 128 * t:hi].T, U32)

    def col_norm_steps(raw, slot):
        for t in range(5):
            hi = min(128 * (t + 1), D)
            for k in range(3):
                w = raw[192 * k:192 * (k + 1), 128 * t:hi].astype(F32)
                wnorm[slot, 8 * k:8 * (k + 1), 128 * t:hi] = jnp.sum(
                    (w * w).reshape(24, 8, hi - 128 * t), axis=0)
                yield

    for _ in ln1_steps(0, x0_copies):
        pass
    cp_wv.start()
    cp_wo.start()
    cp_wk.wait()
    for t in range(3):
        transpose_tile(wkt, wk_raw, t)
    proj_k(0)
    proj_k(1)
    cp_wk2.wait()
    cp_wq.wait()
    for s in range(1, NSEG):
        x_copy(s).start()
    side = _Filler([col_norm_steps(wk_raw, 0), col_norm_steps(wq_raw, 1)], [15, 15])
    transpose_tile(wkt, wk_raw, 3)
    transpose_tile(wkt, wk_raw, 4)
    proj_k(2)
    transpose_tile(wqt, wq_raw, 0)
    side.upto(0.25)
    transpose_tile(wqt, wq_raw, 1)
    proj_k(3)
    side.upto(0.5)
    for c in range(2):
        proj_q(c)
        transpose_tile(wqt, wq_raw, c + 2)
        side.upto(0.75 + 0.25 * c)
    transpose_tile(wqt, wq_raw, 4)
    cp_wv.wait()
    cp_wo.wait()
    side = _Filler([col_norm_steps(wv_raw, 2)], [15])
    for c in range(2, NCH):
        proj_q(c)
        transpose_tile(wvt, wv_raw, c - 2)
        side.upto((c - 1) / 2)
    for c in range(NCH):
        proj_v(c)
        if c + 2 < 5:
            transpose_tile(wvt, wv_raw, c + 2)
        transpose_tile(wot, wo_raw, c)
    transpose_tile(wot, wo_raw, 4)

    for s in range(1, NSEG):
        x_copy(s).wait()
    cp_wg.start()
    cp_wu.start()
    cp_wd.start()

    def max_norm(slot):
        ss = jnp.sum(wnorm[slot], axis=0, keepdims=True)
        return jnp.sqrt(jnp.max(ss, axis=1, keepdims=True))

    nk, nq, nv = max_norm(0), max_norm(1), max_norm(2)

    bound = (QSCALE * DH * D) * nq * nk
    safe = (bound <= SAFE_LOGIT) & (nv * (D ** 0.5) <= SAFE_V)
    flag[0] = jnp.sum(jnp.where(safe, 1, 0).astype(I32))

    def segment(s, carry):
        def side_work():
            return _Filler([_chain(stat_steps(s - 1), out_steps(s - 1)), ln1_steps(s + 1)],
                           [2 * PASS_STEPS, 3 * PASS_STEPS])

        def fast():
            stage_attention_fast(side_work())

        def safe():
            stage_scores_safe()
            side_work().upto(1.0)
            for h in range(H):
                for i in range(NQB):
                    pv_head(h, i)

        jax.lax.cond(flag[0] == 1, fast, safe)

        @pl.when(s + 1 < NSEG)
        def _():
            prev_out_copy(s).start()
            for i in range(NQB):
                attn_block(s, i)
            for g in range(NG):
                mem_update(g)
            for c in range(NCH):
                proj_q(c)
            for c in range(NCH):
                proj_k(c)
            for g in range(NG):
                mem_read(g)
            for c in range(NCH):
                proj_v(c)

        return carry

    jax.lax.fori_loop(0, NSEG, segment, 0)

    out_copy(NSEG - 2).start()
    prev_out_copy(0).wait()
    for i in range(NQB):
        attn_block(NSEG - 1, i)
        if i > 0:
            for _ in stat_steps(NSEG - 1, [i - 1]):
                pass
    for _ in stat_steps(NSEG - 1, [NQB - 1]):
        pass

    r = r_all[...]
    r_sel = jnp.max(jnp.max(r, axis=0, keepdims=True), axis=1, keepdims=True)
    ids = (128 * jax.lax.broadcasted_iota(I32, r.shape, 0)
           + jax.lax.broadcasted_iota(I32, r.shape, 1))
    cand = jnp.min(jnp.where(r == r_sel, ids, S), axis=0, keepdims=True)
    idx = jnp.minimum(jnp.sum(jnp.min(cand, axis=1, keepdims=True)), S - 1)
    for _ in out_steps(NSEG - 1):
        pass
    out_copy(NSEG - 1).start()
    blk = idx >> 7
    m_sel = stat2[blk, 0:1, :]
    rstd_sel = stat2[blk, 1:2, :]
    for r in range(D // RS):
        rows = slice(RS * r, RS * (r + 1))
        hn_sel[rows, :] = ((h_all[blk, rows, :] - m_sel) * rstd_sel).astype(BF16)
    onehot = (jax.lax.broadcasted_iota(I32, (16, 128), 1) == idx - blk * 128).astype(BF16)
    xs = _dot(onehot, hn_sel[...], NT).astype(BF16)
    cp_wg.wait()
    cp_wu.wait()
    cp_wd.wait()

    def down_steps(c, act):
        for r in range(D // RS):
            rows = slice(RS * r, RS * (r + 1))
            part = None if c == 0 else yacc[rows, :]
            for t in range(FC // 128):
                w = wdt_v[rows, FC * c + 128 * t:FC * c + 128 * (t + 1)].astype(F32)
                part = w * act[t] if part is None else part + w * act[t]
            yacc[rows, :] = part
            yield

    nch = FF // FC
    pending = None
    for c in range(nch):
        ga, up = [], []
        for t in range(FC // 128):
            tile = slice(FC * c + 128 * t, FC * c + 128 * (t + 1))
            ga.append(_dot(xs, wg_v[:, tile])[0:1])
            up.append(_dot(xs, wu_v[:, tile])[0:1])
            if pending is not None:
                pending.upto((t + 1) / (FC // 128))
        act = [g * _sigmoid(g) * u for g, u in zip(ga, up)]
        pending = _Filler([down_steps(c, act)], [D // RS])
    pending.upto(1.0)
    y = jnp.sum(yacc[...], axis=1, keepdims=True) * _sigmoid(r_sel)
    sel = jax.lax.broadcasted_iota(I32, (RS, 128), 1) == idx - blk * 128
    for r in range(D // RS):
        rows = slice(RS * r, RS * (r + 1))
        hh = h_all[blk, rows, :]
        stage[rows, :] = (hh + (hh - m_sel) * rstd_sel
                          + jnp.where(sel, y[rows], 0.0)).astype(BF16)
    for s in range(NSEG):
        out_copy(s).wait()
    fix = pltpu.make_async_copy(stage, out_hbm.at[:, hbm_cols(blk)], sem_w.at[7])
    fix.start()
    fix.wait()


@jax.jit
def pallas_sequential_preLN__memory_aug_infini_attn__moe_arch_mod__prompt_kernel(
    A_x: jax.Array,
    A_wq: jax.Array,
    A_wk: jax.Array,
    A_wv: jax.Array,
    A_wo: jax.Array,
    A_beta: jax.Array,
    B_x: jax.Array,
    B_w_r: jax.Array,
    B_w_gate: jax.Array,
    B_w_up: jax.Array,
    B_w_down: jax.Array,
):
    del B_x
    hbm = pl.BlockSpec(memory_space=pltpu.HBM)
    scratch = [
        pltpu.VMEM((H,), BF16),
        pltpu.VMEM((D,), BF16),
        pltpu.VMEM((NSEG * NQB, D, 128), BF16),
        pltpu.VMEM((D, D), BF16),
        pltpu.VMEM((D, D), BF16),
        pltpu.VMEM((D, D), BF16),
        pltpu.VMEM((D, D), BF16),
        pltpu.VMEM((D // 2, D), U32),
        pltpu.VMEM((D // 2, D), U32),
        pltpu.VMEM((D // 2, D), U32),
        pltpu.VMEM((D // 2, D), U32),
        pltpu.VMEM((NQB, D, 128), BF16),
        pltpu.VMEM((D, L), BF16),
        pltpu.VMEM((NG, L // 2, 128), U32),
        pltpu.VMEM((D, L), BF16),
        pltpu.VMEM((D, L), BF16),
        pltpu.VMEM((D, L), BF16),
        pltpu.VMEM((D, L), BF16),
        pltpu.VMEM((H * 32, L), BF16),
        pltpu.VMEM((H, NTILE * 128, 128), BF16),
        pltpu.VMEM((NG, MROWS, 128), F32),
        pltpu.VMEM((NG, MROWS, 128), BF16),
        pltpu.VMEM((NG, MROWS, 128), F32),
        pltpu.VMEM((NQB, D + 24, 128), F32),
        pltpu.VMEM((NQB, D + 24, 128), F32),
        pltpu.VMEM((NSEG * NQB, D, 128), F32),
        pltpu.VMEM((D, 128), BF16),
        pltpu.VMEM((D, 128), F32),
        pltpu.VMEM(((NSEG + 1) * NQB, D, 128), BF16),
        pltpu.VMEM((D, FF), BF16),
        pltpu.VMEM((D, FF), BF16),
        pltpu.VMEM((D, FF), BF16),
        pltpu.VMEM((128, 128), F32),
        pltpu.VMEM((H, 8, 128), F32),
        pltpu.VMEM((D, 128), F32),
        pltpu.VMEM((NSEG * NQB, 8, 128), F32),
        pltpu.VMEM((3, 24, D), F32),
        pltpu.VMEM((NSEG * NQB, 128), F32),
        pltpu.VMEM((D, 128), BF16),
        pltpu.SMEM((1,), I32),
        pltpu.SemaphoreType.DMA((NSEG,)),
        pltpu.SemaphoreType.DMA((NQB,)),
        pltpu.SemaphoreType.DMA((11,)),
        pltpu.SemaphoreType.DMA((NSEG + 1,)),
    ]
    out_t = pl.pallas_call(
        _kernel,
        out_shape=jax.ShapeDtypeStruct((D, S), BF16),
        in_specs=[hbm] * 10,
        out_specs=hbm,
        scratch_shapes=scratch,
        compiler_params=pltpu.CompilerParams(vmem_limit_bytes=100 * 1024 * 1024),
        name="infini_moe",
    )(A_x.reshape(S, D).T, A_wq, A_wk, A_wv, A_wo, A_beta, B_w_r, B_w_gate, B_w_up, B_w_down.T)
    return out_t.T.reshape(1, S, D)
```

```python
import functools

import jax
import jax.numpy as jnp
import jax.experimental.pallas as pl
import jax.experimental.pallas.tpu as pltpu

F32 = jnp.float32
BF16 = jnp.bfloat16
U32 = jnp.uint32
I32 = jnp.int32

S = 2048
D = 576
H = 32
DH = 18
NSEG = 4
L = S // NSEG
FF = 4608
NQB = L // 128
TOFF = (0, 1, 3, 6)
NTILE = 10
NG = 5
WIN = 112
GROUP_HEADS = tuple(tuple(h for h in range(H)
                          if min(max(0, -(-(DH * h + DH - 128) // WIN)), NG - 1) == g)
                    for g in range(NG))
GROUP_OF = {h: g for g in range(NG) for h in GROUP_HEADS[g]}
MROWS = 144
CH = 144
NCH = D // CH
RS = 64
PASS_STEPS = NQB * (D // RS)
FC = 512
LAG = 20
LN_EPS = 1e-5
LOG2E = 1.4426950408889634
QSCALE = (DH ** -0.5) * LOG2E
SAFE_LOGIT = 60.0
SAFE_V = 2.0 ** 50

NN = (((1,), (0,)), ((), ()))
NT = (((1,), (1,)), ((), ()))

for _g, _hs in enumerate(GROUP_HEADS):
    for _h in _hs:
        assert WIN * _g <= DH * _h and DH * _h + DH <= WIN * _g + 128


def _dot(a, b, dims=NN):
    return jax.lax.dot_general(a, b, dims, preferred_element_type=F32)


class _Filler:
    def __init__(self, gens, counts):
        self.gens, self.counts, self.done = gens, counts, [0] * len(gens)

    def upto(self, frac):
        for k, gen in enumerate(self.gens):
            while self.done[k] < min(frac, 1.0) * self.counts[k]:
                next(gen, None)
                self.done[k] += 1
            if frac >= 1.0:
                for _ in gen:
                    pass


def _phi(t):
    return jnp.where(t > 0, t + 1.0, jnp.exp(t))


def _sigmoid(t):
    return 1.0 / (1.0 + jnp.exp(-t))


def _recip(x):
    r = pl.reciprocal(x, approx=True)
    return r * (2.0 - x * r)


def _kernel(xt_hbm, wq_hbm, wk_hbm, wv_hbm, wo_hbm, beta_hbm, wr_hbm, wg_hbm, wu_hbm, wdt_hbm,
            out_hbm,
            beta_ref, wr_ref, xbuf, wq_raw, wk_raw, wv_raw, wo_raw, wqt, wkt, wvt, wot, xn, ktn, kb, qt, pkt, pqt,
            vtn, vt32, pbuf, m_f32, m_bf, keep, amem, ot, h_all, hn_sel, yacc, obuf, wg_v, wu_v, wdt_v,
            gcol, omg, wrcol, wrsum, stat2, wnorm, r_all, stage, flag, sem_x, sem_x0, sem_w, sem_o):
    class _Group:
        def __init__(self, copies):
            self.copies = copies

        def start(self):
            for cp in self.copies:
                cp.start()

        def wait(self):
            for cp in self.copies:
                cp.wait()

    def hbm_cols(blk):
        return pl.ds(pl.multiple_of(blk * 128, 128), 128)

    def x_copy(s):
        return _Group([pltpu.make_async_copy(xt_hbm.at[:, hbm_cols(s * NQB + i)],
                                             xbuf.at[s * NQB + i], sem_x.at[s])
                       for i in range(NQB)])

    def out_copy(s):
        return _Group([pltpu.make_async_copy(obuf.at[s * NQB + i],
                                             out_hbm.at[:, hbm_cols(s * NQB + i)], sem_o.at[s])
                       for i in range(NQB)])

    def prev_out_copy(s):
        src = jnp.where(s > 0, s - 1, NSEG) * NQB
        dst = jnp.where(s > 0, s - 1, NSEG - 1) * NQB
        sem = jnp.where(s > 0, s - 1, NSEG)
        return _Group([pltpu.make_async_copy(obuf.at[src + i], out_hbm.at[:, hbm_cols(dst + i)],
                                             sem_o.at[sem]) for i in range(NQB)])

    cp_beta = pltpu.make_async_copy(beta_hbm, beta_ref, sem_w.at[8])
    cp_wr = pltpu.make_async_copy(wr_hbm, wr_ref, sem_w.at[9])
    ksplit = 384
    cp_wk = pltpu.make_async_copy(wk_hbm.at[:, 0:ksplit], wk_raw.at[:, 0:ksplit], sem_w.at[0])
    cp_wk2 = pltpu.make_async_copy(wk_hbm.at[:, ksplit:D], wk_raw.at[:, ksplit:D], sem_w.at[10])
    x0_copies = [pltpu.make_async_copy(xt_hbm.at[:, 128 * i:128 * (i + 1)], xbuf.at[i],
                                       sem_x0.at[i]) for i in range(NQB)]
    cp_wq = pltpu.make_async_copy(wq_hbm, wq_raw, sem_w.at[1])
    cp_wv = pltpu.make_async_copy(wv_hbm, wv_raw, sem_w.at[2])
    cp_wo = pltpu.make_async_copy(wo_hbm, wo_raw, sem_w.at[3])
    cp_wg = pltpu.make_async_copy(wg_hbm, wg_v, sem_w.at[4])
    cp_wu = pltpu.make_async_copy(wu_hbm, wu_v, sem_w.at[5])
    cp_wd = pltpu.make_async_copy(wdt_hbm, wdt_v, sem_w.at[6])

    def fold8(v):
        return jnp.sum(v.reshape(v.shape[0] // 8, 8, 128), axis=0)

    def col_total(acc):
        return jnp.sum(acc, axis=0, keepdims=True) * (1.0 / D)

    def ln1_steps(s, arrivals=None):
        seg = jnp.minimum(s, NSEG - 1)
        for c in range(NQB):
            if arrivals is not None:
                arrivals[c].wait()
            xs = lambda r: xbuf[seg * NQB + c, RS * r:RS * (r + 1), :].astype(F32)
            acc = None
            for r in range(D // RS):
                part = fold8(xs(r))
                acc = part if acc is None else acc + part
                yield
            m = col_total(acc)
            acc = None
            for r in range(D // RS):
                xc = xs(r) - m
                part = fold8(xc * xc)
                acc = part if acc is None else acc + part
                yield
            rstd = jax.lax.rsqrt(col_total(acc) + LN_EPS)
            for r in range(D // RS):
                xn[c, RS * r:RS * (r + 1), :] = (
                    (xs(r) - m) * rstd).astype(BF16)
                yield

    def xn_all():
        return jnp.concatenate([xn[c] for c in range(NQB)], axis=1)

    def rows_of(c):
        return slice(CH * c, CH * (c + 1))

    def packed(words):
        return pltpu.bitcast(words, BF16)

    def wt_rows(wt, c):
        return packed(wt[CH // 2 * c:CH // 2 * (c + 1), :])

    def transpose_keys(g):
        kb[g] = pltpu.bitcast(ktn[WIN * g:WIN * g + 128, :].T, U32)

    def proj_k(c):
        kt = _dot(wt_rows(wkt, c), xn_all())
        pkt[rows_of(c), :] = _phi(kt).astype(BF16)
        ktn[rows_of(c), :] = kt.astype(BF16)
        if c == 0:
            transpose_keys(0)

    def proj_q(c):
        qf = _dot(wt_rows(wqt, c), xn_all())
        qt[rows_of(c), :] = (qf * QSCALE).astype(BF16)
        pqt[rows_of(c), :] = _phi(qf).astype(BF16)

    def proj_v(c):
        tail = jnp.concatenate([jnp.zeros((6, L), F32), jnp.ones((8, L), F32)], axis=0)
        vt = _dot(wt_rows(wvt, c), xn_all())
        vtn[rows_of(c), :] = vt.astype(BF16)
        for j in range(CH // DH):
            h = (CH // DH) * c + j
            vt32[32 * h:32 * h + 16, :] = vt[DH * j:DH * j + 16].astype(BF16)
            vt32[32 * h + 16:32 * h + 32, :] = jnp.concatenate(
                [vt[DH * j + 16:DH * j + 18], tail], axis=0).astype(BF16)

    def masked_q(w0, i, word_mask):
        qu = pltpu.bitcast(qt[pl.ds(w0, 128), 128 * i:128 * (i + 1)], U32)
        return pltpu.bitcast(jnp.where(word_mask, qu, jnp.uint32(0)), BF16)

    def head_word_mask(lo):
        word = jax.lax.broadcasted_iota(I32, (64, 128), 0)
        return (2 * word >= lo) & (2 * word < lo + DH)

    def causal_mask():
        return (jax.lax.broadcasted_iota(I32, (128, 128), 0)
                <= jax.lax.broadcasted_iota(I32, (128, 128), 1))

    def pv_head(h, i):
        n = 128 * (i + 1)
        r0 = TOFF[i] * 128
        o = _dot(vt32[32 * h:32 * h + 32, 0:n], pbuf[h, r0:r0 + n, :])
        a = omg[h] * _recip(o[24:32, :])
        on = (o[0:24].reshape(3, 8, 128) * a).reshape(24, 128)
        ot[i, DH * h:DH * h + 24, :] = on + amem[i, DH * h:DH * h + 24, :]

    def stage_attention_fast(filler):
        causal = causal_mask()
        for h in range(H + LAG):
            if h < H:
                g = GROUP_OF[h]
                word_mask = head_word_mask(DH * h - WIN * g)
                if h == GROUP_HEADS[g][0] and g + 1 < NG:
                    transpose_keys(g + 1)
            for i in range(NQB):
                n = 128 * (i + 1)
                if h < H:
                    filler.upto((NTILE * h + TOFF[i] + i + 1) / (NTILE * (H - 1)))
                    st = _dot(packed(kb[g, 0:n // 2, :]), masked_q(WIN * g, i, word_mask))
                    p = jnp.exp2(st)
                    r0 = TOFF[i] * 128
                    if i > 0:
                        pbuf[h, r0:r0 + 128 * i, :] = p[:n - 128].astype(BF16)
                    pbuf[h, r0 + 128 * i:r0 + n, :] = jnp.where(
                        causal, p[n - 128:n], 0.0).astype(BF16)
                if h >= LAG:
                    pv_head(h - LAG, i)

    def stage_scores_safe():
        causal = causal_mask()
        for g in range(1, NG):
            transpose_keys(g)

        def head(h, carry):
            g = jnp.clip((DH * h + DH - 128 + WIN - 1) // WIN, 0, NG - 1)
            g = jnp.where(DH * h + DH <= 128, 0, g)
            w0 = pl.multiple_of(WIN * g, 16)
            word_mask = head_word_mask(DH * h - WIN * g)
            for i in range(NQB):
                n = 128 * (i + 1)
                st = _dot(packed(kb[g, 0:n // 2, :]), masked_q(w0, i, word_mask))
                sd = jnp.where(causal, st[n - 128:n], -jnp.inf)
                m = jnp.max(sd, axis=0, keepdims=True)
                if i > 0:
                    m = jnp.maximum(m, jnp.max(st[:n - 128], axis=0, keepdims=True))
                r0 = TOFF[i] * 128
                if i > 0:
                    pbuf[h, r0:r0 + 128 * i, :] = jnp.exp2(st[:n - 128] - m).astype(BF16)
                pbuf[h, r0 + 128 * i:r0 + n, :] = jnp.exp2(sd - m).astype(BF16)
            return carry

        jax.lax.fori_loop(0, H, head, 0)

    def attn_block(s, i):
        blk = s * NQB + i
        otb = ot[i, 0:D, :].astype(BF16)
        acc = None
        for c in range(NCH):
            hh = _dot(wt_rows(wot, c), otb) + xbuf[blk, rows_of(c), :].astype(F32)
            h_all[blk, rows_of(c), :] = hh
            if c == 0:
                pivot = hh[0:1, :]
            d = hh - pivot
            part = (fold8(d), fold8(d * d), fold8(d * wrcol[rows_of(c), :]))
            acc = part if acc is None else tuple(a + b for a, b in zip(acc, part))
        md = col_total(acc[0])
        var = jnp.maximum(col_total(acc[1]) - md * md, 0.0)
        rstd = jax.lax.rsqrt(var + LN_EPS)
        stat2[blk, 0:1, :] = pivot + md
        stat2[blk, 1:2, :] = rstd
        r_all[pl.ds(blk, 1), :] = (jnp.sum(acc[2], axis=0, keepdims=True) - md * wrsum[0:1, :]) * rstd

    def mem_update(g):
        lhs = jnp.concatenate([jnp.ones((16, L), BF16), vtn[WIN * g:WIN * g + 128, :]], axis=0)
        upd = _dot(lhs, pkt[WIN * g:WIN * g + 128, :], NT)
        m_new = m_f32[g] + upd * keep[g]
        m_f32[g] = m_new
        m_bf[g] = m_new.astype(BF16)

    def mem_read(g):
        for i in range(NQB):
            nm = _dot(m_bf[g], pqt[WIN * g:WIN * g + 128, 128 * i:128 * (i + 1)])
            first = GROUP_HEADS[g][0]
            b = gcol[first:first + 8, :] * _recip(nm[0:8, :] + 1e-6)
            for j, h in enumerate(GROUP_HEADS[g]):
                lo = 16 + DH * h - WIN * g
                n = min(24, MROWS - lo)
                amem[i, DH * h:DH * h + n, :] = nm[lo:lo + n] * b[j:j + 1, :]

    def out_steps(s):
        seg = jnp.maximum(s, 0)
        for i in range(NQB):
            blk = seg * NQB + i
            m = stat2[blk, 0:1, :]
            rstd = stat2[blk, 1:2, :]
            for r in range(D // RS):
                rows = slice(RS * r, RS * (r + 1))
                hh = h_all[blk, rows, :]
                obuf[blk, rows, :] = (hh + (hh - m) * rstd).astype(BF16)
                yield

    for cp in [cp_beta, cp_wr] + x0_copies + [cp_wk]:
        cp.start()

    row = jax.lax.broadcasted_iota(I32, (MROWS, 128), 0)
    lane = jax.lax.broadcasted_iota(I32, (MROWS, 128), 1)
    for g in range(NG):
        first, nh = GROUP_HEADS[g][0], len(GROUP_HEADS[g])
        lane_head = ((lane + WIN * g) * 3641) >> 16
        row_head = jnp.where(row < 16, row + first, ((row - 16 + WIN * g) * 3641) >> 16)
        ok = (lane_head == row_head) & (row_head >= first) & (row_head < first + nh)
        keep[g] = jnp.where(ok, 1.0, 0.0)
    m_f32[...] = jnp.zeros_like(m_f32)
    amem[...] = jnp.zeros_like(amem)
    h_all[0:NQB] = jnp.zeros((NQB, D, 128), F32)
    obuf[NSEG * NQB:(NSEG + 1) * NQB] = jnp.zeros((NQB, D, 128), BF16)
    stat2[0:NQB] = jnp.zeros((NQB, 8, 128), F32)

    cp_beta.wait()
    cp_wr.wait()
    cp_wk2.start()
    cp_wq.start()
    beta = beta_ref[...].astype(F32).reshape(1, H)
    gpad = jnp.concatenate([_sigmoid(beta), jnp.zeros((1, 128 - H), F32)], axis=1)
    gcol[...] = jnp.transpose(jnp.broadcast_to(gpad, (128, 128)))
    for h in range(H):
        omg[h] = jnp.broadcast_to(1.0 - gcol[h:h + 1, :], (8, 128))
    wr = jnp.concatenate([wr_ref[...].astype(F32).reshape(1, D), jnp.zeros((1, 64), F32)], axis=1)
    wrcol[...] = jnp.transpose(jnp.broadcast_to(wr, (128, D + 64)))[0:D]
    wrsum[...] = jnp.broadcast_to(jnp.sum(wrcol[...], axis=0, keepdims=True), (8, 128))

    def transpose_tile(dst, raw, t):
        hi = min(128 * (t + 1), D)
        dst[64 * t:hi // 2, :] = pltpu.bitcast(raw[:, 128 * t:hi].T, U32)

    def col_norm_steps(raw, slot):
        for t in range(5):
            hi = min(128 * (t + 1), D)
            for k in range(3):
                w = raw[192 * k:192 * (k + 1), 128 * t:hi].astype(F32)
                wnorm[slot, 8 * k:8 * (k + 1), 128 * t:hi] = jnp.sum(
                    (w * w).reshape(24, 8, hi - 128 * t), axis=0)
                yield

    for _ in ln1_steps(0, x0_copies):
        pass
    cp_wv.start()
    cp_wo.start()
    cp_wk.wait()
    for t in range(3):
        transpose_tile(wkt, wk_raw, t)
    proj_k(0)
    proj_k(1)
    cp_wk2.wait()
    cp_wq.wait()
    for s in range(1, NSEG):
        x_copy(s).start()
    side = _Filler([col_norm_steps(wk_raw, 0), col_norm_steps(wq_raw, 1)], [15, 15])
    transpose_tile(wkt, wk_raw, 3)
    transpose_tile(wkt, wk_raw, 4)
    proj_k(2)
    transpose_tile(wqt, wq_raw, 0)
    side.upto(0.25)
    transpose_tile(wqt, wq_raw, 1)
    proj_k(3)
    side.upto(0.5)
    for c in range(2):
        proj_q(c)
        transpose_tile(wqt, wq_raw, c + 2)
        side.upto(0.75 + 0.25 * c)
    transpose_tile(wqt, wq_raw, 4)
    cp_wv.wait()
    cp_wo.wait()
    side = _Filler([col_norm_steps(wv_raw, 2)], [15])
    for c in range(2, NCH):
        proj_q(c)
        transpose_tile(wvt, wv_raw, c - 2)
        side.upto((c - 1) / 2)
    for c in range(NCH):
        proj_v(c)
        if c + 2 < 5:
            transpose_tile(wvt, wv_raw, c + 2)
        transpose_tile(wot, wo_raw, c)
    transpose_tile(wot, wo_raw, 4)

    for s in range(1, NSEG):
        x_copy(s).wait()
    cp_wg.start()
    cp_wu.start()
    cp_wd.start()

    def max_norm(slot):
        ss = jnp.sum(wnorm[slot], axis=0, keepdims=True)
        return jnp.sqrt(jnp.max(ss, axis=1, keepdims=True))

    nk, nq, nv = max_norm(0), max_norm(1), max_norm(2)

    bound = (QSCALE * DH * D) * nq * nk
    safe = (bound <= SAFE_LOGIT) & (nv * (D ** 0.5) <= SAFE_V)
    flag[0] = jnp.sum(jnp.where(safe, 1, 0).astype(I32))

    def segment(s, carry):
        def side_work():
            return _Filler([out_steps(s - 1), ln1_steps(s + 1)], [PASS_STEPS, 3 * PASS_STEPS])

        def fast():
            stage_attention_fast(side_work())

        def safe():
            stage_scores_safe()
            side_work().upto(1.0)
            for h in range(H):
                for i in range(NQB):
                    pv_head(h, i)

        jax.lax.cond(flag[0] == 1, fast, safe)

        @pl.when(s + 1 < NSEG)
        def _():
            prev_out_copy(s).start()
            for i in range(NQB):
                attn_block(s, i)
            for g in range(NG):
                mem_update(g)
            for c in range(NCH):
                proj_q(c)
            for c in range(NCH):
                proj_k(c)
            for g in range(NG):
                mem_read(g)
            for c in range(NCH):
                proj_v(c)

        return carry

    jax.lax.fori_loop(0, NSEG, segment, 0)

    out_copy(NSEG - 2).start()
    prev_out_copy(0).wait()
    for i in range(NQB):
        attn_block(NSEG - 1, i)

    r = r_all[...]
    r_sel = jnp.max(jnp.max(r, axis=0, keepdims=True), axis=1, keepdims=True)
    ids = (128 * jax.lax.broadcasted_iota(I32, r.shape, 0)
           + jax.lax.broadcasted_iota(I32, r.shape, 1))
    cand = jnp.min(jnp.where(r == r_sel, ids, S), axis=0, keepdims=True)
    idx = jnp.minimum(jnp.sum(jnp.min(cand, axis=1, keepdims=True)), S - 1)
    for _ in out_steps(NSEG - 1):
        pass
    out_copy(NSEG - 1).start()
    blk = idx >> 7
    m_sel = stat2[blk, 0:1, :]
    rstd_sel = stat2[blk, 1:2, :]
    for r in range(D // RS):
        rows = slice(RS * r, RS * (r + 1))
        hn_sel[rows, :] = ((h_all[blk, rows, :] - m_sel) * rstd_sel).astype(BF16)
    onehot = (jax.lax.broadcasted_iota(I32, (16, 128), 1) == idx - blk * 128).astype(BF16)
    xs = _dot(onehot, hn_sel[...], NT).astype(BF16)
    cp_wg.wait()
    cp_wu.wait()
    cp_wd.wait()

    def down_steps(c, act):
        for r in range(D // RS):
            rows = slice(RS * r, RS * (r + 1))
            part = None if c == 0 else yacc[rows, :]
            for t in range(FC // 128):
                w = wdt_v[rows, FC * c + 128 * t:FC * c + 128 * (t + 1)].astype(F32)
                part = w * act[t] if part is None else part + w * act[t]
            yacc[rows, :] = part
            yield

    nch = FF // FC
    pending = None
    for c in range(nch):
        ga, up = [], []
        for t in range(FC // 128):
            tile = slice(FC * c + 128 * t, FC * c + 128 * (t + 1))
            ga.append(_dot(xs, wg_v[:, tile])[0:1])
            up.append(_dot(xs, wu_v[:, tile])[0:1])
            if pending is not None:
                pending.upto((t + 1) / (FC // 128))
        act = [g * _sigmoid(g) * u for g, u in zip(ga, up)]
        pending = _Filler([down_steps(c, act)], [D // RS])
    pending.upto(1.0)
    y = jnp.sum(yacc[...], axis=1, keepdims=True) * _sigmoid(r_sel)
    sel = jax.lax.broadcasted_iota(I32, (RS, 128), 1) == idx - blk * 128
    for r in range(D // RS):
        rows = slice(RS * r, RS * (r + 1))
        hh = h_all[blk, rows, :]
        stage[rows, :] = (hh + (hh - m_sel) * rstd_sel
                          + jnp.where(sel, y[rows], 0.0)).astype(BF16)
    for s in range(NSEG):
        out_copy(s).wait()
    fix = pltpu.make_async_copy(stage, out_hbm.at[:, hbm_cols(blk)], sem_w.at[7])
    fix.start()
    fix.wait()


@jax.jit
def pallas_sequential_preLN__memory_aug_infini_attn__moe_arch_mod__prompt_kernel(
    A_x: jax.Array,
    A_wq: jax.Array,
    A_wk: jax.Array,
    A_wv: jax.Array,
    A_wo: jax.Array,
    A_beta: jax.Array,
    B_x: jax.Array,
    B_w_r: jax.Array,
    B_w_gate: jax.Array,
    B_w_up: jax.Array,
    B_w_down: jax.Array,
):
    del B_x
    hbm = pl.BlockSpec(memory_space=pltpu.HBM)
    scratch = [
        pltpu.VMEM((H,), BF16),
        pltpu.VMEM((D,), BF16),
        pltpu.VMEM((NSEG * NQB, D, 128), BF16),
        pltpu.VMEM((D, D), BF16),
        pltpu.VMEM((D, D), BF16),
        pltpu.VMEM((D, D), BF16),
        pltpu.VMEM((D, D), BF16),
        pltpu.VMEM((D // 2, D), U32),
        pltpu.VMEM((D // 2, D), U32),
        pltpu.VMEM((D // 2, D), U32),
        pltpu.VMEM((D // 2, D), U32),
        pltpu.VMEM((NQB, D, 128), BF16),
        pltpu.VMEM((D, L), BF16),
        pltpu.VMEM((NG, L // 2, 128), U32),
        pltpu.VMEM((D, L), BF16),
        pltpu.VMEM((D, L), BF16),
        pltpu.VMEM((D, L), BF16),
        pltpu.VMEM((D, L), BF16),
        pltpu.VMEM((H * 32, L), BF16),
        pltpu.VMEM((H, NTILE * 128, 128), BF16),
        pltpu.VMEM((NG, MROWS, 128), F32),
        pltpu.VMEM((NG, MROWS, 128), BF16),
        pltpu.VMEM((NG, MROWS, 128), F32),
        pltpu.VMEM((NQB, D + 24, 128), F32),
        pltpu.VMEM((NQB, D + 24, 128), F32),
        pltpu.VMEM((NSEG * NQB, D, 128), F32),
        pltpu.VMEM((D, 128), BF16),
        pltpu.VMEM((D, 128), F32),
        pltpu.VMEM(((NSEG + 1) * NQB, D, 128), BF16),
        pltpu.VMEM((D, FF), BF16),
        pltpu.VMEM((D, FF), BF16),
        pltpu.VMEM((D, FF), BF16),
        pltpu.VMEM((128, 128), F32),
        pltpu.VMEM((H, 8, 128), F32),
        pltpu.VMEM((D, 128), F32),
        pltpu.VMEM((8, 128), F32),
        pltpu.VMEM((NSEG * NQB, 8, 128), F32),
        pltpu.VMEM((3, 24, D), F32),
        pltpu.VMEM((NSEG * NQB, 128), F32),
        pltpu.VMEM((D, 128), BF16),
        pltpu.SMEM((1,), I32),
        pltpu.SemaphoreType.DMA((NSEG,)),
        pltpu.SemaphoreType.DMA((NQB,)),
        pltpu.SemaphoreType.DMA((11,)),
        pltpu.SemaphoreType.DMA((NSEG + 1,)),
    ]
    out_t = pl.pallas_call(
        _kernel,
        out_shape=jax.ShapeDtypeStruct((D, S), BF16),
        in_specs=[hbm] * 10,
        out_specs=hbm,
        scratch_shapes=scratch,
        compiler_params=pltpu.CompilerParams(vmem_limit_bytes=100 * 1024 * 1024),
        name="infini_moe",
    )(A_x.reshape(S, D).T, A_wq, A_wk, A_wv, A_wo, A_beta, B_w_r, B_w_gate, B_w_up, B_w_down.T)
    return out_t.T.reshape(1, S, D)
```

```python
import functools

import jax
import jax.numpy as jnp
import jax.experimental.pallas as pl
import jax.experimental.pallas.tpu as pltpu

F32 = jnp.float32
BF16 = jnp.bfloat16
U32 = jnp.uint32
I32 = jnp.int32

S = 2048
D = 576
H = 32
DH = 18
NSEG = 4
L = S // NSEG
FF = 4608
NQB = L // 128
TOFF = (0, 1, 3, 6)
NTILE = 10
NG = 5
WIN = 112
GROUP_HEADS = tuple(tuple(h for h in range(H)
                          if min(max(0, -(-(DH * h + DH - 128) // WIN)), NG - 1) == g)
                    for g in range(NG))
GROUP_OF = {h: g for g in range(NG) for h in GROUP_HEADS[g]}
MROWS = 144
CH = 144
NCH = D // CH
RS = 64
PASS_STEPS = NQB * (D // RS)
FC = 512
LAG = 20
LN_EPS = 1e-5
LOG2E = 1.4426950408889634
QSCALE = (DH ** -0.5) * LOG2E
SAFE_LOGIT = 60.0
SAFE_V = 2.0 ** 50

NN = (((1,), (0,)), ((), ()))
NT = (((1,), (1,)), ((), ()))

for _g, _hs in enumerate(GROUP_HEADS):
    for _h in _hs:
        assert WIN * _g <= DH * _h and DH * _h + DH <= WIN * _g + 128


def _dot(a, b, dims=NN):
    return jax.lax.dot_general(a, b, dims, preferred_element_type=F32)


class _Filler:
    def __init__(self, gens, counts):
        self.gens, self.counts, self.done = gens, counts, [0] * len(gens)

    def upto(self, frac):
        for k, gen in enumerate(self.gens):
            while self.done[k] < min(frac, 1.0) * self.counts[k]:
                next(gen, None)
                self.done[k] += 1
            if frac >= 1.0:
                for _ in gen:
                    pass


def _phi(t):
    return jnp.where(t > 0, t + 1.0, jnp.exp(t))


def _sigmoid(t):
    return 1.0 / (1.0 + jnp.exp(-t))


def _recip(x):
    r = pl.reciprocal(x, approx=True)
    return r * (2.0 - x * r)


def _kernel(xt_hbm, wq_hbm, wk_hbm, wv_hbm, wo_hbm, beta_hbm, wr_hbm, wg_hbm, wu_hbm, wdt_hbm,
            out_hbm,
            beta_ref, wr_ref, xbuf, wq_raw, wk_raw, wv_raw, wo_raw, wqt, wkt, wvt, wot, xn, ktn, kb, qt, pkt, pqt,
            vtn, vt32, pbuf, m_f32, m_bf, keep, amem, ot, h_all, hn_sel, yacc, obuf, wg_v, wu_v, wdt_v,
            gcol, omg, wrcol, wrsum, stat2, wnorm, r_all, stage, flag, sem_x, sem_x0, sem_w, sem_o):
    class _Group:
        def __init__(self, copies):
            self.copies = copies

        def start(self):
            for cp in self.copies:
                cp.start()

        def wait(self):
            for cp in self.copies:
                cp.wait()

    def hbm_cols(blk):
        return pl.ds(pl.multiple_of(blk * 128, 128), 128)

    def x_copy(s):
        return _Group([pltpu.make_async_copy(xt_hbm.at[:, hbm_cols(s * NQB + i)],
                                             xbuf.at[s * NQB + i], sem_x.at[s])
                       for i in range(NQB)])

    def out_copy(s):
        return _Group([pltpu.make_async_copy(obuf.at[s * NQB + i],
                                             out_hbm.at[:, hbm_cols(s * NQB + i)], sem_o.at[s])
                       for i in range(NQB)])

    def prev_out_copy(s):
        src = jnp.where(s > 0, s - 1, NSEG) * NQB
        dst = jnp.where(s > 0, s - 1, NSEG - 1) * NQB
        sem = jnp.where(s > 0, s - 1, NSEG)
        return _Group([pltpu.make_async_copy(obuf.at[src + i], out_hbm.at[:, hbm_cols(dst + i)],
                                             sem_o.at[sem]) for i in range(NQB)])

    cp_beta = pltpu.make_async_copy(beta_hbm, beta_ref, sem_w.at[8])
    cp_wr = pltpu.make_async_copy(wr_hbm, wr_ref, sem_w.at[9])
    ksplit = 384
    cp_wk = pltpu.make_async_copy(wk_hbm.at[:, 0:ksplit], wk_raw.at[:, 0:ksplit], sem_w.at[0])
    cp_wk2 = pltpu.make_async_copy(wk_hbm.at[:, ksplit:D], wk_raw.at[:, ksplit:D], sem_w.at[10])
    x0_copies = [pltpu.make_async_copy(xt_hbm.at[:, 128 * i:128 * (i + 1)], xbuf.at[i],
                                       sem_x0.at[i]) for i in range(NQB)]
    cp_wq = pltpu.make_async_copy(wq_hbm, wq_raw, sem_w.at[1])
    cp_wv = pltpu.make_async_copy(wv_hbm, wv_raw, sem_w.at[2])
    cp_wo = pltpu.make_async_copy(wo_hbm, wo_raw, sem_w.at[3])
    cp_wg = pltpu.make_async_copy(wg_hbm, wg_v, sem_w.at[4])
    cp_wu = pltpu.make_async_copy(wu_hbm, wu_v, sem_w.at[5])
    cp_wd = pltpu.make_async_copy(wdt_hbm, wdt_v, sem_w.at[6])

    def fold8(v):
        return jnp.sum(v.reshape(v.shape[0] // 8, 8, 128), axis=0)

    def col_total(acc):
        return jnp.sum(acc, axis=0, keepdims=True) * (1.0 / D)

    def ln1_steps(s, arrivals=None):
        seg = jnp.minimum(s, NSEG - 1)
        for c in range(NQB):
            if arrivals is not None:
                arrivals[c].wait()
            xs = lambda r: xbuf[seg * NQB + c, RS * r:RS * (r + 1), :].astype(F32)
            acc = None
            for r in range(D // RS):
                xr = xs(r)
                if r == 0:
                    pivot = xr[0:1, :]
                d = xr - pivot
                part = (fold8(d), fold8(d * d))
                acc = part if acc is None else (acc[0] + part[0], acc[1] + part[1])
                yield
            md = col_total(acc[0])
            m = pivot + md
            rstd = jax.lax.rsqrt(jnp.maximum(col_total(acc[1]) - md * md, 0.0) + LN_EPS)
            for r in range(D // RS):
                xn[c, RS * r:RS * (r + 1), :] = (
                    (xs(r) - m) * rstd).astype(BF16)
                yield

    def xn_all():
        return jnp.concatenate([xn[c] for c in range(NQB)], axis=1)

    def rows_of(c):
        return slice(CH * c, CH * (c + 1))

    def packed(words):
        return pltpu.bitcast(words, BF16)

    def wt_rows(wt, c):
        return packed(wt[CH // 2 * c:CH // 2 * (c + 1), :])

    def transpose_keys(g):
        kb[g] = pltpu.bitcast(ktn[WIN * g:WIN * g + 128, :].T, U32)

    def proj_k(c):
        kt = _dot(wt_rows(wkt, c), xn_all())
        pkt[rows_of(c), :] = _phi(kt).astype(BF16)
        ktn[rows_of(c), :] = kt.astype(BF16)
        if c == 0:
            transpose_keys(0)

    def proj_q(c):
        qf = _dot(wt_rows(wqt, c), xn_all())
        qt[rows_of(c), :] = (qf * QSCALE).astype(BF16)
        pqt[rows_of(c), :] = _phi(qf).astype(BF16)

    def proj_v(c):
        tail = jnp.concatenate([jnp.zeros((6, L), F32), jnp.ones((8, L), F32)], axis=0)
        vt = _dot(wt_rows(wvt, c), xn_all())
        vtn[rows_of(c), :] = vt.astype(BF16)
        for j in range(CH // DH):
            h = (CH // DH) * c + j
            vt32[32 * h:32 * h + 16, :] = vt[DH * j:DH * j + 16].astype(BF16)
            vt32[32 * h + 16:32 * h + 32, :] = jnp.concatenate(
                [vt[DH * j + 16:DH * j + 18], tail], axis=0).astype(BF16)

    def masked_q(w0, i, word_mask):
        qu = pltpu.bitcast(qt[pl.ds(w0, 128), 128 * i:128 * (i + 1)], U32)
        return pltpu.bitcast(jnp.where(word_mask, qu, jnp.uint32(0)), BF16)

    def head_word_mask(lo):
        word = jax.lax.broadcasted_iota(I32, (64, 128), 0)
        return (2 * word >= lo) & (2 * word < lo + DH)

    def causal_mask():
        return (jax.lax.broadcasted_iota(I32, (128, 128), 0)
                <= jax.lax.broadcasted_iota(I32, (128, 128), 1))

    def pv_head(h, i):
        n = 128 * (i + 1)
        r0 = TOFF[i] * 128
        o = _dot(vt32[32 * h:32 * h + 32, 0:n], pbuf[h, r0:r0 + n, :])
        a = omg[h] * _recip(o[24:32, :])
        on = (o[0:24].reshape(3, 8, 128) * a).reshape(24, 128)
        ot[i, DH * h:DH * h + 24, :] = on + amem[i, DH * h:DH * h + 24, :]

    def stage_attention_fast(filler):
        causal = causal_mask()
        for h in range(H + LAG):
            if h < H:
                g = GROUP_OF[h]
                word_mask = head_word_mask(DH * h - WIN * g)
                if h == GROUP_HEADS[g][0] and g + 1 < NG:
                    transpose_keys(g + 1)
            for i in range(NQB):
                n = 128 * (i + 1)
                if h < H:
                    filler.upto((NTILE * h + TOFF[i] + i + 1) / (NTILE * (H - 1)))
                    st = _dot(packed(kb[g, 0:n // 2, :]), masked_q(WIN * g, i, word_mask))
                    p = jnp.exp2(st)
                    r0 = TOFF[i] * 128
                    if i > 0:
                        pbuf[h, r0:r0 + 128 * i, :] = p[:n - 128].astype(BF16)
                    pbuf[h, r0 + 128 * i:r0 + n, :] = jnp.where(
                        causal, p[n - 128:n], 0.0).astype(BF16)
                if h >= LAG:
                    pv_head(h - LAG, i)

    def stage_scores_safe():
        causal = causal_mask()
        for g in range(1, NG):
            transpose_keys(g)

        def head(h, carry):
            g = jnp.clip((DH * h + DH - 128 + WIN - 1) // WIN, 0, NG - 1)
            g = jnp.where(DH * h + DH <= 128, 0, g)
            w0 = pl.multiple_of(WIN * g, 16)
            word_mask = head_word_mask(DH * h - WIN * g)
            for i in range(NQB):
                n = 128 * (i + 1)
                st = _dot(packed(kb[g, 0:n // 2, :]), masked_q(w0, i, word_mask))
                sd = jnp.where(causal, st[n - 128:n], -jnp.inf)
                m = jnp.max(sd, axis=0, keepdims=True)
                if i > 0:
                    m = jnp.maximum(m, jnp.max(st[:n - 128], axis=0, keepdims=True))
                r0 = TOFF[i] * 128
                if i > 0:
                    pbuf[h, r0:r0 + 128 * i, :] = jnp.exp2(st[:n - 128] - m).astype(BF16)
                pbuf[h, r0 + 128 * i:r0 + n, :] = jnp.exp2(sd - m).astype(BF16)
            return carry

        jax.lax.fori_loop(0, H, head, 0)

    def attn_block(s, i):
        blk = s * NQB + i
        otb = ot[i, 0:D, :].astype(BF16)
        acc = None
        for c in range(NCH):
            hh = _dot(wt_rows(wot, c), otb) + xbuf[blk, rows_of(c), :].astype(F32)
            h_all[blk, rows_of(c), :] = hh
            if c == 0:
                pivot = hh[0:1, :]
            d = hh - pivot
            part = (fold8(d), fold8(d * d), fold8(d * wrcol[rows_of(c), :]))
            acc = part if acc is None else tuple(a + b for a, b in zip(acc, part))
        md = col_total(acc[0])
        var = jnp.maximum(col_total(acc[1]) - md * md, 0.0)
        rstd = jax.lax.rsqrt(var + LN_EPS)
        stat2[blk, 0:1, :] = pivot + md
        stat2[blk, 1:2, :] = rstd
        r_all[pl.ds(blk, 1), :] = (jnp.sum(acc[2], axis=0, keepdims=True) - md * wrsum[0:1, :]) * rstd

    def mem_update(g):
        lhs = jnp.concatenate([jnp.ones((16, L), BF16), vtn[WIN * g:WIN * g + 128, :]], axis=0)
        upd = _dot(lhs, pkt[WIN * g:WIN * g + 128, :], NT)
        m_new = m_f32[g] + upd * keep[g]
        m_f32[g] = m_new
        m_bf[g] = m_new.astype(BF16)

    def mem_read(g):
        for i in range(NQB):
            nm = _dot(m_bf[g], pqt[WIN * g:WIN * g + 128, 128 * i:128 * (i + 1)])
            first = GROUP_HEADS[g][0]
            b = gcol[first:first + 8, :] * _recip(nm[0:8, :] + 1e-6)
            for j, h in enumerate(GROUP_HEADS[g]):
                lo = 16 + DH * h - WIN * g
                n = min(24, MROWS - lo)
                amem[i, DH * h:DH * h + n, :] = nm[lo:lo + n] * b[j:j + 1, :]

    def out_steps(s):
        seg = jnp.maximum(s, 0)
        for i in range(NQB):
            blk = seg * NQB + i
            m = stat2[blk, 0:1, :]
            rstd = stat2[blk, 1:2, :]
            for r in range(D // RS):
                rows = slice(RS * r, RS * (r + 1))
                hh = h_all[blk, rows, :]
                obuf[blk, rows, :] = (hh + (hh - m) * rstd).astype(BF16)
                yield

    for cp in [cp_beta, cp_wr] + x0_copies + [cp_wk]:
        cp.start()

    row = jax.lax.broadcasted_iota(I32, (MROWS, 128), 0)
    lane = jax.lax.broadcasted_iota(I32, (MROWS, 128), 1)
    for g in range(NG):
        first, nh = GROUP_HEADS[g][0], len(GROUP_HEADS[g])
        lane_head = ((lane + WIN * g) * 3641) >> 16
        row_head = jnp.where(row < 16, row + first, ((row - 16 + WIN * g) * 3641) >> 16)
        ok = (lane_head == row_head) & (row_head >= first) & (row_head < first + nh)
        keep[g] = jnp.where(ok, 1.0, 0.0)
    m_f32[...] = jnp.zeros_like(m_f32)
    amem[...] = jnp.zeros_like(amem)
    h_all[0:NQB] = jnp.zeros((NQB, D, 128), F32)
    obuf[NSEG * NQB:(NSEG + 1) * NQB] = jnp.zeros((NQB, D, 128), BF16)
    stat2[0:NQB] = jnp.zeros((NQB, 8, 128), F32)

    cp_beta.wait()
    cp_wr.wait()
    cp_wk2.start()
    cp_wq.start()
    beta = beta_ref[...].astype(F32).reshape(1, H)
    gpad = jnp.concatenate([_sigmoid(beta), jnp.zeros((1, 128 - H), F32)], axis=1)
    gcol[...] = jnp.transpose(jnp.broadcast_to(gpad, (128, 128)))
    for h in range(H):
        omg[h] = jnp.broadcast_to(1.0 - gcol[h:h + 1, :], (8, 128))
    wr = jnp.concatenate([wr_ref[...].astype(F32).reshape(1, D), jnp.zeros((1, 64), F32)], axis=1)
    wrcol[...] = jnp.transpose(jnp.broadcast_to(wr, (128, D + 64)))[0:D]
    wrsum[...] = jnp.broadcast_to(jnp.sum(wrcol[...], axis=0, keepdims=True), (8, 128))

    def transpose_tile(dst, raw, t):
        hi = min(128 * (t + 1), D)
        dst[64 * t:hi // 2, :] = pltpu.bitcast(raw[:, 128 * t:hi].T, U32)

    def col_norm_steps(raw, slot):
        for t in range(5):
            hi = min(128 * (t + 1), D)
            for k in range(3):
                w = raw[192 * k:192 * (k + 1), 128 * t:hi].astype(F32)
                wnorm[slot, 8 * k:8 * (k + 1), 128 * t:hi] = jnp.sum(
                    (w * w).reshape(24, 8, hi - 128 * t), axis=0)
                yield

    for _ in ln1_steps(0, x0_copies):
        pass
    cp_wv.start()
    cp_wo.start()
    cp_wk.wait()
    for t in range(3):
        transpose_tile(wkt, wk_raw, t)
    proj_k(0)
    proj_k(1)
    cp_wk2.wait()
    cp_wq.wait()
    for s in range(1, NSEG):
        x_copy(s).start()
    side = _Filler([col_norm_steps(wk_raw, 0), col_norm_steps(wq_raw, 1)], [15, 15])
    transpose_tile(wkt, wk_raw, 3)
    transpose_tile(wkt, wk_raw, 4)
    proj_k(2)
    transpose_tile(wqt, wq_raw, 0)
    side.upto(0.25)
    transpose_tile(wqt, wq_raw, 1)
    proj_k(3)
    side.upto(0.5)
    for c in range(2):
        proj_q(c)
        transpose_tile(wqt, wq_raw, c + 2)
        side.upto(0.75 + 0.25 * c)
    transpose_tile(wqt, wq_raw, 4)
    cp_wv.wait()
    cp_wo.wait()
    side = _Filler([col_norm_steps(wv_raw, 2)], [15])
    for c in range(2, NCH):
        proj_q(c)
        transpose_tile(wvt, wv_raw, c - 2)
        side.upto((c - 1) / 2)
    for c in range(NCH):
        proj_v(c)
        if c + 2 < 5:
            transpose_tile(wvt, wv_raw, c + 2)
        transpose_tile(wot, wo_raw, c)
    transpose_tile(wot, wo_raw, 4)

    for s in range(1, NSEG):
        x_copy(s).wait()
    cp_wg.start()
    cp_wu.start()
    cp_wd.start()

    def max_norm(slot):
        ss = jnp.sum(wnorm[slot], axis=0, keepdims=True)
        return jnp.sqrt(jnp.max(ss, axis=1, keepdims=True))

    nk, nq, nv = max_norm(0), max_norm(1), max_norm(2)

    bound = (QSCALE * DH * D) * nq * nk
    safe = (bound <= SAFE_LOGIT) & (nv * (D ** 0.5) <= SAFE_V)
    flag[0] = jnp.sum(jnp.where(safe, 1, 0).astype(I32))

    def segment(s, carry):
        def side_work():
            return _Filler([out_steps(s - 1), ln1_steps(s + 1)], [PASS_STEPS, 2 * PASS_STEPS])

        def fast():
            stage_attention_fast(side_work())

        def safe():
            stage_scores_safe()
            side_work().upto(1.0)
            for h in range(H):
                for i in range(NQB):
                    pv_head(h, i)

        jax.lax.cond(flag[0] == 1, fast, safe)

        @pl.when(s + 1 < NSEG)
        def _():
            prev_out_copy(s).start()
            for i in range(NQB):
                attn_block(s, i)
            for g in range(NG):
                mem_update(g)
            for c in range(NCH):
                proj_q(c)
            for c in range(NCH):
                proj_k(c)
            for g in range(NG):
                mem_read(g)
            for c in range(NCH):
                proj_v(c)

        return carry

    jax.lax.fori_loop(0, NSEG, segment, 0)

    out_copy(NSEG - 2).start()
    prev_out_copy(0).wait()
    for i in range(NQB):
        attn_block(NSEG - 1, i)

    r = r_all[...]
    r_sel = jnp.max(jnp.max(r, axis=0, keepdims=True), axis=1, keepdims=True)
    ids = (128 * jax.lax.broadcasted_iota(I32, r.shape, 0)
           + jax.lax.broadcasted_iota(I32, r.shape, 1))
    cand = jnp.min(jnp.where(r == r_sel, ids, S), axis=0, keepdims=True)
    idx = jnp.minimum(jnp.sum(jnp.min(cand, axis=1, keepdims=True)), S - 1)
    for _ in out_steps(NSEG - 1):
        pass
    out_copy(NSEG - 1).start()
    blk = idx >> 7
    m_sel = stat2[blk, 0:1, :]
    rstd_sel = stat2[blk, 1:2, :]
    for r in range(D // RS):
        rows = slice(RS * r, RS * (r + 1))
        hn_sel[rows, :] = ((h_all[blk, rows, :] - m_sel) * rstd_sel).astype(BF16)
    onehot = (jax.lax.broadcasted_iota(I32, (16, 128), 1) == idx - blk * 128).astype(BF16)
    xs = _dot(onehot, hn_sel[...], NT).astype(BF16)
    cp_wg.wait()
    cp_wu.wait()
    cp_wd.wait()

    def down_steps(c, act):
        for r in range(D // RS):
            rows = slice(RS * r, RS * (r + 1))
            part = None if c == 0 else yacc[rows, :]
            for t in range(FC // 128):
                w = wdt_v[rows, FC * c + 128 * t:FC * c + 128 * (t + 1)].astype(F32)
                part = w * act[t] if part is None else part + w * act[t]
            yacc[rows, :] = part
            yield

    nch = FF // FC
    pending = None
    for c in range(nch):
        ga, up = [], []
        for t in range(FC // 128):
            tile = slice(FC * c + 128 * t, FC * c + 128 * (t + 1))
            ga.append(_dot(xs, wg_v[:, tile])[0:1])
            up.append(_dot(xs, wu_v[:, tile])[0:1])
            if pending is not None:
                pending.upto((t + 1) / (FC // 128))
        act = [g * _sigmoid(g) * u for g, u in zip(ga, up)]
        pending = _Filler([down_steps(c, act)], [D // RS])
    pending.upto(1.0)
    y = jnp.sum(yacc[...], axis=1, keepdims=True) * _sigmoid(r_sel)
    sel = jax.lax.broadcasted_iota(I32, (RS, 128), 1) == idx - blk * 128
    for r in range(D // RS):
        rows = slice(RS * r, RS * (r + 1))
        hh = h_all[blk, rows, :]
        stage[rows, :] = (hh + (hh - m_sel) * rstd_sel
                          + jnp.where(sel, y[rows], 0.0)).astype(BF16)
    for s in range(NSEG):
        out_copy(s).wait()
    fix = pltpu.make_async_copy(stage, out_hbm.at[:, hbm_cols(blk)], sem_w.at[7])
    fix.start()
    fix.wait()


@jax.jit
def pallas_sequential_preLN__memory_aug_infini_attn__moe_arch_mod__prompt_kernel(
    A_x: jax.Array,
    A_wq: jax.Array,
    A_wk: jax.Array,
    A_wv: jax.Array,
    A_wo: jax.Array,
    A_beta: jax.Array,
    B_x: jax.Array,
    B_w_r: jax.Array,
    B_w_gate: jax.Array,
    B_w_up: jax.Array,
    B_w_down: jax.Array,
):
    del B_x
    hbm = pl.BlockSpec(memory_space=pltpu.HBM)
    scratch = [
        pltpu.VMEM((H,), BF16),
        pltpu.VMEM((D,), BF16),
        pltpu.VMEM((NSEG * NQB, D, 128), BF16),
        pltpu.VMEM((D, D), BF16),
        pltpu.VMEM((D, D), BF16),
        pltpu.VMEM((D, D), BF16),
        pltpu.VMEM((D, D), BF16),
        pltpu.VMEM((D // 2, D), U32),
        pltpu.VMEM((D // 2, D), U32),
        pltpu.VMEM((D // 2, D), U32),
        pltpu.VMEM((D // 2, D), U32),
        pltpu.VMEM((NQB, D, 128), BF16),
        pltpu.VMEM((D, L), BF16),
        pltpu.VMEM((NG, L // 2, 128), U32),
        pltpu.VMEM((D, L), BF16),
        pltpu.VMEM((D, L), BF16),
        pltpu.VMEM((D, L), BF16),
        pltpu.VMEM((D, L), BF16),
        pltpu.VMEM((H * 32, L), BF16),
        pltpu.VMEM((H, NTILE * 128, 128), BF16),
        pltpu.VMEM((NG, MROWS, 128), F32),
        pltpu.VMEM((NG, MROWS, 128), BF16),
        pltpu.VMEM((NG, MROWS, 128), F32),
        pltpu.VMEM((NQB, D + 24, 128), F32),
        pltpu.VMEM((NQB, D + 24, 128), F32),
        pltpu.VMEM((NSEG * NQB, D, 128), F32),
        pltpu.VMEM((D, 128), BF16),
        pltpu.VMEM((D, 128), F32),
        pltpu.VMEM(((NSEG + 1) * NQB, D, 128), BF16),
        pltpu.VMEM((D, FF), BF16),
        pltpu.VMEM((D, FF), BF16),
        pltpu.VMEM((D, FF), BF16),
        pltpu.VMEM((128, 128), F32),
        pltpu.VMEM((H, 8, 128), F32),
        pltpu.VMEM((D, 128), F32),
        pltpu.VMEM((8, 128), F32),
        pltpu.VMEM((NSEG * NQB, 8, 128), F32),
        pltpu.VMEM((3, 24, D), F32),
        pltpu.VMEM((NSEG * NQB, 128), F32),
        pltpu.VMEM((D, 128), BF16),
        pltpu.SMEM((1,), I32),
        pltpu.SemaphoreType.DMA((NSEG,)),
        pltpu.SemaphoreType.DMA((NQB,)),
        pltpu.SemaphoreType.DMA((11,)),
        pltpu.SemaphoreType.DMA((NSEG + 1,)),
    ]
    out_t = pl.pallas_call(
        _kernel,
        out_shape=jax.ShapeDtypeStruct((D, S), BF16),
        in_specs=[hbm] * 10,
        out_specs=hbm,
        scratch_shapes=scratch,
        compiler_params=pltpu.CompilerParams(vmem_limit_bytes=100 * 1024 * 1024),
        name="infini_moe",
    )(A_x.reshape(S, D).T, A_wq, A_wk, A_wv, A_wo, A_beta, B_w_r, B_w_gate, B_w_up, B_w_down.T)
    return out_t.T.reshape(1, S, D)
```

```python
import functools

import jax
import jax.numpy as jnp
import jax.experimental.pallas as pl
import jax.experimental.pallas.tpu as pltpu

F32 = jnp.float32
BF16 = jnp.bfloat16
U32 = jnp.uint32
I32 = jnp.int32

S = 2048
D = 576
H = 32
DH = 18
NSEG = 4
L = S // NSEG
FF = 4608
NQB = L // 128
TOFF = (0, 1, 3, 6)
NTILE = 10
NG = 5
WIN = 112
GROUP_HEADS = tuple(tuple(h for h in range(H)
                          if min(max(0, -(-(DH * h + DH - 128) // WIN)), NG - 1) == g)
                    for g in range(NG))
GROUP_OF = {h: g for g in range(NG) for h in GROUP_HEADS[g]}
MROWS = 144
CH = 144
NCH = D // CH
RS = 64
PASS_STEPS = NQB * (D // RS)
FC = 512
LAG = 20
LN_EPS = 1e-5
LOG2E = 1.4426950408889634
QSCALE = (DH ** -0.5) * LOG2E
SAFE_LOGIT = 60.0
SAFE_V = 2.0 ** 50

NN = (((1,), (0,)), ((), ()))
NT = (((1,), (1,)), ((), ()))

for _g, _hs in enumerate(GROUP_HEADS):
    for _h in _hs:
        assert WIN * _g <= DH * _h and DH * _h + DH <= WIN * _g + 128


def _dot(a, b, dims=NN):
    return jax.lax.dot_general(a, b, dims, preferred_element_type=F32)


class _Filler:
    def __init__(self, gens, counts):
        self.gens, self.counts, self.done = gens, counts, [0] * len(gens)

    def upto(self, frac):
        for k, gen in enumerate(self.gens):
            while self.done[k] < min(frac, 1.0) * self.counts[k]:
                next(gen, None)
                self.done[k] += 1
            if frac >= 1.0:
                for _ in gen:
                    pass


def _phi(t):
    return jnp.where(t > 0, t + 1.0, jnp.exp(t))


def _sigmoid(t):
    return 1.0 / (1.0 + jnp.exp(-t))


def _recip(x):
    r = pl.reciprocal(x, approx=True)
    return r * (2.0 - x * r)


def _kernel(xt_hbm, wq_hbm, wk_hbm, wv_hbm, wo_hbm, beta_hbm, wr_hbm, wg_hbm, wu_hbm, wdt_hbm,
            out_hbm,
            beta_ref, wr_ref, xbuf, wq_raw, wk_raw, wv_raw, wo_raw, wqt, wkt, wvt, wot, xn, ktn, kb, qt, pkt, pqt,
            vtn, vt32, pbuf, m_f32, m_bf, keep, amem, ot, h_all, hn_sel, yacc, obuf, wg_v, wu_v, wdt_v,
            gcol, omg, wrcol, wrsum, stat2, wnorm, r_all, stage, flag, sem_x, sem_x0, sem_w, sem_o):
    class _Group:
        def __init__(self, copies):
            self.copies = copies

        def start(self):
            for cp in self.copies:
                cp.start()

        def wait(self):
            for cp in self.copies:
                cp.wait()

    def hbm_cols(blk):
        return pl.ds(pl.multiple_of(blk * 128, 128), 128)

    def x_copy(s):
        return _Group([pltpu.make_async_copy(xt_hbm.at[:, hbm_cols(s * NQB + i)],
                                             xbuf.at[s * NQB + i], sem_x.at[s])
                       for i in range(NQB)])

    def out_copy(s):
        return _Group([pltpu.make_async_copy(obuf.at[s * NQB + i],
                                             out_hbm.at[:, hbm_cols(s * NQB + i)], sem_o.at[s])
                       for i in range(NQB)])

    def prev_out_copy(s):
        src = jnp.where(s > 0, s - 1, NSEG) * NQB
        dst = jnp.where(s > 0, s - 1, NSEG - 1) * NQB
        sem = jnp.where(s > 0, s - 1, NSEG)
        return _Group([pltpu.make_async_copy(obuf.at[src + i], out_hbm.at[:, hbm_cols(dst + i)],
                                             sem_o.at[sem]) for i in range(NQB)])

    cp_beta = pltpu.make_async_copy(beta_hbm, beta_ref, sem_w.at[8])
    cp_wr = pltpu.make_async_copy(wr_hbm, wr_ref, sem_w.at[9])
    ksplit = 384
    cp_wk = pltpu.make_async_copy(wk_hbm.at[:, 0:ksplit], wk_raw.at[:, 0:ksplit], sem_w.at[0])
    cp_wk2 = pltpu.make_async_copy(wk_hbm.at[:, ksplit:D], wk_raw.at[:, ksplit:D], sem_w.at[10])
    x0_copies = [pltpu.make_async_copy(xt_hbm.at[:, 128 * i:128 * (i + 1)], xbuf.at[i],
                                       sem_x0.at[i]) for i in range(NQB)]
    cp_wq = pltpu.make_async_copy(wq_hbm, wq_raw, sem_w.at[1])
    cp_wv = pltpu.make_async_copy(wv_hbm, wv_raw, sem_w.at[2])
    cp_wo = pltpu.make_async_copy(wo_hbm, wo_raw, sem_w.at[3])
    cp_wg = pltpu.make_async_copy(wg_hbm, wg_v, sem_w.at[4])
    cp_wu = pltpu.make_async_copy(wu_hbm, wu_v, sem_w.at[5])
    cp_wd = pltpu.make_async_copy(wdt_hbm, wdt_v, sem_w.at[6])

    def fold8(v):
        return jnp.sum(v.reshape(v.shape[0] // 8, 8, 128), axis=0)

    def col_total(acc):
        return jnp.sum(acc, axis=0, keepdims=True) * (1.0 / D)

    def ln1_steps(s, arrivals=None):
        seg = jnp.minimum(s, NSEG - 1)
        for c in range(NQB):
            if arrivals is not None:
                arrivals[c].wait()
            xs = lambda r: xbuf[seg * NQB + c, RS * r:RS * (r + 1), :].astype(F32)
            acc = None
            for r in range(D // RS):
                xr = xs(r)
                if r == 0:
                    pivot = xr[0:1, :]
                d = xr - pivot
                part = (fold8(d), fold8(d * d))
                acc = part if acc is None else (acc[0] + part[0], acc[1] + part[1])
                yield
            md = col_total(acc[0])
            m = pivot + md
            rstd = jax.lax.rsqrt(jnp.maximum(col_total(acc[1]) - md * md, 0.0) + LN_EPS)
            for r in range(D // RS):
                xn[c, RS * r:RS * (r + 1), :] = (
                    (xs(r) - m) * rstd).astype(BF16)
                yield

    def xn_all():
        return jnp.concatenate([xn[c] for c in range(NQB)], axis=1)

    def rows_of(c):
        return slice(CH * c, CH * (c + 1))

    def packed(words):
        return pltpu.bitcast(words, BF16)

    def wt_rows(wt, c):
        return packed(wt[CH // 2 * c:CH // 2 * (c + 1), :])

    def transpose_keys(g):
        kb[g] = pltpu.bitcast(ktn[WIN * g:WIN * g + 128, :].T, U32)

    def proj_k(c):
        kt = _dot(wt_rows(wkt, c), xn_all())
        pkt[rows_of(c), :] = _phi(kt).astype(BF16)
        ktn[rows_of(c), :] = kt.astype(BF16)
        if c == 0:
            transpose_keys(0)

    def proj_q(c):
        qf = _dot(wt_rows(wqt, c), xn_all())
        qt[rows_of(c), :] = (qf * QSCALE).astype(BF16)
        pqt[rows_of(c), :] = _phi(qf).astype(BF16)

    def proj_v(c):
        tail = jnp.concatenate([jnp.zeros((6, L), F32), jnp.ones((8, L), F32)], axis=0)
        vt = _dot(wt_rows(wvt, c), xn_all())
        vtn[rows_of(c), :] = vt.astype(BF16)
        for j in range(CH // DH):
            h = (CH // DH) * c + j
            vt32[32 * h:32 * h + 16, :] = vt[DH * j:DH * j + 16].astype(BF16)
            vt32[32 * h + 16:32 * h + 32, :] = jnp.concatenate(
                [vt[DH * j + 16:DH * j + 18], tail], axis=0).astype(BF16)

    def masked_q(w0, i, word_mask):
        qu = pltpu.bitcast(qt[pl.ds(w0, 128), 128 * i:128 * (i + 1)], U32)
        return pltpu.bitcast(jnp.where(word_mask, qu, jnp.uint32(0)), BF16)

    def head_word_mask(lo):
        word = jax.lax.broadcasted_iota(I32, (64, 128), 0)
        return (2 * word >= lo) & (2 * word < lo + DH)

    def causal_mask():
        return (jax.lax.broadcasted_iota(I32, (128, 128), 0)
                <= jax.lax.broadcasted_iota(I32, (128, 128), 1))

    def pv_head(h, i):
        n = 128 * (i + 1)
        r0 = TOFF[i] * 128
        o = _dot(vt32[32 * h:32 * h + 32, 0:n], pbuf[h, r0:r0 + n, :])
        a = omg[h] * _recip(o[24:32, :])
        on = (o[0:24].reshape(3, 8, 128) * a).reshape(24, 128)
        ot[i, DH * h:DH * h + 24, :] = on + amem[i, DH * h:DH * h + 24, :]

    def stage_attention_fast(filler):
        causal = causal_mask()
        for h in range(H + LAG):
            if h < H:
                g = GROUP_OF[h]
                word_mask = head_word_mask(DH * h - WIN * g)
                if h == GROUP_HEADS[g][0] and g + 1 < NG:
                    transpose_keys(g + 1)
            for i in range(NQB):
                n = 128 * (i + 1)
                if h < H:
                    filler.upto((NTILE * h + TOFF[i] + i + 1) / (NTILE * LAG))
                    st = _dot(packed(kb[g, 0:n // 2, :]), masked_q(WIN * g, i, word_mask))
                    p = jnp.exp2(st)
                    r0 = TOFF[i] * 128
                    if i > 0:
                        pbuf[h, r0:r0 + 128 * i, :] = p[:n - 128].astype(BF16)
                    pbuf[h, r0 + 128 * i:r0 + n, :] = jnp.where(
                        causal, p[n - 128:n], 0.0).astype(BF16)
                if h >= LAG:
                    pv_head(h - LAG, i)

    def stage_scores_safe():
        causal = causal_mask()
        for g in range(1, NG):
            transpose_keys(g)

        def head(h, carry):
            g = jnp.clip((DH * h + DH - 128 + WIN - 1) // WIN, 0, NG - 1)
            g = jnp.where(DH * h + DH <= 128, 0, g)
            w0 = pl.multiple_of(WIN * g, 16)
            word_mask = head_word_mask(DH * h - WIN * g)
            for i in range(NQB):
                n = 128 * (i + 1)
                st = _dot(packed(kb[g, 0:n // 2, :]), masked_q(w0, i, word_mask))
                sd = jnp.where(causal, st[n - 128:n], -jnp.inf)
                m = jnp.max(sd, axis=0, keepdims=True)
                if i > 0:
                    m = jnp.maximum(m, jnp.max(st[:n - 128], axis=0, keepdims=True))
                r0 = TOFF[i] * 128
                if i > 0:
                    pbuf[h, r0:r0 + 128 * i, :] = jnp.exp2(st[:n - 128] - m).astype(BF16)
                pbuf[h, r0 + 128 * i:r0 + n, :] = jnp.exp2(sd - m).astype(BF16)
            return carry

        jax.lax.fori_loop(0, H, head, 0)

    def attn_block(s, i):
        blk = s * NQB + i
        otb = ot[i, 0:D, :].astype(BF16)
        acc = None
        for c in range(NCH):
            hh = _dot(wt_rows(wot, c), otb) + xbuf[blk, rows_of(c), :].astype(F32)
            h_all[blk, rows_of(c), :] = hh
            if c == 0:
                pivot = hh[0:1, :]
            d = hh - pivot
            part = (fold8(d), fold8(d * d), fold8(d * wrcol[rows_of(c), :]))
            acc = part if acc is None else tuple(a + b for a, b in zip(acc, part))
        md = col_total(acc[0])
        var = jnp.maximum(col_total(acc[1]) - md * md, 0.0)
        rstd = jax.lax.rsqrt(var + LN_EPS)
        stat2[blk, 0:1, :] = pivot + md
        stat2[blk, 1:2, :] = rstd
        r_all[pl.ds(blk, 1), :] = (jnp.sum(acc[2], axis=0, keepdims=True) - md * wrsum[0:1, :]) * rstd

    def mem_update(g):
        lhs = jnp.concatenate([jnp.ones((16, L), BF16), vtn[WIN * g:WIN * g + 128, :]], axis=0)
        upd = _dot(lhs, pkt[WIN * g:WIN * g + 128, :], NT)
        m_new = m_f32[g] + upd * keep[g]
        m_f32[g] = m_new
        m_bf[g] = m_new.astype(BF16)

    def mem_read(g):
        for i in range(NQB):
            nm = _dot(m_bf[g], pqt[WIN * g:WIN * g + 128, 128 * i:128 * (i + 1)])
            first = GROUP_HEADS[g][0]
            b = gcol[first:first + 8, :] * _recip(nm[0:8, :] + 1e-6)
            for j, h in enumerate(GROUP_HEADS[g]):
                lo = 16 + DH * h - WIN * g
                n = min(24, MROWS - lo)
                amem[i, DH * h:DH * h + n, :] = nm[lo:lo + n] * b[j:j + 1, :]

    def out_steps(s):
        seg = jnp.maximum(s, 0)
        for i in range(NQB):
            blk = seg * NQB + i
            m = stat2[blk, 0:1, :]
            rstd = stat2[blk, 1:2, :]
            for r in range(D // RS):
                rows = slice(RS * r, RS * (r + 1))
                hh = h_all[blk, rows, :]
                obuf[blk, rows, :] = (hh + (hh - m) * rstd).astype(BF16)
                yield

    for cp in [cp_beta, cp_wr] + x0_copies + [cp_wk]:
        cp.start()

    row = jax.lax.broadcasted_iota(I32, (MROWS, 128), 0)
    lane = jax.lax.broadcasted_iota(I32, (MROWS, 128), 1)
    for g in range(NG):
        first, nh = GROUP_HEADS[g][0], len(GROUP_HEADS[g])
        lane_head = ((lane + WIN * g) * 3641) >> 16
        row_head = jnp.where(row < 16, row + first, ((row - 16 + WIN * g) * 3641) >> 16)
        ok = (lane_head == row_head) & (row_head >= first) & (row_head < first + nh)
        keep[g] = jnp.where(ok, 1.0, 0.0)
    m_f32[...] = jnp.zeros_like(m_f32)
    amem[...] = jnp.zeros_like(amem)
    h_all[0:NQB] = jnp.zeros((NQB, D, 128), F32)
    obuf[NSEG * NQB:(NSEG + 1) * NQB] = jnp.zeros((NQB, D, 128), BF16)
    stat2[0:NQB] = jnp.zeros((NQB, 8, 128), F32)

    cp_beta.wait()
    cp_wr.wait()
    cp_wk2.start()
    cp_wq.start()
    beta = beta_ref[...].astype(F32).reshape(1, H)
    gpad = jnp.concatenate([_sigmoid(beta), jnp.zeros((1, 128 - H), F32)], axis=1)
    gcol[...] = jnp.transpose(jnp.broadcast_to(gpad, (128, 128)))
    for h in range(H):
        omg[h] = jnp.broadcast_to(1.0 - gcol[h:h + 1, :], (8, 128))
    wr = jnp.concatenate([wr_ref[...].astype(F32).reshape(1, D), jnp.zeros((1, 64), F32)], axis=1)
    wrcol[...] = jnp.transpose(jnp.broadcast_to(wr, (128, D + 64)))[0:D]
    wrsum[...] = jnp.broadcast_to(jnp.sum(wrcol[...], axis=0, keepdims=True), (8, 128))

    def transpose_tile(dst, raw, t):
        hi = min(128 * (t + 1), D)
        dst[64 * t:hi // 2, :] = pltpu.bitcast(raw[:, 128 * t:hi].T, U32)

    def col_norm_steps(raw, slot):
        for t in range(5):
            hi = min(128 * (t + 1), D)
            for k in range(3):
                w = raw[192 * k:192 * (k + 1), 128 * t:hi].astype(F32)
                wnorm[slot, 8 * k:8 * (k + 1), 128 * t:hi] = jnp.sum(
                    (w * w).reshape(24, 8, hi - 128 * t), axis=0)
                yield

    for _ in ln1_steps(0, x0_copies):
        pass
    cp_wv.start()
    cp_wo.start()
    cp_wk.wait()
    for t in range(3):
        transpose_tile(wkt, wk_raw, t)
    proj_k(0)
    proj_k(1)
    cp_wk2.wait()
    cp_wq.wait()
    for s in range(1, NSEG):
        x_copy(s).start()
    side = _Filler([col_norm_steps(wk_raw, 0), col_norm_steps(wq_raw, 1)], [15, 15])
    transpose_tile(wkt, wk_raw, 3)
    transpose_tile(wkt, wk_raw, 4)
    proj_k(2)
    transpose_tile(wqt, wq_raw, 0)
    side.upto(0.25)
    transpose_tile(wqt, wq_raw, 1)
    proj_k(3)
    side.upto(0.5)
    for c in range(2):
        proj_q(c)
        transpose_tile(wqt, wq_raw, c + 2)
        side.upto(0.75 + 0.25 * c)
    transpose_tile(wqt, wq_raw, 4)
    cp_wv.wait()
    cp_wo.wait()
    side = _Filler([col_norm_steps(wv_raw, 2)], [15])
    for c in range(2, NCH):
        proj_q(c)
        transpose_tile(wvt, wv_raw, c - 2)
        side.upto((c - 1) / 2)
    for c in range(NCH):
        proj_v(c)
        if c + 2 < 5:
            transpose_tile(wvt, wv_raw, c + 2)
        transpose_tile(wot, wo_raw, c)
    transpose_tile(wot, wo_raw, 4)

    for s in range(1, NSEG):
        x_copy(s).wait()
    cp_wg.start()
    cp_wu.start()
    cp_wd.start()

    def max_sq_norm(slot):
        ss = jnp.sum(wnorm[slot], axis=0, keepdims=True)
        return jnp.max(ss, axis=1, keepdims=True)

    bound_sq = (QSCALE * DH * D) ** 2 * max_sq_norm(0) * max_sq_norm(1)
    safe = (bound_sq <= SAFE_LOGIT ** 2) & (max_sq_norm(2) * D <= SAFE_V ** 2)
    flag[0] = jnp.sum(jnp.where(safe, 1, 0).astype(I32))

    def segment(s, carry):
        def side_work():
            return _Filler([out_steps(s - 1), ln1_steps(s + 1)], [PASS_STEPS, 2 * PASS_STEPS])

        def fast():
            stage_attention_fast(side_work())

        def safe():
            stage_scores_safe()
            side_work().upto(1.0)
            for h in range(H):
                for i in range(NQB):
                    pv_head(h, i)

        jax.lax.cond(flag[0] == 1, fast, safe)

        @pl.when(s + 1 < NSEG)
        def _():
            prev_out_copy(s).start()
            for i in range(NQB):
                attn_block(s, i)
            for g in range(NG):
                mem_update(g)
            for c in range(NCH):
                proj_q(c)
            for c in range(NCH):
                proj_k(c)
            for g in range(NG):
                mem_read(g)
            for c in range(NCH):
                proj_v(c)

        return carry

    jax.lax.fori_loop(0, NSEG, segment, 0)

    out_copy(NSEG - 2).start()
    prev_out_copy(0).wait()
    for i in range(NQB):
        attn_block(NSEG - 1, i)

    r = r_all[...]
    r_sel = jnp.max(jnp.max(r, axis=0, keepdims=True), axis=1, keepdims=True)
    ids = (128 * jax.lax.broadcasted_iota(I32, r.shape, 0)
           + jax.lax.broadcasted_iota(I32, r.shape, 1))
    cand = jnp.min(jnp.where(r == r_sel, ids, S), axis=0, keepdims=True)
    idx = jnp.minimum(jnp.sum(jnp.min(cand, axis=1, keepdims=True)), S - 1)
    for _ in out_steps(NSEG - 1):
        pass
    out_copy(NSEG - 1).start()
    blk = idx >> 7
    m_sel = stat2[blk, 0:1, :]
    rstd_sel = stat2[blk, 1:2, :]
    for r in range(D // RS):
        rows = slice(RS * r, RS * (r + 1))
        hn_sel[rows, :] = ((h_all[blk, rows, :] - m_sel) * rstd_sel).astype(BF16)
    onehot = (jax.lax.broadcasted_iota(I32, (16, 128), 1) == idx - blk * 128).astype(BF16)
    xs = _dot(onehot, hn_sel[...], NT).astype(BF16)
    cp_wg.wait()
    cp_wu.wait()
    cp_wd.wait()

    def down_steps(c, act):
        for r in range(D // RS):
            rows = slice(RS * r, RS * (r + 1))
            part = None if c == 0 else yacc[rows, :]
            for t in range(FC // 128):
                w = wdt_v[rows, FC * c + 128 * t:FC * c + 128 * (t + 1)].astype(F32)
                part = w * act[t] if part is None else part + w * act[t]
            yacc[rows, :] = part
            yield

    nch = FF // FC
    pending = None
    for c in range(nch):
        ga, up = [], []
        for t in range(FC // 128):
            tile = slice(FC * c + 128 * t, FC * c + 128 * (t + 1))
            ga.append(_dot(xs, wg_v[:, tile])[0:1])
            up.append(_dot(xs, wu_v[:, tile])[0:1])
            if pending is not None:
                pending.upto((t + 1) / (FC // 128))
        act = [g * _sigmoid(g) * u for g, u in zip(ga, up)]
        pending = _Filler([down_steps(c, act)], [D // RS])
    pending.upto(1.0)
    y = jnp.sum(yacc[...], axis=1, keepdims=True) * _sigmoid(r_sel)
    sel = jax.lax.broadcasted_iota(I32, (RS, 128), 1) == idx - blk * 128
    for r in range(D // RS):
        rows = slice(RS * r, RS * (r + 1))
        hh = h_all[blk, rows, :]
        stage[rows, :] = (hh + (hh - m_sel) * rstd_sel
                          + jnp.where(sel, y[rows], 0.0)).astype(BF16)
    for s in range(NSEG):
        out_copy(s).wait()
    fix = pltpu.make_async_copy(stage, out_hbm.at[:, hbm_cols(blk)], sem_w.at[7])
    fix.start()
    fix.wait()


@jax.jit
def pallas_sequential_preLN__memory_aug_infini_attn__moe_arch_mod__prompt_kernel(
    A_x: jax.Array,
    A_wq: jax.Array,
    A_wk: jax.Array,
    A_wv: jax.Array,
    A_wo: jax.Array,
    A_beta: jax.Array,
    B_x: jax.Array,
    B_w_r: jax.Array,
    B_w_gate: jax.Array,
    B_w_up: jax.Array,
    B_w_down: jax.Array,
):
    del B_x
    hbm = pl.BlockSpec(memory_space=pltpu.HBM)
    scratch = [
        pltpu.VMEM((H,), BF16),
        pltpu.VMEM((D,), BF16),
        pltpu.VMEM((NSEG * NQB, D, 128), BF16),
        pltpu.VMEM((D, D), BF16),
        pltpu.VMEM((D, D), BF16),
        pltpu.VMEM((D, D), BF16),
        pltpu.VMEM((D, D), BF16),
        pltpu.VMEM((D // 2, D), U32),
        pltpu.VMEM((D // 2, D), U32),
        pltpu.VMEM((D // 2, D), U32),
        pltpu.VMEM((D // 2, D), U32),
        pltpu.VMEM((NQB, D, 128), BF16),
        pltpu.VMEM((D, L), BF16),
        pltpu.VMEM((NG, L // 2, 128), U32),
        pltpu.VMEM((D, L), BF16),
        pltpu.VMEM((D, L), BF16),
        pltpu.VMEM((D, L), BF16),
        pltpu.VMEM((D, L), BF16),
        pltpu.VMEM((H * 32, L), BF16),
        pltpu.VMEM((H, NTILE * 128, 128), BF16),
        pltpu.VMEM((NG, MROWS, 128), F32),
        pltpu.VMEM((NG, MROWS, 128), BF16),
        pltpu.VMEM((NG, MROWS, 128), F32),
        pltpu.VMEM((NQB, D + 24, 128), F32),
        pltpu.VMEM((NQB, D + 24, 128), F32),
        pltpu.VMEM((NSEG * NQB, D, 128), F32),
        pltpu.VMEM((D, 128), BF16),
        pltpu.VMEM((D, 128), F32),
        pltpu.VMEM(((NSEG + 1) * NQB, D, 128), BF16),
        pltpu.VMEM((D, FF), BF16),
        pltpu.VMEM((D, FF), BF16),
        pltpu.VMEM((D, FF), BF16),
        pltpu.VMEM((128, 128), F32),
        pltpu.VMEM((H, 8, 128), F32),
        pltpu.VMEM((D, 128), F32),
        pltpu.VMEM((8, 128), F32),
        pltpu.VMEM((NSEG * NQB, 8, 128), F32),
        pltpu.VMEM((3, 24, D), F32),
        pltpu.VMEM((NSEG * NQB, 128), F32),
        pltpu.VMEM((D, 128), BF16),
        pltpu.SMEM((1,), I32),
        pltpu.SemaphoreType.DMA((NSEG,)),
        pltpu.SemaphoreType.DMA((NQB,)),
        pltpu.SemaphoreType.DMA((11,)),
        pltpu.SemaphoreType.DMA((NSEG + 1,)),
    ]
    out_t = pl.pallas_call(
        _kernel,
        out_shape=jax.ShapeDtypeStruct((D, S), BF16),
        in_specs=[hbm] * 10,
        out_specs=hbm,
        scratch_shapes=scratch,
        compiler_params=pltpu.CompilerParams(vmem_limit_bytes=100 * 1024 * 1024),
        name="infini_moe",
    )(A_x.reshape(S, D).T, A_wq, A_wk, A_wv, A_wo, A_beta, B_w_r, B_w_gate, B_w_up, B_w_down.T)
    return out_t.T.reshape(1, S, D)
```
